```python
import jax
import jax.numpy as jnp

def _softmax(x, axis=-1):
    return jax.nn.softmax(x, axis=axis)

def _gelu(x):
    return jax.nn.gelu(x, approximate=True)

def _silu(x):
    return jax.nn.silu(x)

def _sigmoid(x):
    return jax.nn.sigmoid(x)

def _layernorm(x, axis=-1, eps=1e-05):
    m = jnp.mean(x, axis=axis, keepdims=True)
    v = jnp.var(x, axis=axis, keepdims=True)
    return (x - m) / jnp.sqrt(v + eps)

def _scatter_add(tgt, idx, src, axis=0):
    return tgt.at[idx].add(src)

def _segment_sum(src, seg, n):
    return jax.ops.segment_sum(src, seg, n)

class _Rng:

    def __init__(self, key):
        self._k = key

    def _next(self):
        self._k, sub = jax.random.split(self._k)
        return sub

    def normal(self, shape):
        return jax.random.normal(self._next(), shape, dtype=jnp.bfloat16)

    def randint(self, lo, hi, shape):
        return jax.random.randint(self._next(), shape, lo, hi, dtype=jnp.int32)

    def uniform(self, shape, lo=0.0, hi=1.0):
        return jax.random.uniform(self._next(), shape, jnp.bfloat16, lo, hi)

    def permutation(self, n):
        return jax.random.permutation(self._next(), n)
kernel_name = 'parallel_sum__memory_aug_infini_attn__moe_arch_mod__prompt'

def setup_inputs():
    _rng = _Rng(jax.random.key(int.from_bytes(__import__("os").urandom(4), "little")))
    _w = lambda a: (lambda t: t.astype(jnp.bfloat16) if jnp.issubdtype(t.dtype, jnp.floating) else t)(jnp.asarray(a))

    def _A_setup():
        B, S, D, H = (1, 2048, 576, 32)
        N = 4
        L = max(1, S // N)
        sc = D ** (-0.5)
        return {'x': _w((lambda *s: _rng.normal(s) * 0.05)(B, N * L, D)), 'wq': _w((lambda *s: _rng.normal(s) * 0.05)(D, D) * sc), 'wk': _w((lambda *s: _rng.normal(s) * 0.05)(D, D) * sc), 'wv': _w((lambda *s: _rng.normal(s) * 0.05)(D, D) * sc), 'wo': _w((lambda *s: _rng.normal(s) * 0.05)(D, D) * sc), 'beta': _w((lambda *s: _rng.normal(s) * 0.05)(H))}
    _A_in = _A_setup()

    def _B_setup():
        B, S, D, F, C = (1, 2048, 576, 4608, 2)
        return {'x': _w((lambda *s: _rng.normal(s) * 0.05)(B, S, D)), 'w_r': _w((lambda *s: _rng.normal(s) * 0.05)(D)), 'w_gate': _w((lambda *s: _rng.normal(s) * 0.05)(D, F)), 'w_up': _w((lambda *s: _rng.normal(s) * 0.05)(D, F)), 'w_down': _w((lambda *s: _rng.normal(s) * 0.05)(F, D))}
    _B_in = _B_setup()
    return {'A_x': _A_in['x'], 'A_wq': _A_in['wq'], 'A_wk': _A_in['wk'], 'A_wv': _A_in['wv'], 'A_wo': _A_in['wo'], 'A_beta': _A_in['beta'], 'B_x': _B_in['x'], 'B_w_r': _B_in['w_r'], 'B_w_gate': _B_in['w_gate'], 'B_w_up': _B_in['w_up'], 'B_w_down': _B_in['w_down']}

def reference(A_x, A_wq, A_wk, A_wv, A_wo, A_beta, B_x, B_w_r, B_w_gate, B_w_up, B_w_down):

    def _A_ref(x, wq, wk, wv, wo, beta):
        B, S, D = x.shape
        H = 32
        Dh = D // H
        N = 4
        L = S // N
        q = (lambda x, *d: x.transpose(*d))((x @ wq).reshape(B, S, H, Dh), 0, 2, 1, 3).reshape(B, H, N, L, Dh)
        k = (lambda x, *d: x.transpose(*d))((x @ wk).reshape(B, S, H, Dh), 0, 2, 1, 3).reshape(B, H, N, L, Dh)
        v = (lambda x, *d: x.transpose(*d))((x @ wv).reshape(B, S, H, Dh), 0, 2, 1, 3).reshape(B, H, N, L, Dh)
        phi = lambda t: jnp.where(t > 0, t + 1.0, jnp.exp(t))
        scale = Dh ** (-0.5)
        ar = jnp.arange(L)
        mask = (lambda x, dt: x.astype(dt))(ar[:, None] < ar[None, :], x.dtype) * -1000000000.0
        g = _sigmoid(beta).reshape(1, H, 1, 1)
        M = jnp.einsum('bhd,bhe->bhde', q[:, :, 0, 0, :] * 0.0, q[:, :, 0, 0, :] * 0.0)
        z = q[:, :, 0, 0, :] * 0.0
        outs = []
        for s in range(N):
            qs, ks, vs = (q[:, :, s].copy(), k[:, :, s].copy(), v[:, :, s].copy())
            logits = jnp.einsum('bhqd,bhkd->bhqk', qs, ks) * scale + mask
            p = _softmax(logits, axis=-1)
            a_dot = jnp.einsum('bhqk,bhkd->bhqd', p, vs)
            pq = phi(qs)
            num = jnp.einsum('bhld,bhde->bhle', pq, M)
            den = jnp.einsum('bhld,bhd->bhl', pq, z)[..., None] + 1e-06
            a_mem = num / den
            o = g * a_mem + (1.0 - g) * a_dot
            outs.append(o)
            pk = phi(ks)
            M = M + jnp.einsum('bhld,bhle->bhde', pk, vs)
            z = z + jnp.einsum('bhld->bhd', pk)
        o = (lambda x, *d: x.transpose(*d))(jnp.stack(outs, 2).reshape(B, H, S, Dh), 0, 2, 1, 3).reshape(B, S, D)
        return o @ wo

    def _B_ref(x, w_r, w_gate, w_up, w_down):
        B, S, D = x.shape
        C = 2
        r = x @ w_r
        idx = jnp.argsort(-r, axis=-1)[:, :C]
        idx_e = jnp.repeat(idx.reshape(B, C, 1), D, axis=2)
        x_sel = jnp.take_along_axis(x, idx_e, axis=1)
        g = _silu(x_sel @ w_gate)
        u = x_sel @ w_up
        y = g * u @ w_down
        r_sel = _sigmoid(jnp.take_along_axis(r, idx, axis=1))
        y = y * r_sel.reshape(B, C, 1)
        b_off = (jnp.arange(B) * S).reshape(B, 1)
        flat_idx = (idx + b_off).reshape(B * C)
        zero = (x * 0.0).reshape(B * S, D)
        upd = _scatter_add(zero, flat_idx, y.reshape(B * C, D), axis=0)
        return x + upd.reshape(B, S, D)
    x = A_x
    xn = _layernorm(x, axis=-1)
    return x + _A_ref(xn, A_wq, A_wk, A_wv, A_wo, A_beta) + _B_ref(xn, B_w_r, B_w_gate, B_w_up, B_w_down)
```

```python
import jax
import jax.numpy as jnp
from jax import lax
from jax.experimental import pallas as pl
from jax.experimental.pallas import tpu as pltpu

S = 2048
D = 576
H = 32
DH = 18
NSEG = 4
L = 512
FF = 4608
NG = 5
HPG = 7
GW = HPG * DH
NQT = L // 128
PROWS = 3 * D + 16
RROW = 3 * D
MROWS = 144
OROWS = 640
LOG2E = 1.4426950408889634
QSCALE = DH ** -0.5 * LOG2E
NEG = -1e30
SAFE_LOG2 = 40.0
LN_EPS = 1.0013580322265625e-05
F32 = jnp.float32
BF16 = jnp.bfloat16
U32 = jnp.uint32

_NN = (((1,), (0,)), ((), ()))
_NT = (((1,), (1,)), ((), ()))


def _dot(a, b):
    return lax.dot_general(a, b, _NN, preferred_element_type=F32)


def _dot_nt(a, b):
    return lax.dot_general(a, b, _NT, preferred_element_type=F32)


def _iota(shape, dim):
    return lax.broadcasted_iota(jnp.int32, shape, dim)


def _round_bf16(v):
    return v.astype(BF16).astype(F32)


def _pack(v):
    return pltpu.bitcast(v.astype(BF16), U32)


def _unpack(u):
    return pltpu.bitcast(u, BF16)


def _heads_in_group(g):
    return HPG if g < NG - 1 else H - HPG * (NG - 1)


def _phi(t):
    return jnp.where(t > 0, t + 1.0, jnp.exp(t))


def _kernel(x_hbm, wq_hbm, wk_hbm, wv_hbm, wo_hbm, beta_hbm, wr_hbm,
            wg_hbm, wu_hbm, wd_hbm,
            o_ref,
            x_v, wq_v, wk_v, wv_v, wo_v, beta_v, wr_v, wg_v, wu_v, wd_v,
            wall, wot, xn_v, qt_v, k_v, vt_v, mem_v, st_v,
            r_v, yb_v, idx_s, safe_s, gate_v, ot_v, bias_v,
            sems):
    step = pl.program_id(0)

    x_copies = [
        pltpu.make_async_copy(x_hbm.at[:, pl.ds(c * L, L)], x_v.at[c], sems.at[c])
        for c in range(NSEG)
    ]
    pairs = [(wq_hbm, wq_v), (wk_hbm, wk_v), (wv_hbm, wv_v), (wo_hbm, wo_v),
             (beta_hbm, beta_v), (wr_hbm, wr_v),
             (wg_hbm, wg_v), (wu_hbm, wu_v), (wd_hbm, wd_v)]
    (cp_wq, cp_wk, cp_wv, cp_wo, cp_beta, cp_wr, cp_wg, cp_wu, cp_wd) = [
        pltpu.make_async_copy(src, dst, sems.at[NSEG + i])
        for i, (src, dst) in enumerate(pairs)
    ]

    def layer_norm(c):
        xf = x_v[c].astype(F32)
        mean = jnp.sum(xf, axis=0, keepdims=True) * (1.0 / D)
        cen = xf - mean
        var = jnp.sum(cen * cen, axis=0, keepdims=True) * (1.0 / D)
        sd = _round_bf16(jnp.sqrt(_round_bf16(_round_bf16(var) + LN_EPS)))
        xn = (xf - _round_bf16(mean)) * (1.0 / sd)
        xn_v[c] = _pack(xn)

    def init_constants():
        gate = jax.nn.sigmoid(beta_v[...].astype(F32))
        on_diag = _iota((H, H), 0) == _iota((H, H), 1)
        gcol = jnp.sum(jnp.where(on_diag, gate, 0.0), axis=1, keepdims=True)
        gate_v[...] = jnp.broadcast_to(gcol, (H, 128))
        bias_v[...] = jnp.where(_iota((128, 128), 0) > _iota((128, 128), 1), NEG, 0.0)
        router = jnp.broadcast_to(wr_v[...].astype(F32), (16, D))
        wall[RROW // 2:PROWS // 2, :] = _pack(
            jnp.where(_iota((16, D), 0) == 0, router, 0.0))

    def project(c):
        return _dot(_unpack(wall[...]), _unpack(xn_v[c]))

    def store_qkv(c, pt):
        r_v[c:c + 1, :] = _round_bf16(pt[RROW:RROW + 1, :])
        qa = jnp.max(jnp.abs(pt[0:D, :])) * QSCALE
        ka = jnp.max(jnp.abs(pt[D:2 * D, :]))
        safe_s[c] = (qa * ka * (DH * 1.02) <= SAFE_LOG2).astype(jnp.int32)

        tail_row = _iota((8, L), 0)
        for h in range(H):
            base = 2 * D + DH * h
            tail = jnp.where(tail_row < DH - 16, pt[base + 16:base + 24, :],
                             jnp.where(tail_row == DH - 16, 1.0, 0.0))
            blk = jnp.concatenate(
                [pt[base:base + 16, :], tail, jnp.zeros((8, L), F32)], axis=0)
            vt_v[c, h] = _pack(blk)

        rowl = _iota((128, L), 0)
        pqs, pks, vgs = [], [], []
        for g in range(NG):
            used = _heads_in_group(g) * DH
            qg = pt[GW * g:GW * g + 128, :]
            qt_v[c, g] = _pack(qg * QSCALE)
            kg = pt[D + GW * g:D + GW * g + 128, :]
            k_v[c, g] = _pack(kg.T)
            pqs.append(_phi(qg).astype(BF16))
            if c < NSEG - 1:
                pks.append(_phi(kg).astype(BF16))
                lo = 2 * D + GW * g
                if g < NG - 1:
                    vg = pt[lo:lo + 128, :]
                else:
                    vg = jnp.concatenate(
                        [pt[lo:lo + used, :], jnp.zeros((128 - used, L), F32)], axis=0)
                vg = jnp.where(rowl < used, vg, jnp.where(rowl == GW, 1.0, 0.0))
                vgs.append(vg.astype(BF16))
        return pqs, pks, vgs

    def memory_update(states, pks, vgs):
        row = _iota((128, 128), 0)
        lane = _iota((128, 128), 1)
        same_head = (row // DH) == (lane // DH)
        out = []
        for g in range(NG):
            used = _heads_in_group(g) * DH
            upd = _dot_nt(vgs[g], pks[g])
            keep = ((same_head & (row < used)) | (row == GW)) & (lane < used)
            upd = jnp.where(keep, upd, 0.0)
            out.append(upd if states is None else states[g] + upd)
        return out

    def memory_retrieve(c, states, pqs):
        row = _iota((128, 128), 0)
        row8 = _iota((8, 128), 0)
        lane8 = _iota((8, 128), 1) // DH
        for g in range(NG):
            nh = _heads_in_group(g)
            st = states[g]
            mrows = jnp.where(row < GW, st, 0.0)
            zrows = jnp.where(lane8 == row8, st[GW:GW + 1, :], 0.0)
            lhs = jnp.concatenate(
                [mrows, zrows, jnp.zeros((8, 128), F32)], axis=0).astype(BF16)
            ret = _dot(lhs, pqs[g])
            gsel = gate_v[HPG * g:HPG * g + 8, :] if g < NG - 1 else jnp.concatenate(
                [gate_v[HPG * g:H, :], jnp.zeros((8 - nh, 128), F32)], axis=0)
            gwide = jnp.concatenate([gsel] * NQT, axis=1)
            scale = gwide / (ret[128:136, :] + 1e-6)
            pieces = []
            for b in range(16):
                h0 = min((8 * b) // DH, nh - 1)
                h1 = min((8 * b + 7) // DH, nh - 1)
                sc = scale[h0:h0 + 1, :]
                if h1 != h0:
                    first = _iota((8, L), 0) < DH * h1 - 8 * b
                    sc = jnp.where(first, sc, scale[h1:h1 + 1, :])
                pieces.append(ret[8 * b:8 * b + 8, :] * sc)
            mem_v[c, GW * g:GW * g + 128, :] = jnp.concatenate(pieces, axis=0)

    def moe():
        r = r_v[0:NSEG, :]
        idx = _iota((NSEG, L), 0) * L + _iota((NSEG, L), 1)
        m1 = jnp.max(r)
        i1 = jnp.clip(jnp.min(jnp.where(r == m1, idx, S)), 0, S - 1)
        r2 = jnp.where(idx == i1, -jnp.inf, r)
        m2 = jnp.max(r2)
        i2 = jnp.clip(jnp.min(jnp.where(r2 == m2, idx, S)), 0, S - 1)
        idx_s[0] = i1
        idx_s[1] = i2
        row16 = _iota((16, 128), 0)
        lane16 = _iota((16, 128), 1)
        xs = None
        for t, i in enumerate((i1, i2)):
            seg = i // L
            off = i - seg * L
            base = pl.multiple_of((off // 128) * 128, 128)
            cols = _unpack(xn_v[seg, :, pl.ds(base, 128)])
            pick = jnp.where((row16 == t) & (lane16 == off - base), 1.0, 0.0)
            part = _dot_nt(pick.astype(BF16), cols)
            xs = part if xs is None else xs + part
        xs = xs.astype(BF16)
        cp_wg.wait()
        gt = _round_bf16(_dot(xs, wg_v[...]))
        cp_wu.wait()
        up = _round_bf16(_dot(xs, wu_v[...]))
        act = _round_bf16(gt * jax.nn.sigmoid(gt))
        hid = (act * up).astype(BF16)
        cp_wd.wait()
        y = _round_bf16(_dot_nt(hid, wd_v[...]))
        rsel = jnp.where(_iota((16, 1), 0) == 0, m1, m2)
        y = y * _round_bf16(jax.nn.sigmoid(rsel))
        ypad = jnp.concatenate(
            [jnp.concatenate([y, jnp.zeros((16, 64), F32)], axis=1),
             jnp.zeros((112, 640), F32)], axis=0)
        yt = ypad.T
        for t in range(2):
            yb_v[t] = jnp.broadcast_to(yt[0:D, t:t + 1], (D, 128))

    quads = [list(range(4 * q, 4 * q + 4)) for q in range(H // 4)]
    waves = [(quad, j) for quad in quads for j in range(NQT)]

    def attention(shift_by_max):
        rid = _iota((64, 128), 0)

        def scores(w):
            quad, j = waves[w]
            nk = 128 * (j + 1)
            res = []
            for h in quad:
                g, hp = divmod(h, HPG)
                mask = (rid >= (DH // 2) * hp) & (rid < (DH // 2) * (hp + 1))
                qm = _unpack(jnp.where(mask, qt_v[step, g, :, 128 * j:128 * (j + 1)],
                                       jnp.uint32(0)))
                st = _dot(_unpack(k_v[step, g, 0:nk // 2, :]), qm)
                diag = st[nk - 128:, :] + bias_v[...]
                st = diag if j == 0 else jnp.concatenate(
                    [st[:nk - 128, :], diag], axis=0)
                if shift_by_max:
                    st = st - jnp.max(st, axis=0, keepdims=True)
                res.append(jnp.exp2(st).astype(BF16))
            return res

        def values(w, probs):
            quad, j = waves[w]
            nk = 128 * (j + 1)
            for h, p in zip(quad, probs):
                o = _dot(_unpack(vt_v[step, h, :, 0:nk]), p)
                scale = (1.0 - gate_v[h:h + 1, :]) / o[DH:DH + 1, :]
                ot_v[DH * h:DH * h + 24, 128 * j:128 * (j + 1)] = o[0:24, :] * scale

        pending = scores(0)
        for w in range(len(waves)):
            nxt = scores(w + 1) if w + 1 < len(waves) else None
            values(w, pending)
            pending = nxt

    @pl.when(step == 0)
    def _():
        x_copies[0].start()
        cp_wq.start()
        cp_wr.start()
        cp_beta.start()
        cp_wk.start()
        cp_wv.start()
        for c in range(1, NSEG):
            x_copies[c].start()
        cp_wo.start()
        cp_wg.start()
        cp_wu.start()
        cp_wd.start()

        x_copies[0].wait()
        cp_wr.wait()
        cp_beta.wait()
        init_constants()
        layer_norm(0)
        for i, (cp, w_v) in enumerate(((cp_wq, wq_v), (cp_wk, wk_v), (cp_wv, wv_v))):
            cp.wait()
            wall[i * (D // 2):(i + 1) * (D // 2), :] = pltpu.bitcast(w_v[...].T, U32)
        for c in range(1, NSEG):
            x_copies[c].wait()
        cp_wo.wait()

        layer_norm(1)
        pt = project(0)
        wot[...] = pltpu.bitcast(wo_v[...].T, U32)
        mem_v[0] = jnp.zeros(mem_v.shape[1:], F32)
        pqs, pks, vgs = store_qkv(0, pt)
        states = None
        for c in range(1, NSEG):
            if c + 1 < NSEG:
                layer_norm(c + 1)
            pt = project(c)
            states = memory_update(states, pks, vgs)
            pqs, pks, vgs = store_qkv(c, pt)
            memory_retrieve(c, states, pqs)

    safe = safe_s[step] == 1

    @pl.when(safe)
    def _():
        attention(False)

    @pl.when(jnp.logical_not(safe))
    def _():
        attention(True)

    @pl.when(step == 0)
    def _():
        moe()

    heads_out = ot_v[0:D, :] + mem_v[step, 0:D, :]
    attn = _dot(_unpack(wot[...]), heads_out.astype(BF16))
    base = x_v[step].astype(F32) + attn
    xn = _unpack(xn_v[step]).astype(F32)
    col = step * L + _iota((1, L), 1)
    y0 = jnp.concatenate([yb_v[0]] * NQT, axis=1)
    y1 = jnp.concatenate([yb_v[1]] * NQT, axis=1)
    upd = jnp.where(col == idx_s[0], y0, 0.0) + jnp.where(col == idx_s[1], y1, 0.0)
    o_ref[...] = (base + (xn + upd)).astype(BF16)


@jax.jit
def pallas_parallel_sum__memory_aug_infini_attn__moe_arch_mod__prompt_kernel(
    A_x: jax.Array,
    A_wq: jax.Array,
    A_wk: jax.Array,
    A_wv: jax.Array,
    A_wo: jax.Array,
    A_beta: jax.Array,
    B_x: jax.Array,
    B_w_r: jax.Array,
    B_w_gate: jax.Array,
    B_w_up: jax.Array,
    B_w_down: jax.Array,
):
    del B_x
    vm = pltpu.VMEM
    scratch = [
        vm((NSEG, D, L), BF16),
        vm((D, D), BF16),
        vm((D, D), BF16),
        vm((D, D), BF16),
        vm((D, D), BF16),
        vm((1, H), BF16),
        vm((1, D), BF16),
        vm((D, FF), BF16),
        vm((D, FF), BF16),
        vm((D, FF), BF16),
        vm((PROWS // 2, D), U32),
        vm((D // 2, D), U32),
        vm((NSEG, D // 2, L), U32),
        vm((NSEG, NG, 64, L), U32),
        vm((NSEG, NG, L // 2, 128), U32),
        vm((NSEG, H, 16, L), U32),
        vm((NSEG, OROWS, L), F32),
        vm((NG, 128, 128), F32),
        vm((8, L), F32),
        vm((2, D, 128), F32),
        pltpu.SMEM((2,), jnp.int32),
        pltpu.SMEM((NSEG,), jnp.int32),
        vm((H, 128), F32),
        vm((D + 8, L), F32),
        vm((128, 128), F32),
        pltpu.SemaphoreType.DMA((NSEG + 9,)),
    ]
    hbm = pl.BlockSpec(memory_space=pltpu.HBM)
    xt = jnp.transpose(A_x.reshape(S, D))
    out_t = pl.pallas_call(
        _kernel,
        grid=(NSEG,),
        in_specs=[hbm] * 10,
        out_specs=pl.BlockSpec((D, L), lambda s: (0, s)),
        out_shape=jax.ShapeDtypeStruct((D, S), BF16),
        scratch_shapes=scratch,
        compiler_params=pltpu.CompilerParams(
            dimension_semantics=("arbitrary",),
            vmem_limit_bytes=110 * 1024 * 1024,
        ),
        name="infini_moe",
    )(xt, A_wq, A_wk, A_wv, A_wo, A_beta.reshape(1, H),
      B_w_r.reshape(1, D), B_w_gate, B_w_up, jnp.transpose(B_w_down))
    return jnp.transpose(out_t).reshape(1, S, D)
```

```python
import jax
import jax.numpy as jnp
from jax import lax
from jax.experimental import pallas as pl
from jax.experimental.pallas import tpu as pltpu

S = 2048
D = 576
H = 32
DH = 18
NSEG = 4
L = 512
FF = 4608
NG = 5
HPG = 7
GW = HPG * DH
NQT = L // 128
PROWS = 3 * D + 16
RROW = 3 * D
MROWS = 144
OROWS = 640
LOG2E = 1.4426950408889634
QSCALE = DH ** -0.5 * LOG2E
NEG = -1e30
SAFE_LOG2 = 40.0
LN_EPS = 1.0013580322265625e-05
F32 = jnp.float32
BF16 = jnp.bfloat16
U32 = jnp.uint32

_NN = (((1,), (0,)), ((), ()))
_NT = (((1,), (1,)), ((), ()))


def _dot(a, b):
    return lax.dot_general(a, b, _NN, preferred_element_type=F32)


def _dot_nt(a, b):
    return lax.dot_general(a, b, _NT, preferred_element_type=F32)


def _iota(shape, dim):
    return lax.broadcasted_iota(jnp.int32, shape, dim)


def _round_bf16(v):
    return v.astype(BF16).astype(F32)


def _pack(v):
    return pltpu.bitcast(v.astype(BF16), U32)


def _unpack(u):
    return pltpu.bitcast(u, BF16)


def _heads_in_group(g):
    return HPG if g < NG - 1 else H - HPG * (NG - 1)


def _phi(t):
    return jnp.where(t > 0, t + 1.0, jnp.exp(t))


def _kernel(x_hbm, wq_hbm, wk_hbm, wv_hbm, wo_hbm, beta_hbm, wr_hbm,
            wg_hbm, wu_hbm, wd_hbm,
            o_ref,
            x_v, wq_v, wk_v, wv_v, wo_v, beta_v, wr_v, wg_v, wu_v, wd_v,
            wall, wot, xn_v, qt_v, k_v, vt_v, mem_v,
            r_v, yb_v, idx_s, safe_s, gate_v, ot_v, oh_v, bias_v,
            sems):
    step = pl.program_id(0)

    x_copies = [
        pltpu.make_async_copy(x_hbm.at[:, pl.ds(c * L, L)], x_v.at[c], sems.at[c])
        for c in range(NSEG)
    ]
    pairs = [(wq_hbm, wq_v), (wk_hbm, wk_v), (wv_hbm, wv_v), (wo_hbm, wo_v),
             (beta_hbm, beta_v), (wr_hbm, wr_v),
             (wg_hbm, wg_v), (wu_hbm, wu_v), (wd_hbm, wd_v)]
    (cp_wq, cp_wk, cp_wv, cp_wo, cp_beta, cp_wr, cp_wg, cp_wu, cp_wd) = [
        pltpu.make_async_copy(src, dst, sems.at[NSEG + i])
        for i, (src, dst) in enumerate(pairs)
    ]

    def layer_norm(c):
        xf = x_v[c].astype(F32)
        mean = jnp.sum(xf, axis=0, keepdims=True) * (1.0 / D)
        cen = xf - mean
        var = jnp.sum(cen * cen, axis=0, keepdims=True) * (1.0 / D)
        sd = _round_bf16(jnp.sqrt(_round_bf16(_round_bf16(var) + LN_EPS)))
        xn = (xf - _round_bf16(mean)) * (1.0 / sd)
        xn_v[c] = _pack(xn)

    def init_constants():
        gate = jax.nn.sigmoid(beta_v[...].astype(F32).reshape(1, H))
        on_diag = _iota((H, H), 0) == _iota((H, H), 1)
        gcol = jnp.sum(jnp.where(on_diag, gate, 0.0), axis=1, keepdims=True)
        gate_v[...] = jnp.broadcast_to(gcol, (H, 128))
        bias_v[...] = jnp.where(_iota((128, 128), 0) > _iota((128, 128), 1), NEG, 0.0)
        router = jnp.broadcast_to(wr_v[...].astype(F32).reshape(1, D), (16, D))
        wall[RROW // 2:PROWS // 2, :] = _pack(
            jnp.where(_iota((16, D), 0) == 0, router, 0.0))

    def project(c):
        return _dot(_unpack(wall[...]), _unpack(xn_v[c]))

    def store_qkv(c, pt):
        r_v[c:c + 1, :] = _round_bf16(pt[RROW:RROW + 1, :])
        qa = jnp.max(jnp.abs(pt[0:D, :])) * QSCALE
        ka = jnp.max(jnp.abs(pt[D:2 * D, :]))
        safe_s[c] = (qa * ka * (DH * 1.02) <= SAFE_LOG2).astype(jnp.int32)

        tail_row = _iota((8, L), 0)
        for h in range(H):
            base = 2 * D + DH * h
            tail = jnp.where(tail_row < DH - 16, pt[base + 16:base + 24, :],
                             jnp.where(tail_row == DH - 16, 1.0, 0.0))
            blk = jnp.concatenate(
                [pt[base:base + 16, :], tail, jnp.zeros((8, L), F32)], axis=0)
            vt_v[c, h] = _pack(blk)

        rowl = _iota((128, L), 0)
        pqs, pks, vgs = [], [], []
        for g in range(NG):
            used = _heads_in_group(g) * DH
            qg = pt[GW * g:GW * g + 128, :]
            qt_v[c, g] = _pack(qg * QSCALE)
            kg = pt[D + GW * g:D + GW * g + 128, :]
            k_v[c, g] = _pack(kg.T)
            pqs.append(_phi(qg).astype(BF16))
            if c < NSEG - 1:
                pks.append(_phi(kg).astype(BF16))
                lo = 2 * D + GW * g
                if g < NG - 1:
                    vg = pt[lo:lo + 128, :]
                else:
                    vg = jnp.concatenate(
                        [pt[lo:lo + used, :], jnp.zeros((128 - used, L), F32)], axis=0)
                vg = jnp.where(rowl < used, vg, jnp.where(rowl == GW, 1.0, 0.0))
                vgs.append(vg.astype(BF16))
        return pqs, pks, vgs

    def memory_update(states, pks, vgs):
        row = _iota((128, 128), 0)
        lane = _iota((128, 128), 1)
        same_head = (row // DH) == (lane // DH)
        out = []
        for g in range(NG):
            used = _heads_in_group(g) * DH
            upd = _dot_nt(vgs[g], pks[g])
            keep = ((same_head & (row < used)) | (row == GW)) & (lane < used)
            upd = jnp.where(keep, upd, 0.0)
            out.append(upd if states is None else states[g] + upd)
        return out

    def memory_retrieve(c, states, pqs):
        row = _iota((128, 128), 0)
        row8 = _iota((8, 128), 0)
        lane8 = _iota((8, 128), 1) // DH
        for g in range(NG):
            nh = _heads_in_group(g)
            st = states[g]
            mrows = jnp.where(row < GW, st, 0.0)
            zrows = jnp.where(lane8 == row8, st[GW:GW + 1, :], 0.0)
            lhs = jnp.concatenate(
                [mrows, zrows, jnp.zeros((8, 128), F32)], axis=0).astype(BF16)
            ret = _dot(lhs, pqs[g])
            gsel = gate_v[HPG * g:HPG * g + 8, :] if g < NG - 1 else jnp.concatenate(
                [gate_v[HPG * g:H, :], jnp.zeros((8 - nh, 128), F32)], axis=0)
            gwide = jnp.concatenate([gsel] * NQT, axis=1)
            scale = gwide / (ret[128:136, :] + 1e-6)
            pieces = []
            for b in range(16):
                h0 = min((8 * b) // DH, nh - 1)
                h1 = min((8 * b + 7) // DH, nh - 1)
                sc = scale[h0:h0 + 1, :]
                if h1 != h0:
                    first = _iota((8, L), 0) < DH * h1 - 8 * b
                    sc = jnp.where(first, sc, scale[h1:h1 + 1, :])
                pieces.append(ret[8 * b:8 * b + 8, :] * sc)
            mem_v[c, GW * g:GW * g + 128, :] = jnp.concatenate(pieces, axis=0)

    def moe():
        r = r_v[0:NSEG, :]
        idx = _iota((NSEG, L), 0) * L + _iota((NSEG, L), 1)
        m1 = jnp.max(r)
        i1 = jnp.clip(jnp.min(jnp.where(r == m1, idx, S)), 0, S - 1)
        r2 = jnp.where(idx == i1, -jnp.inf, r)
        m2 = jnp.max(r2)
        i2 = jnp.clip(jnp.min(jnp.where(r2 == m2, idx, S)), 0, S - 1)
        idx_s[0] = i1
        idx_s[1] = i2
        row16 = _iota((16, 128), 0)
        lane16 = _iota((16, 128), 1)
        xs = None
        for t, i in enumerate((i1, i2)):
            seg = i // L
            off = i - seg * L
            base = pl.multiple_of((off // 128) * 128, 128)
            cols = _unpack(xn_v[seg, :, pl.ds(base, 128)])
            pick = jnp.where((row16 == t) & (lane16 == off - base), 1.0, 0.0)
            part = _dot_nt(pick.astype(BF16), cols)
            xs = part if xs is None else xs + part
        xs = xs.astype(BF16)
        cp_wg.wait()
        gt = _round_bf16(_dot(xs, wg_v[...]))
        cp_wu.wait()
        up = _round_bf16(_dot(xs, wu_v[...]))
        act = _round_bf16(gt * jax.nn.sigmoid(gt))
        hid = (act * up).astype(BF16)
        cp_wd.wait()
        y = _round_bf16(_dot_nt(hid, wd_v[...]))
        rsel = jnp.where(_iota((16, 1), 0) == 0, m1, m2)
        y = y * _round_bf16(jax.nn.sigmoid(rsel))
        ypad = jnp.concatenate(
            [jnp.concatenate([y, jnp.zeros((16, 64), F32)], axis=1),
             jnp.zeros((112, 640), F32)], axis=0)
        yt = ypad.T
        for t in range(2):
            yb_v[t] = jnp.broadcast_to(yt[0:D, t:t + 1], (D, 128))

    def masked_q(g, hp, j):
        rid = _iota((64, 128), 0)
        mask = (rid >= (DH // 2) * hp) & (rid < (DH // 2) * (hp + 1))
        return _unpack(jnp.where(mask, qt_v[step, g, :, 128 * j:128 * (j + 1)],
                                 jnp.uint32(0)))

    def causal_scores(g, hp, j):
        nk = 128 * (j + 1)
        st = _dot(_unpack(k_v[step, g, 0:nk // 2, :]), masked_q(g, hp, j))
        diag = st[nk - 128:, :] + bias_v[...]
        return diag if j == 0 else jnp.concatenate([st[:nk - 128, :], diag], axis=0)

    def head_output(h, j, p, keep):
        o = _dot(_unpack(vt_v[step, h, :, 0:128 * (j + 1)]), p)
        return o[0:24, :] * (keep / o[DH:DH + 1, :])

    def attention_bounded():
        waves = [(list(range(4 * q, 4 * q + 4)), j)
                 for q in range(H // 4) for j in range(NQT)]

        def scores(w):
            quad, j = waves[w]
            return [jnp.exp2(causal_scores(*divmod(h, HPG), j)).astype(BF16)
                    for h in quad]

        def values(w, probs):
            quad, j = waves[w]
            for h, p in zip(quad, probs):
                ot_v[step, DH * h:DH * h + 24, 128 * j:128 * (j + 1)] = head_output(
                    h, j, p, 1.0 - gate_v[h:h + 1, :])

        pending = scores(0)
        for w in range(len(waves)):
            nxt = scores(w + 1) if w + 1 < len(waves) else None
            values(w, pending)
            pending = nxt

    def attention_max_shifted():
        def one_head(h, carry):
            g = h // HPG
            hp = h - g * HPG
            keep = 1.0 - gate_v[pl.ds(h, 1), :]
            for j in range(NQT):
                st = causal_scores(g, hp, j)
                p = jnp.exp2(st - jnp.max(st, axis=0, keepdims=True)).astype(BF16)
                oh_v[h, :, 128 * j:128 * (j + 1)] = head_output(h, j, p, keep)
            return carry

        lax.fori_loop(0, H, one_head, 0)
        for h in range(H):
            ot_v[step, DH * h:DH * h + 24, :] = oh_v[h]

    @pl.when(step == 0)
    def _():
        for cp in (x_copies[0], cp_wq, cp_wr, cp_beta, cp_wk, cp_wv, x_copies[1],
                   x_copies[2], x_copies[3], cp_wo, cp_wg, cp_wu, cp_wd):
            cp.start()

        half = D // 2
        x_copies[0].wait()
        layer_norm(0)
        cp_wq.wait()
        cp_wr.wait()
        cp_beta.wait()
        init_constants()
        wall[0:half, :] = pltpu.bitcast(wq_v[...].T, U32)
        cp_wk.wait()
        xn0 = _unpack(xn_v[0])
        ptq = _dot(_unpack(wall[0:half, :]), xn0)
        wall[half:2 * half, :] = pltpu.bitcast(wk_v[...].T, U32)
        cp_wv.wait()
        x_copies[1].wait()
        xn0 = _unpack(xn_v[0])
        ptk = _dot(_unpack(wall[half:2 * half, :]), xn0)
        wall[2 * half:3 * half, :] = pltpu.bitcast(wv_v[...].T, U32)
        layer_norm(1)
        ptv = _dot(_unpack(wall[2 * half:PROWS // 2, :]), xn0)
        pt = jnp.concatenate([ptq, ptk, ptv], axis=0)
        mem_v[0] = jnp.zeros(mem_v.shape[1:], F32)
        pq0, pk, vg = store_qkv(0, pt)
        x_copies[2].wait()
        x_copies[3].wait()
        cp_wo.wait()

        layer_norm(2)
        pt = project(1)
        wot[...] = pltpu.bitcast(wo_v[...].T, U32)
        state1 = memory_update(None, pk, vg)
        pq1, pk, vg = store_qkv(1, pt)
        layer_norm(3)
        pt = project(2)
        state2 = memory_update(state1, pk, vg)
        memory_retrieve(1, state1, pq1)
        pq2, pk, vg = store_qkv(2, pt)
        pt = project(3)
        state3 = memory_update(state2, pk, vg)
        memory_retrieve(2, state2, pq2)
        pq3, _, _ = store_qkv(3, pt)
        memory_retrieve(3, state3, pq3)

    @pl.when(step < NSEG)
    def _():
        safe = safe_s[step] == 1

        @pl.when(safe)
        def _():
            attention_bounded()

        @pl.when(jnp.logical_not(safe))
        def _():
            attention_max_shifted()

    @pl.when(step == NSEG)
    def _():
        moe()

    @pl.when(step >= NSEG)
    def _():
        seg = step - NSEG
        heads_out = ot_v[seg, 0:D, :] + mem_v[seg, 0:D, :]
        attn = _dot(_unpack(wot[...]), heads_out.astype(BF16))
        base = x_v[seg].astype(F32) + attn
        xn = _unpack(xn_v[seg]).astype(F32)
        col = seg * L + _iota((1, L), 1)
        y0 = jnp.concatenate([yb_v[0]] * NQT, axis=1)
        y1 = jnp.concatenate([yb_v[1]] * NQT, axis=1)
        upd = jnp.where(col == idx_s[0], y0, 0.0) + jnp.where(col == idx_s[1], y1, 0.0)
        o_ref[...] = (base + (xn + upd)).astype(BF16)


@jax.jit
def pallas_parallel_sum__memory_aug_infini_attn__moe_arch_mod__prompt_kernel(
    A_x: jax.Array,
    A_wq: jax.Array,
    A_wk: jax.Array,
    A_wv: jax.Array,
    A_wo: jax.Array,
    A_beta: jax.Array,
    B_x: jax.Array,
    B_w_r: jax.Array,
    B_w_gate: jax.Array,
    B_w_up: jax.Array,
    B_w_down: jax.Array,
):
    del B_x
    vm = pltpu.VMEM
    scratch = [
        vm((NSEG, D, L), BF16),
        vm((D, D), BF16),
        vm((D, D), BF16),
        vm((D, D), BF16),
        vm((D, D), BF16),
        vm((H,), BF16),
        vm((D,), BF16),
        vm((D, FF), BF16),
        vm((D, FF), BF16),
        vm((D, FF), BF16),
        vm((PROWS // 2, D), U32),
        vm((D // 2, D), U32),
        vm((NSEG, D // 2, L), U32),
        vm((NSEG, NG, 64, L), U32),
        vm((NSEG, NG, L // 2, 128), U32),
        vm((NSEG, H, 16, L), U32),
        vm((NSEG, OROWS, L), F32),
        vm((8, L), F32),
        vm((2, D, 128), F32),
        pltpu.SMEM((2,), jnp.int32),
        pltpu.SMEM((NSEG,), jnp.int32),
        vm((H, 128), F32),
        vm((NSEG, D + 8, L), F32),
        vm((H, 24, L), F32),
        vm((128, 128), F32),
        pltpu.SemaphoreType.DMA((NSEG + 9,)),
    ]
    hbm = pl.BlockSpec(memory_space=pltpu.HBM)
    xt = jnp.transpose(A_x.reshape(S, D))
    out_t = pl.pallas_call(
        _kernel,
        grid=(2 * NSEG,),
        in_specs=[hbm] * 10,
        out_specs=pl.BlockSpec((D, L), lambda s: (0, jnp.maximum(s - NSEG, 0))),
        out_shape=jax.ShapeDtypeStruct((D, S), BF16),
        scratch_shapes=scratch,
        compiler_params=pltpu.CompilerParams(
            dimension_semantics=("arbitrary",),
            vmem_limit_bytes=110 * 1024 * 1024,
        ),
        name="infini_moe",
    )(xt, A_wq, A_wk, A_wv, A_wo, A_beta, B_w_r, B_w_gate, B_w_up,
      jnp.transpose(B_w_down))
    return jnp.transpose(out_t).reshape(1, S, D)
```

```python
import contextlib

import jax
import jax.numpy as jnp
from jax import lax
from jax.experimental import pallas as pl
from jax.experimental.pallas import tpu as pltpu

S = 2048
D = 576
H = 32
DH = 18
NSEG = 4
L = 512
FF = 4608
NG = 5
HPG = 7
GW = HPG * DH
NQT = L // 128
PROWS = 3 * D + 16
RROW = 3 * D
MROWS = 144
FT = FF // 128 // NSEG
OROWS = 640
LOG2E = 1.4426950408889634
QSCALE = DH ** -0.5 * LOG2E
NEG = -1e30
SAFE_LOG2 = 40.0
LN_EPS = 1.0013580322265625e-05
F32 = jnp.float32
BF16 = jnp.bfloat16
U32 = jnp.uint32

PROFILE_SCOPES = False

_NN = (((1,), (0,)), ((), ()))
_NT = (((1,), (1,)), ((), ()))


def _scope(name):
    return jax.named_scope(name) if PROFILE_SCOPES else contextlib.nullcontext()


def _dot(a, b):
    return lax.dot_general(a, b, _NN, preferred_element_type=F32)


def _dot_nt(a, b):
    return lax.dot_general(a, b, _NT, preferred_element_type=F32)


def _iota(shape, dim):
    return lax.broadcasted_iota(jnp.int32, shape, dim)


def _round_bf16(v):
    return v.astype(BF16).astype(F32)


def _pack(v):
    return pltpu.bitcast(v.astype(BF16), U32)


def _unpack(u):
    return pltpu.bitcast(u, BF16)


def _heads_in_group(g):
    return HPG if g < NG - 1 else H - HPG * (NG - 1)


def _phi(t):
    return jnp.where(t > 0, t + 1.0, jnp.exp(t))


def _kernel(x_hbm, wq_hbm, wk_hbm, wv_hbm, wo_hbm, beta_hbm, wr_hbm,
            wg_hbm, wu_hbm, wd_hbm,
            o_ref,
            x_v, wq_v, wk_v, wv_v, wo_v, beta_v, wr_v, wg_v, wu_v, wd_v,
            wall, wot, xn_v, qt_v, k_v, vt_v, mem_v,
            r_v, xb_v, y_v, hid_v, idx_s, rsel_s, zero_s, safe_s,
            gate_v, ot_v, oh_v, bias_v,
            sems):
    step = pl.program_id(0)

    x_copies = [
        pltpu.make_async_copy(x_hbm.at[:, pl.ds(c * L, L)], x_v.at[c], sems.at[c])
        for c in range(NSEG)
    ]
    pairs = [(wq_hbm, wq_v), (wk_hbm, wk_v), (wv_hbm, wv_v), (wo_hbm, wo_v),
             (beta_hbm, beta_v), (wr_hbm, wr_v),
             (wg_hbm, wg_v), (wu_hbm, wu_v), (wd_hbm, wd_v)]
    (cp_wq, cp_wk, cp_wv, cp_wo, cp_beta, cp_wr, cp_wg, cp_wu, cp_wd) = [
        pltpu.make_async_copy(src, dst, sems.at[NSEG + i])
        for i, (src, dst) in enumerate(pairs)
    ]

    def layer_norm(c):
        xf = x_v[c].astype(F32)
        mean = jnp.sum(xf, axis=0, keepdims=True) * (1.0 / D)
        cen = xf - mean
        var = jnp.sum(cen * cen, axis=0, keepdims=True) * (1.0 / D)
        sd = _round_bf16(jnp.sqrt(_round_bf16(_round_bf16(var) + LN_EPS)))
        xn = (xf - _round_bf16(mean)) * (1.0 / sd)
        xn_v[c] = _pack(xn)

    def init_constants():
        gate = jax.nn.sigmoid(beta_v[...].astype(F32).reshape(1, H))
        on_diag = _iota((H, H), 0) == _iota((H, H), 1)
        gcol = jnp.sum(jnp.where(on_diag, gate, 0.0), axis=1, keepdims=True)
        gate_v[...] = jnp.broadcast_to(gcol, (H, 128))
        zero_s[0] = jnp.uint32(0)
        bias_v[...] = jnp.where(_iota((128, 128), 0) > _iota((128, 128), 1), NEG, 0.0)
        router = jnp.broadcast_to(wr_v[...].astype(F32).reshape(1, D), (16, D))
        wall[RROW // 2:PROWS // 2, :] = _pack(
            jnp.where(_iota((16, D), 0) == 0, router, 0.0))

    def project(c):
        return _dot(_unpack(wall[...]), _unpack(xn_v[c]))

    def store_qkv(c, pt):
        r_v[c:c + 1, :] = _round_bf16(pt[RROW:RROW + 1, :])
        qa = jnp.max(jnp.abs(pt[0:D, :])) * QSCALE
        ka = jnp.max(jnp.abs(pt[D:2 * D, :]))
        safe_s[c] = (qa * ka * (DH * 1.02) <= SAFE_LOG2).astype(jnp.int32)

        tail_row = _iota((8, L), 0)
        for h in range(H):
            base = 2 * D + DH * h
            tail = jnp.where(tail_row < DH - 16, pt[base + 16:base + 24, :],
                             jnp.where(tail_row == DH - 16, 1.0, 0.0))
            blk = jnp.concatenate(
                [pt[base:base + 16, :], tail, jnp.zeros((8, L), F32)], axis=0)
            vt_v[c, h] = _pack(blk)

        rowl = _iota((128, L), 0)
        pqs, pks, vgs = [], [], []
        for g in range(NG):
            used = _heads_in_group(g) * DH
            qg = pt[GW * g:GW * g + 128, :]
            qt_v[c, g] = _pack(qg * QSCALE)
            kg = pt[D + GW * g:D + GW * g + 128, :]
            k_v[c, g] = _pack(kg.T)
            pqs.append(_phi(qg).astype(BF16))
            if c < NSEG - 1:
                pks.append(_phi(kg).astype(BF16))
                lo = 2 * D + GW * g
                if g < NG - 1:
                    vg = pt[lo:lo + 128, :]
                else:
                    vg = jnp.concatenate(
                        [pt[lo:lo + used, :], jnp.zeros((128 - used, L), F32)], axis=0)
                vg = jnp.where(rowl < used, vg, jnp.where(rowl == GW, 1.0, 0.0))
                vgs.append(vg.astype(BF16))
        return pqs, pks, vgs

    def memory_update(states, pks, vgs):
        row = _iota((128, 128), 0)
        lane = _iota((128, 128), 1)
        same_head = (row // DH) == (lane // DH)
        out = []
        for g in range(NG):
            used = _heads_in_group(g) * DH
            upd = _dot_nt(vgs[g], pks[g])
            keep = ((same_head & (row < used)) | (row == GW)) & (lane < used)
            upd = jnp.where(keep, upd, 0.0)
            out.append(upd if states is None else states[g] + upd)
        return out

    def memory_retrieve(c, states, pqs):
        row = _iota((128, 128), 0)
        row8 = _iota((8, 128), 0)
        lane8 = _iota((8, 128), 1) // DH
        for g in range(NG):
            nh = _heads_in_group(g)
            st = states[g]
            mrows = jnp.where(row < GW, st, 0.0)
            zrows = jnp.where(lane8 == row8, st[GW:GW + 1, :], 0.0)
            lhs = jnp.concatenate(
                [mrows, zrows, jnp.zeros((8, 128), F32)], axis=0).astype(BF16)
            ret = _dot(lhs, pqs[g])
            gsel = gate_v[HPG * g:HPG * g + 8, :] if g < NG - 1 else jnp.concatenate(
                [gate_v[HPG * g:H, :], jnp.zeros((8 - nh, 128), F32)], axis=0)
            gwide = jnp.concatenate([gsel] * NQT, axis=1)
            scale = gwide / (ret[128:136, :] + 1e-6)
            pieces = []
            for b in range(16):
                h0 = min((8 * b) // DH, nh - 1)
                h1 = min((8 * b + 7) // DH, nh - 1)
                sc = scale[h0:h0 + 1, :]
                if h1 != h0:
                    first = _iota((8, L), 0) < DH * h1 - 8 * b
                    sc = jnp.where(first, sc, scale[h1:h1 + 1, :])
                pieces.append(ret[8 * b:8 * b + 8, :] * sc)
            mem_v[c, GW * g:GW * g + 128, :] = jnp.concatenate(pieces, axis=0)

    def route():
        r = r_v[0:NSEG, :]
        idx = _iota((NSEG, L), 0) * L + _iota((NSEG, L), 1)
        m1 = jnp.max(r)
        i1 = jnp.clip(jnp.min(jnp.where(r == m1, idx, S)), 0, S - 1)
        r2 = jnp.where(idx == i1, -jnp.inf, r)
        m2 = jnp.max(r2)
        i2 = jnp.clip(jnp.min(jnp.where(r2 == m2, idx, S)), 0, S - 1)
        idx_s[0] = i1
        idx_s[1] = i2
        rsel_s[0] = m1
        rsel_s[1] = m2
        krow = _iota((128, 128), 0)
        for t, i in enumerate((i1, i2)):
            seg = i // L
            off = i - seg * L
            base = pl.multiple_of((off // 128) * 128, 128)
            cols = _unpack(xn_v[seg, :, pl.ds(base, 128)])
            pick = jnp.where(krow == off - base, 1.0, 0.0).astype(BF16)
            xb_v[t] = _dot(cols, pick)
        y_v[...] = jnp.zeros(y_v.shape, F32)

    def swiglu(gate_sum, up_sum):
        gt = _round_bf16(jnp.sum(gate_sum, axis=0, keepdims=True))
        up = _round_bf16(jnp.sum(up_sum, axis=0, keepdims=True))
        return _round_bf16(_round_bf16(gt * jax.nn.sigmoid(gt)) * up)

    def ffn_chunk_chained():
        zmask = zero_s[0]

        def nothing(v):
            return pltpu.bitcast(pltpu.bitcast(v, U32) & zmask, F32)

        base = pl.multiple_of(step * (FT * 128), 128)
        link = [None, None]
        hid = {}
        for tile in range(FT):
            cols = pl.ds(base + 128 * tile, 128)
            sums = {}
            for name, w_ref in (("gate", wg_v), ("up", wu_v)):
                acc = [None, None]
                for i in range(D // 16):
                    w = w_ref[16 * i:16 * i + 16, cols].astype(F32)
                    for t in range(2):
                        pr = xb_v[t, 16 * i:16 * i + 16, :] * w
                        if i > 0:
                            lo = acc[t] + pr[0:8, :]
                        elif link[t] is None:
                            lo = pr[0:8, :]
                        else:
                            lo = pr[0:8, :] + nothing(link[t])
                        acc[t] = lo + pr[8:16, :]
                for t in range(2):
                    link[t] = acc[t]
                    sums[name, t] = acc[t]
            for t in range(2):
                hid[t, tile] = swiglu(sums["gate", t], sums["up", t])
        for b in range(D // 16):
            acc = [None, None]
            for tile in range(FT):
                w = wd_v[16 * b:16 * b + 16, pl.ds(base + 128 * tile, 128)].astype(F32)
                for t in range(2):
                    pr = w * hid[t, tile]
                    if tile == 0:
                        lo = pr[0:8, :] + nothing(link[t])
                        acc[t] = [lo, pr[8:16, :] + nothing(lo)]
                    else:
                        acc[t] = [acc[t][0] + pr[0:8, :], acc[t][1] + pr[8:16, :]]
            for t in range(2):
                rows = slice(16 * b, 16 * b + 16)
                y_v[t, rows, :] = y_v[t, rows, :] + jnp.concatenate(acc[t], axis=0)
                link[t] = acc[t][1]

    def ffn_chunk_looped():
        base = step * (FT * 128)

        def gate_up(tile, carry):
            cols = pl.ds(pl.multiple_of(base + 128 * tile, 128), 128)
            wg = wg_v[:, cols].astype(F32)
            wu = wu_v[:, cols].astype(F32)
            for t in range(2):
                h = swiglu(xb_v[t] * wg, xb_v[t] * wu)
                hid_v[t, tile] = jnp.broadcast_to(h, (8, 128))
            return carry

        def down(tile, carry):
            cols = pl.ds(pl.multiple_of(base + 128 * tile, 128), 128)
            w = wd_v[:, cols].astype(F32)
            for t in range(2):
                y_v[t] = y_v[t] + w * hid_v[t, tile][0:1, :]
            return carry

        lax.fori_loop(0, FT, gate_up, 0)
        lax.fori_loop(0, FT, down, 0)

    def masked_q(g, hp, j):
        rid = _iota((64, 128), 0)
        mask = (rid >= (DH // 2) * hp) & (rid < (DH // 2) * (hp + 1))
        return _unpack(jnp.where(mask, qt_v[step, g, :, 128 * j:128 * (j + 1)],
                                 jnp.uint32(0)))

    def causal_scores(g, hp, j):
        nk = 128 * (j + 1)
        st = _dot(_unpack(k_v[step, g, 0:nk // 2, :]), masked_q(g, hp, j))
        diag = st[nk - 128:, :] + bias_v[...]
        return diag if j == 0 else jnp.concatenate([st[:nk - 128, :], diag], axis=0)

    def head_output(h, j, p, keep):
        o = _dot(_unpack(vt_v[step, h, :, 0:128 * (j + 1)]), p)
        den = o[DH:DH + 1, :]
        inv = pl.reciprocal(den, approx=True)
        inv = inv * (2.0 - den * inv)
        return o[0:24, :] * (keep * inv)

    def attention_bounded():
        waves = [(list(range(4 * q, 4 * q + 4)), j)
                 for q in range(H // 4) for j in range(NQT)]

        def scores(w):
            quad, j = waves[w]
            return [jnp.exp2(causal_scores(*divmod(h, HPG), j)).astype(BF16)
                    for h in quad]

        def values(w, probs):
            quad, j = waves[w]
            for h, p in zip(quad, probs):
                ot_v[step, DH * h:DH * h + 24, 128 * j:128 * (j + 1)] = head_output(
                    h, j, p, 1.0 - gate_v[h:h + 1, :])

        pending = scores(0)
        for w in range(len(waves)):
            nxt = scores(w + 1) if w + 1 < len(waves) else None
            values(w, pending)
            pending = nxt
        ffn_chunk_chained()

    def attention_max_shifted():
        def one_head(h, carry):
            g = h // HPG
            hp = h - g * HPG
            keep = 1.0 - gate_v[pl.ds(h, 1), :]
            for j in range(NQT):
                st = causal_scores(g, hp, j)
                p = jnp.exp2(st - jnp.max(st, axis=0, keepdims=True)).astype(BF16)
                oh_v[h, :, 128 * j:128 * (j + 1)] = head_output(h, j, p, keep)
            return carry

        lax.fori_loop(0, H, one_head, 0)
        for h in range(H):
            ot_v[step, DH * h:DH * h + 24, :] = oh_v[h]
        ffn_chunk_looped()

    def output_projection(seg):
        heads_out = ot_v[seg, 0:D, :] + mem_v[seg, 0:D, :]
        attn = _dot(_unpack(wot[...]), heads_out.astype(BF16))
        base = x_v[seg].astype(F32) + attn
        xn = _unpack(xn_v[seg]).astype(F32)
        col = seg * L + _iota((1, L), 1)
        upd = None
        for t in range(2):
            y = _round_bf16(jnp.sum(y_v[t], axis=1, keepdims=True))
            rsel = jnp.full((1, 1), rsel_s[t], F32)
            y = _round_bf16(y * _round_bf16(jax.nn.sigmoid(rsel)))
            part = jnp.where(col == idx_s[t], y, 0.0)
            upd = part if upd is None else upd + part
        o_ref[...] = (base + (xn + upd)).astype(BF16)

    def projections():
        half = D // 2
        xn0 = _unpack(xn_v[0])
        ptq = _dot(_unpack(wall[0:half, :]), xn0)
        wall[half:2 * half, :] = pltpu.bitcast(wk_v[...].T, U32)
        cp_wv.wait()
        x_copies[1].wait()
        xn0 = _unpack(xn_v[0])
        ptk = _dot(_unpack(wall[half:2 * half, :]), xn0)
        wall[2 * half:3 * half, :] = pltpu.bitcast(wv_v[...].T, U32)
        layer_norm(1)
        ptv = _dot(_unpack(wall[2 * half:PROWS // 2, :]), xn0)
        pt = jnp.concatenate([ptq, ptk, ptv], axis=0)
        mem_v[0] = jnp.zeros(mem_v.shape[1:], F32)
        pq0, pk, vg = store_qkv(0, pt)
        x_copies[2].wait()
        x_copies[3].wait()
        cp_wo.wait()

        layer_norm(2)
        pt = project(1)
        wot[...] = pltpu.bitcast(wo_v[...].T, U32)
        state1 = memory_update(None, pk, vg)
        pq1, pk, vg = store_qkv(1, pt)
        layer_norm(3)
        pt = project(2)
        state2 = memory_update(state1, pk, vg)
        memory_retrieve(1, state1, pq1)
        pq2, pk, vg = store_qkv(2, pt)
        pt = project(3)
        state3 = memory_update(state2, pk, vg)
        memory_retrieve(2, state2, pq2)
        pq3, _, _ = store_qkv(3, pt)
        memory_retrieve(3, state3, pq3)
        route()
        cp_wg.wait()
        cp_wu.wait()
        cp_wd.wait()

    @pl.when(step == 0)
    def _():
        for cp in (x_copies[0], cp_wq, cp_wr, cp_beta, cp_wk, cp_wv, x_copies[1],
                   x_copies[2], x_copies[3], cp_wo, cp_wg, cp_wu, cp_wd):
            cp.start()
        with _scope("sc_startup"):
            x_copies[0].wait()
            layer_norm(0)
            cp_wq.wait()
            cp_wr.wait()
            cp_beta.wait()
            init_constants()
            wall[0:D // 2, :] = pltpu.bitcast(wq_v[...].T, U32)
            cp_wk.wait()
        with _scope("sc_projections"):
            projections()

    @pl.when(step < NSEG)
    def _():
        safe = safe_s[step] == 1

        @pl.when(safe)
        def _():
            with _scope("sc_attention"):
                attention_bounded()

        @pl.when(jnp.logical_not(safe))
        def _():
            attention_max_shifted()

    @pl.when(step >= NSEG)
    def _():
        with _scope("sc_outproj"):
            output_projection(step - NSEG)


@jax.jit
def pallas_parallel_sum__memory_aug_infini_attn__moe_arch_mod__prompt_kernel(
    A_x: jax.Array,
    A_wq: jax.Array,
    A_wk: jax.Array,
    A_wv: jax.Array,
    A_wo: jax.Array,
    A_beta: jax.Array,
    B_x: jax.Array,
    B_w_r: jax.Array,
    B_w_gate: jax.Array,
    B_w_up: jax.Array,
    B_w_down: jax.Array,
):
    del B_x
    vm = pltpu.VMEM
    scratch = [
        vm((NSEG, D, L), BF16),
        vm((D, D), BF16),
        vm((D, D), BF16),
        vm((D, D), BF16),
        vm((D, D), BF16),
        vm((H,), BF16),
        vm((D,), BF16),
        vm((D, FF), BF16),
        vm((D, FF), BF16),
        vm((D, FF), BF16),
        vm((PROWS // 2, D), U32),
        vm((D // 2, D), U32),
        vm((NSEG, D // 2, L), U32),
        vm((NSEG, NG, 64, L), U32),
        vm((NSEG, NG, L // 2, 128), U32),
        vm((NSEG, H, 16, L), U32),
        vm((NSEG, OROWS, L), F32),
        vm((8, L), F32),
        vm((2, D, 128), F32),
        vm((2, D, 128), F32),
        vm((2, FT, 8, 128), F32),
        pltpu.SMEM((2,), jnp.int32),
        pltpu.SMEM((2,), F32),
        pltpu.SMEM((1,), U32),
        pltpu.SMEM((NSEG,), jnp.int32),
        vm((H, 128), F32),
        vm((NSEG, D + 8, L), F32),
        vm((H, 24, L), F32),
        vm((128, 128), F32),
        pltpu.SemaphoreType.DMA((NSEG + 9,)),
    ]
    hbm = pl.BlockSpec(memory_space=pltpu.HBM)
    xt = jnp.transpose(A_x.reshape(S, D))
    out_t = pl.pallas_call(
        _kernel,
        grid=(2 * NSEG,),
        in_specs=[hbm] * 10,
        out_specs=pl.BlockSpec((D, L), lambda s: (0, jnp.maximum(s - NSEG, 0))),
        out_shape=jax.ShapeDtypeStruct((D, S), BF16),
        scratch_shapes=scratch,
        compiler_params=pltpu.CompilerParams(
            dimension_semantics=("arbitrary",),
            vmem_limit_bytes=110 * 1024 * 1024,
        ),
        name="infini_moe",
    )(xt, A_wq, A_wk, A_wv, A_wo, A_beta, B_w_r, B_w_gate, B_w_up,
      jnp.transpose(B_w_down))
    return jnp.transpose(out_t).reshape(1, S, D)
```

```python
import contextlib

import jax
import jax.numpy as jnp
from jax import lax
from jax.experimental import pallas as pl
from jax.experimental.pallas import tpu as pltpu

S = 2048
D = 576
H = 32
DH = 18
NSEG = 4
L = 512
FF = 4608
NG = 5
HPG = 7
GW = HPG * DH
NQT = L // 128
PROWS = 3 * D + 16
RROW = 3 * D
MROWS = 144
FT = FF // 128 // NSEG
OROWS = 640
LOG2E = 1.4426950408889634
QSCALE = DH ** -0.5 * LOG2E
NEG = -1e30
SAFE_LOG2 = 40.0
LN_EPS = 1.0013580322265625e-05
F32 = jnp.float32
BF16 = jnp.bfloat16
U32 = jnp.uint32

PROFILE_SCOPES = False

_NN = (((1,), (0,)), ((), ()))
_NT = (((1,), (1,)), ((), ()))


def _scope(name):
    return jax.named_scope(name) if PROFILE_SCOPES else contextlib.nullcontext()


def _dot(a, b):
    return lax.dot_general(a, b, _NN, preferred_element_type=F32)


def _dot_nt(a, b):
    return lax.dot_general(a, b, _NT, preferred_element_type=F32)


def _iota(shape, dim):
    return lax.broadcasted_iota(jnp.int32, shape, dim)


def _round_bf16(v):
    return v.astype(BF16).astype(F32)


def _pack(v):
    return pltpu.bitcast(v.astype(BF16), U32)


def _unpack(u):
    return pltpu.bitcast(u, BF16)


def _rows(index, size):
    if isinstance(index, int):
        return slice(index * size, (index + 1) * size)
    return pl.ds(pl.multiple_of(index * size, 8), size)


def _heads_in_group(g):
    return HPG if g < NG - 1 else H - HPG * (NG - 1)


def _phi(t):
    return jnp.where(t > 0, t + 1.0, jnp.exp(t))


def _kernel(x_hbm, wq_hbm, wk_hbm, wv_hbm, wo_hbm, beta_hbm, wr_hbm,
            wg_hbm, wu_hbm, wd_hbm,
            o_ref,
            x_v, wq_v, wk_v, wv_v, wo_v, beta_v, wr_v, wg_v, wu_v, wd_v,
            wall, wot, xn_v, qt_v, k_v, vt_v, mem_v,
            r_v, xb_v, y_v, hid_v, idx_s, rsel_s, zero_s, safe_s,
            gate_v, ot_v, oh_v, bias_v,
            sems):
    step = pl.program_id(0)

    x_copies = [
        pltpu.make_async_copy(x_hbm.at[:, pl.ds(c * L, L)], x_v.at[c], sems.at[c])
        for c in range(NSEG)
    ]
    pairs = [(wq_hbm, wq_v), (wk_hbm, wk_v), (wv_hbm, wv_v), (wo_hbm, wo_v),
             (beta_hbm, beta_v), (wr_hbm, wr_v),
             (wg_hbm, wg_v), (wu_hbm, wu_v), (wd_hbm, wd_v)]
    (cp_wq, cp_wk, cp_wv, cp_wo, cp_beta, cp_wr, cp_wg, cp_wu, cp_wd) = [
        pltpu.make_async_copy(src, dst, sems.at[NSEG + i])
        for i, (src, dst) in enumerate(pairs)
    ]

    def layer_norm(c):
        xf = x_v[c].astype(F32)
        mean = jnp.sum(xf, axis=0, keepdims=True) * (1.0 / D)
        cen = xf - mean
        var = jnp.sum(cen * cen, axis=0, keepdims=True) * (1.0 / D)
        sd = _round_bf16(jnp.sqrt(_round_bf16(_round_bf16(var) + LN_EPS)))
        xn = (xf - _round_bf16(mean)) * (1.0 / sd)
        xn_v[_rows(c, D // 2), :] = _pack(xn)

    def init_constants():
        gate = jax.nn.sigmoid(beta_v[...].astype(F32).reshape(1, H))
        on_diag = _iota((H, H), 0) == _iota((H, H), 1)
        gcol = jnp.sum(jnp.where(on_diag, gate, 0.0), axis=1, keepdims=True)
        gate_v[...] = jnp.broadcast_to(gcol, (H, 128))
        zero_s[0] = jnp.uint32(0)
        bias_v[...] = jnp.where(_iota((128, 128), 0) > _iota((128, 128), 1), NEG, 0.0)
        router = jnp.broadcast_to(wr_v[...].astype(F32).reshape(1, D), (16, D))
        wall[RROW // 2:PROWS // 2, :] = _pack(
            jnp.where(_iota((16, D), 0) == 0, router, 0.0))

    def project(c):
        return _dot(_unpack(wall[...]), _unpack(xn_v[_rows(c, D // 2), :]))

    def store_qkv(c, pt):
        r_v[c:c + 1, :] = _round_bf16(pt[RROW:RROW + 1, :])
        qa = jnp.max(jnp.abs(pt[0:D, :])) * QSCALE
        ka = jnp.max(jnp.abs(pt[D:2 * D, :]))
        safe_s[c] = (qa * ka * (DH * 1.02) <= SAFE_LOG2).astype(jnp.int32)

        tail_row = _iota((8, L), 0)
        for h in range(H):
            base = 2 * D + DH * h
            tail = jnp.where(tail_row < DH - 16, pt[base + 16:base + 24, :],
                             jnp.where(tail_row == DH - 16, 1.0, 0.0))
            blk = jnp.concatenate(
                [pt[base:base + 16, :], tail, jnp.zeros((8, L), F32)], axis=0)
            vt_v[_rows(c * H + h, 16), :] = _pack(blk)

        rowl = _iota((128, L), 0)
        pqs, pks, vgs = [], [], []
        for g in range(NG):
            used = _heads_in_group(g) * DH
            qg = pt[GW * g:GW * g + 128, :]
            qt_v[_rows(c * NG + g, 64), :] = _pack(qg * QSCALE)
            kg = pt[D + GW * g:D + GW * g + 128, :]
            k_v[_rows(c * NG + g, L // 2), :] = _pack(kg.T)
            pqs.append(_phi(qg).astype(BF16))
            if c < NSEG - 1:
                pks.append(_phi(kg).astype(BF16))
                lo = 2 * D + GW * g
                if g < NG - 1:
                    vg = pt[lo:lo + 128, :]
                else:
                    vg = jnp.concatenate(
                        [pt[lo:lo + used, :], jnp.zeros((128 - used, L), F32)], axis=0)
                vg = jnp.where(rowl < used, vg, jnp.where(rowl == GW, 1.0, 0.0))
                vgs.append(vg.astype(BF16))
        return pqs, pks, vgs

    def memory_update(states, pks, vgs):
        row = _iota((128, 128), 0)
        lane = _iota((128, 128), 1)
        same_head = (row // DH) == (lane // DH)
        out = []
        for g in range(NG):
            used = _heads_in_group(g) * DH
            upd = _dot_nt(vgs[g], pks[g])
            keep = ((same_head & (row < used)) | (row == GW)) & (lane < used)
            upd = jnp.where(keep, upd, 0.0)
            out.append(upd if states is None else states[g] + upd)
        return out

    def memory_retrieve(c, states, pqs):
        row = _iota((128, 128), 0)
        row8 = _iota((8, 128), 0)
        lane8 = _iota((8, 128), 1) // DH
        for g in range(NG):
            nh = _heads_in_group(g)
            st = states[g]
            mrows = jnp.where(row < GW, st, 0.0)
            zrows = jnp.where(lane8 == row8, st[GW:GW + 1, :], 0.0)
            lhs = jnp.concatenate(
                [mrows, zrows, jnp.zeros((8, 128), F32)], axis=0).astype(BF16)
            ret = _dot(lhs, pqs[g])
            gsel = gate_v[HPG * g:HPG * g + 8, :] if g < NG - 1 else jnp.concatenate(
                [gate_v[HPG * g:H, :], jnp.zeros((8 - nh, 128), F32)], axis=0)
            gwide = jnp.concatenate([gsel] * NQT, axis=1)
            scale = gwide / (ret[128:136, :] + 1e-6)
            pieces = []
            for b in range(16):
                h0 = min((8 * b) // DH, nh - 1)
                h1 = min((8 * b + 7) // DH, nh - 1)
                sc = scale[h0:h0 + 1, :]
                if h1 != h0:
                    first = _iota((8, L), 0) < DH * h1 - 8 * b
                    sc = jnp.where(first, sc, scale[h1:h1 + 1, :])
                pieces.append(ret[8 * b:8 * b + 8, :] * sc)
            mem_v[c, GW * g:GW * g + 128, :] = jnp.concatenate(pieces, axis=0)

    def route():
        r = r_v[0:NSEG, :]
        idx = _iota((NSEG, L), 0) * L + _iota((NSEG, L), 1)
        m1 = jnp.max(r)
        i1 = jnp.clip(jnp.min(jnp.where(r == m1, idx, S)), 0, S - 1)
        r2 = jnp.where(idx == i1, -jnp.inf, r)
        m2 = jnp.max(r2)
        i2 = jnp.clip(jnp.min(jnp.where(r2 == m2, idx, S)), 0, S - 1)
        idx_s[0] = i1
        idx_s[1] = i2
        rsel_s[0] = m1
        rsel_s[1] = m2
        krow = _iota((128, 128), 0)
        for t, i in enumerate((i1, i2)):
            seg = i // L
            off = i - seg * L
            base = pl.multiple_of((off // 128) * 128, 128)
            cols = _unpack(xn_v[_rows(seg, D // 2), pl.ds(base, 128)])
            pick = jnp.where(krow == off - base, 1.0, 0.0).astype(BF16)
            xb_v[t] = _dot(cols, pick)
        y_v[...] = jnp.zeros(y_v.shape, F32)

    def swiglu(gate_sum, up_sum):
        gt = _round_bf16(jnp.sum(gate_sum, axis=0, keepdims=True))
        up = _round_bf16(jnp.sum(up_sum, axis=0, keepdims=True))
        return _round_bf16(_round_bf16(gt * jax.nn.sigmoid(gt)) * up)

    def ffn_chunk_chained():
        zmask = zero_s[0]

        def nothing(v):
            return pltpu.bitcast(pltpu.bitcast(v, U32) & zmask, F32)

        base = pl.multiple_of(step * (FT * 128), 128)
        link = [None, None]
        hid = {}
        for tile in range(FT):
            cols = pl.ds(base + 128 * tile, 128)
            sums = {}
            for name, w_ref in (("gate", wg_v), ("up", wu_v)):
                acc = [None, None]
                for i in range(D // 16):
                    w = w_ref[16 * i:16 * i + 16, cols].astype(F32)
                    for t in range(2):
                        pr = xb_v[t, 16 * i:16 * i + 16, :] * w
                        if i > 0:
                            lo = acc[t] + pr[0:8, :]
                        elif link[t] is None:
                            lo = pr[0:8, :]
                        else:
                            lo = pr[0:8, :] + nothing(link[t])
                        acc[t] = lo + pr[8:16, :]
                for t in range(2):
                    link[t] = acc[t]
                    sums[name, t] = acc[t]
            for t in range(2):
                hid[t, tile] = swiglu(sums["gate", t], sums["up", t])
        for b in range(D // 16):
            acc = [None, None]
            for tile in range(FT):
                w = wd_v[16 * b:16 * b + 16, pl.ds(base + 128 * tile, 128)].astype(F32)
                for t in range(2):
                    pr = w * hid[t, tile]
                    if tile == 0:
                        lo = pr[0:8, :] + nothing(link[t])
                        acc[t] = [lo, pr[8:16, :] + nothing(lo)]
                    else:
                        acc[t] = [acc[t][0] + pr[0:8, :], acc[t][1] + pr[8:16, :]]
            for t in range(2):
                rows = slice(16 * b, 16 * b + 16)
                y_v[t, rows, :] = y_v[t, rows, :] + jnp.concatenate(acc[t], axis=0)
                link[t] = acc[t][1]

    def ffn_chunk_looped():
        base = step * (FT * 128)

        def gate_up(tile, carry):
            cols = pl.ds(pl.multiple_of(base + 128 * tile, 128), 128)
            wg = wg_v[:, cols].astype(F32)
            wu = wu_v[:, cols].astype(F32)
            for t in range(2):
                h = swiglu(xb_v[t] * wg, xb_v[t] * wu)
                hid_v[t, tile] = jnp.broadcast_to(h, (8, 128))
            return carry

        def down(tile, carry):
            cols = pl.ds(pl.multiple_of(base + 128 * tile, 128), 128)
            w = wd_v[:, cols].astype(F32)
            for t in range(2):
                y_v[t] = y_v[t] + w * hid_v[t, tile][0:1, :]
            return carry

        lax.fori_loop(0, FT, gate_up, 0)
        lax.fori_loop(0, FT, down, 0)

    def masked_q(g, hp, j):
        rid = _iota((64, 128), 0)
        mask = (rid >= (DH // 2) * hp) & (rid < (DH // 2) * (hp + 1))
        return _unpack(jnp.where(mask, qt_v[_rows(step * NG + g, 64), 128 * j:128 * (j + 1)],
                                 jnp.uint32(0)))

    def causal_scores(g, hp, j):
        nk = 128 * (j + 1)
        first = pl.multiple_of((step * NG + g) * (L // 2), 8)
        st = _dot(_unpack(k_v[pl.ds(first, nk // 2), :]), masked_q(g, hp, j))
        diag = st[nk - 128:, :] + bias_v[...]
        return diag if j == 0 else jnp.concatenate([st[:nk - 128, :], diag], axis=0)

    def head_output(h, j, p, keep):
        o = _dot(_unpack(vt_v[_rows(step * H + h, 16), 0:128 * (j + 1)]), p)
        den = o[DH:DH + 1, :]
        inv = pl.reciprocal(den, approx=True)
        inv = inv * (2.0 - den * inv)
        return o[0:24, :] * (keep * inv)

    def attention_bounded():
        waves = [(list(range(4 * q, 4 * q + 4)), j)
                 for q in range(H // 4) for j in range(NQT)]

        def scores(w):
            quad, j = waves[w]
            return [jnp.exp2(causal_scores(*divmod(h, HPG), j)).astype(BF16)
                    for h in quad]

        def values(w, probs):
            quad, j = waves[w]
            for h, p in zip(quad, probs):
                ot_v[step, DH * h:DH * h + 24, 128 * j:128 * (j + 1)] = head_output(
                    h, j, p, 1.0 - gate_v[h:h + 1, :])

        pending = scores(0)
        for w in range(len(waves)):
            nxt = scores(w + 1) if w + 1 < len(waves) else None
            values(w, pending)
            pending = nxt
        ffn_chunk_chained()

    def attention_max_shifted():
        def one_head(h, carry):
            g = h // HPG
            hp = h - g * HPG
            keep = 1.0 - gate_v[pl.ds(h, 1), :]
            for j in range(NQT):
                st = causal_scores(g, hp, j)
                p = jnp.exp2(st - jnp.max(st, axis=0, keepdims=True)).astype(BF16)
                oh_v[h, :, 128 * j:128 * (j + 1)] = head_output(h, j, p, keep)
            return carry

        lax.fori_loop(0, H, one_head, 0)
        for h in range(H):
            ot_v[step, DH * h:DH * h + 24, :] = oh_v[h]
        ffn_chunk_looped()

    def output_projection(seg):
        heads_out = ot_v[seg, 0:D, :] + mem_v[seg, 0:D, :]
        attn = _dot(_unpack(wot[...]), heads_out.astype(BF16))
        base = x_v[seg].astype(F32) + attn
        xn = _unpack(xn_v[_rows(seg, D // 2), :]).astype(F32)
        col = seg * L + _iota((1, L), 1)
        upd = None
        for t in range(2):
            y = _round_bf16(jnp.sum(y_v[t], axis=1, keepdims=True))
            rsel = jnp.full((1, 1), rsel_s[t], F32)
            y = _round_bf16(y * _round_bf16(jax.nn.sigmoid(rsel)))
            part = jnp.where(col == idx_s[t], y, 0.0)
            upd = part if upd is None else upd + part
        o_ref[...] = (base + (xn + upd)).astype(BF16)

    def projections():
        half = D // 2
        xn0 = _unpack(xn_v[_rows(0, D // 2), :])
        ptq = _dot(_unpack(wall[0:half, :]), xn0)
        wall[half:2 * half, :] = pltpu.bitcast(wk_v[...].T, U32)
        cp_wv.wait()
        x_copies[1].wait()
        xn0 = _unpack(xn_v[_rows(0, D // 2), :])
        ptk = _dot(_unpack(wall[half:2 * half, :]), xn0)
        wall[2 * half:3 * half, :] = pltpu.bitcast(wv_v[...].T, U32)
        layer_norm(1)
        ptv = _dot(_unpack(wall[2 * half:PROWS // 2, :]), xn0)
        pt = jnp.concatenate([ptq, ptk, ptv], axis=0)
        mem_v[0] = jnp.zeros(mem_v.shape[1:], F32)
        pq0, pk, vg = store_qkv(0, pt)
        x_copies[2].wait()
        x_copies[3].wait()
        cp_wo.wait()

        layer_norm(2)
        pt = project(1)
        wot[...] = pltpu.bitcast(wo_v[...].T, U32)
        state1 = memory_update(None, pk, vg)
        pq1, pk, vg = store_qkv(1, pt)
        layer_norm(3)
        pt = project(2)
        state2 = memory_update(state1, pk, vg)
        memory_retrieve(1, state1, pq1)
        pq2, pk, vg = store_qkv(2, pt)
        pt = project(3)
        state3 = memory_update(state2, pk, vg)
        memory_retrieve(2, state2, pq2)
        pq3, _, _ = store_qkv(3, pt)
        memory_retrieve(3, state3, pq3)
        route()
        cp_wg.wait()
        cp_wu.wait()
        cp_wd.wait()

    @pl.when(step == 0)
    def _():
        for cp in (x_copies[0], cp_wq, cp_wr, cp_beta, cp_wk, cp_wv, x_copies[1],
                   x_copies[2], x_copies[3], cp_wo, cp_wg, cp_wu, cp_wd):
            cp.start()
        with _scope("sc_startup"):
            x_copies[0].wait()
            layer_norm(0)
            cp_wq.wait()
            cp_wr.wait()
            cp_beta.wait()
            init_constants()
            wall[0:D // 2, :] = pltpu.bitcast(wq_v[...].T, U32)
            cp_wk.wait()
        with _scope("sc_projections"):
            projections()

    @pl.when(step < NSEG)
    def _():
        safe = safe_s[step] == 1

        @pl.when(safe)
        def _():
            with _scope("sc_attention"):
                attention_bounded()

        @pl.when(jnp.logical_not(safe))
        def _():
            attention_max_shifted()

    @pl.when(step >= NSEG)
    def _():
        with _scope("sc_outproj"):
            output_projection(step - NSEG)


@jax.jit
def pallas_parallel_sum__memory_aug_infini_attn__moe_arch_mod__prompt_kernel(
    A_x: jax.Array,
    A_wq: jax.Array,
    A_wk: jax.Array,
    A_wv: jax.Array,
    A_wo: jax.Array,
    A_beta: jax.Array,
    B_x: jax.Array,
    B_w_r: jax.Array,
    B_w_gate: jax.Array,
    B_w_up: jax.Array,
    B_w_down: jax.Array,
):
    del B_x
    vm = pltpu.VMEM
    scratch = [
        vm((NSEG, D, L), BF16),
        vm((D, D), BF16),
        vm((D, D), BF16),
        vm((D, D), BF16),
        vm((D, D), BF16),
        vm((H,), BF16),
        vm((D,), BF16),
        vm((D, FF), BF16),
        vm((D, FF), BF16),
        vm((D, FF), BF16),
        vm((PROWS // 2, D), U32),
        vm((D // 2, D), U32),
        vm((NSEG * D // 2, L), U32),
        vm((NSEG * NG * 64, L), U32),
        vm((NSEG * NG * L // 2, 128), U32),
        vm((NSEG * H * 16, L), U32),
        vm((NSEG, OROWS, L), F32),
        vm((8, L), F32),
        vm((2, D, 128), F32),
        vm((2, D, 128), F32),
        vm((2, FT, 8, 128), F32),
        pltpu.SMEM((2,), jnp.int32),
        pltpu.SMEM((2,), F32),
        pltpu.SMEM((1,), U32),
        pltpu.SMEM((NSEG,), jnp.int32),
        vm((H, 128), F32),
        vm((NSEG, D + 8, L), F32),
        vm((H, 24, L), F32),
        vm((128, 128), F32),
        pltpu.SemaphoreType.DMA((NSEG + 9,)),
    ]
    hbm = pl.BlockSpec(memory_space=pltpu.HBM)
    xt = jnp.transpose(A_x.reshape(S, D))
    out_t = pl.pallas_call(
        _kernel,
        grid=(2 * NSEG,),
        in_specs=[hbm] * 10,
        out_specs=pl.BlockSpec((D, L), lambda s: (0, jnp.maximum(s - NSEG, 0))),
        out_shape=jax.ShapeDtypeStruct((D, S), BF16),
        scratch_shapes=scratch,
        compiler_params=pltpu.CompilerParams(
            dimension_semantics=("arbitrary",),
            vmem_limit_bytes=110 * 1024 * 1024,
        ),
        name="infini_moe",
    )(xt, A_wq, A_wk, A_wv, A_wo, A_beta, B_w_r, B_w_gate, B_w_up,
      jnp.transpose(B_w_down))
    return jnp.transpose(out_t).reshape(1, S, D)
```

```python
import contextlib

import jax
import jax.numpy as jnp
from jax import lax
from jax.experimental import pallas as pl
from jax.experimental.pallas import tpu as pltpu

S = 2048
D = 576
H = 32
DH = 18
NSEG = 4
L = 512
FF = 4608
NG = 5
HPG = 7
GW = HPG * DH
NQT = L // 128
PROWS = 3 * D + 16
RROW = 3 * D
PBLOCK = 128
MROWS = 144
FT = FF // 128 // NSEG
OROWS = 640
LOG2E = 1.4426950408889634
QSCALE = DH ** -0.5 * LOG2E
NEG = -1e30
SAFE_LOG2 = 40.0
LN_EPS = 1.0013580322265625e-05
F32 = jnp.float32
BF16 = jnp.bfloat16
U32 = jnp.uint32

PROFILE_SCOPES = False

_NN = (((1,), (0,)), ((), ()))
_NT = (((1,), (1,)), ((), ()))


def _scope(name):
    return jax.named_scope(name) if PROFILE_SCOPES else contextlib.nullcontext()


def _dot(a, b):
    return lax.dot_general(a, b, _NN, preferred_element_type=F32)


def _dot_nt(a, b):
    return lax.dot_general(a, b, _NT, preferred_element_type=F32)


def _iota(shape, dim):
    return lax.broadcasted_iota(jnp.int32, shape, dim)


def _round_bf16(v):
    return v.astype(BF16).astype(F32)


def _pack(v):
    return pltpu.bitcast(v.astype(BF16), U32)


def _unpack(u):
    return pltpu.bitcast(u, BF16)


def _rows(index, size):
    if isinstance(index, int):
        return slice(index * size, (index + 1) * size)
    return pl.ds(pl.multiple_of(index * size, 8), size)


def _heads_in_group(g):
    return HPG if g < NG - 1 else H - HPG * (NG - 1)


def _phi(t):
    return jnp.where(t > 0, t + 1.0, jnp.exp(t))


def _kernel(x_hbm, wq_hbm, wk_hbm, wv_hbm, wo_hbm, beta_hbm, wr_hbm,
            wg_hbm, wu_hbm, wd_hbm,
            o_ref,
            x_v, wq_v, wk_v, wv_v, wo_v, beta_v, wr_v, wg_v, wu_v, wd_v,
            wall, wot, xn_v, qt_v, k_v, vt_v, mem_v,
            r_v, xb_v, y_v, hid_v, idx_s, rsel_s, zero_s, safe_s,
            gate_v, ot_v, oh_v, bias_v,
            sems):
    step = pl.program_id(0)

    x_copies = [
        pltpu.make_async_copy(x_hbm.at[:, pl.ds(c * L, L)], x_v.at[c], sems.at[c])
        for c in range(NSEG)
    ]
    pairs = [(wq_hbm, wq_v), (wk_hbm, wk_v), (wv_hbm, wv_v), (wo_hbm, wo_v),
             (beta_hbm, beta_v), (wr_hbm, wr_v),
             (wg_hbm, wg_v), (wu_hbm, wu_v), (wd_hbm, wd_v)]
    (cp_wq, cp_wk, cp_wv, cp_wo, cp_beta, cp_wr, cp_wg, cp_wu, cp_wd) = [
        pltpu.make_async_copy(src, dst, sems.at[NSEG + i])
        for i, (src, dst) in enumerate(pairs)
    ]

    def layer_norm(c):
        for n in range(NQT):
            cols = slice(128 * n, 128 * (n + 1))
            pivot = x_v[c, 0:16, cols].astype(F32)[0:1, :]
            s1 = [None, None]
            s2 = [None, None]
            for i in range(D // 16):
                d = x_v[c, 16 * i:16 * i + 16, cols].astype(F32) - pivot
                for k in range(2):
                    dk = d[8 * k:8 * k + 8, :]
                    s1[k] = dk if s1[k] is None else s1[k] + dk
                    s2[k] = dk * dk if s2[k] is None else s2[k] + dk * dk
            dmean = jnp.sum(s1[0] + s1[1], axis=0, keepdims=True) * (1.0 / D)
            dsq = jnp.sum(s2[0] + s2[1], axis=0, keepdims=True) * (1.0 / D)
            mean = pivot + dmean
            var = jnp.maximum(dsq - dmean * dmean, 0.0)
            sd = _round_bf16(jnp.sqrt(_round_bf16(_round_bf16(var) + LN_EPS)))
            xf = x_v[c, :, cols].astype(F32)
            xn_v[_rows(c, D // 2), cols] = _pack(
                (xf - _round_bf16(mean)) * (1.0 / sd))

    def init_constants():
        gate = jax.nn.sigmoid(beta_v[...].astype(F32).reshape(1, H))
        on_diag = _iota((H, H), 0) == _iota((H, H), 1)
        gcol = jnp.sum(jnp.where(on_diag, gate, 0.0), axis=1, keepdims=True)
        gate_v[...] = jnp.broadcast_to(gcol, (H, 128))
        zero_s[0] = jnp.uint32(0)
        bias_v[...] = jnp.where(_iota((128, 128), 0) > _iota((128, 128), 1), NEG, 0.0)
        router = jnp.broadcast_to(wr_v[...].astype(F32).reshape(1, D), (16, D))
        wall[RROW // 2:PROWS // 2, :] = _pack(
            jnp.where(_iota((16, D), 0) == 0, router, 0.0))

    def project(c):
        xn = _unpack(xn_v[_rows(c, D // 2), :])
        step_rows = PBLOCK // 2
        return jnp.concatenate(
            [_dot(_unpack(wall[r:min(r + step_rows, PROWS // 2), :]), xn)
             for r in range(0, PROWS // 2, step_rows)], axis=0)

    def store_qkv(c, pt):
        r_v[c:c + 1, :] = _round_bf16(pt[RROW:RROW + 1, :])
        qa = jnp.max(jnp.abs(pt[0:D, :])) * QSCALE
        ka = jnp.max(jnp.abs(pt[D:2 * D, :]))
        safe_s[c] = (qa * ka * (DH * 1.02) <= SAFE_LOG2).astype(jnp.int32)

        tail_row = _iota((8, L), 0)
        for h in range(H):
            base = 2 * D + DH * h
            tail = jnp.where(tail_row < DH - 16, pt[base + 16:base + 24, :],
                             jnp.where(tail_row == DH - 16, 1.0, 0.0))
            blk = jnp.concatenate(
                [pt[base:base + 16, :], tail, jnp.zeros((8, L), F32)], axis=0)
            vt_v[_rows(c * H + h, 16), :] = _pack(blk)

        rowl = _iota((128, L), 0)
        pqs, pks, vgs = [], [], []
        for g in range(NG):
            used = _heads_in_group(g) * DH
            qg = pt[GW * g:GW * g + 128, :]
            qt_v[_rows(c * NG + g, 64), :] = _pack(qg * QSCALE)
            kg = pt[D + GW * g:D + GW * g + 128, :]
            k_v[_rows(c * NG + g, L // 2), :] = _pack(kg.T)
            pqs.append(_phi(qg).astype(BF16))
            if c < NSEG - 1:
                pks.append(_phi(kg).astype(BF16))
                lo = 2 * D + GW * g
                if g < NG - 1:
                    vg = pt[lo:lo + 128, :]
                else:
                    vg = jnp.concatenate(
                        [pt[lo:lo + used, :], jnp.zeros((128 - used, L), F32)], axis=0)
                vg = jnp.where(rowl < used, vg, jnp.where(rowl == GW, 1.0, 0.0))
                vgs.append(vg.astype(BF16))
        return pqs, pks, vgs

    def memory_update(states, pks, vgs):
        row = _iota((128, 128), 0)
        lane = _iota((128, 128), 1)
        same_head = (row // DH) == (lane // DH)
        out = []
        for g in range(NG):
            used = _heads_in_group(g) * DH
            upd = _dot_nt(vgs[g], pks[g])
            keep = ((same_head & (row < used)) | (row == GW)) & (lane < used)
            upd = jnp.where(keep, upd, 0.0)
            out.append(upd if states is None else states[g] + upd)
        return out

    def memory_retrieve(c, states, pqs):
        row = _iota((128, 128), 0)
        row8 = _iota((8, 128), 0)
        lane8 = _iota((8, 128), 1) // DH
        for g in range(NG):
            nh = _heads_in_group(g)
            st = states[g]
            mrows = jnp.where(row < GW, st, 0.0)
            zrows = jnp.where(lane8 == row8, st[GW:GW + 1, :], 0.0)
            lhs = jnp.concatenate(
                [mrows, zrows, jnp.zeros((8, 128), F32)], axis=0).astype(BF16)
            ret = _dot(lhs, pqs[g])
            gsel = gate_v[HPG * g:HPG * g + 8, :] if g < NG - 1 else jnp.concatenate(
                [gate_v[HPG * g:H, :], jnp.zeros((8 - nh, 128), F32)], axis=0)
            gwide = jnp.concatenate([gsel] * NQT, axis=1)
            scale = gwide / (ret[128:136, :] + 1e-6)
            pieces = []
            for b in range(16):
                h0 = min((8 * b) // DH, nh - 1)
                h1 = min((8 * b + 7) // DH, nh - 1)
                sc = scale[h0:h0 + 1, :]
                if h1 != h0:
                    first = _iota((8, L), 0) < DH * h1 - 8 * b
                    sc = jnp.where(first, sc, scale[h1:h1 + 1, :])
                pieces.append(ret[8 * b:8 * b + 8, :] * sc)
            mem_v[c - 1, GW * g:GW * g + 128, :] = jnp.concatenate(pieces, axis=0)

    def route():
        r = r_v[0:NSEG, :]
        idx = _iota((NSEG, L), 0) * L + _iota((NSEG, L), 1)
        m1 = jnp.max(r)
        i1 = jnp.clip(jnp.min(jnp.where(r == m1, idx, S)), 0, S - 1)
        r2 = jnp.where(idx == i1, -jnp.inf, r)
        m2 = jnp.max(r2)
        i2 = jnp.clip(jnp.min(jnp.where(r2 == m2, idx, S)), 0, S - 1)
        idx_s[0] = i1
        idx_s[1] = i2
        rsel_s[0] = m1
        rsel_s[1] = m2
        krow = _iota((128, 128), 0)
        for t, i in enumerate((i1, i2)):
            seg = i // L
            off = i - seg * L
            base = pl.multiple_of((off // 128) * 128, 128)
            cols = _unpack(xn_v[_rows(seg, D // 2), pl.ds(base, 128)])
            pick = jnp.where(krow == off - base, 1.0, 0.0).astype(BF16)
            xb_v[t] = _dot(cols, pick)
        y_v[...] = jnp.zeros(y_v.shape, F32)

    def swiglu(gate_sum, up_sum):
        gt = _round_bf16(jnp.sum(gate_sum, axis=0, keepdims=True))
        up = _round_bf16(jnp.sum(up_sum, axis=0, keepdims=True))
        return _round_bf16(_round_bf16(gt * jax.nn.sigmoid(gt)) * up)

    def ffn_chunk_chained():
        zmask = zero_s[0]

        def nothing(v):
            return pltpu.bitcast(pltpu.bitcast(v, U32) & zmask, F32)

        base = pl.multiple_of(step * (FT * 128), 128)
        link = [None, None]
        hid = {}
        for tile in range(FT):
            cols = pl.ds(base + 128 * tile, 128)
            sums = {}
            for name, w_ref in (("gate", wg_v), ("up", wu_v)):
                acc = [None, None]
                for i in range(D // 16):
                    w = w_ref[16 * i:16 * i + 16, cols].astype(F32)
                    for t in range(2):
                        pr = xb_v[t, 16 * i:16 * i + 16, :] * w
                        if i > 0:
                            lo = acc[t] + pr[0:8, :]
                        elif link[t] is None:
                            lo = pr[0:8, :]
                        else:
                            lo = pr[0:8, :] + nothing(link[t])
                        acc[t] = lo + pr[8:16, :]
                for t in range(2):
                    link[t] = acc[t]
                    sums[name, t] = acc[t]
            for t in range(2):
                hid[t, tile] = swiglu(sums["gate", t], sums["up", t])
        for b in range(D // 16):
            acc = [None, None]
            for tile in range(FT):
                w = wd_v[16 * b:16 * b + 16, pl.ds(base + 128 * tile, 128)].astype(F32)
                for t in range(2):
                    pr = w * hid[t, tile]
                    if tile == 0:
                        lo = pr[0:8, :] + nothing(link[t])
                        acc[t] = [lo, pr[8:16, :] + nothing(lo)]
                    else:
                        acc[t] = [acc[t][0] + pr[0:8, :], acc[t][1] + pr[8:16, :]]
            for t in range(2):
                rows = slice(16 * b, 16 * b + 16)
                y_v[t, rows, :] = y_v[t, rows, :] + jnp.concatenate(acc[t], axis=0)
                link[t] = acc[t][1]

    def ffn_chunk_looped():
        base = step * (FT * 128)

        def gate_up(tile, carry):
            cols = pl.ds(pl.multiple_of(base + 128 * tile, 128), 128)
            wg = wg_v[:, cols].astype(F32)
            wu = wu_v[:, cols].astype(F32)
            for t in range(2):
                h = swiglu(xb_v[t] * wg, xb_v[t] * wu)
                hid_v[t, tile] = jnp.broadcast_to(h, (8, 128))
            return carry

        def down(tile, carry):
            cols = pl.ds(pl.multiple_of(base + 128 * tile, 128), 128)
            w = wd_v[:, cols].astype(F32)
            for t in range(2):
                y_v[t] = y_v[t] + w * hid_v[t, tile][0:1, :]
            return carry

        lax.fori_loop(0, FT, gate_up, 0)
        lax.fori_loop(0, FT, down, 0)

    def masked_q(g, hp, j):
        rid = _iota((64, 128), 0)
        mask = (rid >= (DH // 2) * hp) & (rid < (DH // 2) * (hp + 1))
        return _unpack(jnp.where(mask, qt_v[_rows(step * NG + g, 64), 128 * j:128 * (j + 1)],
                                 jnp.uint32(0)))

    def causal_scores(g, hp, j):
        nk = 128 * (j + 1)
        first = pl.multiple_of((step * NG + g) * (L // 2), 8)
        st = _dot(_unpack(k_v[pl.ds(first, nk // 2), :]), masked_q(g, hp, j))
        diag = st[nk - 128:, :] + bias_v[...]
        return diag if j == 0 else jnp.concatenate([st[:nk - 128, :], diag], axis=0)

    def head_output(h, j, p, keep):
        o = _dot(_unpack(vt_v[_rows(step * H + h, 16), 0:128 * (j + 1)]), p)
        den = o[DH:DH + 1, :]
        inv = pl.reciprocal(den, approx=True)
        inv = inv * (2.0 - den * inv)
        return o[0:24, :] * (keep * inv)

    def attention_bounded():
        waves = [(list(range(4 * q, 4 * q + 4)), j)
                 for q in range(H // 4) for j in range(NQT)]

        def scores(w):
            quad, j = waves[w]
            return [jnp.exp2(causal_scores(*divmod(h, HPG), j)).astype(BF16)
                    for h in quad]

        def values(w, probs):
            quad, j = waves[w]
            for h, p in zip(quad, probs):
                ot_v[step, DH * h:DH * h + 24, 128 * j:128 * (j + 1)] = head_output(
                    h, j, p, 1.0 - gate_v[h:h + 1, :])

        pending = scores(0)
        for w in range(len(waves)):
            nxt = scores(w + 1) if w + 1 < len(waves) else None
            values(w, pending)
            pending = nxt
        ffn_chunk_chained()

    def attention_max_shifted():
        def one_head(h, carry):
            g = h // HPG
            hp = h - g * HPG
            keep = 1.0 - gate_v[pl.ds(h, 1), :]
            for j in range(NQT):
                st = causal_scores(g, hp, j)
                p = jnp.exp2(st - jnp.max(st, axis=0, keepdims=True)).astype(BF16)
                oh_v[h, :, 128 * j:128 * (j + 1)] = head_output(h, j, p, keep)
            return carry

        lax.fori_loop(0, H, one_head, 0)
        for h in range(H):
            ot_v[step, DH * h:DH * h + 24, :] = oh_v[h]
        ffn_chunk_looped()

    def output_projection(seg):
        mem = jnp.where(seg > 0, mem_v[jnp.maximum(seg - 1, 0), 0:D, :], 0.0)
        heads_out = ot_v[seg, 0:D, :] + mem
        attn = _dot(_unpack(wot[...]), heads_out.astype(BF16))
        base = x_v[seg].astype(F32) + attn
        xn = _unpack(xn_v[_rows(seg, D // 2), :]).astype(F32)
        col = seg * L + _iota((1, L), 1)
        upd = None
        for t in range(2):
            y = _round_bf16(jnp.sum(y_v[t], axis=1, keepdims=True))
            rsel = jnp.full((1, 1), rsel_s[t], F32)
            y = _round_bf16(y * _round_bf16(jax.nn.sigmoid(rsel)))
            part = jnp.where(col == idx_s[t], y, 0.0)
            upd = part if upd is None else upd + part
        o_ref[...] = (base + (xn + upd)).astype(BF16)

    col_blocks = [(c0, min(128, D - c0)) for c0 in range(0, D, 128)]

    def transpose_block(w_v, section, c0, n):
        r0 = (section * D + c0) // 2
        wall[r0:r0 + n // 2, :] = pltpu.bitcast(w_v[:, c0:c0 + n].T, U32)

    def project_block(section, c0, n, xn):
        r0 = (section * D + c0) // 2
        last = section == 2 and c0 + n == D
        hi = PROWS // 2 if last else r0 + n // 2
        return _dot(_unpack(wall[r0:hi, :]), xn)

    def projections():
        xn0 = _unpack(xn_v[_rows(0, D // 2), :])
        parts = [project_block(0, c0, n, xn0) for c0, n in col_blocks[:3]]
        cp_wk.wait()
        xn0 = _unpack(xn_v[_rows(0, D // 2), :])
        parts += [project_block(0, c0, n, xn0) for c0, n in col_blocks[3:]]
        for c0, n in col_blocks:
            transpose_block(wk_v, 1, c0, n)
        cp_wv.wait()
        x_copies[1].wait()
        xn0 = _unpack(xn_v[_rows(0, D // 2), :])
        parts += [project_block(1, c0, n, xn0) for c0, n in col_blocks]
        for c0, n in col_blocks:
            transpose_block(wv_v, 2, c0, n)
            parts.append(project_block(2, c0, n, xn0))
        layer_norm(1)
        _, pk, vg = store_qkv(0, jnp.concatenate(parts, axis=0))
        x_copies[2].wait()
        x_copies[3].wait()
        cp_wo.wait()

        layer_norm(2)
        pt = project(1)
        wot[...] = pltpu.bitcast(wo_v[...].T, U32)
        state1 = memory_update(None, pk, vg)
        pq1, pk, vg = store_qkv(1, pt)
        layer_norm(3)
        pt = project(2)
        state2 = memory_update(state1, pk, vg)
        pq2, pk, vg = store_qkv(2, pt)
        pt = project(3)
        state3 = memory_update(state2, pk, vg)
        memory_retrieve(1, state1, pq1)
        memory_retrieve(2, state2, pq2)
        pq3, _, _ = store_qkv(3, pt)
        memory_retrieve(3, state3, pq3)
        route()
        cp_wg.wait()
        cp_wu.wait()
        cp_wd.wait()

    @pl.when(step == 0)
    def _():
        for cp in (cp_wq, x_copies[0], cp_wr, cp_beta, cp_wk, cp_wv, x_copies[1],
                   x_copies[2], x_copies[3], cp_wo, cp_wg, cp_wu, cp_wd):
            cp.start()
        with _scope("sc_startup"):
            cp_wr.wait()
            cp_beta.wait()
            cp_wq.wait()
            init_constants()
            for c0, n in col_blocks:
                transpose_block(wq_v, 0, c0, n)
            x_copies[0].wait()
            layer_norm(0)
        with _scope("sc_projections"):
            projections()

    @pl.when(step < NSEG)
    def _():
        safe = safe_s[step] == 1

        @pl.when(safe)
        def _():
            with _scope("sc_attention"):
                attention_bounded()

        @pl.when(jnp.logical_not(safe))
        def _():
            attention_max_shifted()

    @pl.when(step >= NSEG)
    def _():
        with _scope("sc_outproj"):
            output_projection(step - NSEG)


@jax.jit
def pallas_parallel_sum__memory_aug_infini_attn__moe_arch_mod__prompt_kernel(
    A_x: jax.Array,
    A_wq: jax.Array,
    A_wk: jax.Array,
    A_wv: jax.Array,
    A_wo: jax.Array,
    A_beta: jax.Array,
    B_x: jax.Array,
    B_w_r: jax.Array,
    B_w_gate: jax.Array,
    B_w_up: jax.Array,
    B_w_down: jax.Array,
):
    del B_x
    vm = pltpu.VMEM
    scratch = [
        vm((NSEG, D, L), BF16),
        vm((D, D), BF16),
        vm((D, D), BF16),
        vm((D, D), BF16),
        vm((D, D), BF16),
        vm((H,), BF16),
        vm((D,), BF16),
        vm((D, FF), BF16),
        vm((D, FF), BF16),
        vm((D, FF), BF16),
        vm((PROWS // 2, D), U32),
        vm((D // 2, D), U32),
        vm((NSEG * D // 2, L), U32),
        vm((NSEG * NG * 64, L), U32),
        vm((NSEG * NG * L // 2, 128), U32),
        vm((NSEG * H * 16, L), U32),
        vm((NSEG - 1, OROWS, L), F32),
        vm((8, L), F32),
        vm((2, D, 128), F32),
        vm((2, D, 128), F32),
        vm((2, FT, 8, 128), F32),
        pltpu.SMEM((2,), jnp.int32),
        pltpu.SMEM((2,), F32),
        pltpu.SMEM((1,), U32),
        pltpu.SMEM((NSEG,), jnp.int32),
        vm((H, 128), F32),
        vm((NSEG, D + 8, L), F32),
        vm((H, 24, L), F32),
        vm((128, 128), F32),
        pltpu.SemaphoreType.DMA((NSEG + 9,)),
    ]
    hbm = pl.BlockSpec(memory_space=pltpu.HBM)
    xt = jnp.transpose(A_x.reshape(S, D))
    out_t = pl.pallas_call(
        _kernel,
        grid=(2 * NSEG,),
        in_specs=[hbm] * 10,
        out_specs=pl.BlockSpec((D, L), lambda s: (0, jnp.maximum(s - NSEG, 0))),
        out_shape=jax.ShapeDtypeStruct((D, S), BF16),
        scratch_shapes=scratch,
        compiler_params=pltpu.CompilerParams(
            dimension_semantics=("arbitrary",),
            vmem_limit_bytes=110 * 1024 * 1024,
        ),
        name="infini_moe",
    )(xt, A_wq, A_wk, A_wv, A_wo, A_beta, B_w_r, B_w_gate, B_w_up,
      jnp.transpose(B_w_down))
    return jnp.transpose(out_t).reshape(1, S, D)
```

```python
import contextlib

import jax
import jax.numpy as jnp
from jax import lax
from jax.experimental import pallas as pl
from jax.experimental.pallas import tpu as pltpu

S = 2048
D = 576
H = 32
DH = 18
NSEG = 4
L = 512
FF = 4608
NG = 5
HPG = 7
GW = HPG * DH
NQT = L // 128
PROWS = 3 * D + 16
RROW = 3 * D
PBLOCK = 128
MROWS = 144
FT = FF // 128 // NSEG
OROWS = 640
LOG2E = 1.4426950408889634
QSCALE = DH ** -0.5 * LOG2E
NEG = -1e30
SAFE_LOG2 = 40.0
LN_EPS = 1.0013580322265625e-05
F32 = jnp.float32
BF16 = jnp.bfloat16
U32 = jnp.uint32

PROFILE_SCOPES = False

_NN = (((1,), (0,)), ((), ()))
_NT = (((1,), (1,)), ((), ()))


def _scope(name):
    return jax.named_scope(name) if PROFILE_SCOPES else contextlib.nullcontext()


def _dot(a, b):
    return lax.dot_general(a, b, _NN, preferred_element_type=F32)


def _dot_nt(a, b):
    return lax.dot_general(a, b, _NT, preferred_element_type=F32)


def _iota(shape, dim):
    return lax.broadcasted_iota(jnp.int32, shape, dim)


def _round_bf16(v):
    return v.astype(BF16).astype(F32)


def _pack(v):
    return pltpu.bitcast(v.astype(BF16), U32)


def _unpack(u):
    return pltpu.bitcast(u, BF16)


def _rows(index, size):
    if isinstance(index, int):
        return slice(index * size, (index + 1) * size)
    return pl.ds(pl.multiple_of(index * size, 8), size)


def _heads_in_group(g):
    return HPG if g < NG - 1 else H - HPG * (NG - 1)


def _phi(t):
    return jnp.where(t > 0, t + 1.0, jnp.exp(t))


def _kernel(x_hbm, wq_hbm, wk_hbm, wv_hbm, wo_hbm, beta_hbm, wr_hbm,
            wg_hbm, wu_hbm, wd_hbm,
            o_ref,
            x_v, wq_v, wk_v, wv_v, wo_v, beta_v, wr_v, wg_v, wu_v, wd_v,
            wall, wot, xn_v, qt_v, k_v, vt_v, mem_v,
            r_v, xb_v, y_v, hid_v, idx_s, rsel_s, zero_s, safe_s,
            gate_v, ot_v, oh_v, bias_v, half_v,
            sems):
    step = pl.program_id(0)

    x_copies = [
        pltpu.make_async_copy(x_hbm.at[:, pl.ds(c * L, L)], x_v.at[c], sems.at[c])
        for c in range(NSEG)
    ]
    pairs = [(wq_hbm, wq_v), (wk_hbm, wk_v), (wv_hbm, wv_v), (wo_hbm, wo_v),
             (beta_hbm, beta_v), (wr_hbm, wr_v),
             (wg_hbm, wg_v), (wu_hbm, wu_v), (wd_hbm, wd_v)]
    (cp_wq, cp_wk, cp_wv, cp_wo, cp_beta, cp_wr, cp_wg, cp_wu, cp_wd) = [
        pltpu.make_async_copy(src, dst, sems.at[NSEG + i])
        for i, (src, dst) in enumerate(pairs)
    ]

    def layer_norm(c):
        for n in range(NQT):
            cols = slice(128 * n, 128 * (n + 1))
            pivot = x_v[c, 0:16, cols].astype(F32)[0:1, :]
            s1 = [None, None]
            s2 = [None, None]
            for i in range(D // 16):
                d = x_v[c, 16 * i:16 * i + 16, cols].astype(F32) - pivot
                for k in range(2):
                    dk = d[8 * k:8 * k + 8, :]
                    s1[k] = dk if s1[k] is None else s1[k] + dk
                    s2[k] = dk * dk if s2[k] is None else s2[k] + dk * dk
            dmean = jnp.sum(s1[0] + s1[1], axis=0, keepdims=True) * (1.0 / D)
            dsq = jnp.sum(s2[0] + s2[1], axis=0, keepdims=True) * (1.0 / D)
            mean = pivot + dmean
            var = jnp.maximum(dsq - dmean * dmean, 0.0)
            sd = _round_bf16(jnp.sqrt(_round_bf16(_round_bf16(var) + LN_EPS)))
            xf = x_v[c, :, cols].astype(F32)
            xn_v[_rows(c, D // 2), cols] = _pack(
                (xf - _round_bf16(mean)) * (1.0 / sd))

    def init_constants():
        gate = jax.nn.sigmoid(beta_v[...].astype(F32).reshape(1, H))
        on_diag = _iota((H, H), 0) == _iota((H, H), 1)
        gcol = jnp.sum(jnp.where(on_diag, gate, 0.0), axis=1, keepdims=True)
        gate_v[...] = jnp.broadcast_to(gcol, (H, 128))
        zero_s[0] = jnp.uint32(0)
        bias_v[...] = jnp.where(_iota((128, 128), 0) > _iota((128, 128), 1), NEG, 0.0)
        key, lane = _iota((64, 128), 0), _iota((64, 128), 1)
        future = key > (lane & 63)
        half_v[0] = jnp.where(future, NEG, 0.0)
        half_v[1] = jnp.where(future | (lane < 64), NEG, 0.0)
        half_v[2] = jnp.where(future | (lane >= 64), NEG, 0.0)
        router = jnp.broadcast_to(wr_v[...].astype(F32).reshape(1, D), (16, D))
        wall[RROW // 2:PROWS // 2, :] = _pack(
            jnp.where(_iota((16, D), 0) == 0, router, 0.0))

    def project(c):
        xn = _unpack(xn_v[_rows(c, D // 2), :])
        step_rows = PBLOCK // 2
        return jnp.concatenate(
            [_dot(_unpack(wall[r:min(r + step_rows, PROWS // 2), :]), xn)
             for r in range(0, PROWS // 2, step_rows)], axis=0)

    def store_qkv(c, pt):
        r_v[c:c + 1, :] = _round_bf16(pt[RROW:RROW + 1, :])
        qa = jnp.max(jnp.abs(pt[0:D, :])) * QSCALE
        ka = jnp.max(jnp.abs(pt[D:2 * D, :]))
        safe_s[c] = (qa * ka * (DH * 1.02) <= SAFE_LOG2).astype(jnp.int32)

        tail_row = _iota((8, L), 0)
        for h in range(H):
            base = 2 * D + DH * h
            tail = jnp.where(tail_row < DH - 16, pt[base + 16:base + 24, :],
                             jnp.where(tail_row == DH - 16, 1.0, 0.0))
            blk = jnp.concatenate(
                [pt[base:base + 16, :], tail, jnp.zeros((8, L), F32)], axis=0)
            vt_v[_rows(c * H + h, 16), :] = _pack(blk)

        rowl = _iota((128, L), 0)
        pqs, pks, vgs = [], [], []
        for g in range(NG):
            used = _heads_in_group(g) * DH
            qg = pt[GW * g:GW * g + 128, :]
            qt_v[_rows(c * NG + g, 64), :] = _pack(qg * QSCALE)
            kg = pt[D + GW * g:D + GW * g + 128, :]
            k_v[_rows(c * NG + g, L // 2), :] = _pack(kg.T)
            pqs.append(_phi(qg).astype(BF16))
            if c < NSEG - 1:
                pks.append(_phi(kg).astype(BF16))
                lo = 2 * D + GW * g
                if g < NG - 1:
                    vg = pt[lo:lo + 128, :]
                else:
                    vg = jnp.concatenate(
                        [pt[lo:lo + used, :], jnp.zeros((128 - used, L), F32)], axis=0)
                vg = jnp.where(rowl < used, vg, jnp.where(rowl == GW, 1.0, 0.0))
                vgs.append(vg.astype(BF16))
        return pqs, pks, vgs

    def memory_update(states, pks, vgs):
        row = _iota((128, 128), 0)
        lane = _iota((128, 128), 1)
        same_head = (row // DH) == (lane // DH)
        out = []
        for g in range(NG):
            used = _heads_in_group(g) * DH
            upd = _dot_nt(vgs[g], pks[g])
            keep = ((same_head & (row < used)) | (row == GW)) & (lane < used)
            upd = jnp.where(keep, upd, 0.0)
            out.append(upd if states is None else states[g] + upd)
        return out

    def memory_retrieve(c, states, pqs):
        row = _iota((128, 128), 0)
        row8 = _iota((8, 128), 0)
        lane8 = _iota((8, 128), 1) // DH
        for g in range(NG):
            nh = _heads_in_group(g)
            st = states[g]
            mrows = jnp.where(row < GW, st, 0.0)
            zrows = jnp.where(lane8 == row8, st[GW:GW + 1, :], 0.0)
            lhs = jnp.concatenate(
                [mrows, zrows, jnp.zeros((8, 128), F32)], axis=0).astype(BF16)
            ret = _dot(lhs, pqs[g])
            gsel = gate_v[HPG * g:HPG * g + 8, :] if g < NG - 1 else jnp.concatenate(
                [gate_v[HPG * g:H, :], jnp.zeros((8 - nh, 128), F32)], axis=0)
            gwide = jnp.concatenate([gsel] * NQT, axis=1)
            scale = gwide / (ret[128:136, :] + 1e-6)
            pieces = []
            for b in range(16):
                h0 = min((8 * b) // DH, nh - 1)
                h1 = min((8 * b + 7) // DH, nh - 1)
                sc = scale[h0:h0 + 1, :]
                if h1 != h0:
                    first = _iota((8, L), 0) < DH * h1 - 8 * b
                    sc = jnp.where(first, sc, scale[h1:h1 + 1, :])
                pieces.append(ret[8 * b:8 * b + 8, :] * sc)
            mem_v[c - 1, GW * g:GW * g + 128, :] = jnp.concatenate(pieces, axis=0)

    def route():
        r = r_v[0:NSEG, :]
        idx = _iota((NSEG, L), 0) * L + _iota((NSEG, L), 1)
        m1 = jnp.max(r)
        i1 = jnp.clip(jnp.min(jnp.where(r == m1, idx, S)), 0, S - 1)
        r2 = jnp.where(idx == i1, -jnp.inf, r)
        m2 = jnp.max(r2)
        i2 = jnp.clip(jnp.min(jnp.where(r2 == m2, idx, S)), 0, S - 1)
        idx_s[0] = i1
        idx_s[1] = i2
        rsel_s[0] = m1
        rsel_s[1] = m2
        krow = _iota((128, 128), 0)
        for t, i in enumerate((i1, i2)):
            seg = i // L
            off = i - seg * L
            base = pl.multiple_of((off // 128) * 128, 128)
            cols = _unpack(xn_v[_rows(seg, D // 2), pl.ds(base, 128)])
            pick = jnp.where(krow == off - base, 1.0, 0.0).astype(BF16)
            xb_v[t] = _dot(cols, pick)
        y_v[...] = jnp.zeros(y_v.shape, F32)

    def swiglu(gate_sum, up_sum):
        gt = _round_bf16(jnp.sum(gate_sum, axis=0, keepdims=True))
        up = _round_bf16(jnp.sum(up_sum, axis=0, keepdims=True))
        return _round_bf16(_round_bf16(gt * jax.nn.sigmoid(gt)) * up)

    def ffn_chunk_chained():
        zmask = zero_s[0]

        def nothing(v):
            return pltpu.bitcast(pltpu.bitcast(v, U32) & zmask, F32)

        base = pl.multiple_of(step * (FT * 128), 128)
        link = [None, None]
        hid = {}
        for tile in range(FT):
            cols = pl.ds(base + 128 * tile, 128)
            sums = {}
            for name, w_ref in (("gate", wg_v), ("up", wu_v)):
                acc = [None, None]
                for i in range(D // 16):
                    w = w_ref[16 * i:16 * i + 16, cols].astype(F32)
                    for t in range(2):
                        pr = xb_v[t, 16 * i:16 * i + 16, :] * w
                        if i > 0:
                            lo = acc[t] + pr[0:8, :]
                        elif link[t] is None:
                            lo = pr[0:8, :]
                        else:
                            lo = pr[0:8, :] + nothing(link[t])
                        acc[t] = lo + pr[8:16, :]
                for t in range(2):
                    link[t] = acc[t]
                    sums[name, t] = acc[t]
            for t in range(2):
                hid[t, tile] = swiglu(sums["gate", t], sums["up", t])
        for b in range(D // 16):
            acc = [None, None]
            for tile in range(FT):
                w = wd_v[16 * b:16 * b + 16, pl.ds(base + 128 * tile, 128)].astype(F32)
                for t in range(2):
                    pr = w * hid[t, tile]
                    if tile == 0:
                        lo = pr[0:8, :] + nothing(link[t])
                        acc[t] = [lo, pr[8:16, :] + nothing(lo)]
                    else:
                        acc[t] = [acc[t][0] + pr[0:8, :], acc[t][1] + pr[8:16, :]]
            for t in range(2):
                rows = slice(16 * b, 16 * b + 16)
                y_v[t, rows, :] = y_v[t, rows, :] + jnp.concatenate(acc[t], axis=0)
                link[t] = acc[t][1]

    def ffn_chunk_looped():
        base = step * (FT * 128)

        def gate_up(tile, carry):
            cols = pl.ds(pl.multiple_of(base + 128 * tile, 128), 128)
            wg = wg_v[:, cols].astype(F32)
            wu = wu_v[:, cols].astype(F32)
            for t in range(2):
                h = swiglu(xb_v[t] * wg, xb_v[t] * wu)
                hid_v[t, tile] = jnp.broadcast_to(h, (8, 128))
            return carry

        def down(tile, carry):
            cols = pl.ds(pl.multiple_of(base + 128 * tile, 128), 128)
            w = wd_v[:, cols].astype(F32)
            for t in range(2):
                y_v[t] = y_v[t] + w * hid_v[t, tile][0:1, :]
            return carry

        lax.fori_loop(0, FT, gate_up, 0)
        lax.fori_loop(0, FT, down, 0)

    def masked_q_bits(g, hp, j):
        rid = _iota((64, 128), 0)
        mask = (rid >= (DH // 2) * hp) & (rid < (DH // 2) * (hp + 1))
        return jnp.where(mask, qt_v[_rows(step * NG + g, 64), 128 * j:128 * (j + 1)],
                         jnp.uint32(0))

    def keys(g, lo, hi):
        first = pl.multiple_of((step * NG + g) * (L // 2) + lo // 2, 8)
        return _unpack(k_v[pl.ds(first, (hi - lo) // 2), :])

    def causal_scores(g, hp, j):
        nk = 128 * (j + 1)
        st = _dot(keys(g, 0, nk), _unpack(masked_q_bits(g, hp, j)))
        diag = st[nk - 128:, :] + bias_v[...]
        return diag if j == 0 else jnp.concatenate([st[:nk - 128, :], diag], axis=0)

    def head_output(h, j, p, keep):
        o = _dot(_unpack(vt_v[_rows(step * H + h, 16), 0:128 * (j + 1)]), p)
        den = o[DH:DH + 1, :]
        inv = pl.reciprocal(den, approx=True)
        inv = inv * (2.0 - den * inv)
        return o[0:24, :] * (keep * inv)

    def single_probs(h, j):
        return jnp.exp2(causal_scores(*divmod(h, HPG), j)).astype(BF16)

    def pair_probs(pairs, j, flip):
        low = _iota((64, 128), 1) < 64
        qa, qb = {}, {}
        for h in pairs:
            g, hp = divmod(h, HPG)
            qa[h] = masked_q_bits(g, hp, j)
            qb[h] = pltpu.roll(masked_q_bits(g, hp + 1, j), 64, 1)
        off = {}
        if j > 0:
            for h in pairs:
                g = h // HPG
                for hh, q in ((h, qa[h]), (h + 1, qb[h])):
                    off[hh] = jnp.exp2(_dot(keys(g, 0, 128 * j), _unpack(q)))
        early, late = {}, {}
        for h in pairs:
            g = h // HPG
            k0 = 128 * j
            for which in ((0, 1) if flip else (1, 0)):
                if which == 0:
                    early[h] = _dot(keys(g, k0, k0 + 64),
                                    _unpack(jnp.where(low, qa[h], qb[h])))
                else:
                    late[h] = _dot(keys(g, k0, k0 + 128),
                                   _unpack(jnp.where(low, qb[h], qa[h])))
        probs = {}
        for h in pairs:
            p1 = jnp.exp2(early[h] + half_v[0])
            p2 = jnp.exp2(late[h][0:64, :])
            bottom = late[h][64:128, :]
            pa = jnp.concatenate(
                [jnp.where(low, p1, p2), jnp.exp2(bottom + half_v[1])], axis=0)
            pb = jnp.concatenate(
                [jnp.where(low, p2, p1), jnp.exp2(bottom + half_v[2])], axis=0)
            for hh, pd in ((h, pa), (h + 1, pb)):
                full = pd if j == 0 else jnp.concatenate([off[hh], pd], axis=0)
                probs[hh] = full.astype(BF16)
        return probs

    def attention_bounded():
        pairs = [g * HPG + hp for g in range(NG)
                 for hp in range(0, _heads_in_group(g) - 1, 2)]
        paired = set(pairs) | {h + 1 for h in pairs}
        singles = [h for h in range(H) if h not in paired]
        waves = [(pairs[i:i + 2], j) for i in range(0, len(pairs), 2) for j in range(NQT)]
        waves += [(None, j) for j in range(NQT)]

        def scores(w):
            grp, j = waves[w]
            if grp is None:
                return {h: single_probs(h, j) for h in singles}
            return pair_probs(grp, j, w % 2 == 1)

        def values(w, probs):
            grp, j = waves[w]
            for h, p in probs.items():
                o = head_output(h, j, p, 1.0 - gate_v[h:h + 1, :])
                if grp is not None and h - 1 in grp:
                    o = pltpu.roll(o, 64, 1)
                ot_v[step, DH * h:DH * (h + 1), 128 * j:128 * (j + 1)] = o[0:DH, :]

        pending = scores(0)
        for w in range(len(waves)):
            nxt = scores(w + 1) if w + 1 < len(waves) else None
            values(w, pending)
            pending = nxt
        ffn_chunk_chained()

    def attention_max_shifted():
        def one_head(h, carry):
            g = h // HPG
            hp = h - g * HPG
            keep = 1.0 - gate_v[pl.ds(h, 1), :]
            for j in range(NQT):
                st = causal_scores(g, hp, j)
                p = jnp.exp2(st - jnp.max(st, axis=0, keepdims=True)).astype(BF16)
                oh_v[h, :, 128 * j:128 * (j + 1)] = head_output(h, j, p, keep)
            return carry

        lax.fori_loop(0, H, one_head, 0)
        for h in range(H):
            ot_v[step, DH * h:DH * (h + 1), :] = oh_v[h, 0:DH, :]
        ffn_chunk_looped()

    def output_projection(seg):
        mem = jnp.where(seg > 0, mem_v[jnp.maximum(seg - 1, 0), 0:D, :], 0.0)
        heads_out = ot_v[seg, 0:D, :] + mem
        attn = _dot(_unpack(wot[...]), heads_out.astype(BF16))
        base = x_v[seg].astype(F32) + attn
        xn = _unpack(xn_v[_rows(seg, D // 2), :]).astype(F32)
        col = seg * L + _iota((1, L), 1)
        upd = None
        for t in range(2):
            y = _round_bf16(jnp.sum(y_v[t], axis=1, keepdims=True))
            rsel = jnp.full((1, 1), rsel_s[t], F32)
            y = _round_bf16(y * _round_bf16(jax.nn.sigmoid(rsel)))
            part = jnp.where(col == idx_s[t], y, 0.0)
            upd = part if upd is None else upd + part
        o_ref[...] = (base + (xn + upd)).astype(BF16)

    col_blocks = [(c0, min(128, D - c0)) for c0 in range(0, D, 128)]

    def transpose_block(w_v, section, c0, n):
        r0 = (section * D + c0) // 2
        wall[r0:r0 + n // 2, :] = pltpu.bitcast(w_v[:, c0:c0 + n].T, U32)

    def project_block(section, c0, n, xn):
        r0 = (section * D + c0) // 2
        last = section == 2 and c0 + n == D
        hi = PROWS // 2 if last else r0 + n // 2
        return _dot(_unpack(wall[r0:hi, :]), xn)

    def projections():
        xn0 = _unpack(xn_v[_rows(0, D // 2), :])
        parts = [project_block(0, c0, n, xn0) for c0, n in col_blocks[:3]]
        cp_wk.wait()
        xn0 = _unpack(xn_v[_rows(0, D // 2), :])
        parts += [project_block(0, c0, n, xn0) for c0, n in col_blocks[3:]]
        for c0, n in col_blocks:
            transpose_block(wk_v, 1, c0, n)
        cp_wv.wait()
        x_copies[1].wait()
        xn0 = _unpack(xn_v[_rows(0, D // 2), :])
        parts += [project_block(1, c0, n, xn0) for c0, n in col_blocks]
        for c0, n in col_blocks:
            transpose_block(wv_v, 2, c0, n)
            parts.append(project_block(2, c0, n, xn0))
        layer_norm(1)
        _, pk, vg = store_qkv(0, jnp.concatenate(parts, axis=0))
        x_copies[2].wait()
        x_copies[3].wait()
        cp_wo.wait()

        layer_norm(2)
        pt = project(1)
        wot[...] = pltpu.bitcast(wo_v[...].T, U32)
        state1 = memory_update(None, pk, vg)
        pq1, pk, vg = store_qkv(1, pt)
        layer_norm(3)
        pt = project(2)
        state2 = memory_update(state1, pk, vg)
        pq2, pk, vg = store_qkv(2, pt)
        pt = project(3)
        state3 = memory_update(state2, pk, vg)
        memory_retrieve(1, state1, pq1)
        memory_retrieve(2, state2, pq2)
        pq3, _, _ = store_qkv(3, pt)
        memory_retrieve(3, state3, pq3)
        route()
        cp_wg.wait()
        cp_wu.wait()
        cp_wd.wait()

    @pl.when(step == 0)
    def _():
        for cp in (cp_wq, x_copies[0], cp_wr, cp_beta, cp_wk, cp_wv, x_copies[1],
                   x_copies[2], x_copies[3], cp_wo, cp_wg, cp_wu, cp_wd):
            cp.start()
        with _scope("sc_startup"):
            cp_wr.wait()
            cp_beta.wait()
            cp_wq.wait()
            init_constants()
            for c0, n in col_blocks:
                transpose_block(wq_v, 0, c0, n)
            x_copies[0].wait()
            layer_norm(0)
        with _scope("sc_projections"):
            projections()

    @pl.when(step < NSEG)
    def _():
        safe = safe_s[step] == 1

        @pl.when(safe)
        def _():
            with _scope("sc_attention"):
                attention_bounded()

        @pl.when(jnp.logical_not(safe))
        def _():
            attention_max_shifted()

    @pl.when(step >= NSEG)
    def _():
        with _scope("sc_outproj"):
            output_projection(step - NSEG)


@jax.jit
def pallas_parallel_sum__memory_aug_infini_attn__moe_arch_mod__prompt_kernel(
    A_x: jax.Array,
    A_wq: jax.Array,
    A_wk: jax.Array,
    A_wv: jax.Array,
    A_wo: jax.Array,
    A_beta: jax.Array,
    B_x: jax.Array,
    B_w_r: jax.Array,
    B_w_gate: jax.Array,
    B_w_up: jax.Array,
    B_w_down: jax.Array,
):
    del B_x
    vm = pltpu.VMEM
    scratch = [
        vm((NSEG, D, L), BF16),
        vm((D, D), BF16),
        vm((D, D), BF16),
        vm((D, D), BF16),
        vm((D, D), BF16),
        vm((H,), BF16),
        vm((D,), BF16),
        vm((D, FF), BF16),
        vm((D, FF), BF16),
        vm((D, FF), BF16),
        vm((PROWS // 2, D), U32),
        vm((D // 2, D), U32),
        vm((NSEG * D // 2, L), U32),
        vm((NSEG * NG * 64, L), U32),
        vm((NSEG * NG * L // 2, 128), U32),
        vm((NSEG * H * 16, L), U32),
        vm((NSEG - 1, OROWS, L), F32),
        vm((8, L), F32),
        vm((2, D, 128), F32),
        vm((2, D, 128), F32),
        vm((2, FT, 8, 128), F32),
        pltpu.SMEM((2,), jnp.int32),
        pltpu.SMEM((2,), F32),
        pltpu.SMEM((1,), U32),
        pltpu.SMEM((NSEG,), jnp.int32),
        vm((H, 128), F32),
        vm((NSEG, D, L), F32),
        vm((H, 24, L), F32),
        vm((128, 128), F32),
        vm((3, 64, 128), F32),
        pltpu.SemaphoreType.DMA((NSEG + 9,)),
    ]
    hbm = pl.BlockSpec(memory_space=pltpu.HBM)
    xt = jnp.transpose(A_x.reshape(S, D))
    out_t = pl.pallas_call(
        _kernel,
        grid=(2 * NSEG,),
        in_specs=[hbm] * 10,
        out_specs=pl.BlockSpec((D, L), lambda s: (0, jnp.maximum(s - NSEG, 0))),
        out_shape=jax.ShapeDtypeStruct((D, S), BF16),
        scratch_shapes=scratch,
        compiler_params=pltpu.CompilerParams(
            dimension_semantics=("arbitrary",),
            vmem_limit_bytes=110 * 1024 * 1024,
        ),
        name="infini_moe",
    )(xt, A_wq, A_wk, A_wv, A_wo, A_beta, B_w_r, B_w_gate, B_w_up,
      jnp.transpose(B_w_down))
    return jnp.transpose(out_t).reshape(1, S, D)
```

```python
import contextlib

import jax
import jax.numpy as jnp
from jax import lax
from jax.experimental import pallas as pl
from jax.experimental.pallas import tpu as pltpu

S = 2048
D = 576
H = 32
DH = 18
NSEG = 4
L = 512
FF = 4608
NG = 5
HPG = 7
GW = HPG * DH
NQT = L // 128
PROWS = 3 * D + 16
RROW = 3 * D
PBLOCK = 128
MROWS = 144
FT = FF // 128 // NSEG
OROWS = 640
LOG2E = 1.4426950408889634
QSCALE = DH ** -0.5 * LOG2E
NEG = -1e30
SAFE_LOG2 = 40.0
LN_EPS = 1.0013580322265625e-05
F32 = jnp.float32
BF16 = jnp.bfloat16
U32 = jnp.uint32

PROFILE_SCOPES = False

_NN = (((1,), (0,)), ((), ()))
_NT = (((1,), (1,)), ((), ()))


def _scope(name):
    return jax.named_scope(name) if PROFILE_SCOPES else contextlib.nullcontext()


def _dot(a, b):
    return lax.dot_general(a, b, _NN, preferred_element_type=F32)


def _dot_nt(a, b):
    return lax.dot_general(a, b, _NT, preferred_element_type=F32)


def _iota(shape, dim):
    return lax.broadcasted_iota(jnp.int32, shape, dim)


def _round_bf16(v):
    return v.astype(BF16).astype(F32)


def _pack(v):
    return pltpu.bitcast(v.astype(BF16), U32)


def _unpack(u):
    return pltpu.bitcast(u, BF16)


def _rows(index, size):
    if isinstance(index, int):
        return slice(index * size, (index + 1) * size)
    return pl.ds(pl.multiple_of(index * size, 8), size)


def _heads_in_group(g):
    return HPG if g < NG - 1 else H - HPG * (NG - 1)


def _phi(t):
    return jnp.where(t > 0, t + 1.0, jnp.exp(t))


def _kernel(x_hbm, wq_hbm, wk_hbm, wv_hbm, wo_hbm, beta_hbm, wr_hbm,
            wg_hbm, wu_hbm, wd_hbm,
            o_ref,
            x_v, wq_v, wk_v, wv_v, wo_v, beta_v, wr_v, wg_v, wu_v, wd_v,
            wall, wot, xn_v, qt_v, k_v, vt_v, mem_v,
            r_v, xs_v, y_v, hid_v, idx_s, rsel_s, zero_s, safe_s,
            gate_v, ot_v, oh_v, bias_v, half_v,
            sems):
    step = pl.program_id(0)

    x_copies = [
        pltpu.make_async_copy(x_hbm.at[:, pl.ds(c * L, L)], x_v.at[c], sems.at[c])
        for c in range(NSEG)
    ]
    pairs = [(wq_hbm, wq_v), (wk_hbm, wk_v), (wv_hbm, wv_v), (wo_hbm, wo_v),
             (beta_hbm, beta_v), (wr_hbm, wr_v),
             (wg_hbm, wg_v), (wu_hbm, wu_v), (wd_hbm, wd_v)]
    (cp_wq, cp_wk, cp_wv, cp_wo, cp_beta, cp_wr, cp_wg, cp_wu, cp_wd) = [
        pltpu.make_async_copy(src, dst, sems.at[NSEG + i])
        for i, (src, dst) in enumerate(pairs)
    ]

    def nothing(v):
        return pltpu.bitcast(pltpu.bitcast(v, U32) & zero_s[0], F32)

    def layer_norm(c):
        for n in range(NQT):
            cols = slice(128 * n, 128 * (n + 1))
            pivot = x_v[c, 0:16, cols].astype(F32)[0:1, :]
            s1 = [None, None]
            s2 = [None, None]
            for i in range(D // 16):
                d = x_v[c, 16 * i:16 * i + 16, cols].astype(F32) - pivot
                for k in range(2):
                    dk = d[8 * k:8 * k + 8, :]
                    s1[k] = dk if s1[k] is None else s1[k] + dk
                    s2[k] = dk * dk if s2[k] is None else s2[k] + dk * dk
            dmean = jnp.sum(s1[0] + s1[1], axis=0, keepdims=True) * (1.0 / D)
            dsq = jnp.sum(s2[0] + s2[1], axis=0, keepdims=True) * (1.0 / D)
            mean = pivot + dmean
            var = jnp.maximum(dsq - dmean * dmean, 0.0)
            sd = _round_bf16(jnp.sqrt(_round_bf16(_round_bf16(var) + LN_EPS)))
            xf = x_v[c, :, cols].astype(F32)
            xn_v[_rows(c, D // 2), cols] = _pack(
                (xf - _round_bf16(mean)) * (1.0 / sd))

    def init_constants():
        gate = jax.nn.sigmoid(beta_v[...].astype(F32).reshape(1, H))
        on_diag = _iota((H, H), 0) == _iota((H, H), 1)
        gcol = jnp.sum(jnp.where(on_diag, gate, 0.0), axis=1, keepdims=True)
        gate_v[...] = jnp.broadcast_to(gcol, (H, 128))
        zero_s[0] = jnp.uint32(0)
        bias_v[...] = jnp.where(_iota((128, 128), 0) > _iota((128, 128), 1), NEG, 0.0)
        key, lane = _iota((64, 128), 0), _iota((64, 128), 1)
        future = key > (lane & 63)
        half_v[0] = jnp.where(future, NEG, 0.0)
        half_v[1] = jnp.where(future | (lane < 64), NEG, 0.0)
        half_v[2] = jnp.where(future | (lane >= 64), NEG, 0.0)
        router = jnp.broadcast_to(wr_v[...].astype(F32).reshape(1, D), (16, D))
        wall[RROW // 2:PROWS // 2, :] = _pack(
            jnp.where(_iota((16, D), 0) == 0, router, 0.0))

    def project(c, router_first=False):
        xn = _unpack(xn_v[_rows(c, D // 2), :])
        step_rows = PBLOCK // 2
        end = RROW // 2 if router_first else PROWS // 2
        tail = [_dot(_unpack(wall[end:PROWS // 2, :]), xn)] if router_first else []
        return jnp.concatenate(
            [_dot(_unpack(wall[r:min(r + step_rows, end), :]), xn)
             for r in range(0, end, step_rows)] + tail, axis=0)

    def store_qkv(c, pt):
        r_v[c:c + 1, :] = _round_bf16(pt[RROW:RROW + 1, :])
        qa = jnp.max(jnp.abs(pt[0:D, :])) * QSCALE
        ka = jnp.max(jnp.abs(pt[D:2 * D, :]))
        safe_s[c] = (qa * ka * (DH * 1.02) <= SAFE_LOG2).astype(jnp.int32)

        tail_row = _iota((8, L), 0)
        for h in range(H):
            base = 2 * D + DH * h
            tail = jnp.where(tail_row < DH - 16, pt[base + 16:base + 24, :],
                             jnp.where(tail_row == DH - 16, 1.0, 0.0))
            blk = jnp.concatenate(
                [pt[base:base + 16, :], tail, jnp.zeros((8, L), F32)], axis=0)
            vt_v[_rows(c * H + h, 16), :] = _pack(blk)

        rowl = _iota((128, L), 0)
        pqs, pks, vgs = [], [], []
        for g in range(NG):
            used = _heads_in_group(g) * DH
            qg = pt[GW * g:GW * g + 128, :]
            qt_v[_rows(c * NG + g, 64), :] = _pack(qg * QSCALE)
            kg = pt[D + GW * g:D + GW * g + 128, :]
            k_v[_rows(c * NG + g, L // 2), :] = _pack(kg.T)
            pqs.append(_phi(qg).astype(BF16))
            if c < NSEG - 1:
                pks.append(_phi(kg).astype(BF16))
                lo = 2 * D + GW * g
                if g < NG - 1:
                    vg = pt[lo:lo + 128, :]
                else:
                    vg = jnp.concatenate(
                        [pt[lo:lo + used, :], jnp.zeros((128 - used, L), F32)], axis=0)
                vg = jnp.where(rowl < used, vg, jnp.where(rowl == GW, 1.0, 0.0))
                vgs.append(vg.astype(BF16))
        return pqs, pks, vgs

    def memory_update(states, pks, vgs):
        row = _iota((128, 128), 0)
        lane = _iota((128, 128), 1)
        same_head = (row // DH) == (lane // DH)
        out = []
        for g in range(NG):
            used = _heads_in_group(g) * DH
            upd = _dot_nt(vgs[g], pks[g])
            keep = ((same_head & (row < used)) | (row == GW)) & (lane < used)
            upd = jnp.where(keep, upd, 0.0)
            out.append(upd if states is None else states[g] + upd)
        return out

    def memory_retrieve(c, states, pqs):
        row = _iota((128, 128), 0)
        row8 = _iota((8, 128), 0)
        lane8 = _iota((8, 128), 1) // DH
        for g in range(NG):
            nh = _heads_in_group(g)
            st = states[g]
            mrows = jnp.where(row < GW, st, 0.0)
            zrows = jnp.where(lane8 == row8, st[GW:GW + 1, :], 0.0)
            lhs = jnp.concatenate(
                [mrows, zrows, jnp.zeros((8, 128), F32)], axis=0).astype(BF16)
            ret = _dot(lhs, pqs[g])
            gsel = gate_v[HPG * g:HPG * g + 8, :] if g < NG - 1 else jnp.concatenate(
                [gate_v[HPG * g:H, :], jnp.zeros((8 - nh, 128), F32)], axis=0)
            gwide = jnp.concatenate([gsel] * NQT, axis=1)
            scale = gwide / (ret[128:136, :] + 1e-6)
            pieces = []
            for b in range(16):
                h0 = min((8 * b) // DH, nh - 1)
                h1 = min((8 * b + 7) // DH, nh - 1)
                sc = scale[h0:h0 + 1, :]
                if h1 != h0:
                    first = _iota((8, L), 0) < DH * h1 - 8 * b
                    sc = jnp.where(first, sc, scale[h1:h1 + 1, :])
                pieces.append(ret[8 * b:8 * b + 8, :] * sc)
            mem_v[c - 1, GW * g:GW * g + 128, :] = jnp.concatenate(pieces, axis=0)

    def route():
        r = r_v[0:NSEG, :]
        idx = _iota((NSEG, L), 0) * L + _iota((NSEG, L), 1)
        m1 = jnp.max(r)
        i1 = jnp.clip(jnp.min(jnp.where(r == m1, idx, S)), 0, S - 1)
        r2 = jnp.where(idx == i1, -jnp.inf, r)
        m2 = jnp.max(r2)
        i2 = jnp.clip(jnp.min(jnp.where(r2 == m2, idx, S)), 0, S - 1)
        idx_s[0] = i1
        idx_s[1] = i2
        rsel_s[0] = m1
        rsel_s[1] = m2
        row16 = _iota((16, 128), 0)
        lane16 = _iota((16, 128), 1)
        xs = None
        for t, i in enumerate((i1, i2)):
            seg = i // L
            off = i - seg * L
            base = pl.multiple_of((off // 128) * 128, 128)
            cols = _unpack(xn_v[_rows(seg, D // 2), pl.ds(base, 128)])
            pick = jnp.where((row16 == t) & (lane16 == off - base), 1.0, 0.0)
            part = _dot_nt(pick.astype(BF16), cols)
            xs = part if xs is None else xs + part
        xs_v[...] = _pack(xs)
        y_v[...] = jnp.zeros(y_v.shape, F32)

    def ffn_hidden():
        xs = _unpack(xs_v[...])
        gt = _round_bf16(_dot(xs, wg_v[...]))
        up = _round_bf16(_dot(xs, wu_v[...]))
        hid = _round_bf16(_round_bf16(gt * jax.nn.sigmoid(gt)) * up)
        for t in range(2):
            for tile in range(FF // 128):
                hid_v[t, tile] = jnp.broadcast_to(
                    hid[t:t + 1, 128 * tile:128 * (tile + 1)], (8, 128))

    def ffn_down_chained():
        base = pl.multiple_of(step * (FT * 128), 128)
        link = [None, None]
        for b in range(D // 8):
            acc = [None, None]
            for tile in range(FT):
                w = wd_v[8 * b:8 * b + 8, pl.ds(base + 128 * tile, 128)].astype(F32)
                for t in range(2):
                    pr = w * hid_v[t, step * FT + tile]
                    if tile > 0:
                        acc[t] = acc[t] + pr
                    else:
                        acc[t] = pr if link[t] is None else pr + nothing(link[t])
            for t in range(2):
                rows = slice(8 * b, 8 * b + 8)
                y_v[t, rows, :] = y_v[t, rows, :] + acc[t]
                link[t] = acc[t]

    def ffn_down_looped():
        def down(tile, carry):
            col = step * FT + tile
            w = wd_v[:, pl.ds(pl.multiple_of(128 * col, 128), 128)].astype(F32)
            for t in range(2):
                y_v[t] = y_v[t] + w * hid_v[t, col][0:1, :]
            return carry

        lax.fori_loop(0, FT, down, 0)

    def masked_q_bits(g, hp, j):
        rid = _iota((64, 128), 0)
        mask = (rid >= (DH // 2) * hp) & (rid < (DH // 2) * (hp + 1))
        return jnp.where(mask, qt_v[_rows(step * NG + g, 64), 128 * j:128 * (j + 1)],
                         jnp.uint32(0))

    def keys(g, lo, hi):
        first = pl.multiple_of((step * NG + g) * (L // 2) + lo // 2, 8)
        return _unpack(k_v[pl.ds(first, (hi - lo) // 2), :])

    def causal_scores(g, hp, j):
        nk = 128 * (j + 1)
        st = _dot(keys(g, 0, nk), _unpack(masked_q_bits(g, hp, j)))
        diag = st[nk - 128:, :] + bias_v[...]
        return diag if j == 0 else jnp.concatenate([st[:nk - 128, :], diag], axis=0)

    def head_output(h, j, p, keep):
        o = _dot(_unpack(vt_v[_rows(step * H + h, 16), 0:128 * (j + 1)]), p)
        den = o[DH:DH + 1, :]
        inv = pl.reciprocal(den, approx=True)
        inv = inv * (2.0 - den * inv)
        return o[0:24, :] * (keep * inv)

    def single_probs(h, j):
        return jnp.exp2(causal_scores(*divmod(h, HPG), j)).astype(BF16)

    def pair_probs(pairs, j, flip):
        low = _iota((64, 128), 1) < 64
        qa, qb = {}, {}
        for h in pairs:
            g, hp = divmod(h, HPG)
            qa[h] = masked_q_bits(g, hp, j)
            qb[h] = pltpu.roll(masked_q_bits(g, hp + 1, j), 64, 1)
        off = {}
        if j > 0:
            for h in pairs:
                g = h // HPG
                for hh, q in ((h, qa[h]), (h + 1, qb[h])):
                    off[hh] = jnp.exp2(_dot(keys(g, 0, 128 * j), _unpack(q)))
        early, late = {}, {}
        for h in pairs:
            g = h // HPG
            k0 = 128 * j
            for which in ((0, 1) if flip else (1, 0)):
                if which == 0:
                    early[h] = _dot(keys(g, k0, k0 + 64),
                                    _unpack(jnp.where(low, qa[h], qb[h])))
                else:
                    late[h] = _dot(keys(g, k0, k0 + 128),
                                   _unpack(jnp.where(low, qb[h], qa[h])))
        probs = {}
        for h in pairs:
            p1 = jnp.exp2(early[h] + half_v[0])
            p2 = jnp.exp2(late[h][0:64, :])
            bottom = late[h][64:128, :]
            pa = jnp.concatenate(
                [jnp.where(low, p1, p2), jnp.exp2(bottom + half_v[1])], axis=0)
            pb = jnp.concatenate(
                [jnp.where(low, p2, p1), jnp.exp2(bottom + half_v[2])], axis=0)
            for hh, pd in ((h, pa), (h + 1, pb)):
                full = pd if j == 0 else jnp.concatenate([off[hh], pd], axis=0)
                probs[hh] = full.astype(BF16)
        return probs

    def attention_bounded():
        pairs = [g * HPG + hp for g in range(NG)
                 for hp in range(0, _heads_in_group(g) - 1, 2)]
        paired = set(pairs) | {h + 1 for h in pairs}
        singles = [h for h in range(H) if h not in paired]
        waves = [(pairs[i:i + 2], j) for i in range(0, len(pairs), 2) for j in range(NQT)]
        waves += [(None, j) for j in range(NQT)]

        def scores(w):
            grp, j = waves[w]
            if grp is None:
                return {h: single_probs(h, j) for h in singles}
            return pair_probs(grp, j, w % 2 == 1)

        def values(w, probs):
            grp, j = waves[w]
            for h, p in probs.items():
                o = head_output(h, j, p, 1.0 - gate_v[h:h + 1, :])
                if grp is not None and h - 1 in grp:
                    o = pltpu.roll(o, 64, 1)
                ot_v[step, DH * h:DH * (h + 1), 128 * j:128 * (j + 1)] = o[0:DH, :]

        pending = scores(0)
        for w in range(len(waves)):
            nxt = scores(w + 1) if w + 1 < len(waves) else None
            values(w, pending)
            pending = nxt
        ffn_down_chained()

    def attention_max_shifted():
        def one_head(h, carry):
            g = h // HPG
            hp = h - g * HPG
            keep = 1.0 - gate_v[pl.ds(h, 1), :]
            for j in range(NQT):
                st = causal_scores(g, hp, j)
                p = jnp.exp2(st - jnp.max(st, axis=0, keepdims=True)).astype(BF16)
                oh_v[h, :, 128 * j:128 * (j + 1)] = head_output(h, j, p, keep)
            return carry

        lax.fori_loop(0, H, one_head, 0)
        for h in range(H):
            ot_v[step, DH * h:DH * (h + 1), :] = oh_v[h, 0:DH, :]
        ffn_down_looped()

    def output_projection(seg):
        mem = jnp.where(seg > 0, mem_v[jnp.maximum(seg - 1, 0), 0:D, :], 0.0)
        heads_out = ot_v[seg, 0:D, :] + mem
        attn = _dot(_unpack(wot[...]), heads_out.astype(BF16))
        base = x_v[seg].astype(F32) + attn
        xn = _unpack(xn_v[_rows(seg, D // 2), :]).astype(F32)
        col = seg * L + _iota((1, L), 1)
        upd = None
        for t in range(2):
            y = _round_bf16(jnp.sum(y_v[t], axis=1, keepdims=True))
            rsel = jnp.full((1, 1), rsel_s[t], F32)
            y = _round_bf16(y * _round_bf16(jax.nn.sigmoid(rsel)))
            part = jnp.where(col == idx_s[t], y, 0.0)
            upd = part if upd is None else upd + part
        o_ref[...] = (base + (xn + upd)).astype(BF16)

    col_blocks = [(c0, min(128, D - c0)) for c0 in range(0, D, 128)]

    def transpose_block(w_v, section, c0, n):
        r0 = (section * D + c0) // 2
        wall[r0:r0 + n // 2, :] = pltpu.bitcast(w_v[:, c0:c0 + n].T, U32)

    def project_block(section, c0, n, xn):
        r0 = (section * D + c0) // 2
        last = section == 2 and c0 + n == D
        hi = PROWS // 2 if last else r0 + n // 2
        return _dot(_unpack(wall[r0:hi, :]), xn)

    def projections():
        xn0 = _unpack(xn_v[_rows(0, D // 2), :])
        parts = [project_block(0, c0, n, xn0) for c0, n in col_blocks[:3]]
        cp_wk.wait()
        xn0 = _unpack(xn_v[_rows(0, D // 2), :])
        parts += [project_block(0, c0, n, xn0) for c0, n in col_blocks[3:]]
        for c0, n in col_blocks:
            transpose_block(wk_v, 1, c0, n)
        cp_wv.wait()
        x_copies[1].wait()
        xn0 = _unpack(xn_v[_rows(0, D // 2), :])
        parts += [project_block(1, c0, n, xn0) for c0, n in col_blocks]
        for c0, n in col_blocks:
            transpose_block(wv_v, 2, c0, n)
            parts.append(project_block(2, c0, n, xn0))
        layer_norm(1)
        _, pk, vg = store_qkv(0, jnp.concatenate(parts, axis=0))
        x_copies[2].wait()
        x_copies[3].wait()
        cp_wo.wait()

        layer_norm(2)
        pt = project(1)
        wot[...] = pltpu.bitcast(wo_v[...].T, U32)
        state1 = memory_update(None, pk, vg)
        pq1, pk, vg = store_qkv(1, pt)
        layer_norm(3)
        pt = project(2)
        state2 = memory_update(state1, pk, vg)
        pq2, pk, vg = store_qkv(2, pt)
        cp_wg.wait()
        cp_wu.wait()
        pt = project(3, router_first=True)
        pq3, _, _ = store_qkv(3, pt)
        route()
        ffn_hidden()
        state3 = memory_update(state2, pk, vg)
        memory_retrieve(1, state1, pq1)
        memory_retrieve(2, state2, pq2)
        memory_retrieve(3, state3, pq3)
        cp_wd.wait()

    @pl.when(step == 0)
    def _():
        for cp in (cp_wq, x_copies[0], cp_wr, cp_beta, cp_wk, cp_wv, x_copies[1],
                   x_copies[2], x_copies[3], cp_wo, cp_wg, cp_wu, cp_wd):
            cp.start()
        with _scope("sc_startup"):
            cp_wr.wait()
            cp_beta.wait()
            cp_wq.wait()
            init_constants()
            for c0, n in col_blocks:
                transpose_block(wq_v, 0, c0, n)
            x_copies[0].wait()
            layer_norm(0)
        with _scope("sc_projections"):
            projections()

    @pl.when(step < NSEG)
    def _():
        safe = safe_s[step] == 1

        @pl.when(safe)
        def _():
            with _scope("sc_attention"):
                attention_bounded()

        @pl.when(jnp.logical_not(safe))
        def _():
            attention_max_shifted()

    @pl.when(step >= NSEG)
    def _():
        with _scope("sc_outproj"):
            output_projection(step - NSEG)


@jax.jit
def pallas_parallel_sum__memory_aug_infini_attn__moe_arch_mod__prompt_kernel(
    A_x: jax.Array,
    A_wq: jax.Array,
    A_wk: jax.Array,
    A_wv: jax.Array,
    A_wo: jax.Array,
    A_beta: jax.Array,
    B_x: jax.Array,
    B_w_r: jax.Array,
    B_w_gate: jax.Array,
    B_w_up: jax.Array,
    B_w_down: jax.Array,
):
    del B_x
    vm = pltpu.VMEM
    scratch = [
        vm((NSEG, D, L), BF16),
        vm((D, D), BF16),
        vm((D, D), BF16),
        vm((D, D), BF16),
        vm((D, D), BF16),
        vm((H,), BF16),
        vm((D,), BF16),
        vm((D, FF), BF16),
        vm((D, FF), BF16),
        vm((D, FF), BF16),
        vm((PROWS // 2, D), U32),
        vm((D // 2, D), U32),
        vm((NSEG * D // 2, L), U32),
        vm((NSEG * NG * 64, L), U32),
        vm((NSEG * NG * L // 2, 128), U32),
        vm((NSEG * H * 16, L), U32),
        vm((NSEG - 1, OROWS, L), F32),
        vm((8, L), F32),
        vm((8, D), U32),
        vm((2, D, 128), F32),
        vm((2, FF // 128, 8, 128), F32),
        pltpu.SMEM((2,), jnp.int32),
        pltpu.SMEM((2,), F32),
        pltpu.SMEM((1,), U32),
        pltpu.SMEM((NSEG,), jnp.int32),
        vm((H, 128), F32),
        vm((NSEG, D, L), F32),
        vm((H, 24, L), F32),
        vm((128, 128), F32),
        vm((3, 64, 128), F32),
        pltpu.SemaphoreType.DMA((NSEG + 9,)),
    ]
    hbm = pl.BlockSpec(memory_space=pltpu.HBM)
    xt = jnp.transpose(A_x.reshape(S, D))
    out_t = pl.pallas_call(
        _kernel,
        grid=(2 * NSEG,),
        in_specs=[hbm] * 10,
        out_specs=pl.BlockSpec((D, L), lambda s: (0, jnp.maximum(s - NSEG, 0))),
        out_shape=jax.ShapeDtypeStruct((D, S), BF16),
        scratch_shapes=scratch,
        compiler_params=pltpu.CompilerParams(
            dimension_semantics=("arbitrary",),
            vmem_limit_bytes=110 * 1024 * 1024,
        ),
        name="infini_moe",
    )(xt, A_wq, A_wk, A_wv, A_wo, A_beta, B_w_r, B_w_gate, B_w_up,
      jnp.transpose(B_w_down))
    return jnp.transpose(out_t).reshape(1, S, D)
```

```python
import contextlib

import jax
import jax.numpy as jnp
from jax import lax
from jax.experimental import pallas as pl
from jax.experimental.pallas import tpu as pltpu

S = 2048
D = 576
H = 32
DH = 18
NSEG = 4
L = 512
FF = 4608
NG = 5
HPG = 7
GW = HPG * DH
NQT = L // 128
PROWS = 3 * D + 16
RROW = 3 * D
PBLOCK = 128
MROWS = 144
FT = FF // 128 // NSEG
OROWS = 640
LOG2E = 1.4426950408889634
QSCALE = DH ** -0.5 * LOG2E
NEG = -1e30
LN_EPS = 1.0013580322265625e-05
F32 = jnp.float32
BF16 = jnp.bfloat16
U32 = jnp.uint32

PROFILE_SCOPES = False

_NN = (((1,), (0,)), ((), ()))
_NT = (((1,), (1,)), ((), ()))


def _scope(name):
    return jax.named_scope(name) if PROFILE_SCOPES else contextlib.nullcontext()


def _dot(a, b):
    return lax.dot_general(a, b, _NN, preferred_element_type=F32)


def _dot_nt(a, b):
    return lax.dot_general(a, b, _NT, preferred_element_type=F32)


def _iota(shape, dim):
    return lax.broadcasted_iota(jnp.int32, shape, dim)


def _round_bf16(v):
    return v.astype(BF16).astype(F32)


def _pack(v):
    return pltpu.bitcast(v.astype(BF16), U32)


def _unpack(u):
    return pltpu.bitcast(u, BF16)


def _rows(index, size):
    if isinstance(index, int):
        return slice(index * size, (index + 1) * size)
    return pl.ds(pl.multiple_of(index * size, 8), size)


def _heads_in_group(g):
    return HPG if g < NG - 1 else H - HPG * (NG - 1)


def _phi(t):
    return jnp.where(t > 0, t + 1.0, jnp.exp(t))


def _kernel(x_hbm, wq_hbm, wk_hbm, wv_hbm, wo_hbm, beta_hbm, wr_hbm,
            wg_hbm, wu_hbm, wd_hbm,
            o_ref,
            x_v, wq_v, wk_v, wv_v, wo_v, beta_v, wr_v, wg_v, wu_v, wd_v,
            wall, wot, xn_v, qt_v, k_v, vt_v, mem_v,
            r_v, xs_v, y_v, hid_v, idx_s, rsel_s, zero_s, safe_s,
            gate_v, ot_v, oh_v, bias_v, half_v,
            sems):
    step = pl.program_id(0)

    x_copies = [
        pltpu.make_async_copy(x_hbm.at[:, pl.ds(c * L, L)], x_v.at[c], sems.at[c])
        for c in range(NSEG)
    ]
    pairs = [(wq_hbm, wq_v), (wk_hbm, wk_v), (wv_hbm, wv_v), (wo_hbm, wo_v),
             (beta_hbm, beta_v), (wr_hbm, wr_v),
             (wg_hbm, wg_v), (wu_hbm, wu_v), (wd_hbm, wd_v)]
    (cp_wq, cp_wk, cp_wv, cp_wo, cp_beta, cp_wr, cp_wg, cp_wu, cp_wd) = [
        pltpu.make_async_copy(src, dst, sems.at[NSEG + i])
        for i, (src, dst) in enumerate(pairs)
    ]

    def nothing(v):
        return pltpu.bitcast(pltpu.bitcast(v, U32) & zero_s[0], F32)

    def layer_norm(c):
        for n in range(NQT):
            cols = slice(128 * n, 128 * (n + 1))
            pivot = x_v[c, 0:16, cols].astype(F32)[0:1, :]
            s1 = [None, None]
            s2 = [None, None]
            for i in range(D // 16):
                d = x_v[c, 16 * i:16 * i + 16, cols].astype(F32) - pivot
                for k in range(2):
                    dk = d[8 * k:8 * k + 8, :]
                    s1[k] = dk if s1[k] is None else s1[k] + dk
                    s2[k] = dk * dk if s2[k] is None else s2[k] + dk * dk
            dmean = jnp.sum(s1[0] + s1[1], axis=0, keepdims=True) * (1.0 / D)
            dsq = jnp.sum(s2[0] + s2[1], axis=0, keepdims=True) * (1.0 / D)
            mean = pivot + dmean
            var = jnp.maximum(dsq - dmean * dmean, 0.0)
            sd = _round_bf16(jnp.sqrt(_round_bf16(_round_bf16(var) + LN_EPS)))
            xf = x_v[c, :, cols].astype(F32)
            xn_v[_rows(c, D // 2), cols] = _pack(
                (xf - _round_bf16(mean)) * (1.0 / sd))

    def init_constants():
        gate = jax.nn.sigmoid(beta_v[...].astype(F32).reshape(1, H))
        on_diag = _iota((H, H), 0) == _iota((H, H), 1)
        gcol = jnp.sum(jnp.where(on_diag, gate, 0.0), axis=1, keepdims=True)
        gate_v[...] = jnp.broadcast_to(gcol, (H, 128))
        zero_s[0] = jnp.uint32(0)
        bias_v[...] = jnp.where(_iota((128, 128), 0) > _iota((128, 128), 1), NEG, 0.0)
        key, lane = _iota((64, 128), 0), _iota((64, 128), 1)
        future = key > (lane & 63)
        half_v[0] = jnp.where(future, NEG, 0.0)
        half_v[1] = jnp.where(future | (lane < 64), NEG, 0.0)
        half_v[2] = jnp.where(future | (lane >= 64), NEG, 0.0)
        router = jnp.broadcast_to(wr_v[...].astype(F32).reshape(1, D), (16, D))
        wall[RROW // 2:PROWS // 2, :] = _pack(
            jnp.where(_iota((16, D), 0) == 0, router, 0.0))

    def project(c, router_first=False):
        xn = _unpack(xn_v[_rows(c, D // 2), :])
        step_rows = PBLOCK // 2
        end = RROW // 2 if router_first else PROWS // 2
        tail = [_dot(_unpack(wall[end:PROWS // 2, :]), xn)] if router_first else []
        return jnp.concatenate(
            [_dot(_unpack(wall[r:min(r + step_rows, end), :]), xn)
             for r in range(0, end, step_rows)] + tail, axis=0)

    seen = [None]

    def record_logit_bound():
        big = (seen[0] >> 30) & 1
        safe_s[0] = (jnp.max(big.astype(jnp.int32)) == 0).astype(jnp.int32)

    def store_qkv(c, pt):
        r_v[c:c + 1, :] = _round_bf16(pt[RROW:RROW + 1, :])
        tail_row = _iota((8, L), 0)
        for h in range(H):
            base = 2 * D + DH * h
            tail = jnp.where(tail_row < DH - 16, pt[base + 16:base + 24, :],
                             jnp.where(tail_row == DH - 16, 1.0, 0.0))
            blk = jnp.concatenate(
                [pt[base:base + 16, :], tail, jnp.zeros((8, L), F32)], axis=0)
            vt_v[_rows(c * H + h, 16), :] = _pack(blk)

        rowl = _iota((128, L), 0)
        pqs, pks, vgs = [], [], []
        for g in range(NG):
            used = _heads_in_group(g) * DH
            qg = pt[GW * g:GW * g + 128, :]
            qs = qg * QSCALE
            qt_v[_rows(c * NG + g, 64), :] = _pack(qs)
            kg = pt[D + GW * g:D + GW * g + 128, :]
            for operand in (qs, kg):
                bits = pltpu.bitcast(operand, U32)
                for blk in range(0, 128, 8):
                    for col in range(0, L, 128):
                        piece = bits[blk:blk + 8, col:col + 128]
                        seen[0] = piece if seen[0] is None else seen[0] | piece
            k_v[_rows(c * NG + g, L // 2), :] = _pack(kg.T)
            pqs.append(_phi(qg).astype(BF16))
            if c < NSEG - 1:
                pks.append(_phi(kg).astype(BF16))
                lo = 2 * D + GW * g
                if g < NG - 1:
                    vg = pt[lo:lo + 128, :]
                else:
                    vg = jnp.concatenate(
                        [pt[lo:lo + used, :], jnp.zeros((128 - used, L), F32)], axis=0)
                vg = jnp.where(rowl < used, vg, jnp.where(rowl == GW, 1.0, 0.0))
                vgs.append(vg.astype(BF16))
        return pqs, pks, vgs

    def memory_update(states, pks, vgs):
        row = _iota((128, 128), 0)
        lane = _iota((128, 128), 1)
        same_head = (row // DH) == (lane // DH)
        out = []
        for g in range(NG):
            used = _heads_in_group(g) * DH
            upd = _dot_nt(vgs[g], pks[g])
            keep = ((same_head & (row < used)) | (row == GW)) & (lane < used)
            upd = jnp.where(keep, upd, 0.0)
            out.append(upd if states is None else states[g] + upd)
        return out

    def memory_retrieve(c, states, pqs):
        row = _iota((128, 128), 0)
        row8 = _iota((8, 128), 0)
        lane8 = _iota((8, 128), 1) // DH
        for g in range(NG):
            nh = _heads_in_group(g)
            st = states[g]
            mrows = jnp.where(row < GW, st, 0.0)
            zrows = jnp.where(lane8 == row8, st[GW:GW + 1, :], 0.0)
            lhs = jnp.concatenate(
                [mrows, zrows, jnp.zeros((8, 128), F32)], axis=0).astype(BF16)
            ret = _dot(lhs, pqs[g])
            gsel = gate_v[HPG * g:HPG * g + 8, :] if g < NG - 1 else jnp.concatenate(
                [gate_v[HPG * g:H, :], jnp.zeros((8 - nh, 128), F32)], axis=0)
            gwide = jnp.concatenate([gsel] * NQT, axis=1)
            scale = gwide / (ret[128:136, :] + 1e-6)
            pieces = []
            for b in range(16):
                h0 = min((8 * b) // DH, nh - 1)
                h1 = min((8 * b + 7) // DH, nh - 1)
                sc = scale[h0:h0 + 1, :]
                if h1 != h0:
                    first = _iota((8, L), 0) < DH * h1 - 8 * b
                    sc = jnp.where(first, sc, scale[h1:h1 + 1, :])
                pieces.append(ret[8 * b:8 * b + 8, :] * sc)
            mem_v[c - 1, GW * g:GW * g + 128, :] = jnp.concatenate(pieces, axis=0)

    def route():
        r = r_v[0:NSEG, :]
        idx = _iota((NSEG, L), 0) * L + _iota((NSEG, L), 1)
        m1 = jnp.max(r)
        i1 = jnp.clip(jnp.min(jnp.where(r == m1, idx, S)), 0, S - 1)
        r2 = jnp.where(idx == i1, -jnp.inf, r)
        m2 = jnp.max(r2)
        i2 = jnp.clip(jnp.min(jnp.where(r2 == m2, idx, S)), 0, S - 1)
        idx_s[0] = i1
        idx_s[1] = i2
        rsel_s[0] = m1
        rsel_s[1] = m2
        row16 = _iota((16, 128), 0)
        lane16 = _iota((16, 128), 1)
        xs = None
        for t, i in enumerate((i1, i2)):
            seg = i // L
            off = i - seg * L
            base = pl.multiple_of((off // 128) * 128, 128)
            cols = _unpack(xn_v[_rows(seg, D // 2), pl.ds(base, 128)])
            pick = jnp.where((row16 == t) & (lane16 == off - base), 1.0, 0.0)
            part = _dot_nt(pick.astype(BF16), cols)
            xs = part if xs is None else xs + part
        xs_v[...] = _pack(xs)
        y_v[...] = jnp.zeros(y_v.shape, F32)

    def ffn_hidden():
        xs = _unpack(xs_v[...])
        gt = _round_bf16(_dot(xs, wg_v[...]))
        up = _round_bf16(_dot(xs, wu_v[...]))
        hid = _round_bf16(_round_bf16(gt * jax.nn.sigmoid(gt)) * up)
        for t in range(2):
            for tile in range(FF // 128):
                hid_v[t, tile] = jnp.broadcast_to(
                    hid[t:t + 1, 128 * tile:128 * (tile + 1)], (8, 128))

    def ffn_down_chained():
        base = pl.multiple_of(step * (FT * 128), 128)
        link = [None, None]
        for b in range(D // 8):
            acc = [None, None]
            for tile in range(FT):
                w = wd_v[8 * b:8 * b + 8, pl.ds(base + 128 * tile, 128)].astype(F32)
                for t in range(2):
                    pr = w * hid_v[t, step * FT + tile]
                    if tile > 0:
                        acc[t] = acc[t] + pr
                    else:
                        acc[t] = pr if link[t] is None else pr + nothing(link[t])
            for t in range(2):
                rows = slice(8 * b, 8 * b + 8)
                y_v[t, rows, :] = y_v[t, rows, :] + acc[t]
                link[t] = acc[t]

    def ffn_down_looped():
        def down(tile, carry):
            col = step * FT + tile
            w = wd_v[:, pl.ds(pl.multiple_of(128 * col, 128), 128)].astype(F32)
            for t in range(2):
                y_v[t] = y_v[t] + w * hid_v[t, col][0:1, :]
            return carry

        lax.fori_loop(0, FT, down, 0)

    def masked_q_bits(g, hp, j):
        rid = _iota((64, 128), 0)
        mask = (rid >= (DH // 2) * hp) & (rid < (DH // 2) * (hp + 1))
        return jnp.where(mask, qt_v[_rows(step * NG + g, 64), 128 * j:128 * (j + 1)],
                         jnp.uint32(0))

    def keys(g, lo, hi):
        first = pl.multiple_of((step * NG + g) * (L // 2) + lo // 2, 8)
        return _unpack(k_v[pl.ds(first, (hi - lo) // 2), :])

    def causal_scores(g, hp, j):
        nk = 128 * (j + 1)
        st = _dot(keys(g, 0, nk), _unpack(masked_q_bits(g, hp, j)))
        diag = st[nk - 128:, :] + bias_v[...]
        return diag if j == 0 else jnp.concatenate([st[:nk - 128, :], diag], axis=0)

    def head_output(h, j, p, keep):
        o = _dot(_unpack(vt_v[_rows(step * H + h, 16), 0:128 * (j + 1)]), p)
        den = o[DH:DH + 1, :]
        inv = pl.reciprocal(den, approx=True)
        inv = inv * (2.0 - den * inv)
        return o[0:24, :] * (keep * inv)

    def single_probs(h, j):
        return jnp.exp2(causal_scores(*divmod(h, HPG), j)).astype(BF16)

    def pair_probs(pairs, j, flip):
        low = _iota((64, 128), 1) < 64
        qa, qb = {}, {}
        for h in pairs:
            g, hp = divmod(h, HPG)
            qa[h] = masked_q_bits(g, hp, j)
            qb[h] = pltpu.roll(masked_q_bits(g, hp + 1, j), 64, 1)
        off = {}
        if j > 0:
            for h in pairs:
                g = h // HPG
                for hh, q in ((h, qa[h]), (h + 1, qb[h])):
                    off[hh] = jnp.exp2(_dot(keys(g, 0, 128 * j), _unpack(q)))
        early, late = {}, {}
        for h in pairs:
            g = h // HPG
            k0 = 128 * j
            for which in ((0, 1) if flip else (1, 0)):
                if which == 0:
                    early[h] = _dot(keys(g, k0, k0 + 64),
                                    _unpack(jnp.where(low, qa[h], qb[h])))
                else:
                    late[h] = _dot(keys(g, k0, k0 + 128),
                                   _unpack(jnp.where(low, qb[h], qa[h])))
        probs = {}
        for h in pairs:
            p1 = jnp.exp2(early[h] + half_v[0])
            p2 = jnp.exp2(late[h][0:64, :])
            bottom = late[h][64:128, :]
            pa = jnp.concatenate(
                [jnp.where(low, p1, p2), jnp.exp2(bottom + half_v[1])], axis=0)
            pb = jnp.concatenate(
                [jnp.where(low, p2, p1), jnp.exp2(bottom + half_v[2])], axis=0)
            for hh, pd in ((h, pa), (h + 1, pb)):
                full = pd if j == 0 else jnp.concatenate([off[hh], pd], axis=0)
                probs[hh] = full.astype(BF16)
        return probs

    def attention_bounded():
        pairs = [g * HPG + hp for g in range(NG)
                 for hp in range(0, _heads_in_group(g) - 1, 2)]
        paired = set(pairs) | {h + 1 for h in pairs}
        singles = [h for h in range(H) if h not in paired]
        waves = [(pairs[i:i + 2], j) for i in range(0, len(pairs), 2) for j in range(NQT)]
        waves += [(None, j) for j in range(NQT)]

        def scores(w):
            grp, j = waves[w]
            if grp is None:
                return {h: single_probs(h, j) for h in singles}
            return pair_probs(grp, j, w % 2 == 1)

        def values(w, probs):
            grp, j = waves[w]
            for h, p in probs.items():
                o = head_output(h, j, p, 1.0 - gate_v[h:h + 1, :])
                if grp is not None and h - 1 in grp:
                    o = pltpu.roll(o, 64, 1)
                ot_v[step, DH * h:DH * (h + 1), 128 * j:128 * (j + 1)] = o[0:DH, :]

        pending = scores(0)
        for w in range(len(waves)):
            nxt = scores(w + 1) if w + 1 < len(waves) else None
            values(w, pending)
            pending = nxt
        ffn_down_chained()

    def attention_max_shifted():
        def one_head(h, carry):
            g = h // HPG
            hp = h - g * HPG
            keep = 1.0 - gate_v[pl.ds(h, 1), :]
            for j in range(NQT):
                st = causal_scores(g, hp, j)
                p = jnp.exp2(st - jnp.max(st, axis=0, keepdims=True)).astype(BF16)
                oh_v[h, :, 128 * j:128 * (j + 1)] = head_output(h, j, p, keep)
            return carry

        lax.fori_loop(0, H, one_head, 0)
        for h in range(H):
            ot_v[step, DH * h:DH * (h + 1), :] = oh_v[h, 0:DH, :]
        ffn_down_looped()

    def output_projection(seg):
        mem = jnp.where(seg > 0, mem_v[jnp.maximum(seg - 1, 0), 0:D, :], 0.0)
        heads_out = ot_v[seg, 0:D, :] + mem
        attn = _dot(_unpack(wot[...]), heads_out.astype(BF16))
        base = x_v[seg].astype(F32) + attn
        xn = _unpack(xn_v[_rows(seg, D // 2), :]).astype(F32)
        col = seg * L + _iota((1, L), 1)
        upd = None
        for t in range(2):
            y = _round_bf16(jnp.sum(y_v[t], axis=1, keepdims=True))
            rsel = jnp.full((1, 1), rsel_s[t], F32)
            y = _round_bf16(y * _round_bf16(jax.nn.sigmoid(rsel)))
            part = jnp.where(col == idx_s[t], y, 0.0)
            upd = part if upd is None else upd + part
        o_ref[...] = (base + (xn + upd)).astype(BF16)

    col_blocks = [(c0, min(128, D - c0)) for c0 in range(0, D, 128)]

    def transpose_block(w_v, section, c0, n):
        r0 = (section * D + c0) // 2
        wall[r0:r0 + n // 2, :] = pltpu.bitcast(w_v[:, c0:c0 + n].T, U32)

    def project_block(section, c0, n, xn):
        r0 = (section * D + c0) // 2
        last = section == 2 and c0 + n == D
        hi = PROWS // 2 if last else r0 + n // 2
        return _dot(_unpack(wall[r0:hi, :]), xn)

    def projections():
        xn0 = _unpack(xn_v[_rows(0, D // 2), :])
        parts = [project_block(0, c0, n, xn0) for c0, n in col_blocks[:3]]
        cp_wk.wait()
        xn0 = _unpack(xn_v[_rows(0, D // 2), :])
        parts += [project_block(0, c0, n, xn0) for c0, n in col_blocks[3:]]
        for c0, n in col_blocks:
            transpose_block(wk_v, 1, c0, n)
        cp_wv.wait()
        x_copies[1].wait()
        xn0 = _unpack(xn_v[_rows(0, D // 2), :])
        parts += [project_block(1, c0, n, xn0) for c0, n in col_blocks]
        for c0, n in col_blocks:
            transpose_block(wv_v, 2, c0, n)
            parts.append(project_block(2, c0, n, xn0))
        layer_norm(1)
        _, pk, vg = store_qkv(0, jnp.concatenate(parts, axis=0))
        x_copies[2].wait()
        x_copies[3].wait()
        cp_wo.wait()

        layer_norm(2)
        pt = project(1)
        wot[...] = pltpu.bitcast(wo_v[...].T, U32)
        state1 = memory_update(None, pk, vg)
        pq1, pk, vg = store_qkv(1, pt)
        layer_norm(3)
        pt = project(2)
        state2 = memory_update(state1, pk, vg)
        pq2, pk, vg = store_qkv(2, pt)
        cp_wg.wait()
        cp_wu.wait()
        pt = project(3, router_first=True)
        pq3, _, _ = store_qkv(3, pt)
        route()
        ffn_hidden()
        state3 = memory_update(state2, pk, vg)
        memory_retrieve(1, state1, pq1)
        memory_retrieve(2, state2, pq2)
        memory_retrieve(3, state3, pq3)
        record_logit_bound()
        cp_wd.wait()

    @pl.when(step == 0)
    def _():
        for cp in (cp_wq, x_copies[0], cp_wr, cp_beta, cp_wk, cp_wv, x_copies[1],
                   x_copies[2], x_copies[3], cp_wo, cp_wg, cp_wu, cp_wd):
            cp.start()
        with _scope("sc_startup"):
            cp_wr.wait()
            cp_beta.wait()
            cp_wq.wait()
            init_constants()
            for c0, n in col_blocks:
                transpose_block(wq_v, 0, c0, n)
            x_copies[0].wait()
            layer_norm(0)
        with _scope("sc_projections"):
            projections()

    @pl.when(step < NSEG)
    def _():
        safe = safe_s[0] == 1

        @pl.when(safe)
        def _():
            with _scope("sc_attention"):
                attention_bounded()

        @pl.when(jnp.logical_not(safe))
        def _():
            attention_max_shifted()

    @pl.when(step >= NSEG)
    def _():
        with _scope("sc_outproj"):
            output_projection(step - NSEG)


@jax.jit
def pallas_parallel_sum__memory_aug_infini_attn__moe_arch_mod__prompt_kernel(
    A_x: jax.Array,
    A_wq: jax.Array,
    A_wk: jax.Array,
    A_wv: jax.Array,
    A_wo: jax.Array,
    A_beta: jax.Array,
    B_x: jax.Array,
    B_w_r: jax.Array,
    B_w_gate: jax.Array,
    B_w_up: jax.Array,
    B_w_down: jax.Array,
):
    del B_x
    vm = pltpu.VMEM
    scratch = [
        vm((NSEG, D, L), BF16),
        vm((D, D), BF16),
        vm((D, D), BF16),
        vm((D, D), BF16),
        vm((D, D), BF16),
        vm((H,), BF16),
        vm((D,), BF16),
        vm((D, FF), BF16),
        vm((D, FF), BF16),
        vm((D, FF), BF16),
        vm((PROWS // 2, D), U32),
        vm((D // 2, D), U32),
        vm((NSEG * D // 2, L), U32),
        vm((NSEG * NG * 64, L), U32),
        vm((NSEG * NG * L // 2, 128), U32),
        vm((NSEG * H * 16, L), U32),
        vm((NSEG - 1, OROWS, L), F32),
        vm((8, L), F32),
        vm((8, D), U32),
        vm((2, D, 128), F32),
        vm((2, FF // 128, 8, 128), F32),
        pltpu.SMEM((2,), jnp.int32),
        pltpu.SMEM((2,), F32),
        pltpu.SMEM((1,), U32),
        pltpu.SMEM((1,), jnp.int32),
        vm((H, 128), F32),
        vm((NSEG, D, L), F32),
        vm((H, 24, L), F32),
        vm((128, 128), F32),
        vm((3, 64, 128), F32),
        pltpu.SemaphoreType.DMA((NSEG + 9,)),
    ]
    hbm = pl.BlockSpec(memory_space=pltpu.HBM)
    xt = jnp.transpose(A_x.reshape(S, D))
    out_t = pl.pallas_call(
        _kernel,
        grid=(2 * NSEG,),
        in_specs=[hbm] * 10,
        out_specs=pl.BlockSpec((D, L), lambda s: (0, jnp.maximum(s - NSEG, 0))),
        out_shape=jax.ShapeDtypeStruct((D, S), BF16),
        scratch_shapes=scratch,
        compiler_params=pltpu.CompilerParams(
            dimension_semantics=("arbitrary",),
            vmem_limit_bytes=110 * 1024 * 1024,
        ),
        name="infini_moe",
    )(xt, A_wq, A_wk, A_wv, A_wo, A_beta, B_w_r, B_w_gate, B_w_up,
      jnp.transpose(B_w_down))
    return jnp.transpose(out_t).reshape(1, S, D)
```

```python
import contextlib

import jax
import jax.numpy as jnp
from jax import lax
from jax.experimental import pallas as pl
from jax.experimental.pallas import tpu as pltpu

S = 2048
D = 576
H = 32
DH = 18
NSEG = 4
L = 512
FF = 4608
NG = 5
HPG = 7
GW = HPG * DH
NQT = L // 128
PROWS = 3 * D + 16
RROW = 3 * D
PBLOCK = 128
MROWS = 144
FT = FF // 128 // NSEG
OROWS = 640
LOG2E = 1.4426950408889634
QSCALE = DH ** -0.5 * LOG2E
NEG = -1e30
LN_EPS = 1.0013580322265625e-05
F32 = jnp.float32
BF16 = jnp.bfloat16
U32 = jnp.uint32

PROFILE_SCOPES = False

_NN = (((1,), (0,)), ((), ()))
_NT = (((1,), (1,)), ((), ()))


def _scope(name):
    return jax.named_scope(name) if PROFILE_SCOPES else contextlib.nullcontext()


def _dot(a, b):
    return lax.dot_general(a, b, _NN, preferred_element_type=F32)


def _dot_nt(a, b):
    return lax.dot_general(a, b, _NT, preferred_element_type=F32)


def _iota(shape, dim):
    return lax.broadcasted_iota(jnp.int32, shape, dim)


def _round_bf16(v):
    return v.astype(BF16).astype(F32)


def _pack(v):
    return pltpu.bitcast(v.astype(BF16), U32)


def _unpack(u):
    return pltpu.bitcast(u, BF16)


def _rows(index, size):
    if isinstance(index, int):
        return slice(index * size, (index + 1) * size)
    return pl.ds(pl.multiple_of(index * size, 8), size)


def _heads_in_group(g):
    return HPG if g < NG - 1 else H - HPG * (NG - 1)


def _phi(t):
    return jnp.where(t > 0, t + 1.0, jnp.exp(t))


def _kernel(x_hbm, wq_hbm, wk_hbm, wv_hbm, wo_hbm, beta_hbm, wr_hbm,
            wg_hbm, wu_hbm, wd_hbm,
            o_ref,
            x_v, wq_v, wk_v, wv_v, wo_v, beta_v, wr_v, wg_v, wu_v, wd_v,
            wall, wot, xn_v, qt_v, k_v, vt_v, mem_v,
            r_v, xs_v, y_v, hid_v, idx_s, rsel_s, zero_s, safe_s,
            gate_v, ot_v, oh_v, bias_v, half_v,
            sems):
    step = pl.program_id(0)

    x_copies = [
        pltpu.make_async_copy(x_hbm.at[:, pl.ds(c * L, L)], x_v.at[c], sems.at[c])
        for c in range(NSEG)
    ]
    pairs = [(wq_hbm, wq_v), (wk_hbm, wk_v), (wv_hbm, wv_v), (wo_hbm, wo_v),
             (beta_hbm, beta_v), (wr_hbm, wr_v),
             (wg_hbm, wg_v), (wu_hbm, wu_v), (wd_hbm, wd_v)]
    (cp_wq, cp_wk, cp_wv, cp_wo, cp_beta, cp_wr, cp_wg, cp_wu, cp_wd) = [
        pltpu.make_async_copy(src, dst, sems.at[NSEG + i])
        for i, (src, dst) in enumerate(pairs)
    ]

    def nothing(v):
        return pltpu.bitcast(pltpu.bitcast(v, U32) & zero_s[0], F32)

    def layer_norm(c, serial=True):
        link = None
        for n in range(NQT):
            cols = slice(128 * n, 128 * (n + 1))
            pivot = x_v[c, 0:16, cols].astype(F32)[0:1, :]
            pivot8 = jnp.broadcast_to(pivot, (8, 128))
            shift = pivot8
            s1 = s2 = None
            for i in range(D // 16):
                last = s1 if s1 is not None else link
                if serial and last is not None:
                    shift = pivot8 + nothing(last)
                x16 = x_v[c, 16 * i:16 * i + 16, cols].astype(F32)
                for k in range(2):
                    d = x16[8 * k:8 * k + 8, :] - shift
                    s1 = d if s1 is None else s1 + d
                    s2 = d * d if s2 is None else s2 + d * d
            dmean = jnp.sum(s1, axis=0, keepdims=True) * (1.0 / D)
            dsq = jnp.sum(s2, axis=0, keepdims=True) * (1.0 / D)
            var = jnp.maximum(dsq - dmean * dmean, 0.0)
            sd = _round_bf16(jnp.sqrt(_round_bf16(_round_bf16(var) + LN_EPS)))
            mean8 = jnp.broadcast_to(_round_bf16(pivot + dmean), (8, 128))
            inv8 = jnp.broadcast_to(1.0 / sd, (8, 128))
            center = mean8
            for i in range(D // 32):
                if serial and i > 0:
                    center = mean8 + nothing(link)
                x32 = x_v[c, 32 * i:32 * i + 32, cols].astype(F32)
                z = [(x32[8 * k:8 * k + 8, :] - center) * inv8 for k in range(4)]
                link = z[3]
                r0 = c * (D // 2) + 16 * i
                xn_v[r0:r0 + 16, cols] = _pack(jnp.concatenate(z, axis=0))

    def init_constants():
        gate = jax.nn.sigmoid(beta_v[...].astype(F32).reshape(1, H))
        on_diag = _iota((H, H), 0) == _iota((H, H), 1)
        gcol = jnp.sum(jnp.where(on_diag, gate, 0.0), axis=1, keepdims=True)
        gate_v[...] = jnp.broadcast_to(gcol, (H, 128))
        zero_s[0] = jnp.uint32(0)
        bias_v[...] = jnp.where(_iota((128, 128), 0) > _iota((128, 128), 1), NEG, 0.0)
        key, lane = _iota((64, 128), 0), _iota((64, 128), 1)
        future = key > (lane & 63)
        half_v[0] = jnp.where(future, NEG, 0.0)
        half_v[1] = jnp.where(future | (lane < 64), NEG, 0.0)
        half_v[2] = jnp.where(future | (lane >= 64), NEG, 0.0)
        router = jnp.broadcast_to(wr_v[...].astype(F32).reshape(1, D), (16, D))
        wall[RROW // 2:PROWS // 2, :] = _pack(
            jnp.where(_iota((16, D), 0) == 0, router, 0.0))

    def project(c, router_first=False):
        xn = _unpack(xn_v[_rows(c, D // 2), :])
        step_rows = PBLOCK // 2
        end = RROW // 2 if router_first else PROWS // 2
        tail = [_dot(_unpack(wall[end:PROWS // 2, :]), xn)] if router_first else []
        return jnp.concatenate(
            [_dot(_unpack(wall[r:min(r + step_rows, end), :]), xn)
             for r in range(0, end, step_rows)] + tail, axis=0)

    seen = [None]

    def record_logit_bound():
        big = (seen[0] >> 30) & 1
        safe_s[0] = (jnp.max(big.astype(jnp.int32)) == 0).astype(jnp.int32)

    def store_qkv(c, pt):
        r_v[c:c + 1, :] = _round_bf16(pt[RROW:RROW + 1, :])
        tail_row = _iota((8, L), 0)
        for h in range(H):
            base = 2 * D + DH * h
            tail = jnp.where(tail_row < DH - 16, pt[base + 16:base + 24, :],
                             jnp.where(tail_row == DH - 16, 1.0, 0.0))
            blk = jnp.concatenate(
                [pt[base:base + 16, :], tail, jnp.zeros((8, L), F32)], axis=0)
            vt_v[_rows(c * H + h, 16), :] = _pack(blk)

        rowl = _iota((128, L), 0)
        pqs, pks, vgs = [], [], []
        for g in range(NG):
            used = _heads_in_group(g) * DH
            qg = pt[GW * g:GW * g + 128, :]
            qs = qg * QSCALE
            qt_v[_rows(c * NG + g, 64), :] = _pack(qs)
            kg = pt[D + GW * g:D + GW * g + 128, :]
            for operand in (qs, kg):
                bits = pltpu.bitcast(operand, U32)
                for blk in range(0, 128 if g < NG - 1 else used, 8):
                    for col in range(0, L, 128):
                        piece = bits[blk:blk + 8, col:col + 128]
                        seen[0] = piece if seen[0] is None else seen[0] | piece
            k_v[_rows(c * NG + g, L // 2), :] = _pack(kg.T)
            pqs.append(_phi(qg).astype(BF16))
            if c < NSEG - 1:
                pks.append(_phi(kg).astype(BF16))
                lo = 2 * D + GW * g
                if g < NG - 1:
                    vg = pt[lo:lo + 128, :]
                else:
                    vg = jnp.concatenate(
                        [pt[lo:lo + used, :], jnp.zeros((128 - used, L), F32)], axis=0)
                vg = jnp.where(rowl < used, vg, jnp.where(rowl == GW, 1.0, 0.0))
                vgs.append(vg.astype(BF16))
        return pqs, pks, vgs

    def memory_update(states, pks, vgs):
        row = _iota((128, 128), 0)
        lane = _iota((128, 128), 1)
        same_head = (row // DH) == (lane // DH)
        out = []
        for g in range(NG):
            used = _heads_in_group(g) * DH
            upd = _dot_nt(vgs[g], pks[g])
            keep = ((same_head & (row < used)) | (row == GW)) & (lane < used)
            upd = jnp.where(keep, upd, 0.0)
            out.append(upd if states is None else states[g] + upd)
        return out

    def memory_retrieve(c, states, pqs):
        row = _iota((128, 128), 0)
        row8 = _iota((8, 128), 0)
        lane8 = _iota((8, 128), 1) // DH
        for g in range(NG):
            nh = _heads_in_group(g)
            st = states[g]
            mrows = jnp.where(row < GW, st, 0.0)
            zrows = jnp.where(lane8 == row8, st[GW:GW + 1, :], 0.0)
            lhs = jnp.concatenate(
                [mrows, zrows, jnp.zeros((8, 128), F32)], axis=0).astype(BF16)
            ret = _dot(lhs, pqs[g])
            gsel = gate_v[HPG * g:HPG * g + 8, :] if g < NG - 1 else jnp.concatenate(
                [gate_v[HPG * g:H, :], jnp.zeros((8 - nh, 128), F32)], axis=0)
            gwide = jnp.concatenate([gsel] * NQT, axis=1)
            scale = gwide / (ret[128:136, :] + 1e-6)
            pieces = []
            for b in range(16):
                h0 = min((8 * b) // DH, nh - 1)
                h1 = min((8 * b + 7) // DH, nh - 1)
                sc = scale[h0:h0 + 1, :]
                if h1 != h0:
                    first = _iota((8, L), 0) < DH * h1 - 8 * b
                    sc = jnp.where(first, sc, scale[h1:h1 + 1, :])
                pieces.append(ret[8 * b:8 * b + 8, :] * sc)
            mem_v[c - 1, GW * g:GW * g + 128, :] = jnp.concatenate(pieces, axis=0)

    def route():
        r = r_v[0:NSEG, :]
        idx = _iota((NSEG, L), 0) * L + _iota((NSEG, L), 1)
        m1 = jnp.max(r)
        i1 = jnp.clip(jnp.min(jnp.where(r == m1, idx, S)), 0, S - 1)
        r2 = jnp.where(idx == i1, -jnp.inf, r)
        m2 = jnp.max(r2)
        i2 = jnp.clip(jnp.min(jnp.where(r2 == m2, idx, S)), 0, S - 1)
        idx_s[0] = i1
        idx_s[1] = i2
        rsel_s[0] = m1
        rsel_s[1] = m2
        row16 = _iota((16, 128), 0)
        lane16 = _iota((16, 128), 1)
        xs = None
        for t, i in enumerate((i1, i2)):
            seg = i // L
            off = i - seg * L
            base = pl.multiple_of((off // 128) * 128, 128)
            cols = _unpack(xn_v[_rows(seg, D // 2), pl.ds(base, 128)])
            pick = jnp.where((row16 == t) & (lane16 == off - base), 1.0, 0.0)
            part = _dot_nt(pick.astype(BF16), cols)
            xs = part if xs is None else xs + part
        xs_v[...] = _pack(xs)
        y_v[...] = jnp.zeros(y_v.shape, F32)

    def ffn_hidden():
        xs = _unpack(xs_v[...])
        gt = _round_bf16(_dot(xs, wg_v[...]))
        up = _round_bf16(_dot(xs, wu_v[...]))
        hid = _round_bf16(_round_bf16(gt * jax.nn.sigmoid(gt)) * up)
        for t in range(2):
            for tile in range(FF // 128):
                hid_v[t, tile] = jnp.broadcast_to(
                    hid[t:t + 1, 128 * tile:128 * (tile + 1)], (8, 128))

    def ffn_down_chained():
        base = pl.multiple_of(step * (FT * 128), 128)
        link = [None, None]
        for b in range(D // 8):
            acc = [None, None]
            for tile in range(FT):
                w = wd_v[8 * b:8 * b + 8, pl.ds(base + 128 * tile, 128)].astype(F32)
                for t in range(2):
                    pr = w * hid_v[t, step * FT + tile]
                    if tile > 0:
                        acc[t] = acc[t] + pr
                    else:
                        acc[t] = pr if link[t] is None else pr + nothing(link[t])
            for t in range(2):
                rows = slice(8 * b, 8 * b + 8)
                y_v[t, rows, :] = y_v[t, rows, :] + acc[t]
                link[t] = acc[t]

    def ffn_down_looped():
        def down(tile, carry):
            col = step * FT + tile
            w = wd_v[:, pl.ds(pl.multiple_of(128 * col, 128), 128)].astype(F32)
            for t in range(2):
                y_v[t] = y_v[t] + w * hid_v[t, col][0:1, :]
            return carry

        lax.fori_loop(0, FT, down, 0)

    def masked_q_bits(g, hp, j):
        rid = _iota((64, 128), 0)
        mask = (rid >= (DH // 2) * hp) & (rid < (DH // 2) * (hp + 1))
        return jnp.where(mask, qt_v[_rows(step * NG + g, 64), 128 * j:128 * (j + 1)],
                         jnp.uint32(0))

    def keys(g, lo, hi):
        first = pl.multiple_of((step * NG + g) * (L // 2) + lo // 2, 8)
        return _unpack(k_v[pl.ds(first, (hi - lo) // 2), :])

    def causal_scores(g, hp, j):
        nk = 128 * (j + 1)
        st = _dot(keys(g, 0, nk), _unpack(masked_q_bits(g, hp, j)))
        diag = st[nk - 128:, :] + bias_v[...]
        return diag if j == 0 else jnp.concatenate([st[:nk - 128, :], diag], axis=0)

    def head_output(h, j, p, keep):
        o = _dot(_unpack(vt_v[_rows(step * H + h, 16), 0:128 * (j + 1)]), p)
        den = o[DH:DH + 1, :]
        inv = pl.reciprocal(den, approx=True)
        inv = inv * (2.0 - den * inv)
        return o[0:24, :] * (keep * inv)

    def single_probs(h, j):
        return jnp.exp2(causal_scores(*divmod(h, HPG), j)).astype(BF16)

    def pair_probs(pairs, j, flip):
        low = _iota((64, 128), 1) < 64
        qa, qb = {}, {}
        for h in pairs:
            g, hp = divmod(h, HPG)
            qa[h] = masked_q_bits(g, hp, j)
            qb[h] = pltpu.roll(masked_q_bits(g, hp + 1, j), 64, 1)
        off = {}
        if j > 0:
            for h in pairs:
                g = h // HPG
                for hh, q in ((h, qa[h]), (h + 1, qb[h])):
                    off[hh] = jnp.exp2(_dot(keys(g, 0, 128 * j), _unpack(q)))
        early, late = {}, {}
        for h in pairs:
            g = h // HPG
            k0 = 128 * j
            for which in ((0, 1) if flip else (1, 0)):
                if which == 0:
                    early[h] = _dot(keys(g, k0, k0 + 64),
                                    _unpack(jnp.where(low, qa[h], qb[h])))
                else:
                    late[h] = _dot(keys(g, k0, k0 + 128),
                                   _unpack(jnp.where(low, qb[h], qa[h])))
        probs = {}
        for h in pairs:
            p1 = jnp.exp2(early[h] + half_v[0])
            p2 = jnp.exp2(late[h][0:64, :])
            bottom = late[h][64:128, :]
            pa = jnp.concatenate(
                [jnp.where(low, p1, p2), jnp.exp2(bottom + half_v[1])], axis=0)
            pb = jnp.concatenate(
                [jnp.where(low, p2, p1), jnp.exp2(bottom + half_v[2])], axis=0)
            for hh, pd in ((h, pa), (h + 1, pb)):
                full = pd if j == 0 else jnp.concatenate([off[hh], pd], axis=0)
                probs[hh] = full.astype(BF16)
        return probs

    def attention_bounded():
        pairs = [g * HPG + hp for g in range(NG)
                 for hp in range(0, _heads_in_group(g) - 1, 2)]
        paired = set(pairs) | {h + 1 for h in pairs}
        singles = [h for h in range(H) if h not in paired]
        waves = [(pairs[i:i + 2], j) for i in range(0, len(pairs), 2) for j in range(NQT)]
        waves += [(None, j) for j in range(NQT)]

        def scores(w):
            grp, j = waves[w]
            if grp is None:
                return {h: single_probs(h, j) for h in singles}
            return pair_probs(grp, j, w % 2 == 1)

        def values(w, probs):
            grp, j = waves[w]
            for h, p in probs.items():
                o = head_output(h, j, p, 1.0 - gate_v[h:h + 1, :])
                if grp is not None and h - 1 in grp:
                    o = pltpu.roll(o, 64, 1)
                ot_v[step, DH * h:DH * (h + 1), 128 * j:128 * (j + 1)] = o[0:DH, :]

        pending = scores(0)
        for w in range(len(waves)):
            nxt = scores(w + 1) if w + 1 < len(waves) else None
            values(w, pending)
            pending = nxt
        ffn_down_chained()

    def attention_max_shifted():
        def one_head(h, carry):
            g = h // HPG
            hp = h - g * HPG
            keep = 1.0 - gate_v[pl.ds(h, 1), :]
            for j in range(NQT):
                st = causal_scores(g, hp, j)
                p = jnp.exp2(st - jnp.max(st, axis=0, keepdims=True)).astype(BF16)
                oh_v[h, :, 128 * j:128 * (j + 1)] = head_output(h, j, p, keep)
            return carry

        lax.fori_loop(0, H, one_head, 0)
        for h in range(H):
            ot_v[step, DH * h:DH * (h + 1), :] = oh_v[h, 0:DH, :]
        ffn_down_looped()

    def output_projection(seg):
        mem = jnp.where(seg > 0, mem_v[jnp.maximum(seg - 1, 0), 0:D, :], 0.0)
        heads_out = ot_v[seg, 0:D, :] + mem
        attn = _dot(_unpack(wot[...]), heads_out.astype(BF16))
        base = x_v[seg].astype(F32) + attn
        xn = _unpack(xn_v[_rows(seg, D // 2), :]).astype(F32)
        col = seg * L + _iota((1, L), 1)
        upd = None
        for t in range(2):
            y = _round_bf16(jnp.sum(y_v[t], axis=1, keepdims=True))
            rsel = jnp.full((1, 1), rsel_s[t], F32)
            y = _round_bf16(y * _round_bf16(jax.nn.sigmoid(rsel)))
            part = jnp.where(col == idx_s[t], y, 0.0)
            upd = part if upd is None else upd + part
        o_ref[...] = (base + (xn + upd)).astype(BF16)

    col_blocks = [(c0, min(128, D - c0)) for c0 in range(0, D, 128)]

    def transpose_block(w_v, section, c0, n):
        r0 = (section * D + c0) // 2
        wall[r0:r0 + n // 2, :] = pltpu.bitcast(w_v[:, c0:c0 + n].T, U32)

    def project_block(section, c0, n, xn):
        r0 = (section * D + c0) // 2
        last = section == 2 and c0 + n == D
        hi = PROWS // 2 if last else r0 + n // 2
        return _dot(_unpack(wall[r0:hi, :]), xn)

    def projections():
        xn0 = _unpack(xn_v[_rows(0, D // 2), :])
        parts = [project_block(0, c0, n, xn0) for c0, n in col_blocks[:3]]
        cp_wk.wait()
        xn0 = _unpack(xn_v[_rows(0, D // 2), :])
        parts += [project_block(0, c0, n, xn0) for c0, n in col_blocks[3:]]
        for c0, n in col_blocks:
            transpose_block(wk_v, 1, c0, n)
        cp_wv.wait()
        x_copies[1].wait()
        xn0 = _unpack(xn_v[_rows(0, D // 2), :])
        parts += [project_block(1, c0, n, xn0) for c0, n in col_blocks]
        for c0, n in col_blocks:
            transpose_block(wv_v, 2, c0, n)
            parts.append(project_block(2, c0, n, xn0))
        layer_norm(1)
        _, pk, vg = store_qkv(0, jnp.concatenate(parts, axis=0))
        x_copies[2].wait()
        x_copies[3].wait()
        cp_wo.wait()

        layer_norm(2)
        pt = project(1)
        wot[...] = pltpu.bitcast(wo_v[...].T, U32)
        state1 = memory_update(None, pk, vg)
        pq1, pk, vg = store_qkv(1, pt)
        layer_norm(3)
        pt = project(2)
        state2 = memory_update(state1, pk, vg)
        pq2, pk, vg = store_qkv(2, pt)
        cp_wg.wait()
        cp_wu.wait()
        pt = project(3, router_first=True)
        pq3, _, _ = store_qkv(3, pt)
        route()
        ffn_hidden()
        state3 = memory_update(state2, pk, vg)
        memory_retrieve(1, state1, pq1)
        memory_retrieve(2, state2, pq2)
        memory_retrieve(3, state3, pq3)
        record_logit_bound()
        cp_wd.wait()

    @pl.when(step == 0)
    def _():
        for cp in (cp_wq, x_copies[0], cp_wr, cp_beta, cp_wk, cp_wv, x_copies[1],
                   x_copies[2], x_copies[3], cp_wo, cp_wg, cp_wu, cp_wd):
            cp.start()
        with _scope("sc_startup"):
            cp_wr.wait()
            cp_beta.wait()
            cp_wq.wait()
            init_constants()
            for c0, n in col_blocks:
                transpose_block(wq_v, 0, c0, n)
            x_copies[0].wait()
            layer_norm(0, serial=False)
        with _scope("sc_projections"):
            projections()

    @pl.when(step < NSEG)
    def _():
        safe = safe_s[0] == 1

        @pl.when(safe)
        def _():
            with _scope("sc_attention"):
                attention_bounded()

        @pl.when(jnp.logical_not(safe))
        def _():
            attention_max_shifted()

    @pl.when(step >= NSEG)
    def _():
        with _scope("sc_outproj"):
            output_projection(step - NSEG)


@jax.jit
def pallas_parallel_sum__memory_aug_infini_attn__moe_arch_mod__prompt_kernel(
    A_x: jax.Array,
    A_wq: jax.Array,
    A_wk: jax.Array,
    A_wv: jax.Array,
    A_wo: jax.Array,
    A_beta: jax.Array,
    B_x: jax.Array,
    B_w_r: jax.Array,
    B_w_gate: jax.Array,
    B_w_up: jax.Array,
    B_w_down: jax.Array,
):
    del B_x
    vm = pltpu.VMEM
    scratch = [
        vm((NSEG, D, L), BF16),
        vm((D, D), BF16),
        vm((D, D), BF16),
        vm((D, D), BF16),
        vm((D, D), BF16),
        vm((H,), BF16),
        vm((D,), BF16),
        vm((D, FF), BF16),
        vm((D, FF), BF16),
        vm((D, FF), BF16),
        vm((PROWS // 2, D), U32),
        vm((D // 2, D), U32),
        vm((NSEG * D // 2, L), U32),
        vm((NSEG * NG * 64, L), U32),
        vm((NSEG * NG * L // 2, 128), U32),
        vm((NSEG * H * 16, L), U32),
        vm((NSEG - 1, OROWS, L), F32),
        vm((8, L), F32),
        vm((8, D), U32),
        vm((2, D, 128), F32),
        vm((2, FF // 128, 8, 128), F32),
        pltpu.SMEM((2,), jnp.int32),
        pltpu.SMEM((2,), F32),
        pltpu.SMEM((1,), U32),
        pltpu.SMEM((1,), jnp.int32),
        vm((H, 128), F32),
        vm((NSEG, D, L), F32),
        vm((H, 24, L), F32),
        vm((128, 128), F32),
        vm((3, 64, 128), F32),
        pltpu.SemaphoreType.DMA((NSEG + 9,)),
    ]
    hbm = pl.BlockSpec(memory_space=pltpu.HBM)
    xt = jnp.transpose(A_x.reshape(S, D))
    out_t = pl.pallas_call(
        _kernel,
        grid=(2 * NSEG,),
        in_specs=[hbm] * 10,
        out_specs=pl.BlockSpec((D, L), lambda s: (0, jnp.maximum(s - NSEG, 0))),
        out_shape=jax.ShapeDtypeStruct((D, S), BF16),
        scratch_shapes=scratch,
        compiler_params=pltpu.CompilerParams(
            dimension_semantics=("arbitrary",),
            vmem_limit_bytes=110 * 1024 * 1024,
        ),
        name="infini_moe",
    )(xt, A_wq, A_wk, A_wv, A_wo, A_beta, B_w_r, B_w_gate, B_w_up,
      jnp.transpose(B_w_down))
    return jnp.transpose(out_t).reshape(1, S, D)
```

```python
import contextlib

import jax
import jax.numpy as jnp
from jax import lax
from jax.experimental import pallas as pl
from jax.experimental.pallas import tpu as pltpu

S = 2048
D = 576
H = 32
DH = 18
NSEG = 4
L = 512
FF = 4608
NG = 5
HPG = 7
GW = HPG * DH
NQT = L // 128
PROWS = 3 * D + 16
RROW = 3 * D
PBLOCK = 128
MROWS = 144
FT = FF // 128 // NSEG
OROWS = 640
LOG2E = 1.4426950408889634
QSCALE = DH ** -0.5 * LOG2E
NEG = -1e30
LN_EPS = 1.0013580322265625e-05
F32 = jnp.float32
BF16 = jnp.bfloat16
U32 = jnp.uint32

PROFILE_SCOPES = False

_NN = (((1,), (0,)), ((), ()))
_NT = (((1,), (1,)), ((), ()))


def _scope(name):
    return jax.named_scope(name) if PROFILE_SCOPES else contextlib.nullcontext()


def _dot(a, b):
    return lax.dot_general(a, b, _NN, preferred_element_type=F32)


def _dot_nt(a, b):
    return lax.dot_general(a, b, _NT, preferred_element_type=F32)


def _iota(shape, dim):
    return lax.broadcasted_iota(jnp.int32, shape, dim)


def _round_bf16(v):
    return v.astype(BF16).astype(F32)


def _pack(v):
    return pltpu.bitcast(v.astype(BF16), U32)


def _unpack(u):
    return pltpu.bitcast(u, BF16)


def _rows(index, size):
    if isinstance(index, int):
        return slice(index * size, (index + 1) * size)
    return pl.ds(pl.multiple_of(index * size, 8), size)


def _heads_in_group(g):
    return HPG if g < NG - 1 else H - HPG * (NG - 1)


def _phi(t):
    return jnp.where(t > 0, t + 1.0, jnp.exp(t))


def _kernel(x_hbm, wq_hbm, wk_hbm, wv_hbm, wo_hbm, beta_hbm, wr_hbm,
            wg_hbm, wu_hbm, wd_hbm,
            o_ref,
            x_v, wq_v, wk_v, wv_v, wo_v, beta_v, wr_v, wg_v, wu_v, wd_v,
            wall, wot, xn_v, qt_v, k_v, vt_v, mem_v,
            r_v, xs_v, y_v, hid_v, idx_s, rsel_s, zero_s, safe_s,
            gate_v, ot_v, oh_v, bias_v, half_v,
            sems):
    step = pl.program_id(0)

    x_copies = [None] + [
        pltpu.make_async_copy(x_hbm.at[:, pl.ds(c * L, L)], x_v.at[c], sems.at[c])
        for c in range(1, NSEG)
    ]
    x0_copies = [
        pltpu.make_async_copy(x_hbm.at[:, pl.ds(256 * n, 256)],
                              x_v.at[0, :, pl.ds(256 * n, 256)],
                              sems.at[NSEG + 9 + n])
        for n in range(2)
    ]
    pairs = [(wq_hbm, wq_v), (wk_hbm, wk_v), (wv_hbm, wv_v), (wo_hbm, wo_v),
             (beta_hbm, beta_v), (wr_hbm, wr_v),
             (wg_hbm, wg_v), (wu_hbm, wu_v), (wd_hbm, wd_v)]
    (cp_wq, cp_wk, cp_wv, cp_wo, cp_beta, cp_wr, cp_wg, cp_wu, cp_wd) = [
        pltpu.make_async_copy(src, dst, sems.at[NSEG + i])
        for i, (src, dst) in enumerate(pairs)
    ]

    def nothing(v):
        return pltpu.bitcast(pltpu.bitcast(v, U32) & zero_s[0], F32)

    def layer_norm(c, serial=True, tiles=range(NQT)):
        link = None
        for n in tiles:
            cols = slice(128 * n, 128 * (n + 1))
            pivot = x_v[c, 0:16, cols].astype(F32)[0:1, :]
            pivot8 = jnp.broadcast_to(pivot, (8, 128))
            shift = pivot8
            s1 = s2 = None
            for i in range(D // 16):
                last = s1 if s1 is not None else link
                if serial and last is not None:
                    shift = pivot8 + nothing(last)
                x16 = x_v[c, 16 * i:16 * i + 16, cols].astype(F32)
                for k in range(2):
                    d = x16[8 * k:8 * k + 8, :] - shift
                    s1 = d if s1 is None else s1 + d
                    s2 = d * d if s2 is None else s2 + d * d
            dmean = jnp.sum(s1, axis=0, keepdims=True) * (1.0 / D)
            dsq = jnp.sum(s2, axis=0, keepdims=True) * (1.0 / D)
            var = jnp.maximum(dsq - dmean * dmean, 0.0)
            sd = _round_bf16(jnp.sqrt(_round_bf16(_round_bf16(var) + LN_EPS)))
            mean8 = jnp.broadcast_to(_round_bf16(pivot + dmean), (8, 128))
            inv8 = jnp.broadcast_to(1.0 / sd, (8, 128))
            center = mean8
            for i in range(D // 32):
                if serial and i > 0:
                    center = mean8 + nothing(link)
                x32 = x_v[c, 32 * i:32 * i + 32, cols].astype(F32)
                z = [(x32[8 * k:8 * k + 8, :] - center) * inv8 for k in range(4)]
                link = z[3]
                r0 = c * (D // 2) + 16 * i
                xn_v[r0:r0 + 16, cols] = _pack(jnp.concatenate(z, axis=0))

    def init_constants():
        gate = jax.nn.sigmoid(beta_v[...].astype(F32).reshape(1, H))
        on_diag = _iota((H, H), 0) == _iota((H, H), 1)
        gcol = jnp.sum(jnp.where(on_diag, gate, 0.0), axis=1, keepdims=True)
        gate_v[...] = jnp.broadcast_to(gcol, (H, 128))
        zero_s[0] = jnp.uint32(0)
        bias_v[...] = jnp.where(_iota((128, 128), 0) > _iota((128, 128), 1), NEG, 0.0)
        key, lane = _iota((64, 128), 0), _iota((64, 128), 1)
        future = key > (lane & 63)
        half_v[0] = jnp.where(future, NEG, 0.0)
        half_v[1] = jnp.where(future | (lane < 64), NEG, 0.0)
        half_v[2] = jnp.where(future | (lane >= 64), NEG, 0.0)
        router = jnp.broadcast_to(wr_v[...].astype(F32).reshape(1, D), (16, D))
        wall[RROW // 2:PROWS // 2, :] = _pack(
            jnp.where(_iota((16, D), 0) == 0, router, 0.0))

    def project(c, router_first=False):
        xn = _unpack(xn_v[_rows(c, D // 2), :])
        step_rows = PBLOCK // 2
        end = RROW // 2 if router_first else PROWS // 2
        tail = [_dot(_unpack(wall[end:PROWS // 2, :]), xn)] if router_first else []
        return jnp.concatenate(
            [_dot(_unpack(wall[r:min(r + step_rows, end), :]), xn)
             for r in range(0, end, step_rows)] + tail, axis=0)

    seen = [None]

    def record_logit_bound():
        big = (seen[0] >> 30) & 1
        safe_s[0] = (jnp.max(big.astype(jnp.int32)) == 0).astype(jnp.int32)

    def store_qkv(c, pt):
        r_v[c:c + 1, :] = _round_bf16(pt[RROW:RROW + 1, :])
        tail_row = _iota((8, L), 0)
        for h in range(H):
            base = 2 * D + DH * h
            tail = jnp.where(tail_row < DH - 16, pt[base + 16:base + 24, :],
                             jnp.where(tail_row == DH - 16, 1.0, 0.0))
            blk = jnp.concatenate(
                [pt[base:base + 16, :], tail, jnp.zeros((8, L), F32)], axis=0)
            vt_v[_rows(c * H + h, 16), :] = _pack(blk)

        rowl = _iota((128, L), 0)
        pqs, pks, vgs = [], [], []
        for g in range(NG):
            used = _heads_in_group(g) * DH
            qg = pt[GW * g:GW * g + 128, :]
            qs = qg * QSCALE
            qt_v[_rows(c * NG + g, 64), :] = _pack(qs)
            kg = pt[D + GW * g:D + GW * g + 128, :]
            for operand in (qs, kg):
                bits = pltpu.bitcast(operand, U32)
                for blk in range(0, 128 if g < NG - 1 else used, 8):
                    for col in range(0, L, 128):
                        piece = bits[blk:blk + 8, col:col + 128]
                        seen[0] = piece if seen[0] is None else seen[0] | piece
            k_v[_rows(c * NG + g, L // 2), :] = _pack(kg.T)
            pqs.append(_phi(qg).astype(BF16))
            if c < NSEG - 1:
                pks.append(_phi(kg).astype(BF16))
                lo = 2 * D + GW * g
                if g < NG - 1:
                    vg = pt[lo:lo + 128, :]
                else:
                    vg = jnp.concatenate(
                        [pt[lo:lo + used, :], jnp.zeros((128 - used, L), F32)], axis=0)
                vg = jnp.where(rowl < used, vg, jnp.where(rowl == GW, 1.0, 0.0))
                vgs.append(vg.astype(BF16))
        return pqs, pks, vgs

    def memory_update(states, pks, vgs):
        row = _iota((128, 128), 0)
        lane = _iota((128, 128), 1)
        same_head = (row // DH) == (lane // DH)
        out = []
        for g in range(NG):
            used = _heads_in_group(g) * DH
            upd = _dot_nt(vgs[g], pks[g])
            keep = ((same_head & (row < used)) | (row == GW)) & (lane < used)
            upd = jnp.where(keep, upd, 0.0)
            out.append(upd if states is None else states[g] + upd)
        return out

    def memory_retrieve(c, states, pqs):
        row = _iota((128, 128), 0)
        row8 = _iota((8, 128), 0)
        lane8 = _iota((8, 128), 1) // DH
        for g in range(NG):
            nh = _heads_in_group(g)
            st = states[g]
            mrows = jnp.where(row < GW, st, 0.0)
            zrows = jnp.where(lane8 == row8, st[GW:GW + 1, :], 0.0)
            lhs = jnp.concatenate(
                [mrows, zrows, jnp.zeros((8, 128), F32)], axis=0).astype(BF16)
            ret = _dot(lhs, pqs[g])
            gsel = gate_v[HPG * g:HPG * g + 8, :] if g < NG - 1 else jnp.concatenate(
                [gate_v[HPG * g:H, :], jnp.zeros((8 - nh, 128), F32)], axis=0)
            gwide = jnp.concatenate([gsel] * NQT, axis=1)
            scale = gwide / (ret[128:136, :] + 1e-6)
            pieces = []
            for b in range(16):
                h0 = min((8 * b) // DH, nh - 1)
                h1 = min((8 * b + 7) // DH, nh - 1)
                sc = scale[h0:h0 + 1, :]
                if h1 != h0:
                    first = _iota((8, L), 0) < DH * h1 - 8 * b
                    sc = jnp.where(first, sc, scale[h1:h1 + 1, :])
                pieces.append(ret[8 * b:8 * b + 8, :] * sc)
            mem_v[c - 1, GW * g:GW * g + 128, :] = jnp.concatenate(pieces, axis=0)

    def route():
        r = r_v[0:NSEG, :]
        idx = _iota((NSEG, L), 0) * L + _iota((NSEG, L), 1)
        m1 = jnp.max(r)
        i1 = jnp.clip(jnp.min(jnp.where(r == m1, idx, S)), 0, S - 1)
        r2 = jnp.where(idx == i1, -jnp.inf, r)
        m2 = jnp.max(r2)
        i2 = jnp.clip(jnp.min(jnp.where(r2 == m2, idx, S)), 0, S - 1)
        idx_s[0] = i1
        idx_s[1] = i2
        rsel_s[0] = m1
        rsel_s[1] = m2
        row16 = _iota((16, 128), 0)
        lane16 = _iota((16, 128), 1)
        xs = None
        for t, i in enumerate((i1, i2)):
            seg = i // L
            off = i - seg * L
            base = pl.multiple_of((off // 128) * 128, 128)
            cols = _unpack(xn_v[_rows(seg, D // 2), pl.ds(base, 128)])
            pick = jnp.where((row16 == t) & (lane16 == off - base), 1.0, 0.0)
            part = _dot_nt(pick.astype(BF16), cols)
            xs = part if xs is None else xs + part
        xs_v[...] = _pack(xs)
        y_v[...] = jnp.zeros(y_v.shape, F32)

    def ffn_hidden():
        xs = _unpack(xs_v[...])
        gt = _round_bf16(_dot(xs, wg_v[...]))
        up = _round_bf16(_dot(xs, wu_v[...]))
        hid = _round_bf16(_round_bf16(gt * jax.nn.sigmoid(gt)) * up)
        for t in range(2):
            for tile in range(FF // 128):
                hid_v[t, tile] = jnp.broadcast_to(
                    hid[t:t + 1, 128 * tile:128 * (tile + 1)], (8, 128))

    def ffn_down_chained():
        base = pl.multiple_of(step * (FT * 128), 128)
        link = [None, None]
        for b in range(D // 8):
            acc = [None, None]
            for tile in range(FT):
                w = wd_v[8 * b:8 * b + 8, pl.ds(base + 128 * tile, 128)].astype(F32)
                for t in range(2):
                    pr = w * hid_v[t, step * FT + tile]
                    if tile > 0:
                        acc[t] = acc[t] + pr
                    else:
                        acc[t] = pr if link[t] is None else pr + nothing(link[t])
            for t in range(2):
                rows = slice(8 * b, 8 * b + 8)
                y_v[t, rows, :] = y_v[t, rows, :] + acc[t]
                link[t] = acc[t]

    def ffn_down_looped():
        def down(tile, carry):
            col = step * FT + tile
            w = wd_v[:, pl.ds(pl.multiple_of(128 * col, 128), 128)].astype(F32)
            for t in range(2):
                y_v[t] = y_v[t] + w * hid_v[t, col][0:1, :]
            return carry

        lax.fori_loop(0, FT, down, 0)

    def masked_q_bits(g, hp, j):
        rid = _iota((64, 128), 0)
        mask = (rid >= (DH // 2) * hp) & (rid < (DH // 2) * (hp + 1))
        return jnp.where(mask, qt_v[_rows(step * NG + g, 64), 128 * j:128 * (j + 1)],
                         jnp.uint32(0))

    def keys(g, lo, hi):
        first = pl.multiple_of((step * NG + g) * (L // 2) + lo // 2, 8)
        return _unpack(k_v[pl.ds(first, (hi - lo) // 2), :])

    def causal_scores(g, hp, j):
        nk = 128 * (j + 1)
        st = _dot(keys(g, 0, nk), _unpack(masked_q_bits(g, hp, j)))
        diag = st[nk - 128:, :] + bias_v[...]
        return diag if j == 0 else jnp.concatenate([st[:nk - 128, :], diag], axis=0)

    def head_output(h, j, p, keep):
        o = _dot(_unpack(vt_v[_rows(step * H + h, 16), 0:128 * (j + 1)]), p)
        den = o[DH:DH + 1, :]
        inv = pl.reciprocal(den, approx=True)
        inv = inv * (2.0 - den * inv)
        return o[0:24, :] * (keep * inv)

    def single_probs(h, j):
        return jnp.exp2(causal_scores(*divmod(h, HPG), j)).astype(BF16)

    def pair_probs(pairs, j, flip):
        low = _iota((64, 128), 1) < 64
        qa, qb = {}, {}
        for h in pairs:
            g, hp = divmod(h, HPG)
            qa[h] = masked_q_bits(g, hp, j)
            qb[h] = pltpu.roll(masked_q_bits(g, hp + 1, j), 64, 1)
        off = {}
        if j > 0:
            for h in pairs:
                g = h // HPG
                for hh, q in ((h, qa[h]), (h + 1, qb[h])):
                    off[hh] = jnp.exp2(_dot(keys(g, 0, 128 * j), _unpack(q)))
        early, late = {}, {}
        for h in pairs:
            g = h // HPG
            k0 = 128 * j
            for which in ((0, 1) if flip else (1, 0)):
                if which == 0:
                    early[h] = _dot(keys(g, k0, k0 + 64),
                                    _unpack(jnp.where(low, qa[h], qb[h])))
                else:
                    late[h] = _dot(keys(g, k0, k0 + 128),
                                   _unpack(jnp.where(low, qb[h], qa[h])))
        probs = {}
        for h in pairs:
            p1 = jnp.exp2(early[h] + half_v[0])
            p2 = jnp.exp2(late[h][0:64, :])
            bottom = late[h][64:128, :]
            pa = jnp.concatenate(
                [jnp.where(low, p1, p2), jnp.exp2(bottom + half_v[1])], axis=0)
            pb = jnp.concatenate(
                [jnp.where(low, p2, p1), jnp.exp2(bottom + half_v[2])], axis=0)
            for hh, pd in ((h, pa), (h + 1, pb)):
                full = pd if j == 0 else jnp.concatenate([off[hh], pd], axis=0)
                probs[hh] = full.astype(BF16)
        return probs

    def attention_bounded():
        pairs = [g * HPG + hp for g in range(NG)
                 for hp in range(0, _heads_in_group(g) - 1, 2)]
        paired = set(pairs) | {h + 1 for h in pairs}
        singles = [h for h in range(H) if h not in paired]
        waves = [(pairs[i:i + 2], j) for i in range(0, len(pairs), 2) for j in range(NQT)]
        waves += [(None, j) for j in range(NQT)]

        def scores(w):
            grp, j = waves[w]
            if grp is None:
                return {h: single_probs(h, j) for h in singles}
            return pair_probs(grp, j, w % 2 == 1)

        def values(w, probs):
            grp, j = waves[w]
            for h, p in probs.items():
                o = head_output(h, j, p, 1.0 - gate_v[h:h + 1, :])
                if grp is not None and h - 1 in grp:
                    o = pltpu.roll(o, 64, 1)
                ot_v[step, DH * h:DH * (h + 1), 128 * j:128 * (j + 1)] = o[0:DH, :]

        pending = scores(0)
        for w in range(len(waves)):
            nxt = scores(w + 1) if w + 1 < len(waves) else None
            values(w, pending)
            pending = nxt
        ffn_down_chained()

    def attention_max_shifted():
        def one_head(h, carry):
            g = h // HPG
            hp = h - g * HPG
            keep = 1.0 - gate_v[pl.ds(h, 1), :]
            for j in range(NQT):
                st = causal_scores(g, hp, j)
                p = jnp.exp2(st - jnp.max(st, axis=0, keepdims=True)).astype(BF16)
                oh_v[h, :, 128 * j:128 * (j + 1)] = head_output(h, j, p, keep)
            return carry

        lax.fori_loop(0, H, one_head, 0)
        for h in range(H):
            ot_v[step, DH * h:DH * (h + 1), :] = oh_v[h, 0:DH, :]
        ffn_down_looped()

    def output_projection(seg):
        mem = jnp.where(seg > 0, mem_v[jnp.maximum(seg - 1, 0), 0:D, :], 0.0)
        heads_out = ot_v[seg, 0:D, :] + mem
        attn = _dot(_unpack(wot[...]), heads_out.astype(BF16))
        base = x_v[seg].astype(F32) + attn
        xn = _unpack(xn_v[_rows(seg, D // 2), :]).astype(F32)
        col = seg * L + _iota((1, L), 1)
        upd = None
        for t in range(2):
            y = _round_bf16(jnp.sum(y_v[t], axis=1, keepdims=True))
            rsel = jnp.full((1, 1), rsel_s[t], F32)
            y = _round_bf16(y * _round_bf16(jax.nn.sigmoid(rsel)))
            part = jnp.where(col == idx_s[t], y, 0.0)
            upd = part if upd is None else upd + part
        o_ref[...] = (base + (xn + upd)).astype(BF16)

    col_blocks = [(c0, min(128, D - c0)) for c0 in range(0, D, 128)]

    def transpose_block(w_v, section, c0, n):
        r0 = (section * D + c0) // 2
        wall[r0:r0 + n // 2, :] = pltpu.bitcast(w_v[:, c0:c0 + n].T, U32)

    def project_block(section, c0, n, xn):
        r0 = (section * D + c0) // 2
        last = section == 2 and c0 + n == D
        hi = PROWS // 2 if last else r0 + n // 2
        return _dot(_unpack(wall[r0:hi, :]), xn)

    def query_half0(half):
        layer_norm(0, serial=False, tiles=[2 * half, 2 * half + 1])
        xn = _unpack(xn_v[0:D // 2, 256 * half:256 * (half + 1)])
        return jnp.concatenate(
            [_dot(_unpack(wall[r:r + D // 4, :]), xn) for r in (0, D // 4)], axis=0)

    def projections():
        qtiles = []
        for half in range(2):
            x0_copies[half].wait()
            if half == 1:
                cp_wk.wait()
            qtiles.append(query_half0(half))
        for c0, n in col_blocks:
            transpose_block(wk_v, 1, c0, n)
        parts = [jnp.concatenate(qtiles, axis=1)]
        cp_wv.wait()
        x_copies[1].wait()
        xn0 = _unpack(xn_v[_rows(0, D // 2), :])
        parts += [project_block(1, c0, n, xn0) for c0, n in col_blocks]
        for c0, n in col_blocks:
            transpose_block(wv_v, 2, c0, n)
            parts.append(project_block(2, c0, n, xn0))
        layer_norm(1)
        _, pk, vg = store_qkv(0, jnp.concatenate(parts, axis=0))
        x_copies[2].wait()
        x_copies[3].wait()
        cp_wo.wait()

        layer_norm(2)
        pt = project(1)
        wot[...] = pltpu.bitcast(wo_v[...].T, U32)
        state1 = memory_update(None, pk, vg)
        pq1, pk, vg = store_qkv(1, pt)
        layer_norm(3)
        pt = project(2)
        state2 = memory_update(state1, pk, vg)
        pq2, pk, vg = store_qkv(2, pt)
        cp_wg.wait()
        cp_wu.wait()
        pt = project(3, router_first=True)
        pq3, _, _ = store_qkv(3, pt)
        route()
        ffn_hidden()
        state3 = memory_update(state2, pk, vg)
        memory_retrieve(1, state1, pq1)
        memory_retrieve(2, state2, pq2)
        memory_retrieve(3, state3, pq3)
        record_logit_bound()
        cp_wd.wait()

    @pl.when(step == 0)
    def _():
        for cp in (cp_wq, cp_wr, cp_beta, *x0_copies, cp_wk, cp_wv, x_copies[1],
                   x_copies[2], x_copies[3], cp_wo, cp_wg, cp_wu, cp_wd):
            cp.start()
        with _scope("sc_startup"):
            cp_wr.wait()
            cp_beta.wait()
            cp_wq.wait()
            init_constants()
            for c0, n in col_blocks:
                transpose_block(wq_v, 0, c0, n)
        with _scope("sc_projections"):
            projections()

    @pl.when(step < NSEG)
    def _():
        safe = safe_s[0] == 1

        @pl.when(safe)
        def _():
            with _scope("sc_attention"):
                attention_bounded()

        @pl.when(jnp.logical_not(safe))
        def _():
            attention_max_shifted()

    @pl.when(step >= NSEG)
    def _():
        with _scope("sc_outproj"):
            output_projection(step - NSEG)


@jax.jit
def pallas_parallel_sum__memory_aug_infini_attn__moe_arch_mod__prompt_kernel(
    A_x: jax.Array,
    A_wq: jax.Array,
    A_wk: jax.Array,
    A_wv: jax.Array,
    A_wo: jax.Array,
    A_beta: jax.Array,
    B_x: jax.Array,
    B_w_r: jax.Array,
    B_w_gate: jax.Array,
    B_w_up: jax.Array,
    B_w_down: jax.Array,
):
    del B_x
    vm = pltpu.VMEM
    scratch = [
        vm((NSEG, D, L), BF16),
        vm((D, D), BF16),
        vm((D, D), BF16),
        vm((D, D), BF16),
        vm((D, D), BF16),
        vm((H,), BF16),
        vm((D,), BF16),
        vm((D, FF), BF16),
        vm((D, FF), BF16),
        vm((D, FF), BF16),
        vm((PROWS // 2, D), U32),
        vm((D // 2, D), U32),
        vm((NSEG * D // 2, L), U32),
        vm((NSEG * NG * 64, L), U32),
        vm((NSEG * NG * L // 2, 128), U32),
        vm((NSEG * H * 16, L), U32),
        vm((NSEG - 1, OROWS, L), F32),
        vm((8, L), F32),
        vm((8, D), U32),
        vm((2, D, 128), F32),
        vm((2, FF // 128, 8, 128), F32),
        pltpu.SMEM((2,), jnp.int32),
        pltpu.SMEM((2,), F32),
        pltpu.SMEM((1,), U32),
        pltpu.SMEM((1,), jnp.int32),
        vm((H, 128), F32),
        vm((NSEG, D, L), F32),
        vm((H, 24, L), F32),
        vm((128, 128), F32),
        vm((3, 64, 128), F32),
        pltpu.SemaphoreType.DMA((NSEG + 9 + 2,)),
    ]
    hbm = pl.BlockSpec(memory_space=pltpu.HBM)
    xt = jnp.transpose(A_x.reshape(S, D))
    out_t = pl.pallas_call(
        _kernel,
        grid=(2 * NSEG,),
        in_specs=[hbm] * 10,
        out_specs=pl.BlockSpec((D, L), lambda s: (0, jnp.maximum(s - NSEG, 0))),
        out_shape=jax.ShapeDtypeStruct((D, S), BF16),
        scratch_shapes=scratch,
        compiler_params=pltpu.CompilerParams(
            dimension_semantics=("arbitrary",),
            vmem_limit_bytes=110 * 1024 * 1024,
        ),
        name="infini_moe",
    )(xt, A_wq, A_wk, A_wv, A_wo, A_beta, B_w_r, B_w_gate, B_w_up,
      jnp.transpose(B_w_down))
    return jnp.transpose(out_t).reshape(1, S, D)
```

```python
import contextlib

import jax
import jax.numpy as jnp
from jax import lax
from jax.experimental import pallas as pl
from jax.experimental.pallas import tpu as pltpu

S = 2048
D = 576
H = 32
DH = 18
NSEG = 4
L = 512
FF = 4608
NG = 5
HPG = 7
GW = HPG * DH
NQT = L // 128
PROWS = 3 * D + 16
RROW = 3 * D
PBLOCK = 128
MROWS = 144
FT = FF // 128 // NSEG
OROWS = 640
LOG2E = 1.4426950408889634
QSCALE = DH ** -0.5 * LOG2E
NEG = -1e30
LN_EPS = 1.0013580322265625e-05
F32 = jnp.float32
BF16 = jnp.bfloat16
U32 = jnp.uint32

PROFILE_SCOPES = False

_NN = (((1,), (0,)), ((), ()))
_NT = (((1,), (1,)), ((), ()))


def _scope(name):
    return jax.named_scope(name) if PROFILE_SCOPES else contextlib.nullcontext()


def _dot(a, b):
    return lax.dot_general(a, b, _NN, preferred_element_type=F32)


def _dot_nt(a, b):
    return lax.dot_general(a, b, _NT, preferred_element_type=F32)


def _iota(shape, dim):
    return lax.broadcasted_iota(jnp.int32, shape, dim)


def _round_bf16(v):
    return v.astype(BF16).astype(F32)


def _pack(v):
    return pltpu.bitcast(v.astype(BF16), U32)


def _unpack(u):
    return pltpu.bitcast(u, BF16)


def _rows(index, size):
    if isinstance(index, int):
        return slice(index * size, (index + 1) * size)
    return pl.ds(pl.multiple_of(index * size, 8), size)


def _heads_in_group(g):
    return HPG if g < NG - 1 else H - HPG * (NG - 1)


def _phi(t):
    return jnp.where(t > 0, t + 1.0, jnp.exp(t))


def _kernel(x_hbm, wq_hbm, wk_hbm, wv_hbm, wo_hbm, beta_hbm, wr_hbm,
            wg_hbm, wu_hbm, wd_hbm,
            o_hbm,
            x_v, wq_v, wk_v, wv_v, wo_v, beta_v, wr_v, wg_v, wu_v, wd_v,
            wall, wot, xn_v, qt_v, k_v, vt_v, mem_v,
            r_v, xs_v, y_v, hid_v, idx_s, rsel_s, zero_s, safe_s,
            gate_v, ot_v, oh_v, bias_v, half_v, out_v, out_sems,
            sems):
    step = pl.program_id(0)

    x_copies = [None] + [
        pltpu.make_async_copy(x_hbm.at[:, pl.ds(c * L, L)], x_v.at[c], sems.at[c])
        for c in range(1, NSEG)
    ]
    x0_copies = [
        pltpu.make_async_copy(x_hbm.at[:, pl.ds(256 * n, 256)],
                              x_v.at[0, :, pl.ds(256 * n, 256)],
                              sems.at[NSEG + 9 + n])
        for n in range(2)
    ]
    pairs = [(wq_hbm, wq_v), (wk_hbm, wk_v), (wv_hbm, wv_v), (wo_hbm, wo_v),
             (beta_hbm, beta_v), (wr_hbm, wr_v),
             (wg_hbm, wg_v), (wu_hbm, wu_v), (wd_hbm, wd_v)]
    (cp_wq, cp_wk, cp_wv, cp_wo, cp_beta, cp_wr, cp_wg, cp_wu, cp_wd) = [
        pltpu.make_async_copy(src, dst, sems.at[NSEG + i])
        for i, (src, dst) in enumerate(pairs)
    ]

    def nothing(v):
        return pltpu.bitcast(pltpu.bitcast(v, U32) & zero_s[0], F32)

    def layer_norm(c, serial=True, tiles=range(NQT)):
        link = None
        for n in tiles:
            cols = slice(128 * n, 128 * (n + 1))
            pivot = x_v[c, 0:16, cols].astype(F32)[0:1, :]
            pivot8 = jnp.broadcast_to(pivot, (8, 128))
            shift = pivot8
            s1 = s2 = None
            for i in range(D // 16):
                last = s1 if s1 is not None else link
                if serial and last is not None:
                    shift = pivot8 + nothing(last)
                x16 = x_v[c, 16 * i:16 * i + 16, cols].astype(F32)
                for k in range(2):
                    d = x16[8 * k:8 * k + 8, :] - shift
                    s1 = d if s1 is None else s1 + d
                    s2 = d * d if s2 is None else s2 + d * d
            dmean = jnp.sum(s1, axis=0, keepdims=True) * (1.0 / D)
            dsq = jnp.sum(s2, axis=0, keepdims=True) * (1.0 / D)
            var = jnp.maximum(dsq - dmean * dmean, 0.0)
            sd = _round_bf16(jnp.sqrt(_round_bf16(_round_bf16(var) + LN_EPS)))
            mean8 = jnp.broadcast_to(_round_bf16(pivot + dmean), (8, 128))
            inv8 = jnp.broadcast_to(1.0 / sd, (8, 128))
            center = mean8
            for i in range(D // 32):
                if serial and i > 0:
                    center = mean8 + nothing(link)
                x32 = x_v[c, 32 * i:32 * i + 32, cols].astype(F32)
                z = [(x32[8 * k:8 * k + 8, :] - center) * inv8 for k in range(4)]
                link = z[3]
                r0 = c * (D // 2) + 16 * i
                xn_v[r0:r0 + 16, cols] = _pack(jnp.concatenate(z, axis=0))

    def init_constants():
        gate = jax.nn.sigmoid(beta_v[...].astype(F32).reshape(1, H))
        on_diag = _iota((H, H), 0) == _iota((H, H), 1)
        gcol = jnp.sum(jnp.where(on_diag, gate, 0.0), axis=1, keepdims=True)
        gate_v[...] = jnp.broadcast_to(gcol, (H, 128))
        zero_s[0] = jnp.uint32(0)
        bias_v[...] = jnp.where(_iota((128, 128), 0) > _iota((128, 128), 1), NEG, 0.0)
        key, lane = _iota((64, 128), 0), _iota((64, 128), 1)
        future = key > (lane & 63)
        half_v[0] = jnp.where(future, NEG, 0.0)
        half_v[1] = jnp.where(future | (lane < 64), NEG, 0.0)
        half_v[2] = jnp.where(future | (lane >= 64), NEG, 0.0)
        router = jnp.broadcast_to(wr_v[...].astype(F32).reshape(1, D), (16, D))
        wall[RROW // 2:PROWS // 2, :] = _pack(
            jnp.where(_iota((16, D), 0) == 0, router, 0.0))

    def project(c, router_first=False):
        xn = _unpack(xn_v[_rows(c, D // 2), :])
        step_rows = PBLOCK // 2
        end = RROW // 2 if router_first else PROWS // 2
        tail = [_dot(_unpack(wall[end:PROWS // 2, :]), xn)] if router_first else []
        return jnp.concatenate(
            [_dot(_unpack(wall[r:min(r + step_rows, end), :]), xn)
             for r in range(0, end, step_rows)] + tail, axis=0)

    seen = [None]

    def record_logit_bound():
        big = (seen[0] >> 30) & 1
        safe_s[0] = (jnp.max(big.astype(jnp.int32)) == 0).astype(jnp.int32)

    def store_qkv(c, pt):
        r_v[c:c + 1, :] = _round_bf16(pt[RROW:RROW + 1, :])
        tail_row = _iota((8, L), 0)
        for h in range(H):
            base = 2 * D + DH * h
            tail = jnp.where(tail_row < DH - 16, pt[base + 16:base + 24, :],
                             jnp.where(tail_row == DH - 16, 1.0, 0.0))
            blk = jnp.concatenate(
                [pt[base:base + 16, :], tail, jnp.zeros((8, L), F32)], axis=0)
            vt_v[_rows(c * H + h, 16), :] = _pack(blk)

        rowl = _iota((128, L), 0)
        pqs, pks, vgs = [], [], []
        for g in range(NG):
            used = _heads_in_group(g) * DH
            qg = pt[GW * g:GW * g + 128, :]
            qs = qg * QSCALE
            qt_v[_rows(c * NG + g, 64), :] = _pack(qs)
            kg = pt[D + GW * g:D + GW * g + 128, :]
            for operand in (qs, kg):
                bits = pltpu.bitcast(operand, U32)
                for blk in range(0, 128 if g < NG - 1 else used, 8):
                    for col in range(0, L, 128):
                        piece = bits[blk:blk + 8, col:col + 128]
                        seen[0] = piece if seen[0] is None else seen[0] | piece
            k_v[_rows(c * NG + g, L // 2), :] = _pack(kg.T)
            pqs.append(_phi(qg).astype(BF16))
            if c < NSEG - 1:
                pks.append(_phi(kg).astype(BF16))
                lo = 2 * D + GW * g
                if g < NG - 1:
                    vg = pt[lo:lo + 128, :]
                else:
                    vg = jnp.concatenate(
                        [pt[lo:lo + used, :], jnp.zeros((128 - used, L), F32)], axis=0)
                vg = jnp.where(rowl < used, vg, jnp.where(rowl == GW, 1.0, 0.0))
                vgs.append(vg.astype(BF16))
        return pqs, pks, vgs

    def memory_update(states, pks, vgs):
        row = _iota((128, 128), 0)
        lane = _iota((128, 128), 1)
        same_head = (row // DH) == (lane // DH)
        out = []
        for g in range(NG):
            used = _heads_in_group(g) * DH
            upd = _dot_nt(vgs[g], pks[g])
            keep = ((same_head & (row < used)) | (row == GW)) & (lane < used)
            upd = jnp.where(keep, upd, 0.0)
            out.append(upd if states is None else states[g] + upd)
        return out

    def memory_retrieve(c, states, pqs):
        row = _iota((128, 128), 0)
        row8 = _iota((8, 128), 0)
        lane8 = _iota((8, 128), 1) // DH
        for g in range(NG):
            nh = _heads_in_group(g)
            st = states[g]
            mrows = jnp.where(row < GW, st, 0.0)
            zrows = jnp.where(lane8 == row8, st[GW:GW + 1, :], 0.0)
            lhs = jnp.concatenate(
                [mrows, zrows, jnp.zeros((8, 128), F32)], axis=0).astype(BF16)
            ret = _dot(lhs, pqs[g])
            gsel = gate_v[HPG * g:HPG * g + 8, :] if g < NG - 1 else jnp.concatenate(
                [gate_v[HPG * g:H, :], jnp.zeros((8 - nh, 128), F32)], axis=0)
            gwide = jnp.concatenate([gsel] * NQT, axis=1)
            scale = gwide / (ret[128:136, :] + 1e-6)
            pieces = []
            for b in range(16):
                h0 = min((8 * b) // DH, nh - 1)
                h1 = min((8 * b + 7) // DH, nh - 1)
                sc = scale[h0:h0 + 1, :]
                if h1 != h0:
                    first = _iota((8, L), 0) < DH * h1 - 8 * b
                    sc = jnp.where(first, sc, scale[h1:h1 + 1, :])
                pieces.append(ret[8 * b:8 * b + 8, :] * sc)
            mem_v[c - 1, GW * g:GW * g + 128, :] = jnp.concatenate(pieces, axis=0)

    def route():
        r = r_v[0:NSEG, :]
        idx = _iota((NSEG, L), 0) * L + _iota((NSEG, L), 1)
        m1 = jnp.max(r)
        i1 = jnp.clip(jnp.min(jnp.where(r == m1, idx, S)), 0, S - 1)
        r2 = jnp.where(idx == i1, -jnp.inf, r)
        m2 = jnp.max(r2)
        i2 = jnp.clip(jnp.min(jnp.where(r2 == m2, idx, S)), 0, S - 1)
        idx_s[0] = i1
        idx_s[1] = i2
        rsel_s[0] = m1
        rsel_s[1] = m2
        row16 = _iota((16, 128), 0)
        lane16 = _iota((16, 128), 1)
        xs = None
        for t, i in enumerate((i1, i2)):
            seg = i // L
            off = i - seg * L
            base = pl.multiple_of((off // 128) * 128, 128)
            cols = _unpack(xn_v[_rows(seg, D // 2), pl.ds(base, 128)])
            pick = jnp.where((row16 == t) & (lane16 == off - base), 1.0, 0.0)
            part = _dot_nt(pick.astype(BF16), cols)
            xs = part if xs is None else xs + part
        xs_v[...] = _pack(xs)
        y_v[...] = jnp.zeros(y_v.shape, F32)

    def ffn_hidden():
        xs = _unpack(xs_v[...])
        gt = _round_bf16(_dot(xs, wg_v[...]))
        up = _round_bf16(_dot(xs, wu_v[...]))
        hid = _round_bf16(_round_bf16(gt * jax.nn.sigmoid(gt)) * up)
        for t in range(2):
            for tile in range(FF // 128):
                hid_v[t, tile] = jnp.broadcast_to(
                    hid[t:t + 1, 128 * tile:128 * (tile + 1)], (8, 128))

    def ffn_down_chained():
        base = pl.multiple_of(step * (FT * 128), 128)
        link = [None, None]
        for b in range(D // 8):
            acc = [None, None]
            for tile in range(FT):
                w = wd_v[8 * b:8 * b + 8, pl.ds(base + 128 * tile, 128)].astype(F32)
                for t in range(2):
                    pr = w * hid_v[t, step * FT + tile]
                    if tile > 0:
                        acc[t] = acc[t] + pr
                    else:
                        acc[t] = pr if link[t] is None else pr + nothing(link[t])
            for t in range(2):
                rows = slice(8 * b, 8 * b + 8)
                y_v[t, rows, :] = y_v[t, rows, :] + acc[t]
                link[t] = acc[t]

    def ffn_down_looped():
        def down(tile, carry):
            col = step * FT + tile
            w = wd_v[:, pl.ds(pl.multiple_of(128 * col, 128), 128)].astype(F32)
            for t in range(2):
                y_v[t] = y_v[t] + w * hid_v[t, col][0:1, :]
            return carry

        lax.fori_loop(0, FT, down, 0)

    def masked_q_bits(g, hp, j):
        rid = _iota((64, 128), 0)
        mask = (rid >= (DH // 2) * hp) & (rid < (DH // 2) * (hp + 1))
        return jnp.where(mask, qt_v[_rows(step * NG + g, 64), 128 * j:128 * (j + 1)],
                         jnp.uint32(0))

    def keys(g, lo, hi):
        first = pl.multiple_of((step * NG + g) * (L // 2) + lo // 2, 8)
        return _unpack(k_v[pl.ds(first, (hi - lo) // 2), :])

    def causal_scores(g, hp, j):
        nk = 128 * (j + 1)
        st = _dot(keys(g, 0, nk), _unpack(masked_q_bits(g, hp, j)))
        diag = st[nk - 128:, :] + bias_v[...]
        return diag if j == 0 else jnp.concatenate([st[:nk - 128, :], diag], axis=0)

    def head_output(h, j, p, keep):
        o = _dot(_unpack(vt_v[_rows(step * H + h, 16), 0:128 * (j + 1)]), p)
        den = o[DH:DH + 1, :]
        inv = pl.reciprocal(den, approx=True)
        inv = inv * (2.0 - den * inv)
        return o[0:24, :] * (keep * inv)

    def single_probs(h, j):
        return jnp.exp2(causal_scores(*divmod(h, HPG), j)).astype(BF16)

    def pair_probs(pairs, j, flip):
        low = _iota((64, 128), 1) < 64
        qa, qb = {}, {}
        for h in pairs:
            g, hp = divmod(h, HPG)
            qa[h] = masked_q_bits(g, hp, j)
            qb[h] = pltpu.roll(masked_q_bits(g, hp + 1, j), 64, 1)
        off = {}
        if j > 0:
            for h in pairs:
                g = h // HPG
                for hh, q in ((h, qa[h]), (h + 1, qb[h])):
                    off[hh] = jnp.exp2(_dot(keys(g, 0, 128 * j), _unpack(q)))
        early, late = {}, {}
        for h in pairs:
            g = h // HPG
            k0 = 128 * j
            for which in ((0, 1) if flip else (1, 0)):
                if which == 0:
                    early[h] = _dot(keys(g, k0, k0 + 64),
                                    _unpack(jnp.where(low, qa[h], qb[h])))
                else:
                    late[h] = _dot(keys(g, k0, k0 + 128),
                                   _unpack(jnp.where(low, qb[h], qa[h])))
        probs = {}
        for h in pairs:
            p1 = jnp.exp2(early[h] + half_v[0])
            p2 = jnp.exp2(late[h][0:64, :])
            bottom = late[h][64:128, :]
            pa = jnp.concatenate(
                [jnp.where(low, p1, p2), jnp.exp2(bottom + half_v[1])], axis=0)
            pb = jnp.concatenate(
                [jnp.where(low, p2, p1), jnp.exp2(bottom + half_v[2])], axis=0)
            for hh, pd in ((h, pa), (h + 1, pb)):
                full = pd if j == 0 else jnp.concatenate([off[hh], pd], axis=0)
                probs[hh] = full.astype(BF16)
        return probs

    def attention_bounded():
        pairs = [g * HPG + hp for g in range(NG)
                 for hp in range(0, _heads_in_group(g) - 1, 2)]
        paired = set(pairs) | {h + 1 for h in pairs}
        singles = [h for h in range(H) if h not in paired]
        waves = [(pairs[i:i + 2], j) for i in range(0, len(pairs), 2) for j in range(NQT)]
        waves += [(None, j) for j in range(NQT)]

        def scores(w):
            grp, j = waves[w]
            if grp is None:
                return {h: single_probs(h, j) for h in singles}
            return pair_probs(grp, j, w % 2 == 1)

        def values(w, probs):
            grp, j = waves[w]
            for h, p in probs.items():
                o = head_output(h, j, p, 1.0 - gate_v[h:h + 1, :])
                if grp is not None and h - 1 in grp:
                    o = pltpu.roll(o, 64, 1)
                ot_v[step, DH * h:DH * (h + 1), 128 * j:128 * (j + 1)] = o[0:DH, :]

        pending = scores(0)
        for w in range(len(waves)):
            nxt = scores(w + 1) if w + 1 < len(waves) else None
            values(w, pending)
            pending = nxt
        ffn_down_chained()

    def attention_max_shifted():
        def one_head(h, carry):
            g = h // HPG
            hp = h - g * HPG
            keep = 1.0 - gate_v[pl.ds(h, 1), :]
            for j in range(NQT):
                st = causal_scores(g, hp, j)
                p = jnp.exp2(st - jnp.max(st, axis=0, keepdims=True)).astype(BF16)
                oh_v[h, :, 128 * j:128 * (j + 1)] = head_output(h, j, p, keep)
            return carry

        lax.fori_loop(0, H, one_head, 0)
        for h in range(H):
            ot_v[step, DH * h:DH * (h + 1), :] = oh_v[h, 0:DH, :]
        ffn_down_looped()

    def output_projection(seg):
        heads_out = ot_v[seg, 0:D, :]
        if seg > 0:
            heads_out = heads_out + mem_v[seg - 1, 0:D, :]
        attn = _dot(_unpack(wot[...]), heads_out.astype(BF16))
        base = x_v[seg].astype(F32) + attn
        xn = _unpack(xn_v[_rows(seg, D // 2), :]).astype(F32)
        col = seg * L + _iota((1, L), 1)
        upd = None
        for t in range(2):
            y = _round_bf16(jnp.sum(y_v[t], axis=1, keepdims=True))
            rsel = jnp.full((1, 1), rsel_s[t], F32)
            y = _round_bf16(y * _round_bf16(jax.nn.sigmoid(rsel)))
            part = jnp.where(col == idx_s[t], y, 0.0)
            upd = part if upd is None else upd + part
        result = base + (xn + upd)
        copies = []
        for n in range(NQT):
            cols = slice(128 * n, 128 * (n + 1))
            out_v[seg * D:(seg + 1) * D, cols] = result[:, cols].astype(BF16)
            cp = pltpu.make_async_copy(
                out_v.at[pl.ds(seg * D, D), pl.ds(128 * n, 128)],
                o_hbm.at[:, pl.ds(seg * L + 128 * n, 128)],
                out_sems.at[NQT * seg + n])
            cp.start()
            copies.append(cp)
        return copies

    col_blocks = [(c0, min(128, D - c0)) for c0 in range(0, D, 128)]

    def transpose_block(w_v, section, c0, n):
        r0 = (section * D + c0) // 2
        wall[r0:r0 + n // 2, :] = pltpu.bitcast(w_v[:, c0:c0 + n].T, U32)

    def project_block(section, c0, n, xn):
        r0 = (section * D + c0) // 2
        last = section == 2 and c0 + n == D
        hi = PROWS // 2 if last else r0 + n // 2
        return _dot(_unpack(wall[r0:hi, :]), xn)

    def query_half0(half):
        layer_norm(0, serial=False, tiles=[2 * half, 2 * half + 1])
        xn = _unpack(xn_v[0:D // 2, 256 * half:256 * (half + 1)])
        return jnp.concatenate(
            [_dot(_unpack(wall[r:r + D // 4, :]), xn) for r in (0, D // 4)], axis=0)

    def projections():
        qtiles = []
        for half in range(2):
            x0_copies[half].wait()
            if half == 1:
                cp_wk.wait()
            qtiles.append(query_half0(half))
        for c0, n in col_blocks:
            transpose_block(wk_v, 1, c0, n)
        parts = [jnp.concatenate(qtiles, axis=1)]
        cp_wv.wait()
        x_copies[1].wait()
        xn0 = _unpack(xn_v[_rows(0, D // 2), :])
        parts += [project_block(1, c0, n, xn0) for c0, n in col_blocks]
        for c0, n in col_blocks:
            transpose_block(wv_v, 2, c0, n)
            parts.append(project_block(2, c0, n, xn0))
        layer_norm(1)
        _, pk, vg = store_qkv(0, jnp.concatenate(parts, axis=0))
        x_copies[2].wait()
        x_copies[3].wait()
        cp_wo.wait()

        layer_norm(2)
        pt = project(1)
        wot[...] = pltpu.bitcast(wo_v[...].T, U32)
        state1 = memory_update(None, pk, vg)
        pq1, pk, vg = store_qkv(1, pt)
        layer_norm(3)
        pt = project(2)
        state2 = memory_update(state1, pk, vg)
        pq2, pk, vg = store_qkv(2, pt)
        cp_wg.wait()
        cp_wu.wait()
        pt = project(3, router_first=True)
        pq3, _, _ = store_qkv(3, pt)
        route()
        ffn_hidden()
        state3 = memory_update(state2, pk, vg)
        memory_retrieve(1, state1, pq1)
        memory_retrieve(2, state2, pq2)
        memory_retrieve(3, state3, pq3)
        record_logit_bound()
        cp_wd.wait()

    @pl.when(step == 0)
    def _():
        for cp in (cp_wq, cp_wr, cp_beta, *x0_copies, cp_wk, cp_wv, x_copies[1],
                   x_copies[2], x_copies[3], cp_wo, cp_wg, cp_wu, cp_wd):
            cp.start()
        with _scope("sc_startup"):
            cp_wr.wait()
            cp_beta.wait()
            cp_wq.wait()
            init_constants()
            for c0, n in col_blocks:
                transpose_block(wq_v, 0, c0, n)
        with _scope("sc_projections"):
            projections()

    @pl.when(step < NSEG)
    def _():
        safe = safe_s[0] == 1

        @pl.when(safe)
        def _():
            with _scope("sc_attention"):
                attention_bounded()

        @pl.when(jnp.logical_not(safe))
        def _():
            attention_max_shifted()

    @pl.when(step == NSEG)
    def _():
        with _scope("sc_outproj"):
            pending = []
            for seg in range(NSEG):
                pending += output_projection(seg)
            for cp in pending:
                cp.wait()


@jax.jit
def pallas_parallel_sum__memory_aug_infini_attn__moe_arch_mod__prompt_kernel(
    A_x: jax.Array,
    A_wq: jax.Array,
    A_wk: jax.Array,
    A_wv: jax.Array,
    A_wo: jax.Array,
    A_beta: jax.Array,
    B_x: jax.Array,
    B_w_r: jax.Array,
    B_w_gate: jax.Array,
    B_w_up: jax.Array,
    B_w_down: jax.Array,
):
    del B_x
    vm = pltpu.VMEM
    scratch = [
        vm((NSEG, D, L), BF16),
        vm((D, D), BF16),
        vm((D, D), BF16),
        vm((D, D), BF16),
        vm((D, D), BF16),
        vm((H,), BF16),
        vm((D,), BF16),
        vm((D, FF), BF16),
        vm((D, FF), BF16),
        vm((D, FF), BF16),
        vm((PROWS // 2, D), U32),
        vm((D // 2, D), U32),
        vm((NSEG * D // 2, L), U32),
        vm((NSEG * NG * 64, L), U32),
        vm((NSEG * NG * L // 2, 128), U32),
        vm((NSEG * H * 16, L), U32),
        vm((NSEG - 1, OROWS, L), F32),
        vm((8, L), F32),
        vm((8, D), U32),
        vm((2, D, 128), F32),
        vm((2, FF // 128, 8, 128), F32),
        pltpu.SMEM((2,), jnp.int32),
        pltpu.SMEM((2,), F32),
        pltpu.SMEM((1,), U32),
        pltpu.SMEM((1,), jnp.int32),
        vm((H, 128), F32),
        vm((NSEG, D, L), F32),
        vm((H, 24, L), F32),
        vm((128, 128), F32),
        vm((3, 64, 128), F32),
        vm((NSEG * D, L), BF16),
        pltpu.SemaphoreType.DMA((NSEG * NQT,)),
        pltpu.SemaphoreType.DMA((NSEG + 9 + 2,)),
    ]
    hbm = pl.BlockSpec(memory_space=pltpu.HBM)
    xt = jnp.transpose(A_x.reshape(S, D))
    out_t = pl.pallas_call(
        _kernel,
        grid=(NSEG + 1,),
        in_specs=[hbm] * 10,
        out_specs=hbm,
        out_shape=jax.ShapeDtypeStruct((D, S), BF16),
        scratch_shapes=scratch,
        compiler_params=pltpu.CompilerParams(
            dimension_semantics=("arbitrary",),
            vmem_limit_bytes=110 * 1024 * 1024,
        ),
        name="infini_moe",
    )(xt, A_wq, A_wk, A_wv, A_wo, A_beta, B_w_r, B_w_gate, B_w_up,
      jnp.transpose(B_w_down))
    return jnp.transpose(out_t).reshape(1, S, D)
```

```python
import contextlib

import jax
import jax.numpy as jnp
from jax import lax
from jax.experimental import pallas as pl
from jax.experimental.pallas import tpu as pltpu

S = 2048
D = 576
H = 32
DH = 18
NSEG = 4
L = 512
FF = 4608
NG = 5
HPG = 7
GW = HPG * DH
NQT = L // 128
PROWS = 3 * D + 16
RROW = 3 * D
PBLOCK = 128
MROWS = 144
FT = FF // 128 // NSEG
OROWS = 640
LOG2E = 1.4426950408889634
QSCALE = DH ** -0.5 * LOG2E
NEG = -1e30
LN_EPS = 1.0013580322265625e-05
F32 = jnp.float32
BF16 = jnp.bfloat16
U32 = jnp.uint32

PROFILE_SCOPES = False

_NN = (((1,), (0,)), ((), ()))
_NT = (((1,), (1,)), ((), ()))


def _scope(name):
    return jax.named_scope(name) if PROFILE_SCOPES else contextlib.nullcontext()


def _dot(a, b):
    return lax.dot_general(a, b, _NN, preferred_element_type=F32)


def _dot_nt(a, b):
    return lax.dot_general(a, b, _NT, preferred_element_type=F32)


def _iota(shape, dim):
    return lax.broadcasted_iota(jnp.int32, shape, dim)


def _round_bf16(v):
    return v.astype(BF16).astype(F32)


def _pack(v):
    return pltpu.bitcast(v.astype(BF16), U32)


def _unpack(u):
    return pltpu.bitcast(u, BF16)


def _rows(index, size):
    if isinstance(index, int):
        return slice(index * size, (index + 1) * size)
    return pl.ds(pl.multiple_of(index * size, 8), size)


def _heads_in_group(g):
    return HPG if g < NG - 1 else H - HPG * (NG - 1)


def _phi(t):
    return jnp.where(t > 0, t + 1.0, jnp.exp(t))


def _kernel(x_hbm, wq_hbm, wk_hbm, wv_hbm, wo_hbm, beta_hbm, wr_hbm,
            wg_hbm, wu_hbm, wd_hbm,
            o_hbm,
            x_v, wq_v, wk_v, wv_v, wo_v, beta_v, wr_v, wg_v, wu_v, wd_v,
            wall, wot, xn_v, qt_v, k_v, vt_v, mem_v,
            r_v, xs_v, y_v, hid_v, idx_s, rsel_s, zero_s, safe_s,
            gate_v, ot_v, oh_v, bias_v, half_v, out_v, out_sems,
            sems):
    step = pl.program_id(0)

    x_copies = [None] + [
        pltpu.make_async_copy(x_hbm.at[:, pl.ds(c * L, L)], x_v.at[c], sems.at[c])
        for c in range(1, NSEG)
    ]
    x0_copies = [
        pltpu.make_async_copy(x_hbm.at[:, pl.ds(256 * n, 256)],
                              x_v.at[0, :, pl.ds(256 * n, 256)],
                              sems.at[NSEG + 9 + n])
        for n in range(2)
    ]
    pairs = [(wq_hbm, wq_v), (wk_hbm, wk_v), (wv_hbm, wv_v), (wo_hbm, wo_v),
             (beta_hbm, beta_v), (wr_hbm, wr_v),
             (wg_hbm, wg_v), (wu_hbm, wu_v), (wd_hbm, wd_v)]
    (cp_wq, cp_wk, cp_wv, cp_wo, cp_beta, cp_wr, cp_wg, cp_wu, cp_wd) = [
        pltpu.make_async_copy(src, dst, sems.at[NSEG + i])
        for i, (src, dst) in enumerate(pairs)
    ]

    def nothing(v):
        return pltpu.bitcast(pltpu.bitcast(v, U32) & zero_s[0], F32)

    def layer_norm(c, serial=True, tiles=range(NQT)):
        link = None
        for n in tiles:
            cols = slice(128 * n, 128 * (n + 1))
            pivot = x_v[c, 0:16, cols].astype(F32)[0:1, :]
            pivot8 = jnp.broadcast_to(pivot, (8, 128))
            shift = pivot8
            s1 = s2 = None
            for i in range(D // 16):
                last = s1 if s1 is not None else link
                if serial and last is not None:
                    shift = pivot8 + nothing(last)
                x16 = x_v[c, 16 * i:16 * i + 16, cols].astype(F32)
                for k in range(2):
                    d = x16[8 * k:8 * k + 8, :] - shift
                    s1 = d if s1 is None else s1 + d
                    s2 = d * d if s2 is None else s2 + d * d
            dmean = jnp.sum(s1, axis=0, keepdims=True) * (1.0 / D)
            dsq = jnp.sum(s2, axis=0, keepdims=True) * (1.0 / D)
            var = jnp.maximum(dsq - dmean * dmean, 0.0)
            sd = _round_bf16(jnp.sqrt(_round_bf16(_round_bf16(var) + LN_EPS)))
            mean8 = jnp.broadcast_to(_round_bf16(pivot + dmean), (8, 128))
            inv8 = jnp.broadcast_to(1.0 / sd, (8, 128))
            center = mean8
            for i in range(D // 32):
                if serial and i > 0:
                    center = mean8 + nothing(link)
                x32 = x_v[c, 32 * i:32 * i + 32, cols].astype(F32)
                z = [(x32[8 * k:8 * k + 8, :] - center) * inv8 for k in range(4)]
                link = z[3]
                r0 = c * (D // 2) + 16 * i
                xn_v[r0:r0 + 16, cols] = _pack(jnp.concatenate(z, axis=0))

    def init_constants():
        gate = jax.nn.sigmoid(beta_v[...].astype(F32).reshape(1, H))
        on_diag = _iota((H, H), 0) == _iota((H, H), 1)
        gcol = jnp.sum(jnp.where(on_diag, gate, 0.0), axis=1, keepdims=True)
        gate_v[...] = jnp.broadcast_to(gcol, (H, 128))
        zero_s[0] = jnp.uint32(0)
        bias_v[...] = jnp.where(_iota((128, 128), 0) > _iota((128, 128), 1), NEG, 0.0)
        key, lane = _iota((64, 128), 0), _iota((64, 128), 1)
        future = key > (lane & 63)
        half_v[0] = jnp.where(future, NEG, 0.0)
        half_v[1] = jnp.where(future | (lane < 64), NEG, 0.0)
        half_v[2] = jnp.where(future | (lane >= 64), NEG, 0.0)
        router = jnp.broadcast_to(wr_v[...].astype(F32).reshape(1, D), (16, D))
        wall[RROW // 2:PROWS // 2, :] = _pack(
            jnp.where(_iota((16, D), 0) == 0, router, 0.0))

    def project(c, router_first=False):
        xn = _unpack(xn_v[_rows(c, D // 2), :])
        step_rows = PBLOCK // 2
        end = RROW // 2 if router_first else PROWS // 2
        tail = [_dot(_unpack(wall[end:PROWS // 2, :]), xn)] if router_first else []
        return jnp.concatenate(
            [_dot(_unpack(wall[r:min(r + step_rows, end), :]), xn)
             for r in range(0, end, step_rows)] + tail, axis=0)

    seen = [None]

    def record_logit_bound():
        big = (seen[0] >> 30) & 1
        safe_s[0] = (jnp.max(big.astype(jnp.int32)) == 0).astype(jnp.int32)

    def store_qkv(c, pt):
        r_v[c:c + 1, :] = _round_bf16(pt[RROW:RROW + 1, :])
        tail_row = _iota((8, L), 0)
        for h in range(H):
            base = 2 * D + DH * h
            tail = jnp.where(tail_row < DH - 16, pt[base + 16:base + 24, :],
                             jnp.where(tail_row == DH - 16, 1.0, 0.0))
            blk = jnp.concatenate(
                [pt[base:base + 16, :], tail, jnp.zeros((8, L), F32)], axis=0)
            vt_v[_rows(c * H + h, 16), :] = _pack(blk)

        rowl = _iota((128, L), 0)
        pqs, pks, vgs = [], [], []
        for g in range(NG):
            used = _heads_in_group(g) * DH
            qg = pt[GW * g:GW * g + 128, :]
            qs = qg * QSCALE
            qt_v[_rows(c * NG + g, 64), :] = _pack(qs)
            kg = pt[D + GW * g:D + GW * g + 128, :]
            for operand in (qs, kg):
                bits = pltpu.bitcast(operand, U32)
                for blk in range(0, 128 if g < NG - 1 else used, 8):
                    for col in range(0, L, 128):
                        piece = bits[blk:blk + 8, col:col + 128]
                        seen[0] = piece if seen[0] is None else seen[0] | piece
            k_v[_rows(c * NG + g, L // 2), :] = _pack(kg.T)
            pqs.append(_phi(qg).astype(BF16))
            if c < NSEG - 1:
                pks.append(_phi(kg).astype(BF16))
                lo = 2 * D + GW * g
                if g < NG - 1:
                    vg = pt[lo:lo + 128, :]
                else:
                    vg = jnp.concatenate(
                        [pt[lo:lo + used, :], jnp.zeros((128 - used, L), F32)], axis=0)
                vg = jnp.where(rowl < used, vg, jnp.where(rowl == GW, 1.0, 0.0))
                vgs.append(vg.astype(BF16))
        return pqs, pks, vgs

    def memory_update(states, pks, vgs):
        row = _iota((128, 128), 0)
        lane = _iota((128, 128), 1)
        same_head = (row // DH) == (lane // DH)
        out = []
        for g in range(NG):
            used = _heads_in_group(g) * DH
            upd = _dot_nt(vgs[g], pks[g])
            keep = ((same_head & (row < used)) | (row == GW)) & (lane < used)
            upd = jnp.where(keep, upd, 0.0)
            out.append(upd if states is None else states[g] + upd)
        return out

    def memory_retrieve(c, states, pqs):
        row = _iota((128, 128), 0)
        row8 = _iota((8, 128), 0)
        lane8 = _iota((8, 128), 1) // DH
        for g in range(NG):
            nh = _heads_in_group(g)
            st = states[g]
            mrows = jnp.where(row < GW, st, 0.0)
            zrows = jnp.where(lane8 == row8, st[GW:GW + 1, :], 0.0)
            lhs = jnp.concatenate(
                [mrows, zrows, jnp.zeros((8, 128), F32)], axis=0).astype(BF16)
            ret = _dot(lhs, pqs[g])
            gsel = gate_v[HPG * g:HPG * g + 8, :] if g < NG - 1 else jnp.concatenate(
                [gate_v[HPG * g:H, :], jnp.zeros((8 - nh, 128), F32)], axis=0)
            gwide = jnp.concatenate([gsel] * NQT, axis=1)
            scale = gwide / (ret[128:136, :] + 1e-6)
            pieces = []
            for b in range(16):
                h0 = min((8 * b) // DH, nh - 1)
                h1 = min((8 * b + 7) // DH, nh - 1)
                sc = scale[h0:h0 + 1, :]
                if h1 != h0:
                    first = _iota((8, L), 0) < DH * h1 - 8 * b
                    sc = jnp.where(first, sc, scale[h1:h1 + 1, :])
                pieces.append(ret[8 * b:8 * b + 8, :] * sc)
            mem_v[c - 1, GW * g:GW * g + 128, :] = jnp.concatenate(pieces, axis=0)

    def route():
        r = r_v[0:NSEG, :]
        idx = _iota((NSEG, L), 0) * L + _iota((NSEG, L), 1)
        m1 = jnp.max(r)
        i1 = jnp.clip(jnp.min(jnp.where(r == m1, idx, S)), 0, S - 1)
        r2 = jnp.where(idx == i1, -jnp.inf, r)
        m2 = jnp.max(r2)
        i2 = jnp.clip(jnp.min(jnp.where(r2 == m2, idx, S)), 0, S - 1)
        idx_s[0] = i1
        idx_s[1] = i2
        rsel_s[0] = m1
        rsel_s[1] = m2
        row16 = _iota((16, 128), 0)
        lane16 = _iota((16, 128), 1)
        xs = None
        for t, i in enumerate((i1, i2)):
            seg = i // L
            off = i - seg * L
            base = pl.multiple_of((off // 128) * 128, 128)
            cols = _unpack(xn_v[_rows(seg, D // 2), pl.ds(base, 128)])
            pick = jnp.where((row16 == t) & (lane16 == off - base), 1.0, 0.0)
            part = _dot_nt(pick.astype(BF16), cols)
            xs = part if xs is None else xs + part
        xs_v[...] = _pack(xs)
        y_v[...] = jnp.zeros(y_v.shape, F32)

    def ffn_hidden():
        xs = _unpack(xs_v[...])
        gt = _round_bf16(_dot(xs, wg_v[...]))
        up = _round_bf16(_dot(xs, wu_v[...]))
        hid = _round_bf16(_round_bf16(gt * jax.nn.sigmoid(gt)) * up)
        for t in range(2):
            for tile in range(FF // 128):
                hid_v[t, tile] = jnp.broadcast_to(
                    hid[t:t + 1, 128 * tile:128 * (tile + 1)], (8, 128))

    def ffn_down_chained():
        base = pl.multiple_of(step * (FT * 128), 128)
        link = [None, None]
        for b in range(D // 8):
            acc = [None, None]
            for tile in range(FT):
                w = wd_v[8 * b:8 * b + 8, pl.ds(base + 128 * tile, 128)].astype(F32)
                for t in range(2):
                    pr = w * hid_v[t, step * FT + tile]
                    if tile > 0:
                        acc[t] = acc[t] + pr
                    else:
                        acc[t] = pr if link[t] is None else pr + nothing(link[t])
            for t in range(2):
                rows = slice(8 * b, 8 * b + 8)
                y_v[t, rows, :] = y_v[t, rows, :] + acc[t]
                link[t] = acc[t]

    def ffn_down_looped():
        def down(tile, carry):
            col = step * FT + tile
            w = wd_v[:, pl.ds(pl.multiple_of(128 * col, 128), 128)].astype(F32)
            for t in range(2):
                y_v[t] = y_v[t] + w * hid_v[t, col][0:1, :]
            return carry

        lax.fori_loop(0, FT, down, 0)

    def masked_q_bits(g, hp, j):
        rid = _iota((64, 128), 0)
        mask = (rid >= (DH // 2) * hp) & (rid < (DH // 2) * (hp + 1))
        return jnp.where(mask, qt_v[_rows(step * NG + g, 64), 128 * j:128 * (j + 1)],
                         jnp.uint32(0))

    def keys(g, lo, hi):
        first = pl.multiple_of((step * NG + g) * (L // 2) + lo // 2, 8)
        return _unpack(k_v[pl.ds(first, (hi - lo) // 2), :])

    def causal_scores(g, hp, j):
        nk = 128 * (j + 1)
        st = _dot(keys(g, 0, nk), _unpack(masked_q_bits(g, hp, j)))
        diag = st[nk - 128:, :] + bias_v[...]
        return diag if j == 0 else jnp.concatenate([st[:nk - 128, :], diag], axis=0)

    def head_output(h, j, p, keep):
        o = _dot(_unpack(vt_v[_rows(step * H + h, 16), 0:128 * (j + 1)]), p)
        den = o[DH:DH + 1, :]
        inv = pl.reciprocal(den, approx=True)
        inv = inv * (2.0 - den * inv)
        return o[0:24, :] * (keep * inv)

    def single_probs(h, j):
        return jnp.exp2(causal_scores(*divmod(h, HPG), j)).astype(BF16)

    def pair_probs(pairs, j, flip):
        low = _iota((64, 128), 1) < 64
        qa, qb = {}, {}
        for h in pairs:
            g, hp = divmod(h, HPG)
            qa[h] = masked_q_bits(g, hp, j)
            qb[h] = pltpu.roll(masked_q_bits(g, hp + 1, j), 64, 1)
        off = {}
        if j > 0:
            for h in pairs:
                g = h // HPG
                for hh, q in ((h, qa[h]), (h + 1, qb[h])):
                    off[hh] = jnp.exp2(_dot(keys(g, 0, 128 * j), _unpack(q)))
        early, late = {}, {}
        for h in pairs:
            g = h // HPG
            k0 = 128 * j
            for which in ((0, 1) if flip else (1, 0)):
                if which == 0:
                    early[h] = _dot(keys(g, k0, k0 + 64),
                                    _unpack(jnp.where(low, qa[h], qb[h])))
                else:
                    late[h] = _dot(keys(g, k0, k0 + 128),
                                   _unpack(jnp.where(low, qb[h], qa[h])))
        probs = {}
        for h in pairs:
            p1 = jnp.exp2(early[h] + half_v[0])
            p2 = jnp.exp2(late[h][0:64, :])
            bottom = late[h][64:128, :]
            pa = jnp.concatenate(
                [jnp.where(low, p1, p2), jnp.exp2(bottom + half_v[1])], axis=0)
            pb = jnp.concatenate(
                [jnp.where(low, p2, p1), jnp.exp2(bottom + half_v[2])], axis=0)
            for hh, pd in ((h, pa), (h + 1, pb)):
                full = pd if j == 0 else jnp.concatenate([off[hh], pd], axis=0)
                probs[hh] = full.astype(BF16)
        return probs

    def attention_bounded():
        pairs = [g * HPG + hp for g in range(NG)
                 for hp in range(0, _heads_in_group(g) - 1, 2)]
        paired = set(pairs) | {h + 1 for h in pairs}
        singles = [h for h in range(H) if h not in paired]
        waves = [(pairs[i:i + 2], j) for i in range(0, len(pairs), 2) for j in range(NQT)]
        waves += [(None, j) for j in range(NQT)]

        def scores(w):
            grp, j = waves[w]
            if grp is None:
                return {h: single_probs(h, j) for h in singles}
            return pair_probs(grp, j, w % 2 == 1)

        def values(w, probs):
            grp, j = waves[w]
            for h, p in probs.items():
                o = head_output(h, j, p, 1.0 - gate_v[h:h + 1, :])
                if grp is not None and h - 1 in grp:
                    o = pltpu.roll(o, 64, 1)
                ot_v[step, DH * h:DH * (h + 1), 128 * j:128 * (j + 1)] = o[0:DH, :]

        pending = scores(0)
        for w in range(len(waves)):
            nxt = scores(w + 1) if w + 1 < len(waves) else None
            values(w, pending)
            pending = nxt
        ffn_down_chained()

    def attention_max_shifted():
        def one_tile(item, carry):
            h = item // NQT
            j = item - h * NQT
            g = h // HPG
            hp = h - g * HPG
            cols = pl.ds(pl.multiple_of(128 * j, 128), 128)
            rid = _iota((64, 128), 0)
            mask = (rid >= (DH // 2) * hp) & (rid < (DH // 2) * (hp + 1))
            qm = jnp.where(mask, qt_v[_rows(step * NG + g, 64), cols], jnp.uint32(0))
            st = _dot(keys(g, 0, L), _unpack(qm))
            future = _iota((L, 128), 0) > 128 * j + _iota((L, 128), 1)
            st = jnp.where(future, NEG, st)
            p = jnp.exp2(st - jnp.max(st, axis=0, keepdims=True)).astype(BF16)
            keep = 1.0 - gate_v[pl.ds(h, 1), :]
            oh_v[h, :, cols] = head_output(h, NQT - 1, p, keep)
            return carry

        lax.fori_loop(0, H * NQT, one_tile, 0)
        for h in range(H):
            ot_v[step, DH * h:DH * (h + 1), :] = oh_v[h, 0:DH, :]
        ffn_down_looped()

    def output_projection(seg):
        heads_out = ot_v[seg, 0:D, :]
        if seg > 0:
            heads_out = heads_out + mem_v[seg - 1, 0:D, :]
        attn = _dot(_unpack(wot[...]), heads_out.astype(BF16))
        base = x_v[seg].astype(F32) + attn
        xn = _unpack(xn_v[_rows(seg, D // 2), :]).astype(F32)
        col = seg * L + _iota((1, L), 1)
        upd = None
        for t in range(2):
            y = _round_bf16(jnp.sum(y_v[t], axis=1, keepdims=True))
            rsel = jnp.full((1, 1), rsel_s[t], F32)
            y = _round_bf16(y * _round_bf16(jax.nn.sigmoid(rsel)))
            part = jnp.where(col == idx_s[t], y, 0.0)
            upd = part if upd is None else upd + part
        result = base + (xn + upd)
        copies = []
        for n in range(NQT):
            cols = slice(128 * n, 128 * (n + 1))
            out_v[seg * D:(seg + 1) * D, cols] = result[:, cols].astype(BF16)
            cp = pltpu.make_async_copy(
                out_v.at[pl.ds(seg * D, D), pl.ds(128 * n, 128)],
                o_hbm.at[:, pl.ds(seg * L + 128 * n, 128)],
                out_sems.at[NQT * seg + n])
            cp.start()
            copies.append(cp)
        return copies

    col_blocks = [(c0, min(128, D - c0)) for c0 in range(0, D, 128)]

    def transpose_block(w_v, section, c0, n):
        r0 = (section * D + c0) // 2
        wall[r0:r0 + n // 2, :] = pltpu.bitcast(w_v[:, c0:c0 + n].T, U32)

    def project_block(section, c0, n, xn):
        r0 = (section * D + c0) // 2
        last = section == 2 and c0 + n == D
        hi = PROWS // 2 if last else r0 + n // 2
        return _dot(_unpack(wall[r0:hi, :]), xn)

    def query_half0(half):
        layer_norm(0, serial=False, tiles=[2 * half, 2 * half + 1])
        xn = _unpack(xn_v[0:D // 2, 256 * half:256 * (half + 1)])
        return jnp.concatenate(
            [_dot(_unpack(wall[r:r + D // 4, :]), xn) for r in (0, D // 4)], axis=0)

    def projections():
        qtiles = []
        for half in range(2):
            x0_copies[half].wait()
            if half == 1:
                cp_wk.wait()
            qtiles.append(query_half0(half))
        for c0, n in col_blocks:
            transpose_block(wk_v, 1, c0, n)
        parts = [jnp.concatenate(qtiles, axis=1)]
        cp_wv.wait()
        x_copies[1].wait()
        xn0 = _unpack(xn_v[_rows(0, D // 2), :])
        parts += [project_block(1, c0, n, xn0) for c0, n in col_blocks]
        for c0, n in col_blocks:
            transpose_block(wv_v, 2, c0, n)
            parts.append(project_block(2, c0, n, xn0))
        layer_norm(1)
        _, pk, vg = store_qkv(0, jnp.concatenate(parts, axis=0))
        x_copies[2].wait()
        x_copies[3].wait()
        cp_wo.wait()

        layer_norm(2)
        pt = project(1)
        wot[...] = pltpu.bitcast(wo_v[...].T, U32)
        state1 = memory_update(None, pk, vg)
        pq1, pk, vg = store_qkv(1, pt)
        layer_norm(3)
        pt = project(2)
        state2 = memory_update(state1, pk, vg)
        pq2, pk, vg = store_qkv(2, pt)
        cp_wg.wait()
        cp_wu.wait()
        pt = project(3, router_first=True)
        pq3, _, _ = store_qkv(3, pt)
        route()
        ffn_hidden()
        state3 = memory_update(state2, pk, vg)
        memory_retrieve(1, state1, pq1)
        memory_retrieve(2, state2, pq2)
        memory_retrieve(3, state3, pq3)
        record_logit_bound()
        cp_wd.wait()

    @pl.when(step == 0)
    def _():
        for cp in (cp_wq, cp_wr, cp_beta, *x0_copies, cp_wk, cp_wv, x_copies[1],
                   x_copies[2], x_copies[3], cp_wo, cp_wg, cp_wu, cp_wd):
            cp.start()
        with _scope("sc_startup"):
            cp_wr.wait()
            cp_beta.wait()
            cp_wq.wait()
            init_constants()
            for c0, n in col_blocks:
                transpose_block(wq_v, 0, c0, n)
        with _scope("sc_projections"):
            projections()

    @pl.when(step < NSEG)
    def _():
        safe = safe_s[0] == 1

        @pl.when(safe)
        def _():
            with _scope("sc_attention"):
                attention_bounded()

        @pl.when(jnp.logical_not(safe))
        def _():
            attention_max_shifted()

    @pl.when(step == NSEG)
    def _():
        with _scope("sc_outproj"):
            pending = []
            for seg in range(NSEG):
                pending += output_projection(seg)
            for cp in pending:
                cp.wait()


@jax.jit
def pallas_parallel_sum__memory_aug_infini_attn__moe_arch_mod__prompt_kernel(
    A_x: jax.Array,
    A_wq: jax.Array,
    A_wk: jax.Array,
    A_wv: jax.Array,
    A_wo: jax.Array,
    A_beta: jax.Array,
    B_x: jax.Array,
    B_w_r: jax.Array,
    B_w_gate: jax.Array,
    B_w_up: jax.Array,
    B_w_down: jax.Array,
):
    del B_x
    vm = pltpu.VMEM
    scratch = [
        vm((NSEG, D, L), BF16),
        vm((D, D), BF16),
        vm((D, D), BF16),
        vm((D, D), BF16),
        vm((D, D), BF16),
        vm((H,), BF16),
        vm((D,), BF16),
        vm((D, FF), BF16),
        vm((D, FF), BF16),
        vm((D, FF), BF16),
        vm((PROWS // 2, D), U32),
        vm((D // 2, D), U32),
        vm((NSEG * D // 2, L), U32),
        vm((NSEG * NG * 64, L), U32),
        vm((NSEG * NG * L // 2, 128), U32),
        vm((NSEG * H * 16, L), U32),
        vm((NSEG - 1, OROWS, L), F32),
        vm((8, L), F32),
        vm((8, D), U32),
        vm((2, D, 128), F32),
        vm((2, FF // 128, 8, 128), F32),
        pltpu.SMEM((2,), jnp.int32),
        pltpu.SMEM((2,), F32),
        pltpu.SMEM((1,), U32),
        pltpu.SMEM((1,), jnp.int32),
        vm((H, 128), F32),
        vm((NSEG, D, L), F32),
        vm((H, 24, L), F32),
        vm((128, 128), F32),
        vm((3, 64, 128), F32),
        vm((NSEG * D, L), BF16),
        pltpu.SemaphoreType.DMA((NSEG * NQT,)),
        pltpu.SemaphoreType.DMA((NSEG + 9 + 2,)),
    ]
    hbm = pl.BlockSpec(memory_space=pltpu.HBM)
    xt = jnp.transpose(A_x.reshape(S, D))
    out_t = pl.pallas_call(
        _kernel,
        grid=(NSEG + 1,),
        in_specs=[hbm] * 10,
        out_specs=hbm,
        out_shape=jax.ShapeDtypeStruct((D, S), BF16),
        scratch_shapes=scratch,
        compiler_params=pltpu.CompilerParams(
            dimension_semantics=("arbitrary",),
            vmem_limit_bytes=110 * 1024 * 1024,
        ),
        name="infini_moe",
    )(xt, A_wq, A_wk, A_wv, A_wo, A_beta, B_w_r, B_w_gate, B_w_up,
      jnp.transpose(B_w_down))
    return jnp.transpose(out_t).reshape(1, S, D)
```

```python
import contextlib

import jax
import jax.numpy as jnp
from jax import lax
from jax.experimental import pallas as pl
from jax.experimental.pallas import tpu as pltpu

S = 2048
D = 576
H = 32
DH = 18
NSEG = 4
L = 512
FF = 4608
NG = 5
HPG = 7
GW = HPG * DH
NQT = L // 128
PROWS = 3 * D + 16
RROW = 3 * D
PBLOCK = 128
MROWS = 144
FT = FF // 128 // NSEG
OROWS = 640
LOG2E = 1.4426950408889634
QSCALE = DH ** -0.5 * LOG2E
NEG = -1e30
LN_EPS = 1.0013580322265625e-05
F32 = jnp.float32
BF16 = jnp.bfloat16
U32 = jnp.uint32

PROFILE_SCOPES = False

_NN = (((1,), (0,)), ((), ()))
_NT = (((1,), (1,)), ((), ()))


def _scope(name):
    return jax.named_scope(name) if PROFILE_SCOPES else contextlib.nullcontext()


def _dot(a, b):
    return lax.dot_general(a, b, _NN, preferred_element_type=F32)


def _dot_nt(a, b):
    return lax.dot_general(a, b, _NT, preferred_element_type=F32)


def _iota(shape, dim):
    return lax.broadcasted_iota(jnp.int32, shape, dim)


def _round_bf16(v):
    return v.astype(BF16).astype(F32)


def _pack(v):
    return pltpu.bitcast(v.astype(BF16), U32)


def _unpack(u):
    return pltpu.bitcast(u, BF16)


def _rows(index, size):
    if isinstance(index, int):
        return slice(index * size, (index + 1) * size)
    return pl.ds(pl.multiple_of(index * size, 8), size)


def _heads_in_group(g):
    return HPG if g < NG - 1 else H - HPG * (NG - 1)


def _phi(t):
    return jnp.where(t > 0, t + 1.0, jnp.exp(t))


def _kernel(x_hbm, wq_hbm, wk_hbm, wv_hbm, wo_hbm, beta_hbm, wr_hbm,
            wg_hbm, wu_hbm, wd_hbm,
            o_hbm,
            x_v, wq_v, wk_v, wv_v, wo_v, beta_v, wr_v, wg_v, wu_v, wd_v,
            wall, wot, xn_v, qt_v, k_v, vt_v, mem_v,
            r_v, xs_v, y_v, hid_v, idx_s, rsel_s, zero_s, safe_s,
            gate_v, ot_v, oh_v, bias_v, half_v, out_v, out_sems,
            sems):
    step = pl.program_id(0)

    x_copies = [None] + [
        pltpu.make_async_copy(x_hbm.at[:, pl.ds(c * L, L)], x_v.at[c], sems.at[c])
        for c in range(1, NSEG)
    ]
    x0_copies = [
        pltpu.make_async_copy(x_hbm.at[:, pl.ds(256 * n, 256)],
                              x_v.at[0, :, pl.ds(256 * n, 256)],
                              sems.at[NSEG + 9 + n])
        for n in range(2)
    ]
    pairs = [(wq_hbm, wq_v), (wk_hbm, wk_v), (wv_hbm, wv_v), (wo_hbm, wo_v),
             (beta_hbm, beta_v), (wr_hbm, wr_v),
             (wg_hbm, wg_v), (wu_hbm, wu_v), (wd_hbm, wd_v)]
    (cp_wq, cp_wk, cp_wv, cp_wo, cp_beta, cp_wr, cp_wg, cp_wu, cp_wd) = [
        pltpu.make_async_copy(src, dst, sems.at[NSEG + i])
        for i, (src, dst) in enumerate(pairs)
    ]

    def nothing(v):
        return pltpu.bitcast(pltpu.bitcast(v, U32) & zero_s[0], F32)

    def layer_norm(c, serial=True, tiles=range(NQT)):
        link = None
        for n in tiles:
            cols = slice(128 * n, 128 * (n + 1))
            pivot = x_v[c, 0:16, cols].astype(F32)[0:1, :]
            pivot8 = jnp.broadcast_to(pivot, (8, 128))
            shift = pivot8
            s1 = s2 = None
            for i in range(D // 16):
                last = s1 if s1 is not None else link
                if serial and last is not None:
                    shift = pivot8 + nothing(last)
                x16 = x_v[c, 16 * i:16 * i + 16, cols].astype(F32)
                for k in range(2):
                    d = x16[8 * k:8 * k + 8, :] - shift
                    s1 = d if s1 is None else s1 + d
                    s2 = d * d if s2 is None else s2 + d * d
            dmean = jnp.sum(s1, axis=0, keepdims=True) * (1.0 / D)
            dsq = jnp.sum(s2, axis=0, keepdims=True) * (1.0 / D)
            var = jnp.maximum(dsq - dmean * dmean, 0.0)
            sd = _round_bf16(jnp.sqrt(_round_bf16(_round_bf16(var) + LN_EPS)))
            mean8 = jnp.broadcast_to(_round_bf16(pivot + dmean), (8, 128))
            inv8 = jnp.broadcast_to(1.0 / sd, (8, 128))
            center = mean8
            for i in range(D // 32):
                if serial and i > 0:
                    center = mean8 + nothing(link)
                x32 = x_v[c, 32 * i:32 * i + 32, cols].astype(F32)
                z = [(x32[8 * k:8 * k + 8, :] - center) * inv8 for k in range(4)]
                link = z[3]
                r0 = c * (D // 2) + 16 * i
                xn_v[r0:r0 + 16, cols] = _pack(jnp.concatenate(z, axis=0))

    def init_constants():
        gate = jax.nn.sigmoid(beta_v[...].astype(F32).reshape(1, H))
        on_diag = _iota((H, H), 0) == _iota((H, H), 1)
        gcol = jnp.sum(jnp.where(on_diag, gate, 0.0), axis=1, keepdims=True)
        gate_v[...] = jnp.broadcast_to(gcol, (H, 128))
        zero_s[0] = jnp.uint32(0)
        bias_v[...] = jnp.where(_iota((128, 128), 0) > _iota((128, 128), 1), NEG, 0.0)
        key, lane = _iota((64, 128), 0), _iota((64, 128), 1)
        future = key > (lane & 63)
        half_v[0] = jnp.where(future, NEG, 0.0)
        half_v[1] = jnp.where(future | (lane < 64), NEG, 0.0)
        half_v[2] = jnp.where(future | (lane >= 64), NEG, 0.0)
        router = jnp.broadcast_to(wr_v[...].astype(F32).reshape(1, D), (16, D))
        wall[RROW // 2:PROWS // 2, :] = _pack(
            jnp.where(_iota((16, D), 0) == 0, router, 0.0))

    def project(c, router_first=False):
        xn = _unpack(xn_v[_rows(c, D // 2), :])
        step_rows = PBLOCK // 2
        end = RROW // 2 if router_first else PROWS // 2
        tail = [_dot(_unpack(wall[end:PROWS // 2, :]), xn)] if router_first else []
        return jnp.concatenate(
            [_dot(_unpack(wall[r:min(r + step_rows, end), :]), xn)
             for r in range(0, end, step_rows)] + tail, axis=0)

    seen = [None]

    def record_logit_bound():
        big = (seen[0] >> 30) & 1
        safe_s[0] = (jnp.max(big.astype(jnp.int32)) == 0).astype(jnp.int32)

    def store_qkv(c, pt):
        r_v[c:c + 1, :] = _round_bf16(pt[RROW:RROW + 1, :])
        tail_row = _iota((8, L), 0)
        for h in range(H):
            base = 2 * D + DH * h
            tail = jnp.where(tail_row < DH - 16, pt[base + 16:base + 24, :],
                             jnp.where(tail_row == DH - 16, 1.0, 0.0))
            blk = jnp.concatenate(
                [pt[base:base + 16, :], tail, jnp.zeros((8, L), F32)], axis=0)
            vt_v[_rows(c * H + h, 16), :] = _pack(blk)

        rowl = _iota((128, L), 0)
        pqs, pks, vgs = [], [], []
        for g in range(NG):
            used = _heads_in_group(g) * DH
            qg = pt[GW * g:GW * g + 128, :]
            qs = qg * QSCALE
            qt_v[_rows(c * NG + g, 64), :] = _pack(qs)
            kg = pt[D + GW * g:D + GW * g + 128, :]
            for operand in (qs, kg):
                bits = pltpu.bitcast(operand, U32)
                for blk in range(0, 128 if g < NG - 1 else used, 8):
                    for col in range(0, L, 128):
                        piece = bits[blk:blk + 8, col:col + 128]
                        seen[0] = piece if seen[0] is None else seen[0] | piece
            k_v[_rows(c * NG + g, L // 2), :] = _pack(kg.T)
            pqs.append(_phi(qg).astype(BF16))
            if c < NSEG - 1:
                pks.append(_phi(kg).astype(BF16))
                lo = 2 * D + GW * g
                if g < NG - 1:
                    vg = pt[lo:lo + 128, :]
                else:
                    vg = jnp.concatenate(
                        [pt[lo:lo + used, :], jnp.zeros((128 - used, L), F32)], axis=0)
                vg = jnp.where(rowl < used, vg, jnp.where(rowl == GW, 1.0, 0.0))
                vgs.append(vg.astype(BF16))
        return pqs, pks, vgs

    def memory_update(states, pks, vgs):
        row = _iota((128, 128), 0)
        lane = _iota((128, 128), 1)
        same_head = (row // DH) == (lane // DH)
        out = []
        for g in range(NG):
            used = _heads_in_group(g) * DH
            upd = _dot_nt(vgs[g], pks[g])
            keep = ((same_head & (row < used)) | (row == GW)) & (lane < used)
            upd = jnp.where(keep, upd, 0.0)
            out.append(upd if states is None else states[g] + upd)
        return out

    def memory_retrieve(c, states, pqs):
        row = _iota((128, 128), 0)
        row8 = _iota((8, 128), 0)
        lane8 = _iota((8, 128), 1) // DH
        for g in range(NG):
            nh = _heads_in_group(g)
            st = states[g]
            mrows = jnp.where(row < GW, st, 0.0)
            zrows = jnp.where(lane8 == row8, st[GW:GW + 1, :], 0.0)
            lhs = jnp.concatenate(
                [mrows, zrows, jnp.zeros((8, 128), F32)], axis=0).astype(BF16)
            ret = _dot(lhs, pqs[g])
            gsel = gate_v[HPG * g:HPG * g + 8, :] if g < NG - 1 else jnp.concatenate(
                [gate_v[HPG * g:H, :], jnp.zeros((8 - nh, 128), F32)], axis=0)
            gwide = jnp.concatenate([gsel] * NQT, axis=1)
            scale = gwide / (ret[128:136, :] + 1e-6)
            pieces = []
            for b in range(16):
                h0 = min((8 * b) // DH, nh - 1)
                h1 = min((8 * b + 7) // DH, nh - 1)
                sc = scale[h0:h0 + 1, :]
                if h1 != h0:
                    first = _iota((8, L), 0) < DH * h1 - 8 * b
                    sc = jnp.where(first, sc, scale[h1:h1 + 1, :])
                pieces.append(ret[8 * b:8 * b + 8, :] * sc)
            mem_v[c - 1, GW * g:GW * g + 128, :] = jnp.concatenate(pieces, axis=0)

    def route():
        r = r_v[0:NSEG, :]
        idx = _iota((NSEG, L), 0) * L + _iota((NSEG, L), 1)
        m1 = jnp.max(r)
        i1 = jnp.clip(jnp.min(jnp.where(r == m1, idx, S)), 0, S - 1)
        r2 = jnp.where(idx == i1, -jnp.inf, r)
        m2 = jnp.max(r2)
        i2 = jnp.clip(jnp.min(jnp.where(r2 == m2, idx, S)), 0, S - 1)
        idx_s[0] = i1
        idx_s[1] = i2
        rsel_s[0] = m1
        rsel_s[1] = m2
        row16 = _iota((16, 128), 0)
        lane16 = _iota((16, 128), 1)
        xs = None
        for t, i in enumerate((i1, i2)):
            seg = i // L
            off = i - seg * L
            base = pl.multiple_of((off // 128) * 128, 128)
            cols = _unpack(xn_v[_rows(seg, D // 2), pl.ds(base, 128)])
            pick = jnp.where((row16 == t) & (lane16 == off - base), 1.0, 0.0)
            part = _dot_nt(pick.astype(BF16), cols)
            xs = part if xs is None else xs + part
        xs_v[...] = _pack(xs)
        y_v[...] = jnp.zeros(y_v.shape, F32)

    def ffn_hidden():
        xs = _unpack(xs_v[...])
        gt = _round_bf16(_dot(xs, wg_v[...]))
        up = _round_bf16(_dot(xs, wu_v[...]))
        hid = _round_bf16(_round_bf16(gt * jax.nn.sigmoid(gt)) * up)
        for t in range(2):
            for tile in range(FF // 128):
                hid_v[t, tile] = jnp.broadcast_to(
                    hid[t:t + 1, 128 * tile:128 * (tile + 1)], (8, 128))

    def ffn_down_chained():
        base = pl.multiple_of(step * (FT * 128), 128)
        link = [None, None]
        for b in range(D // 8):
            acc = [None, None]
            for tile in range(FT):
                w = wd_v[8 * b:8 * b + 8, pl.ds(base + 128 * tile, 128)].astype(F32)
                for t in range(2):
                    pr = w * hid_v[t, step * FT + tile]
                    if tile > 0:
                        acc[t] = acc[t] + pr
                    else:
                        acc[t] = pr if link[t] is None else pr + nothing(link[t])
            for t in range(2):
                rows = slice(8 * b, 8 * b + 8)
                y_v[t, rows, :] = y_v[t, rows, :] + acc[t]
                link[t] = acc[t]

    def ffn_down_looped():
        def down(tile, carry):
            col = step * FT + tile
            w = wd_v[:, pl.ds(pl.multiple_of(128 * col, 128), 128)].astype(F32)
            for t in range(2):
                y_v[t] = y_v[t] + w * hid_v[t, col][0:1, :]
            return carry

        lax.fori_loop(0, FT, down, 0)

    def masked_q_bits(g, hp, j):
        rid = _iota((64, 128), 0)
        mask = (rid >= (DH // 2) * hp) & (rid < (DH // 2) * (hp + 1))
        return jnp.where(mask, qt_v[_rows(step * NG + g, 64), 128 * j:128 * (j + 1)],
                         jnp.uint32(0))

    def keys(g, lo, hi):
        first = pl.multiple_of((step * NG + g) * (L // 2) + lo // 2, 8)
        return _unpack(k_v[pl.ds(first, (hi - lo) // 2), :])

    def causal_scores(g, hp, j):
        nk = 128 * (j + 1)
        st = _dot(keys(g, 0, nk), _unpack(masked_q_bits(g, hp, j)))
        diag = st[nk - 128:, :] + bias_v[...]
        return diag if j == 0 else jnp.concatenate([st[:nk - 128, :], diag], axis=0)

    def head_output(h, j, p, keep):
        o = _dot(_unpack(vt_v[_rows(step * H + h, 16), 0:128 * (j + 1)]), p)
        den = o[DH:DH + 1, :]
        inv = pl.reciprocal(den, approx=True)
        inv = inv * (2.0 - den * inv)
        return o[0:24, :] * (keep * inv)

    def single_probs(h, j):
        return jnp.exp2(causal_scores(*divmod(h, HPG), j)).astype(BF16)

    def pair_probs(pairs, j, flip):
        low = _iota((64, 128), 1) < 64
        qa, qb = {}, {}
        for h in pairs:
            g, hp = divmod(h, HPG)
            qa[h] = masked_q_bits(g, hp, j)
            qb[h] = pltpu.roll(masked_q_bits(g, hp + 1, j), 64, 1)
        off = {}
        if j > 0:
            for h in pairs:
                g = h // HPG
                for hh, q in ((h, qa[h]), (h + 1, qb[h])):
                    off[hh] = jnp.exp2(_dot(keys(g, 0, 128 * j), _unpack(q)))
        early, late = {}, {}
        for h in pairs:
            g = h // HPG
            k0 = 128 * j
            for which in ((0, 1) if flip else (1, 0)):
                if which == 0:
                    early[h] = _dot(keys(g, k0, k0 + 64),
                                    _unpack(jnp.where(low, qa[h], qb[h])))
                else:
                    late[h] = _dot(keys(g, k0, k0 + 128),
                                   _unpack(jnp.where(low, qb[h], qa[h])))
        probs = {}
        for h in pairs:
            p1 = jnp.exp2(early[h] + half_v[0])
            p2 = jnp.exp2(late[h][0:64, :])
            bottom = late[h][64:128, :]
            pa = jnp.concatenate(
                [jnp.where(low, p1, p2), jnp.exp2(bottom + half_v[1])], axis=0)
            pb = jnp.concatenate(
                [jnp.where(low, p2, p1), jnp.exp2(bottom + half_v[2])], axis=0)
            for hh, pd in ((h, pa), (h + 1, pb)):
                full = pd if j == 0 else jnp.concatenate([off[hh], pd], axis=0)
                probs[hh] = full.astype(BF16)
        return probs

    def attention_bounded():
        pairs = [g * HPG + hp for g in range(NG)
                 for hp in range(0, _heads_in_group(g) - 1, 2)]
        paired = set(pairs) | {h + 1 for h in pairs}
        singles = [h for h in range(H) if h not in paired]
        waves = [(pairs[i:i + 2], j) for i in range(0, len(pairs), 2) for j in range(NQT)]
        waves += [(None, j) for j in range(NQT)]

        def scores(w):
            grp, j = waves[w]
            if grp is None:
                return {h: single_probs(h, j) for h in singles}
            return pair_probs(grp, j, w % 2 == 1)

        def values(w, probs):
            grp, j = waves[w]
            for h, p in probs.items():
                o = head_output(h, j, p, 1.0 - gate_v[h:h + 1, :])
                if grp is not None and h - 1 in grp:
                    o = pltpu.roll(o, 64, 1)
                ot_v[step, DH * h:DH * (h + 1), 128 * j:128 * (j + 1)] = o[0:DH, :]

        pending = scores(0)
        for w in range(len(waves)):
            nxt = scores(w + 1) if w + 1 < len(waves) else None
            values(w, pending)
            pending = nxt
        ffn_down_chained()

    def attention_max_shifted():
        def one_tile(item, carry):
            h = item // NQT
            j = item - h * NQT
            g = h // HPG
            hp = h - g * HPG
            cols = pl.ds(pl.multiple_of(128 * j, 128), 128)
            rid = _iota((64, 128), 0)
            mask = (rid >= (DH // 2) * hp) & (rid < (DH // 2) * (hp + 1))
            qm = jnp.where(mask, qt_v[_rows(step * NG + g, 64), cols], jnp.uint32(0))
            st = _dot(keys(g, 0, L), _unpack(qm))
            future = _iota((L, 128), 0) > 128 * j + _iota((L, 128), 1)
            st = jnp.where(future, NEG, st)
            p = jnp.exp2(st - jnp.max(st, axis=0, keepdims=True)).astype(BF16)
            keep = 1.0 - gate_v[pl.ds(h, 1), :]
            oh_v[h, :, cols] = head_output(h, NQT - 1, p, keep)
            return carry

        lax.fori_loop(0, H * NQT, one_tile, 0)
        for h in range(H):
            ot_v[step, DH * h:DH * (h + 1), :] = oh_v[h, 0:DH, :]
        ffn_down_looped()

    def routed_columns():
        ys = []
        for t in range(2):
            y = _round_bf16(jnp.sum(y_v[t], axis=1, keepdims=True))
            rsel = jnp.full((1, 1), rsel_s[t], F32)
            ys.append(_round_bf16(y * _round_bf16(jax.nn.sigmoid(rsel))))
        return ys

    def output_copy(seg, n):
        return pltpu.make_async_copy(
            out_v.at[pl.ds(seg * D, D), pl.ds(128 * n, 128)],
            o_hbm.at[:, pl.ds(seg * L + 128 * n, 128)],
            out_sems.at[NQT * seg + n])

    def output_projection(seg, ys):
        heads_out = ot_v[seg, 0:D, :]
        if seg > 0:
            heads_out = heads_out + mem_v[seg - 1, 0:D, :]
        attn = _dot(_unpack(wot[...]), heads_out.astype(BF16))
        base = x_v[seg].astype(F32) + attn
        xn = _unpack(xn_v[_rows(seg, D // 2), :]).astype(F32)
        col = seg * L + _iota((1, L), 1)
        upd = (jnp.where(col == idx_s[0], ys[0], 0.0)
               + jnp.where(col == idx_s[1], ys[1], 0.0))
        result = base + (xn + upd)
        for n in range(NQT):
            cols = slice(128 * n, 128 * (n + 1))
            out_v[seg * D:(seg + 1) * D, cols] = result[:, cols].astype(BF16)
            output_copy(seg, n).start()

    col_blocks = [(c0, min(128, D - c0)) for c0 in range(0, D, 128)]

    def transpose_block(w_v, section, c0, n):
        r0 = (section * D + c0) // 2
        wall[r0:r0 + n // 2, :] = pltpu.bitcast(w_v[:, c0:c0 + n].T, U32)

    def project_block(section, c0, n, xn):
        r0 = (section * D + c0) // 2
        last = section == 2 and c0 + n == D
        hi = PROWS // 2 if last else r0 + n // 2
        return _dot(_unpack(wall[r0:hi, :]), xn)

    def query_half0(half):
        layer_norm(0, serial=False, tiles=[2 * half, 2 * half + 1])
        xn = _unpack(xn_v[0:D // 2, 256 * half:256 * (half + 1)])
        return jnp.concatenate(
            [_dot(_unpack(wall[r:r + D // 4, :]), xn) for r in (0, D // 4)], axis=0)

    def projections():
        qtiles = []
        for half in range(2):
            x0_copies[half].wait()
            if half == 1:
                cp_wk.wait()
            qtiles.append(query_half0(half))
        for c0, n in col_blocks:
            transpose_block(wk_v, 1, c0, n)
        parts = [jnp.concatenate(qtiles, axis=1)]
        cp_wv.wait()
        x_copies[1].wait()
        xn0 = _unpack(xn_v[_rows(0, D // 2), :])
        parts += [project_block(1, c0, n, xn0) for c0, n in col_blocks]
        for c0, n in col_blocks:
            transpose_block(wv_v, 2, c0, n)
            parts.append(project_block(2, c0, n, xn0))
        layer_norm(1)
        _, pk, vg = store_qkv(0, jnp.concatenate(parts, axis=0))
        x_copies[2].wait()
        x_copies[3].wait()
        cp_wo.wait()

        layer_norm(2)
        pt = project(1)
        wot[...] = pltpu.bitcast(wo_v[...].T, U32)
        state1 = memory_update(None, pk, vg)
        pq1, pk, vg = store_qkv(1, pt)
        layer_norm(3)
        pt = project(2)
        state2 = memory_update(state1, pk, vg)
        pq2, pk, vg = store_qkv(2, pt)
        cp_wg.wait()
        cp_wu.wait()
        pt = project(3, router_first=True)
        pq3, _, _ = store_qkv(3, pt)
        route()
        ffn_hidden()
        state3 = memory_update(state2, pk, vg)
        memory_retrieve(1, state1, pq1)
        memory_retrieve(2, state2, pq2)
        memory_retrieve(3, state3, pq3)
        record_logit_bound()
        cp_wd.wait()

    @pl.when(step == 0)
    def _():
        for cp in (cp_wq, cp_wr, cp_beta, *x0_copies, cp_wk, cp_wv, x_copies[1],
                   x_copies[2], x_copies[3], cp_wo, cp_wg, cp_wu, cp_wd):
            cp.start()
        with _scope("sc_startup"):
            cp_wr.wait()
            cp_beta.wait()
            cp_wq.wait()
            init_constants()
            for c0, n in col_blocks:
                transpose_block(wq_v, 0, c0, n)
        with _scope("sc_projections"):
            projections()

    @pl.when(step < NSEG)
    def _():
        safe = safe_s[0] == 1

        @pl.when(safe)
        def _():
            with _scope("sc_attention"):
                attention_bounded()

        @pl.when(jnp.logical_not(safe))
        def _():
            attention_max_shifted()

    @pl.when(step == NSEG)
    def _():
        with _scope("sc_outproj"):
            ys = routed_columns()
            for seg in range(NSEG):
                output_projection(seg, ys)
            for seg in range(NSEG):
                for n in range(NQT):
                    output_copy(seg, n).wait()


@jax.jit
def pallas_parallel_sum__memory_aug_infini_attn__moe_arch_mod__prompt_kernel(
    A_x: jax.Array,
    A_wq: jax.Array,
    A_wk: jax.Array,
    A_wv: jax.Array,
    A_wo: jax.Array,
    A_beta: jax.Array,
    B_x: jax.Array,
    B_w_r: jax.Array,
    B_w_gate: jax.Array,
    B_w_up: jax.Array,
    B_w_down: jax.Array,
):
    del B_x
    vm = pltpu.VMEM
    scratch = [
        vm((NSEG, D, L), BF16),
        vm((D, D), BF16),
        vm((D, D), BF16),
        vm((D, D), BF16),
        vm((D, D), BF16),
        vm((H,), BF16),
        vm((D,), BF16),
        vm((D, FF), BF16),
        vm((D, FF), BF16),
        vm((D, FF), BF16),
        vm((PROWS // 2, D), U32),
        vm((D // 2, D), U32),
        vm((NSEG * D // 2, L), U32),
        vm((NSEG * NG * 64, L), U32),
        vm((NSEG * NG * L // 2, 128), U32),
        vm((NSEG * H * 16, L), U32),
        vm((NSEG - 1, OROWS, L), F32),
        vm((8, L), F32),
        vm((8, D), U32),
        vm((2, D, 128), F32),
        vm((2, FF // 128, 8, 128), F32),
        pltpu.SMEM((2,), jnp.int32),
        pltpu.SMEM((2,), F32),
        pltpu.SMEM((1,), U32),
        pltpu.SMEM((1,), jnp.int32),
        vm((H, 128), F32),
        vm((NSEG, D, L), F32),
        vm((H, 24, L), F32),
        vm((128, 128), F32),
        vm((3, 64, 128), F32),
        vm((NSEG * D, L), BF16),
        pltpu.SemaphoreType.DMA((NSEG * NQT,)),
        pltpu.SemaphoreType.DMA((NSEG + 9 + 2,)),
    ]
    hbm = pl.BlockSpec(memory_space=pltpu.HBM)
    xt = jnp.transpose(A_x.reshape(S, D))
    out_t = pl.pallas_call(
        _kernel,
        grid=(NSEG + 1,),
        in_specs=[hbm] * 10,
        out_specs=hbm,
        out_shape=jax.ShapeDtypeStruct((D, S), BF16),
        scratch_shapes=scratch,
        compiler_params=pltpu.CompilerParams(
            dimension_semantics=("arbitrary",),
            vmem_limit_bytes=110 * 1024 * 1024,
        ),
        name="infini_moe",
    )(xt, A_wq, A_wk, A_wv, A_wo, A_beta, B_w_r, B_w_gate, B_w_up,
      jnp.transpose(B_w_down))
    return jnp.transpose(out_t).reshape(1, S, D)
```

```python
import contextlib

import jax
import jax.numpy as jnp
from jax import lax
from jax.experimental import pallas as pl
from jax.experimental.pallas import tpu as pltpu

S = 2048
D = 576
H = 32
DH = 18
NSEG = 4
L = 512
FF = 4608
NG = 5
HPG = 7
GW = HPG * DH
NQT = L // 128
PROWS = 3 * D + 16
RROW = 3 * D
EARLY_K = 1
PBLOCK = 128
MROWS = 144
FT = FF // 128 // NSEG
OROWS = 640
LOG2E = 1.4426950408889634
QSCALE = DH ** -0.5 * LOG2E
NEG = -1e30
LN_EPS = 1.0013580322265625e-05
F32 = jnp.float32
BF16 = jnp.bfloat16
U32 = jnp.uint32

PROFILE_SCOPES = False

_NN = (((1,), (0,)), ((), ()))
_NT = (((1,), (1,)), ((), ()))


def _scope(name):
    return jax.named_scope(name) if PROFILE_SCOPES else contextlib.nullcontext()


def _dot(a, b):
    return lax.dot_general(a, b, _NN, preferred_element_type=F32)


def _dot_nt(a, b):
    return lax.dot_general(a, b, _NT, preferred_element_type=F32)


def _iota(shape, dim):
    return lax.broadcasted_iota(jnp.int32, shape, dim)


def _round_bf16(v):
    return v.astype(BF16).astype(F32)


def _pack(v):
    return pltpu.bitcast(v.astype(BF16), U32)


def _unpack(u):
    return pltpu.bitcast(u, BF16)


def _rows(index, size):
    if isinstance(index, int):
        return slice(index * size, (index + 1) * size)
    return pl.ds(pl.multiple_of(index * size, 8), size)


def _heads_in_group(g):
    return HPG if g < NG - 1 else H - HPG * (NG - 1)


def _phi(t):
    return jnp.where(t > 0, t + 1.0, jnp.exp(t))


def _kernel(x_hbm, wq_hbm, wk_hbm, wv_hbm, wo_hbm, beta_hbm, wr_hbm,
            wg_hbm, wu_hbm, wd_hbm,
            o_hbm,
            x_v, wq_v, wk_v, wv_v, wo_v, beta_v, wr_v, wg_v, wu_v, wd_v,
            wall, wot, xn_v, qt_v, k_v, vt_v, mem_v,
            r_v, xs_v, y_v, hid_v, idx_s, rsel_s, zero_s, safe_s,
            gate_v, ot_v, oh_v, bias_v, half_v, out_v, out_sems,
            sems):
    step = pl.program_id(0)

    x_copies = [None] + [
        pltpu.make_async_copy(x_hbm.at[:, pl.ds(c * L, L)], x_v.at[c], sems.at[c])
        for c in range(1, NSEG)
    ]
    x0_copies = [
        pltpu.make_async_copy(x_hbm.at[:, pl.ds(256 * n, 256)],
                              x_v.at[0, :, pl.ds(256 * n, 256)],
                              sems.at[NSEG + 9 + n])
        for n in range(2)
    ]
    pairs = [(wq_hbm, wq_v), (wk_hbm, wk_v), (wv_hbm, wv_v), (wo_hbm, wo_v),
             (beta_hbm, beta_v), (wr_hbm, wr_v),
             (wg_hbm, wg_v), (wu_hbm, wu_v), (wd_hbm, wd_v)]
    (cp_wq, cp_wk, cp_wv, cp_wo, cp_beta, cp_wr, cp_wg, cp_wu, cp_wd) = [
        pltpu.make_async_copy(src, dst, sems.at[NSEG + i])
        for i, (src, dst) in enumerate(pairs)
    ]

    def nothing(v):
        return pltpu.bitcast(pltpu.bitcast(v, U32) & zero_s[0], F32)

    def layer_norm(c, serial=True, tiles=range(NQT)):
        link = None
        for n in tiles:
            cols = slice(128 * n, 128 * (n + 1))
            pivot = x_v[c, 0:16, cols].astype(F32)[0:1, :]
            pivot8 = jnp.broadcast_to(pivot, (8, 128))
            shift = pivot8
            s1 = s2 = None
            for i in range(D // 16):
                last = s1 if s1 is not None else link
                if serial and last is not None:
                    shift = pivot8 + nothing(last)
                x16 = x_v[c, 16 * i:16 * i + 16, cols].astype(F32)
                for k in range(2):
                    d = x16[8 * k:8 * k + 8, :] - shift
                    s1 = d if s1 is None else s1 + d
                    s2 = d * d if s2 is None else s2 + d * d
            dmean = jnp.sum(s1, axis=0, keepdims=True) * (1.0 / D)
            dsq = jnp.sum(s2, axis=0, keepdims=True) * (1.0 / D)
            var = jnp.maximum(dsq - dmean * dmean, 0.0)
            sd = _round_bf16(jnp.sqrt(_round_bf16(_round_bf16(var) + LN_EPS)))
            mean8 = jnp.broadcast_to(_round_bf16(pivot + dmean), (8, 128))
            inv8 = jnp.broadcast_to(1.0 / sd, (8, 128))
            center = mean8
            for i in range(D // 32):
                if serial and i > 0:
                    center = mean8 + nothing(link)
                x32 = x_v[c, 32 * i:32 * i + 32, cols].astype(F32)
                z = [(x32[8 * k:8 * k + 8, :] - center) * inv8 for k in range(4)]
                link = z[3]
                r0 = c * (D // 2) + 16 * i
                xn_v[r0:r0 + 16, cols] = _pack(jnp.concatenate(z, axis=0))

    def init_constants():
        gate = jax.nn.sigmoid(beta_v[...].astype(F32).reshape(1, H))
        on_diag = _iota((H, H), 0) == _iota((H, H), 1)
        gcol = jnp.sum(jnp.where(on_diag, gate, 0.0), axis=1, keepdims=True)
        gate_v[...] = jnp.broadcast_to(gcol, (H, 128))
        zero_s[0] = jnp.uint32(0)
        bias_v[...] = jnp.where(_iota((128, 128), 0) > _iota((128, 128), 1), NEG, 0.0)
        key, lane = _iota((64, 128), 0), _iota((64, 128), 1)
        future = key > (lane & 63)
        half_v[0] = jnp.where(future, NEG, 0.0)
        half_v[1] = jnp.where(future | (lane < 64), NEG, 0.0)
        half_v[2] = jnp.where(future | (lane >= 64), NEG, 0.0)
        router = jnp.broadcast_to(wr_v[...].astype(F32).reshape(1, D), (16, D))
        wall[RROW // 2:PROWS // 2, :] = _pack(
            jnp.where(_iota((16, D), 0) == 0, router, 0.0))

    def project(c, router_first=False):
        xn = _unpack(xn_v[_rows(c, D // 2), :])
        step_rows = PBLOCK // 2
        end = RROW // 2 if router_first else PROWS // 2
        tail = [_dot(_unpack(wall[end:PROWS // 2, :]), xn)] if router_first else []
        return jnp.concatenate(
            [_dot(_unpack(wall[r:min(r + step_rows, end), :]), xn)
             for r in range(0, end, step_rows)] + tail, axis=0)

    seen = [None]

    def record_logit_bound():
        big = (seen[0] >> 30) & 1
        safe_s[0] = (jnp.max(big.astype(jnp.int32)) == 0).astype(jnp.int32)

    def store_qkv(c, pt):
        r_v[c:c + 1, :] = _round_bf16(pt[RROW:RROW + 1, :])
        tail_row = _iota((8, L), 0)
        for h in range(H):
            base = 2 * D + DH * h
            tail = jnp.where(tail_row < DH - 16, pt[base + 16:base + 24, :],
                             jnp.where(tail_row == DH - 16, 1.0, 0.0))
            blk = jnp.concatenate(
                [pt[base:base + 16, :], tail, jnp.zeros((8, L), F32)], axis=0)
            vt_v[_rows(c * H + h, 16), :] = _pack(blk)

        rowl = _iota((128, L), 0)
        pqs, pks, vgs = [], [], []
        for g in range(NG):
            used = _heads_in_group(g) * DH
            qg = pt[GW * g:GW * g + 128, :]
            qs = qg * QSCALE
            qt_v[_rows(c * NG + g, 64), :] = _pack(qs)
            kg = pt[D + GW * g:D + GW * g + 128, :]
            for operand in (qs, kg):
                bits = pltpu.bitcast(operand, U32)
                for blk in range(0, 128 if g < NG - 1 else used, 8):
                    for col in range(0, L, 128):
                        piece = bits[blk:blk + 8, col:col + 128]
                        seen[0] = piece if seen[0] is None else seen[0] | piece
            k_v[_rows(c * NG + g, L // 2), :] = _pack(kg.T)
            pqs.append(_phi(qg).astype(BF16))
            if c < NSEG - 1:
                pks.append(_phi(kg).astype(BF16))
                lo = 2 * D + GW * g
                if g < NG - 1:
                    vg = pt[lo:lo + 128, :]
                else:
                    vg = jnp.concatenate(
                        [pt[lo:lo + used, :], jnp.zeros((128 - used, L), F32)], axis=0)
                vg = jnp.where(rowl < used, vg, jnp.where(rowl == GW, 1.0, 0.0))
                vgs.append(vg.astype(BF16))
        return pqs, pks, vgs

    def memory_update(states, pks, vgs):
        row = _iota((128, 128), 0)
        lane = _iota((128, 128), 1)
        same_head = (row // DH) == (lane // DH)
        out = []
        for g in range(NG):
            used = _heads_in_group(g) * DH
            upd = _dot_nt(vgs[g], pks[g])
            keep = ((same_head & (row < used)) | (row == GW)) & (lane < used)
            upd = jnp.where(keep, upd, 0.0)
            out.append(upd if states is None else states[g] + upd)
        return out

    def memory_retrieve(c, states, pqs):
        row = _iota((128, 128), 0)
        row8 = _iota((8, 128), 0)
        lane8 = _iota((8, 128), 1) // DH
        for g in range(NG):
            nh = _heads_in_group(g)
            st = states[g]
            mrows = jnp.where(row < GW, st, 0.0)
            zrows = jnp.where(lane8 == row8, st[GW:GW + 1, :], 0.0)
            lhs = jnp.concatenate(
                [mrows, zrows, jnp.zeros((8, 128), F32)], axis=0).astype(BF16)
            ret = _dot(lhs, pqs[g])
            gsel = gate_v[HPG * g:HPG * g + 8, :] if g < NG - 1 else jnp.concatenate(
                [gate_v[HPG * g:H, :], jnp.zeros((8 - nh, 128), F32)], axis=0)
            gwide = jnp.concatenate([gsel] * NQT, axis=1)
            scale = gwide / (ret[128:136, :] + 1e-6)
            pieces = []
            for b in range(16):
                h0 = min((8 * b) // DH, nh - 1)
                h1 = min((8 * b + 7) // DH, nh - 1)
                sc = scale[h0:h0 + 1, :]
                if h1 != h0:
                    first = _iota((8, L), 0) < DH * h1 - 8 * b
                    sc = jnp.where(first, sc, scale[h1:h1 + 1, :])
                pieces.append(ret[8 * b:8 * b + 8, :] * sc)
            mem_v[c - 1, GW * g:GW * g + 128, :] = jnp.concatenate(pieces, axis=0)

    def route():
        r = r_v[0:NSEG, :]
        idx = _iota((NSEG, L), 0) * L + _iota((NSEG, L), 1)
        m1 = jnp.max(r)
        i1 = jnp.clip(jnp.min(jnp.where(r == m1, idx, S)), 0, S - 1)
        r2 = jnp.where(idx == i1, -jnp.inf, r)
        m2 = jnp.max(r2)
        i2 = jnp.clip(jnp.min(jnp.where(r2 == m2, idx, S)), 0, S - 1)
        idx_s[0] = i1
        idx_s[1] = i2
        rsel_s[0] = m1
        rsel_s[1] = m2
        row16 = _iota((16, 128), 0)
        lane16 = _iota((16, 128), 1)
        xs = None
        for t, i in enumerate((i1, i2)):
            seg = i // L
            off = i - seg * L
            base = pl.multiple_of((off // 128) * 128, 128)
            cols = _unpack(xn_v[_rows(seg, D // 2), pl.ds(base, 128)])
            pick = jnp.where((row16 == t) & (lane16 == off - base), 1.0, 0.0)
            part = _dot_nt(pick.astype(BF16), cols)
            xs = part if xs is None else xs + part
        xs_v[...] = _pack(xs)
        y_v[...] = jnp.zeros(y_v.shape, F32)

    def ffn_hidden():
        xs = _unpack(xs_v[...])
        gt = _round_bf16(_dot(xs, wg_v[...]))
        up = _round_bf16(_dot(xs, wu_v[...]))
        hid = _round_bf16(_round_bf16(gt * jax.nn.sigmoid(gt)) * up)
        for t in range(2):
            for tile in range(FF // 128):
                hid_v[t, tile] = jnp.broadcast_to(
                    hid[t:t + 1, 128 * tile:128 * (tile + 1)], (8, 128))

    def ffn_down_chained():
        base = pl.multiple_of(step * (FT * 128), 128)
        link = [None, None]
        for b in range(D // 8):
            acc = [None, None]
            for tile in range(FT):
                w = wd_v[8 * b:8 * b + 8, pl.ds(base + 128 * tile, 128)].astype(F32)
                for t in range(2):
                    pr = w * hid_v[t, step * FT + tile]
                    if tile > 0:
                        acc[t] = acc[t] + pr
                    else:
                        acc[t] = pr if link[t] is None else pr + nothing(link[t])
            for t in range(2):
                rows = slice(8 * b, 8 * b + 8)
                y_v[t, rows, :] = y_v[t, rows, :] + acc[t]
                link[t] = acc[t]

    def ffn_down_looped():
        def down(tile, carry):
            col = step * FT + tile
            w = wd_v[:, pl.ds(pl.multiple_of(128 * col, 128), 128)].astype(F32)
            for t in range(2):
                y_v[t] = y_v[t] + w * hid_v[t, col][0:1, :]
            return carry

        lax.fori_loop(0, FT, down, 0)

    def masked_q_bits(g, hp, j):
        rid = _iota((64, 128), 0)
        mask = (rid >= (DH // 2) * hp) & (rid < (DH // 2) * (hp + 1))
        return jnp.where(mask, qt_v[_rows(step * NG + g, 64), 128 * j:128 * (j + 1)],
                         jnp.uint32(0))

    def keys(g, lo, hi):
        first = pl.multiple_of((step * NG + g) * (L // 2) + lo // 2, 8)
        return _unpack(k_v[pl.ds(first, (hi - lo) // 2), :])

    def causal_scores(g, hp, j):
        nk = 128 * (j + 1)
        st = _dot(keys(g, 0, nk), _unpack(masked_q_bits(g, hp, j)))
        diag = st[nk - 128:, :] + bias_v[...]
        return diag if j == 0 else jnp.concatenate([st[:nk - 128, :], diag], axis=0)

    def head_output(h, j, p, keep):
        o = _dot(_unpack(vt_v[_rows(step * H + h, 16), 0:128 * (j + 1)]), p)
        den = o[DH:DH + 1, :]
        inv = pl.reciprocal(den, approx=True)
        inv = inv * (2.0 - den * inv)
        return o[0:24, :] * (keep * inv)

    def single_probs(h, j):
        return jnp.exp2(causal_scores(*divmod(h, HPG), j)).astype(BF16)

    def pair_probs(pairs, j, flip):
        low = _iota((64, 128), 1) < 64
        qa, qb = {}, {}
        for h in pairs:
            g, hp = divmod(h, HPG)
            qa[h] = masked_q_bits(g, hp, j)
            qb[h] = pltpu.roll(masked_q_bits(g, hp + 1, j), 64, 1)
        off = {}
        if j > 0:
            for h in pairs:
                g = h // HPG
                for hh, q in ((h, qa[h]), (h + 1, qb[h])):
                    off[hh] = jnp.exp2(_dot(keys(g, 0, 128 * j), _unpack(q)))
        early, late = {}, {}
        for h in pairs:
            g = h // HPG
            k0 = 128 * j
            for which in ((0, 1) if flip else (1, 0)):
                if which == 0:
                    early[h] = _dot(keys(g, k0, k0 + 64),
                                    _unpack(jnp.where(low, qa[h], qb[h])))
                else:
                    late[h] = _dot(keys(g, k0, k0 + 128),
                                   _unpack(jnp.where(low, qb[h], qa[h])))
        probs = {}
        for h in pairs:
            p1 = jnp.exp2(early[h] + half_v[0])
            p2 = jnp.exp2(late[h][0:64, :])
            bottom = late[h][64:128, :]
            pa = jnp.concatenate(
                [jnp.where(low, p1, p2), jnp.exp2(bottom + half_v[1])], axis=0)
            pb = jnp.concatenate(
                [jnp.where(low, p2, p1), jnp.exp2(bottom + half_v[2])], axis=0)
            for hh, pd in ((h, pa), (h + 1, pb)):
                full = pd if j == 0 else jnp.concatenate([off[hh], pd], axis=0)
                probs[hh] = full.astype(BF16)
        return probs

    def attention_bounded():
        pairs = [g * HPG + hp for g in range(NG)
                 for hp in range(0, _heads_in_group(g) - 1, 2)]
        paired = set(pairs) | {h + 1 for h in pairs}
        singles = [h for h in range(H) if h not in paired]
        waves = [(pairs[i:i + 2], j) for i in range(0, len(pairs), 2) for j in range(NQT)]
        waves += [(None, j) for j in range(NQT)]

        def scores(w):
            grp, j = waves[w]
            if grp is None:
                return {h: single_probs(h, j) for h in singles}
            return pair_probs(grp, j, w % 2 == 1)

        def values(w, probs):
            grp, j = waves[w]
            for h, p in probs.items():
                o = head_output(h, j, p, 1.0 - gate_v[h:h + 1, :])
                if grp is not None and h - 1 in grp:
                    o = pltpu.roll(o, 64, 1)
                ot_v[step, DH * h:DH * (h + 1), 128 * j:128 * (j + 1)] = o[0:DH, :]

        pending = scores(0)
        for w in range(len(waves)):
            nxt = scores(w + 1) if w + 1 < len(waves) else None
            values(w, pending)
            pending = nxt
        ffn_down_chained()

    def attention_max_shifted():
        def one_tile(item, carry):
            h = item // NQT
            j = item - h * NQT
            g = h // HPG
            hp = h - g * HPG
            cols = pl.ds(pl.multiple_of(128 * j, 128), 128)
            rid = _iota((64, 128), 0)
            mask = (rid >= (DH // 2) * hp) & (rid < (DH // 2) * (hp + 1))
            qm = jnp.where(mask, qt_v[_rows(step * NG + g, 64), cols], jnp.uint32(0))
            st = _dot(keys(g, 0, L), _unpack(qm))
            future = _iota((L, 128), 0) > 128 * j + _iota((L, 128), 1)
            st = jnp.where(future, NEG, st)
            p = jnp.exp2(st - jnp.max(st, axis=0, keepdims=True)).astype(BF16)
            keep = 1.0 - gate_v[pl.ds(h, 1), :]
            oh_v[h, :, cols] = head_output(h, NQT - 1, p, keep)
            return carry

        lax.fori_loop(0, H * NQT, one_tile, 0)
        for h in range(H):
            ot_v[step, DH * h:DH * (h + 1), :] = oh_v[h, 0:DH, :]
        ffn_down_looped()

    def routed_columns():
        ys = []
        for t in range(2):
            y = _round_bf16(jnp.sum(y_v[t], axis=1, keepdims=True))
            rsel = jnp.full((1, 1), rsel_s[t], F32)
            ys.append(_round_bf16(y * _round_bf16(jax.nn.sigmoid(rsel))))
        return ys

    def output_copy(seg, n):
        return pltpu.make_async_copy(
            out_v.at[pl.ds(seg * D, D), pl.ds(128 * n, 128)],
            o_hbm.at[:, pl.ds(seg * L + 128 * n, 128)],
            out_sems.at[NQT * seg + n])

    def output_projection(seg, ys):
        heads_out = ot_v[seg, 0:D, :]
        if seg > 0:
            heads_out = heads_out + mem_v[seg - 1, 0:D, :]
        attn = _dot(_unpack(wot[...]), heads_out.astype(BF16))
        base = x_v[seg].astype(F32) + attn
        xn = _unpack(xn_v[_rows(seg, D // 2), :]).astype(F32)
        col = seg * L + _iota((1, L), 1)
        upd = (jnp.where(col == idx_s[0], ys[0], 0.0)
               + jnp.where(col == idx_s[1], ys[1], 0.0))
        result = base + (xn + upd)
        for n in range(NQT):
            cols = slice(128 * n, 128 * (n + 1))
            out_v[seg * D:(seg + 1) * D, cols] = result[:, cols].astype(BF16)
            output_copy(seg, n).start()

    col_blocks = [(c0, min(128, D - c0)) for c0 in range(0, D, 128)]

    def transpose_block(w_v, section, c0, n):
        r0 = (section * D + c0) // 2
        wall[r0:r0 + n // 2, :] = pltpu.bitcast(w_v[:, c0:c0 + n].T, U32)

    def project_block(section, c0, n, xn):
        r0 = (section * D + c0) // 2
        last = section == 2 and c0 + n == D
        hi = PROWS // 2 if last else r0 + n // 2
        return _dot(_unpack(wall[r0:hi, :]), xn)

    def query_half0(half):
        layer_norm(0, serial=False, tiles=[2 * half, 2 * half + 1])
        xn = _unpack(xn_v[0:D // 2, 256 * half:256 * (half + 1)])
        top = _dot(_unpack(wall[0:D // 4, :]), xn)
        if half == 0:
            for c0, n in col_blocks[3:]:
                transpose_block(wq_v, 0, c0, n)
        bottom = _dot(_unpack(wall[D // 4:D // 2, :]), xn)
        return jnp.concatenate([top, bottom], axis=0)

    def projections():
        qtiles = []
        for half in range(2):
            x0_copies[half].wait()
            if half == 1:
                cp_wk.wait()
            qtiles.append(query_half0(half))
        for c0, n in col_blocks:
            transpose_block(wk_v, 1, c0, n)
        parts = [jnp.concatenate(qtiles, axis=1)]
        xn0 = _unpack(xn_v[_rows(0, D // 2), :])
        parts += [project_block(1, c0, n, xn0) for c0, n in col_blocks[:EARLY_K]]
        cp_wv.wait()
        x_copies[1].wait()
        xn0 = _unpack(xn_v[_rows(0, D // 2), :])
        parts += [project_block(1, c0, n, xn0) for c0, n in col_blocks[EARLY_K:]]
        for c0, n in col_blocks:
            transpose_block(wv_v, 2, c0, n)
            parts.append(project_block(2, c0, n, xn0))
        layer_norm(1)
        _, pk, vg = store_qkv(0, jnp.concatenate(parts, axis=0))
        x_copies[2].wait()
        x_copies[3].wait()
        cp_wo.wait()

        layer_norm(2)
        pt = project(1)
        wot[...] = pltpu.bitcast(wo_v[...].T, U32)
        state1 = memory_update(None, pk, vg)
        pq1, pk, vg = store_qkv(1, pt)
        layer_norm(3)
        pt = project(2)
        state2 = memory_update(state1, pk, vg)
        pq2, pk, vg = store_qkv(2, pt)
        cp_wg.wait()
        cp_wu.wait()
        pt = project(3, router_first=True)
        pq3, _, _ = store_qkv(3, pt)
        route()
        ffn_hidden()
        state3 = memory_update(state2, pk, vg)
        memory_retrieve(1, state1, pq1)
        memory_retrieve(2, state2, pq2)
        memory_retrieve(3, state3, pq3)
        record_logit_bound()
        cp_wd.wait()

    @pl.when(step == 0)
    def _():
        for cp in (cp_wq, cp_wr, cp_beta, *x0_copies, cp_wk, cp_wv, x_copies[1],
                   x_copies[2], x_copies[3], cp_wo, cp_wg, cp_wu, cp_wd):
            cp.start()
        with _scope("sc_startup"):
            cp_wr.wait()
            cp_beta.wait()
            cp_wq.wait()
            init_constants()
            for c0, n in col_blocks[:3]:
                transpose_block(wq_v, 0, c0, n)
        with _scope("sc_projections"):
            projections()

    @pl.when(step < NSEG)
    def _():
        safe = safe_s[0] == 1

        @pl.when(safe)
        def _():
            with _scope("sc_attention"):
                attention_bounded()

        @pl.when(jnp.logical_not(safe))
        def _():
            attention_max_shifted()

    @pl.when(step == NSEG)
    def _():
        with _scope("sc_outproj"):
            ys = routed_columns()
            for seg in range(NSEG):
                output_projection(seg, ys)
            for seg in range(NSEG):
                for n in range(NQT):
                    output_copy(seg, n).wait()


@jax.jit
def pallas_parallel_sum__memory_aug_infini_attn__moe_arch_mod__prompt_kernel(
    A_x: jax.Array,
    A_wq: jax.Array,
    A_wk: jax.Array,
    A_wv: jax.Array,
    A_wo: jax.Array,
    A_beta: jax.Array,
    B_x: jax.Array,
    B_w_r: jax.Array,
    B_w_gate: jax.Array,
    B_w_up: jax.Array,
    B_w_down: jax.Array,
):
    del B_x
    vm = pltpu.VMEM
    scratch = [
        vm((NSEG, D, L), BF16),
        vm((D, D), BF16),
        vm((D, D), BF16),
        vm((D, D), BF16),
        vm((D, D), BF16),
        vm((H,), BF16),
        vm((D,), BF16),
        vm((D, FF), BF16),
        vm((D, FF), BF16),
        vm((D, FF), BF16),
        vm((PROWS // 2, D), U32),
        vm((D // 2, D), U32),
        vm((NSEG * D // 2, L), U32),
        vm((NSEG * NG * 64, L), U32),
        vm((NSEG * NG * L // 2, 128), U32),
        vm((NSEG * H * 16, L), U32),
        vm((NSEG - 1, OROWS, L), F32),
        vm((8, L), F32),
        vm((8, D), U32),
        vm((2, D, 128), F32),
        vm((2, FF // 128, 8, 128), F32),
        pltpu.SMEM((2,), jnp.int32),
        pltpu.SMEM((2,), F32),
        pltpu.SMEM((1,), U32),
        pltpu.SMEM((1,), jnp.int32),
        vm((H, 128), F32),
        vm((NSEG, D, L), F32),
        vm((H, 24, L), F32),
        vm((128, 128), F32),
        vm((3, 64, 128), F32),
        vm((NSEG * D, L), BF16),
        pltpu.SemaphoreType.DMA((NSEG * NQT,)),
        pltpu.SemaphoreType.DMA((NSEG + 9 + 2,)),
    ]
    hbm = pl.BlockSpec(memory_space=pltpu.HBM)
    xt = jnp.transpose(A_x.reshape(S, D))
    out_t = pl.pallas_call(
        _kernel,
        grid=(NSEG + 1,),
        in_specs=[hbm] * 10,
        out_specs=hbm,
        out_shape=jax.ShapeDtypeStruct((D, S), BF16),
        scratch_shapes=scratch,
        compiler_params=pltpu.CompilerParams(
            dimension_semantics=("arbitrary",),
            vmem_limit_bytes=110 * 1024 * 1024,
        ),
        name="infini_moe",
    )(xt, A_wq, A_wk, A_wv, A_wo, A_beta, B_w_r, B_w_gate, B_w_up,
      jnp.transpose(B_w_down))
    return jnp.transpose(out_t).reshape(1, S, D)
```

```python
import contextlib

import jax
import jax.numpy as jnp
from jax import lax
from jax.experimental import pallas as pl
from jax.experimental.pallas import tpu as pltpu

S = 2048
D = 576
H = 32
DH = 18
NSEG = 4
L = 512
FF = 4608
NG = 5
HPG = 7
GW = HPG * DH
NQT = L // 128
PROWS = 3 * D + 16
RROW = 3 * D
EARLY_K = 1
PBLOCK = 128
MROWS = 144
FT = FF // 128 // NSEG
OROWS = 640
LOG2E = 1.4426950408889634
QSCALE = DH ** -0.5 * LOG2E
NEG = -1e30
LN_EPS = 1.0013580322265625e-05
F32 = jnp.float32
BF16 = jnp.bfloat16
U32 = jnp.uint32

PROFILE_SCOPES = False

_NN = (((1,), (0,)), ((), ()))
_NT = (((1,), (1,)), ((), ()))


def _scope(name):
    return jax.named_scope(name) if PROFILE_SCOPES else contextlib.nullcontext()


def _dot(a, b):
    return lax.dot_general(a, b, _NN, preferred_element_type=F32)


def _dot_nt(a, b):
    return lax.dot_general(a, b, _NT, preferred_element_type=F32)


def _iota(shape, dim):
    return lax.broadcasted_iota(jnp.int32, shape, dim)


def _round_bf16(v):
    return v.astype(BF16).astype(F32)


def _pack(v):
    return pltpu.bitcast(v.astype(BF16), U32)


def _unpack(u):
    return pltpu.bitcast(u, BF16)


def _rows(index, size):
    if isinstance(index, int):
        return slice(index * size, (index + 1) * size)
    return pl.ds(pl.multiple_of(index * size, 8), size)


def _heads_in_group(g):
    return HPG if g < NG - 1 else H - HPG * (NG - 1)


def _phi(t):
    return jnp.where(t > 0, t + 1.0, jnp.exp(t))


def _kernel(x_hbm, wq_hbm, wk_hbm, wv_hbm, wo_hbm, beta_hbm, wr_hbm,
            wg_hbm, wu_hbm, wd_hbm,
            o_hbm,
            x_v, wq_v, wk_v, wv_v, wo_v, beta_v, wr_v, wg_v, wu_v, wd_v,
            wall, wot, xn_v, qt_v, k_v, vt_v, mem_v,
            r_v, xs_v, y_v, hid_v, idx_s, rsel_s, zero_s, safe_s,
            gate_v, ot_v, oh_v, bias_v, half_v, out_v, out_sems,
            sems):
    step = pl.program_id(0)

    x_copies = [None] + [
        pltpu.make_async_copy(x_hbm.at[:, pl.ds(c * L, L)], x_v.at[c], sems.at[c])
        for c in range(1, NSEG)
    ]
    x0_copies = [
        pltpu.make_async_copy(x_hbm.at[:, pl.ds(256 * n, 256)],
                              x_v.at[0, :, pl.ds(256 * n, 256)],
                              sems.at[NSEG + 9 + n])
        for n in range(2)
    ]
    pairs = [(wq_hbm, wq_v), (wk_hbm, wk_v), (wv_hbm, wv_v), (wo_hbm, wo_v),
             (beta_hbm, beta_v), (wr_hbm, wr_v),
             (wg_hbm, wg_v), (wu_hbm, wu_v), (wd_hbm, wd_v)]
    (cp_wq, cp_wk, cp_wv, cp_wo, cp_beta, cp_wr, cp_wg, cp_wu, cp_wd) = [
        pltpu.make_async_copy(src, dst, sems.at[NSEG + i])
        for i, (src, dst) in enumerate(pairs)
    ]

    def nothing(v):
        return pltpu.bitcast(pltpu.bitcast(v, U32) & zero_s[0], F32)

    def layer_norm(c, serial=True, tiles=range(NQT)):
        link = None
        for n in tiles:
            cols = slice(128 * n, 128 * (n + 1))
            pivot = x_v[c, 0:16, cols].astype(F32)[0:1, :]
            pivot8 = jnp.broadcast_to(pivot, (8, 128))
            shift = pivot8
            s1 = s2 = None
            for i in range(D // 16):
                last = s1 if s1 is not None else link
                if serial and last is not None:
                    shift = pivot8 + nothing(last)
                x16 = x_v[c, 16 * i:16 * i + 16, cols].astype(F32)
                for k in range(2):
                    d = x16[8 * k:8 * k + 8, :] - shift
                    s1 = d if s1 is None else s1 + d
                    s2 = d * d if s2 is None else s2 + d * d
            dmean = jnp.sum(s1, axis=0, keepdims=True) * (1.0 / D)
            dsq = jnp.sum(s2, axis=0, keepdims=True) * (1.0 / D)
            var = jnp.maximum(dsq - dmean * dmean, 0.0)
            sd = _round_bf16(jnp.sqrt(_round_bf16(_round_bf16(var) + LN_EPS)))
            mean8 = jnp.broadcast_to(_round_bf16(pivot + dmean), (8, 128))
            inv8 = jnp.broadcast_to(1.0 / sd, (8, 128))
            center = mean8
            for i in range(D // 32):
                if serial and i > 0:
                    center = mean8 + nothing(link)
                x32 = x_v[c, 32 * i:32 * i + 32, cols].astype(F32)
                z = [(x32[8 * k:8 * k + 8, :] - center) * inv8 for k in range(4)]
                link = z[3]
                r0 = c * (D // 2) + 16 * i
                xn_v[r0:r0 + 16, cols] = _pack(jnp.concatenate(z, axis=0))

    def init_constants():
        gate = jax.nn.sigmoid(beta_v[...].astype(F32).reshape(1, H))
        on_diag = _iota((H, H), 0) == _iota((H, H), 1)
        gcol = jnp.sum(jnp.where(on_diag, gate, 0.0), axis=1, keepdims=True)
        gate_v[...] = jnp.broadcast_to(gcol, (H, 128))
        zero_s[0] = jnp.uint32(0)
        bias_v[...] = jnp.where(_iota((128, 128), 0) > _iota((128, 128), 1), NEG, 0.0)
        key, lane = _iota((64, 128), 0), _iota((64, 128), 1)
        future = key > (lane & 63)
        half_v[0] = jnp.where(future, NEG, 0.0)
        half_v[1] = jnp.where(future | (lane < 64), NEG, 0.0)
        half_v[2] = jnp.where(future | (lane >= 64), NEG, 0.0)
        router = jnp.broadcast_to(wr_v[...].astype(F32).reshape(1, D), (16, D))
        wall[RROW // 2:PROWS // 2, :] = _pack(
            jnp.where(_iota((16, D), 0) == 0, router, 0.0))

    def project(c, router_first=False):
        xn = _unpack(xn_v[_rows(c, D // 2), :])
        step_rows = PBLOCK // 2
        end = RROW // 2 if router_first else PROWS // 2
        tail = [_dot(_unpack(wall[end:PROWS // 2, :]), xn)] if router_first else []
        return jnp.concatenate(
            [_dot(_unpack(wall[r:min(r + step_rows, end), :]), xn)
             for r in range(0, end, step_rows)] + tail, axis=0)

    seen = [None]

    def record_logit_bound():
        big = (seen[0] >> 30) & 1
        safe_s[0] = (jnp.max(big.astype(jnp.int32)) == 0).astype(jnp.int32)

    def store_qkv(c, pt):
        r_v[c:c + 1, :] = _round_bf16(pt[RROW:RROW + 1, :])
        tail_row = _iota((8, L), 0)
        for h in range(H):
            base = 2 * D + DH * h
            tail = jnp.where(tail_row < DH - 16, pt[base + 16:base + 24, :],
                             jnp.where(tail_row == DH - 16, 1.0, 0.0))
            blk = jnp.concatenate(
                [pt[base:base + 16, :], tail, jnp.zeros((8, L), F32)], axis=0)
            vt_v[_rows(c * H + h, 16), :] = _pack(blk)

        rowl = _iota((128, L), 0)
        pqs, pks, vgs = [], [], []
        for g in range(NG):
            used = _heads_in_group(g) * DH
            qg = pt[GW * g:GW * g + 128, :]
            qs = qg * QSCALE
            qt_v[_rows(c * NG + g, 64), :] = _pack(qs)
            kg = pt[D + GW * g:D + GW * g + 128, :]
            for operand in (qs, kg):
                bits = pltpu.bitcast(operand, U32)
                for blk in range(0, 128 if g < NG - 1 else used, 8):
                    for col in range(0, L, 128):
                        piece = bits[blk:blk + 8, col:col + 128]
                        seen[0] = piece if seen[0] is None else seen[0] | piece
            k_v[_rows(c * NG + g, L // 2), :] = _pack(kg.T)
            pqs.append(_phi(qg).astype(BF16))
            if c < NSEG - 1:
                pks.append(_phi(kg).astype(BF16))
                lo = 2 * D + GW * g
                if g < NG - 1:
                    vg = pt[lo:lo + 128, :]
                else:
                    vg = jnp.concatenate(
                        [pt[lo:lo + used, :], jnp.zeros((128 - used, L), F32)], axis=0)
                vg = jnp.where(rowl < used, vg, jnp.where(rowl == GW, 1.0, 0.0))
                vgs.append(vg.astype(BF16))
        return pqs, pks, vgs

    def memory_update(states, pks, vgs):
        row = _iota((128, 128), 0)
        lane = _iota((128, 128), 1)
        same_head = (row // DH) == (lane // DH)
        out = []
        for g in range(NG):
            used = _heads_in_group(g) * DH
            upd = _dot_nt(vgs[g], pks[g])
            keep = ((same_head & (row < used)) | (row == GW)) & (lane < used)
            upd = jnp.where(keep, upd, 0.0)
            out.append(upd if states is None else states[g] + upd)
        return out

    def memory_retrieve(c, states, pqs):
        row = _iota((128, 128), 0)
        row8 = _iota((8, 128), 0)
        lane8 = _iota((8, 128), 1) // DH
        for g in range(NG):
            nh = _heads_in_group(g)
            st = states[g]
            mrows = jnp.where(row < GW, st, 0.0)
            zrows = jnp.where(lane8 == row8, st[GW:GW + 1, :], 0.0)
            lhs = jnp.concatenate(
                [mrows, zrows, jnp.zeros((8, 128), F32)], axis=0).astype(BF16)
            ret = _dot(lhs, pqs[g])
            gsel = gate_v[HPG * g:HPG * g + 8, :] if g < NG - 1 else jnp.concatenate(
                [gate_v[HPG * g:H, :], jnp.zeros((8 - nh, 128), F32)], axis=0)
            gwide = jnp.concatenate([gsel] * NQT, axis=1)
            scale = gwide / (ret[128:136, :] + 1e-6)
            pieces = []
            for b in range(16):
                h0 = min((8 * b) // DH, nh - 1)
                h1 = min((8 * b + 7) // DH, nh - 1)
                sc = scale[h0:h0 + 1, :]
                if h1 != h0:
                    first = _iota((8, L), 0) < DH * h1 - 8 * b
                    sc = jnp.where(first, sc, scale[h1:h1 + 1, :])
                pieces.append(ret[8 * b:8 * b + 8, :] * sc)
            mem_v[c - 1, GW * g:GW * g + 128, :] = jnp.concatenate(pieces, axis=0)

    def route():
        r = r_v[0:NSEG, :]
        idx = _iota((NSEG, L), 0) * L + _iota((NSEG, L), 1)
        m1 = jnp.max(r)
        i1 = jnp.clip(jnp.min(jnp.where(r == m1, idx, S)), 0, S - 1)
        r2 = jnp.where(idx == i1, -jnp.inf, r)
        m2 = jnp.max(r2)
        i2 = jnp.clip(jnp.min(jnp.where(r2 == m2, idx, S)), 0, S - 1)
        idx_s[0] = i1
        idx_s[1] = i2
        rsel_s[0] = m1
        rsel_s[1] = m2
        row16 = _iota((16, 128), 0)
        lane16 = _iota((16, 128), 1)
        xs = None
        for t, i in enumerate((i1, i2)):
            seg = i // L
            off = i - seg * L
            base = pl.multiple_of((off // 128) * 128, 128)
            cols = _unpack(xn_v[_rows(seg, D // 2), pl.ds(base, 128)])
            pick = jnp.where((row16 == t) & (lane16 == off - base), 1.0, 0.0)
            part = _dot_nt(pick.astype(BF16), cols)
            xs = part if xs is None else xs + part
        xs_v[...] = _pack(xs)
        y_v[...] = jnp.zeros(y_v.shape, F32)

    def ffn_hidden():
        xs = _unpack(xs_v[...])
        gt = _round_bf16(_dot(xs, wg_v[...]))
        up = _round_bf16(_dot(xs, wu_v[...]))
        hid = _round_bf16(_round_bf16(gt * jax.nn.sigmoid(gt)) * up)
        for t in range(2):
            for tile in range(FF // 128):
                hid_v[t, tile] = jnp.broadcast_to(
                    hid[t:t + 1, 128 * tile:128 * (tile + 1)], (8, 128))

    def ffn_down_chained():
        base = pl.multiple_of(step * (FT * 128), 128)
        link = [None, None]
        for b in range(D // 8):
            acc = [None, None]
            for tile in range(FT):
                w = wd_v[8 * b:8 * b + 8, pl.ds(base + 128 * tile, 128)].astype(F32)
                for t in range(2):
                    pr = w * hid_v[t, step * FT + tile]
                    if tile > 0:
                        acc[t] = acc[t] + pr
                    else:
                        acc[t] = pr if link[t] is None else pr + nothing(link[t])
            for t in range(2):
                rows = slice(8 * b, 8 * b + 8)
                y_v[t, rows, :] = y_v[t, rows, :] + acc[t]
                link[t] = acc[t]

    def ffn_down_looped():
        def down(tile, carry):
            col = step * FT + tile
            w = wd_v[:, pl.ds(pl.multiple_of(128 * col, 128), 128)].astype(F32)
            for t in range(2):
                y_v[t] = y_v[t] + w * hid_v[t, col][0:1, :]
            return carry

        lax.fori_loop(0, FT, down, 0)

    def masked_q_bits(g, hp, j):
        rid = _iota((64, 128), 0)
        mask = (rid >= (DH // 2) * hp) & (rid < (DH // 2) * (hp + 1))
        return jnp.where(mask, qt_v[_rows(step * NG + g, 64), 128 * j:128 * (j + 1)],
                         jnp.uint32(0))

    def keys(g, lo, hi):
        first = pl.multiple_of((step * NG + g) * (L // 2) + lo // 2, 8)
        return _unpack(k_v[pl.ds(first, (hi - lo) // 2), :])

    def causal_scores(g, hp, j):
        nk = 128 * (j + 1)
        st = _dot(keys(g, 0, nk), _unpack(masked_q_bits(g, hp, j)))
        diag = st[nk - 128:, :] + bias_v[...]
        return diag if j == 0 else jnp.concatenate([st[:nk - 128, :], diag], axis=0)

    def head_output(h, j, p, keep):
        o = _dot(_unpack(vt_v[_rows(step * H + h, 16), 0:128 * (j + 1)]), p)
        den = o[DH:DH + 1, :]
        inv = pl.reciprocal(den, approx=True)
        inv = inv * (2.0 - den * inv)
        return o[0:24, :] * (keep * inv)

    def single_probs(h, j):
        return jnp.exp2(causal_scores(*divmod(h, HPG), j)).astype(BF16)

    def pair_probs(pairs, j, flip):
        low = _iota((64, 128), 1) < 64
        qa, qb = {}, {}
        for h in pairs:
            g, hp = divmod(h, HPG)
            qa[h] = masked_q_bits(g, hp, j)
            qb[h] = pltpu.roll(masked_q_bits(g, hp + 1, j), 64, 1)
        off = {}
        if j > 0:
            for h in pairs:
                g = h // HPG
                for hh, q in ((h, qa[h]), (h + 1, qb[h])):
                    off[hh] = jnp.exp2(_dot(keys(g, 0, 128 * j), _unpack(q)))
        early, late = {}, {}
        for h in pairs:
            g = h // HPG
            k0 = 128 * j
            for which in ((0, 1) if flip else (1, 0)):
                if which == 0:
                    early[h] = _dot(keys(g, k0, k0 + 64),
                                    _unpack(jnp.where(low, qa[h], qb[h])))
                else:
                    late[h] = _dot(keys(g, k0, k0 + 128),
                                   _unpack(jnp.where(low, qb[h], qa[h])))
        probs = {}
        for h in pairs:
            p1 = jnp.exp2(early[h] + half_v[0])
            p2 = jnp.exp2(late[h][0:64, :])
            bottom = late[h][64:128, :]
            pa = jnp.concatenate(
                [jnp.where(low, p1, p2), jnp.exp2(bottom + half_v[1])], axis=0)
            pb = jnp.concatenate(
                [jnp.where(low, p2, p1), jnp.exp2(bottom + half_v[2])], axis=0)
            for hh, pd in ((h, pa), (h + 1, pb)):
                full = pd if j == 0 else jnp.concatenate([off[hh], pd], axis=0)
                probs[hh] = full.astype(BF16)
        return probs

    def attention_bounded():
        pairs = [g * HPG + hp for g in range(NG)
                 for hp in range(0, _heads_in_group(g) - 1, 2)]
        paired = set(pairs) | {h + 1 for h in pairs}
        singles = [h for h in range(H) if h not in paired]
        waves = [(pairs[i:i + 2], j) for i in range(0, len(pairs), 2) for j in range(NQT)]
        waves += [(None, j) for j in range(NQT)]

        def scores(w):
            grp, j = waves[w]
            if grp is None:
                return {h: single_probs(h, j) for h in singles}
            return pair_probs(grp, j, w % 2 == 1)

        def values(w, probs):
            grp, j = waves[w]
            for h, p in probs.items():
                o = head_output(h, j, p, 1.0 - gate_v[h:h + 1, :])
                if grp is not None and h - 1 in grp:
                    o = pltpu.roll(o, 64, 1)
                ot_v[step, DH * h:DH * (h + 1), 128 * j:128 * (j + 1)] = o[0:DH, :]

        pending = scores(0)
        for w in range(len(waves)):
            nxt = scores(w + 1) if w + 1 < len(waves) else None
            values(w, pending)
            pending = nxt
        ffn_down_chained()

    def attention_max_shifted():
        def one_tile(item, carry):
            h = item // NQT
            j = item - h * NQT
            g = h // HPG
            hp = h - g * HPG
            cols = pl.ds(pl.multiple_of(128 * j, 128), 128)
            rid = _iota((64, 128), 0)
            mask = (rid >= (DH // 2) * hp) & (rid < (DH // 2) * (hp + 1))
            qm = jnp.where(mask, qt_v[_rows(step * NG + g, 64), cols], jnp.uint32(0))
            st = _dot(keys(g, 0, L), _unpack(qm))
            future = _iota((L, 128), 0) > 128 * j + _iota((L, 128), 1)
            st = jnp.where(future, NEG, st)
            p = jnp.exp2(st - jnp.max(st, axis=0, keepdims=True)).astype(BF16)
            keep = 1.0 - gate_v[pl.ds(h, 1), :]
            oh_v[h, :, cols] = head_output(h, NQT - 1, p, keep)
            return carry

        def compact(q, carry):
            rows = jnp.concatenate([oh_v[4 * q + k, 0:DH, :] for k in range(4)], axis=0)
            ot_v[step, pl.ds(pl.multiple_of(4 * DH * q, 8), 4 * DH), :] = rows
            return carry

        lax.fori_loop(0, H * NQT, one_tile, 0)
        lax.fori_loop(0, H // 4, compact, 0)
        ffn_down_looped()

    def routed_columns():
        ys = []
        for t in range(2):
            y = _round_bf16(jnp.sum(y_v[t], axis=1, keepdims=True))
            rsel = jnp.full((1, 1), rsel_s[t], F32)
            ys.append(_round_bf16(y * _round_bf16(jax.nn.sigmoid(rsel))))
        return ys

    def output_copy(seg, n):
        return pltpu.make_async_copy(
            out_v.at[pl.ds(seg * D, D), pl.ds(128 * n, 128)],
            o_hbm.at[:, pl.ds(seg * L + 128 * n, 128)],
            out_sems.at[NQT * seg + n])

    def output_projection(seg, ys):
        heads_out = ot_v[seg, 0:D, :]
        if seg > 0:
            heads_out = heads_out + mem_v[seg - 1, 0:D, :]
        attn = _dot(_unpack(wot[...]), heads_out.astype(BF16))
        base = x_v[seg].astype(F32) + attn
        xn = _unpack(xn_v[_rows(seg, D // 2), :]).astype(F32)
        col = seg * L + _iota((1, L), 1)
        upd = (jnp.where(col == idx_s[0], ys[0], 0.0)
               + jnp.where(col == idx_s[1], ys[1], 0.0))
        result = base + (xn + upd)
        for n in range(NQT):
            cols = slice(128 * n, 128 * (n + 1))
            out_v[seg * D:(seg + 1) * D, cols] = result[:, cols].astype(BF16)
            output_copy(seg, n).start()

    col_blocks = [(c0, min(128, D - c0)) for c0 in range(0, D, 128)]

    def transpose_block(w_v, section, c0, n):
        r0 = (section * D + c0) // 2
        wall[r0:r0 + n // 2, :] = pltpu.bitcast(w_v[:, c0:c0 + n].T, U32)

    def project_block(section, c0, n, xn):
        r0 = (section * D + c0) // 2
        last = section == 2 and c0 + n == D
        hi = PROWS // 2 if last else r0 + n // 2
        return _dot(_unpack(wall[r0:hi, :]), xn)

    def query_half0(half):
        layer_norm(0, serial=False, tiles=[2 * half, 2 * half + 1])
        xn = _unpack(xn_v[0:D // 2, 256 * half:256 * (half + 1)])
        top = _dot(_unpack(wall[0:D // 4, :]), xn)
        if half == 0:
            for c0, n in col_blocks[3:]:
                transpose_block(wq_v, 0, c0, n)
        bottom = _dot(_unpack(wall[D // 4:D // 2, :]), xn)
        return jnp.concatenate([top, bottom], axis=0)

    def projections():
        qtiles = []
        for half in range(2):
            x0_copies[half].wait()
            if half == 1:
                cp_wk.wait()
            qtiles.append(query_half0(half))
        for c0, n in col_blocks:
            transpose_block(wk_v, 1, c0, n)
        parts = [jnp.concatenate(qtiles, axis=1)]
        xn0 = _unpack(xn_v[_rows(0, D // 2), :])
        parts += [project_block(1, c0, n, xn0) for c0, n in col_blocks[:EARLY_K]]
        cp_wv.wait()
        x_copies[1].wait()
        xn0 = _unpack(xn_v[_rows(0, D // 2), :])
        parts += [project_block(1, c0, n, xn0) for c0, n in col_blocks[EARLY_K:]]
        for c0, n in col_blocks:
            transpose_block(wv_v, 2, c0, n)
            parts.append(project_block(2, c0, n, xn0))
        layer_norm(1)
        _, pk, vg = store_qkv(0, jnp.concatenate(parts, axis=0))
        x_copies[2].wait()
        x_copies[3].wait()
        cp_wo.wait()

        layer_norm(2)
        pt = project(1)
        wot[...] = pltpu.bitcast(wo_v[...].T, U32)
        state1 = memory_update(None, pk, vg)
        pq1, pk, vg = store_qkv(1, pt)
        layer_norm(3)
        pt = project(2)
        state2 = memory_update(state1, pk, vg)
        pq2, pk, vg = store_qkv(2, pt)
        cp_wg.wait()
        cp_wu.wait()
        pt = project(3, router_first=True)
        pq3, _, _ = store_qkv(3, pt)
        route()
        ffn_hidden()
        state3 = memory_update(state2, pk, vg)
        memory_retrieve(1, state1, pq1)
        memory_retrieve(2, state2, pq2)
        memory_retrieve(3, state3, pq3)
        record_logit_bound()
        cp_wd.wait()

    @pl.when(step == 0)
    def _():
        for cp in (cp_wq, cp_wr, cp_beta, *x0_copies, cp_wk, cp_wv, x_copies[1],
                   x_copies[2], x_copies[3], cp_wo, cp_wg, cp_wu, cp_wd):
            cp.start()
        with _scope("sc_startup"):
            cp_wr.wait()
            cp_beta.wait()
            cp_wq.wait()
            init_constants()
            for c0, n in col_blocks[:3]:
                transpose_block(wq_v, 0, c0, n)
        with _scope("sc_projections"):
            projections()

    @pl.when(step < NSEG)
    def _():
        safe = safe_s[0] == 1

        @pl.when(safe)
        def _():
            with _scope("sc_attention"):
                attention_bounded()

        @pl.when(jnp.logical_not(safe))
        def _():
            attention_max_shifted()

    @pl.when(step == NSEG)
    def _():
        with _scope("sc_outproj"):
            ys = routed_columns()
            for seg in range(NSEG):
                output_projection(seg, ys)
            for seg in range(NSEG):
                for n in range(NQT):
                    output_copy(seg, n).wait()


@jax.jit
def pallas_parallel_sum__memory_aug_infini_attn__moe_arch_mod__prompt_kernel(
    A_x: jax.Array,
    A_wq: jax.Array,
    A_wk: jax.Array,
    A_wv: jax.Array,
    A_wo: jax.Array,
    A_beta: jax.Array,
    B_x: jax.Array,
    B_w_r: jax.Array,
    B_w_gate: jax.Array,
    B_w_up: jax.Array,
    B_w_down: jax.Array,
):
    del B_x
    vm = pltpu.VMEM
    scratch = [
        vm((NSEG, D, L), BF16),
        vm((D, D), BF16),
        vm((D, D), BF16),
        vm((D, D), BF16),
        vm((D, D), BF16),
        vm((H,), BF16),
        vm((D,), BF16),
        vm((D, FF), BF16),
        vm((D, FF), BF16),
        vm((D, FF), BF16),
        vm((PROWS // 2, D), U32),
        vm((D // 2, D), U32),
        vm((NSEG * D // 2, L), U32),
        vm((NSEG * NG * 64, L), U32),
        vm((NSEG * NG * L // 2, 128), U32),
        vm((NSEG * H * 16, L), U32),
        vm((NSEG - 1, OROWS, L), F32),
        vm((8, L), F32),
        vm((8, D), U32),
        vm((2, D, 128), F32),
        vm((2, FF // 128, 8, 128), F32),
        pltpu.SMEM((2,), jnp.int32),
        pltpu.SMEM((2,), F32),
        pltpu.SMEM((1,), U32),
        pltpu.SMEM((1,), jnp.int32),
        vm((H, 128), F32),
        vm((NSEG, D, L), F32),
        vm((H, 24, L), F32),
        vm((128, 128), F32),
        vm((3, 64, 128), F32),
        vm((NSEG * D, L), BF16),
        pltpu.SemaphoreType.DMA((NSEG * NQT,)),
        pltpu.SemaphoreType.DMA((NSEG + 9 + 2,)),
    ]
    hbm = pl.BlockSpec(memory_space=pltpu.HBM)
    xt = jnp.transpose(A_x.reshape(S, D))
    out_t = pl.pallas_call(
        _kernel,
        grid=(NSEG + 1,),
        in_specs=[hbm] * 10,
        out_specs=hbm,
        out_shape=jax.ShapeDtypeStruct((D, S), BF16),
        scratch_shapes=scratch,
        compiler_params=pltpu.CompilerParams(
            dimension_semantics=("arbitrary",),
            vmem_limit_bytes=110 * 1024 * 1024,
        ),
        name="infini_moe",
    )(xt, A_wq, A_wk, A_wv, A_wo, A_beta, B_w_r, B_w_gate, B_w_up,
      jnp.transpose(B_w_down))
    return jnp.transpose(out_t).reshape(1, S, D)
```

```python
import contextlib

import jax
import jax.numpy as jnp
from jax import lax
from jax.experimental import pallas as pl
from jax.experimental.pallas import tpu as pltpu

S = 2048
D = 576
H = 32
DH = 18
NSEG = 4
L = 512
FF = 4608
NG = 5
HPG = 7
GW = HPG * DH
NQT = L // 128
PROWS = 3 * D + 16
RROW = 3 * D
EARLY_K = 1
PBLOCK = 128
FT = FF // 128 // NSEG
LOG2E = 1.4426950408889634
QSCALE = DH ** -0.5 * LOG2E
NEG = -1e30
LN_EPS = 1.0013580322265625e-05
F32 = jnp.float32
BF16 = jnp.bfloat16
U32 = jnp.uint32

PROFILE_SCOPES = False

_NN = (((1,), (0,)), ((), ()))
_NT = (((1,), (1,)), ((), ()))


def _scope(name):
    return jax.named_scope(name) if PROFILE_SCOPES else contextlib.nullcontext()


def _dot(a, b):
    return lax.dot_general(a, b, _NN, preferred_element_type=F32)


def _dot_nt(a, b):
    return lax.dot_general(a, b, _NT, preferred_element_type=F32)


def _iota(shape, dim):
    return lax.broadcasted_iota(jnp.int32, shape, dim)


def _round_bf16(v):
    return v.astype(BF16).astype(F32)


def _pack(v):
    return pltpu.bitcast(v.astype(BF16), U32)


def _unpack(u):
    return pltpu.bitcast(u, BF16)


def _rows(index, size):
    if isinstance(index, int):
        return slice(index * size, (index + 1) * size)
    return pl.ds(pl.multiple_of(index * size, 8), size)


def _heads_in_group(g):
    return HPG if g < NG - 1 else H - HPG * (NG - 1)


def _memory_rows(g):
    used = _heads_in_group(g) * DH
    return (128, GW) if g < NG - 1 else (used + 8, used)


def _phi(t):
    return jnp.where(t > 0, t + 1.0, jnp.exp(t))


def _kernel(x_hbm, wq_hbm, wk_hbm, wv_hbm, wo_hbm, beta_hbm, wr_hbm,
            wg_hbm, wu_hbm, wd_hbm,
            o_hbm,
            x_v, wq_v, wk_v, wv_v, wo_v, beta_v, wr_v, wg_v, wu_v, wd_v,
            wall, wot, xn_v, qt_v, k_v, vt_v, mem_v,
            r_v, xs_v, y_v, hid_v, idx_s, rsel_s, zero_s, safe_s,
            gate_v, ot_v, oh_v, bias_v, half_v, out_v, out_sems,
            sems):
    step = pl.program_id(0)

    x_copies = [None] + [
        pltpu.make_async_copy(x_hbm.at[:, pl.ds(c * L, L)], x_v.at[c], sems.at[c])
        for c in range(1, NSEG)
    ]
    x0_copies = [
        pltpu.make_async_copy(x_hbm.at[:, pl.ds(256 * n, 256)],
                              x_v.at[0, :, pl.ds(256 * n, 256)],
                              sems.at[NSEG + 9 + n])
        for n in range(2)
    ]
    pairs = [(wq_hbm, wq_v), (wk_hbm, wk_v), (wv_hbm, wv_v), (wo_hbm, wo_v),
             (beta_hbm, beta_v), (wr_hbm, wr_v),
             (wg_hbm, wg_v), (wu_hbm, wu_v), (wd_hbm, wd_v)]
    (cp_wq, cp_wk, cp_wv, cp_wo, cp_beta, cp_wr, cp_wg, cp_wu, cp_wd) = [
        pltpu.make_async_copy(src, dst, sems.at[NSEG + i])
        for i, (src, dst) in enumerate(pairs)
    ]

    def nothing(v):
        return pltpu.bitcast(pltpu.bitcast(v, U32) & zero_s[0], F32)

    def layer_norm(c, serial=True, tiles=range(NQT)):
        link = None
        for n in tiles:
            cols = slice(128 * n, 128 * (n + 1))
            pivot = x_v[c, 0:16, cols].astype(F32)[0:1, :]
            pivot8 = jnp.broadcast_to(pivot, (8, 128))
            shift = pivot8
            s1 = s2 = None
            for i in range(D // 16):
                last = s1 if s1 is not None else link
                if serial and last is not None:
                    shift = pivot8 + nothing(last)
                x16 = x_v[c, 16 * i:16 * i + 16, cols].astype(F32)
                for k in range(2):
                    d = x16[8 * k:8 * k + 8, :] - shift
                    s1 = d if s1 is None else s1 + d
                    s2 = d * d if s2 is None else s2 + d * d
            dmean = jnp.sum(s1, axis=0, keepdims=True) * (1.0 / D)
            dsq = jnp.sum(s2, axis=0, keepdims=True) * (1.0 / D)
            var = jnp.maximum(dsq - dmean * dmean, 0.0)
            sd = _round_bf16(jnp.sqrt(_round_bf16(_round_bf16(var) + LN_EPS)))
            mean8 = jnp.broadcast_to(_round_bf16(pivot + dmean), (8, 128))
            inv8 = jnp.broadcast_to(1.0 / sd, (8, 128))
            center = mean8
            for i in range(D // 32):
                if serial and i > 0:
                    center = mean8 + nothing(link)
                x32 = x_v[c, 32 * i:32 * i + 32, cols].astype(F32)
                z = [(x32[8 * k:8 * k + 8, :] - center) * inv8 for k in range(4)]
                link = z[3]
                r0 = c * (D // 2) + 16 * i
                xn_v[r0:r0 + 16, cols] = _pack(jnp.concatenate(z, axis=0))

    def init_constants():
        gate = jax.nn.sigmoid(beta_v[...].astype(F32).reshape(1, H))
        on_diag = _iota((H, H), 0) == _iota((H, H), 1)
        gcol = jnp.sum(jnp.where(on_diag, gate, 0.0), axis=1, keepdims=True)
        gate_v[...] = jnp.broadcast_to(gcol, (H, 128))
        zero_s[0] = jnp.uint32(0)
        bias_v[...] = jnp.where(_iota((128, 128), 0) > _iota((128, 128), 1), NEG, 0.0)
        key, lane = _iota((64, 128), 0), _iota((64, 128), 1)
        future = key > (lane & 63)
        half_v[0] = jnp.where(future, NEG, 0.0)
        half_v[1] = jnp.where(future | (lane < 64), NEG, 0.0)
        half_v[2] = jnp.where(future | (lane >= 64), NEG, 0.0)
        router = jnp.broadcast_to(wr_v[...].astype(F32).reshape(1, D), (16, D))
        wall[RROW // 2:PROWS // 2, :] = _pack(
            jnp.where(_iota((16, D), 0) == 0, router, 0.0))

    def project(c, router_first=False):
        xn = _unpack(xn_v[_rows(c, D // 2), :])
        step_rows = PBLOCK // 2
        end = RROW // 2 if router_first else PROWS // 2
        tail = [_dot(_unpack(wall[end:PROWS // 2, :]), xn)] if router_first else []
        return jnp.concatenate(
            [_dot(_unpack(wall[r:min(r + step_rows, end), :]), xn)
             for r in range(0, end, step_rows)] + tail, axis=0)

    seen = [None]

    def record_logit_bound():
        big = (seen[0] >> 30) & 1
        safe_s[0] = (jnp.max(big.astype(jnp.int32)) == 0).astype(jnp.int32)

    def store_qkv(c, pt):
        r_v[c:c + 1, :] = _round_bf16(pt[RROW:RROW + 1, :])
        tail_row = _iota((8, L), 0)
        for h in range(H):
            base = 2 * D + DH * h
            tail = jnp.where(tail_row < DH - 16, pt[base + 16:base + 24, :],
                             jnp.where(tail_row == DH - 16, 1.0, 0.0))
            blk = jnp.concatenate(
                [pt[base:base + 16, :], tail, jnp.zeros((8, L), F32)], axis=0)
            vt_v[_rows(c * H + h, 16), :] = _pack(blk)

        pqs, pks, vgs = [], [], []
        for g in range(NG):
            used = _heads_in_group(g) * DH
            qg = pt[GW * g:GW * g + 128, :]
            qs = qg * QSCALE
            qt_v[_rows(c * NG + g, 64), :] = _pack(qs)
            kg = pt[D + GW * g:D + GW * g + 128, :]
            for operand in (qs, kg):
                bits = pltpu.bitcast(operand, U32)
                for blk in range(0, 128 if g < NG - 1 else used, 8):
                    for col in range(0, L, 128):
                        piece = bits[blk:blk + 8, col:col + 128]
                        seen[0] = piece if seen[0] is None else seen[0] | piece
            k_v[_rows(c * NG + g, L // 2), :] = _pack(kg.T)
            pqs.append(_phi(qg).astype(BF16))
            if c < NSEG - 1:
                pks.append(_phi(kg).astype(BF16))
                lo = 2 * D + GW * g
                rows, zrow = _memory_rows(g)
                rid = _iota((rows, L), 0)
                vg = jnp.where(rid < used, pt[lo:lo + rows, :],
                               jnp.where(rid == zrow, 1.0, 0.0))
                vgs.append(vg.astype(BF16))
        return pqs, pks, vgs

    def memory_update(states, pks, vgs):
        out = []
        for g in range(NG):
            used = _heads_in_group(g) * DH
            rows, zrow = _memory_rows(g)
            row = _iota((rows, 128), 0)
            lane = _iota((rows, 128), 1)
            same_head = (row // DH) == (lane // DH)
            upd = _dot_nt(vgs[g], pks[g])
            keep = ((same_head & (row < used)) | (row == zrow)) & (lane < used)
            upd = jnp.where(keep, upd, 0.0)
            out.append(upd if states is None else states[g] + upd)
        return out

    def memory_retrieve(c, states, pqs):
        row8 = _iota((8, 128), 0)
        lane8 = _iota((8, 128), 1) // DH
        for g in range(NG):
            nh = _heads_in_group(g)
            rows, zrow = _memory_rows(g)
            st = states[g]
            mrows = jnp.where(_iota((rows, 128), 0) < zrow, st, 0.0)
            zrows = jnp.where(lane8 == row8, st[zrow:zrow + 1, :], 0.0)
            lhs = jnp.concatenate(
                [mrows, zrows, jnp.zeros((8, 128), F32)], axis=0).astype(BF16)
            ret = _dot(lhs, pqs[g])
            gsel = gate_v[HPG * g:HPG * g + 8, :] if g < NG - 1 else jnp.concatenate(
                [gate_v[HPG * g:H, :], jnp.zeros((8 - nh, 128), F32)], axis=0)
            gwide = jnp.concatenate([gsel] * NQT, axis=1)
            scale = gwide / (ret[rows:rows + 8, :] + 1e-6)
            out_rows = 128 if g < NG - 1 else nh * DH
            pieces = []
            for b in range(out_rows // 8):
                h0 = min((8 * b) // DH, nh - 1)
                h1 = min((8 * b + 7) // DH, nh - 1)
                sc = scale[h0:h0 + 1, :]
                if h1 != h0:
                    first = _iota((8, L), 0) < DH * h1 - 8 * b
                    sc = jnp.where(first, sc, scale[h1:h1 + 1, :])
                pieces.append(ret[8 * b:8 * b + 8, :] * sc)
            mem_v[c - 1, GW * g:GW * g + out_rows, :] = jnp.concatenate(pieces, axis=0)

    def route():
        r = r_v[0:NSEG, :]
        idx = _iota((NSEG, L), 0) * L + _iota((NSEG, L), 1)
        m1 = jnp.max(r)
        i1 = jnp.clip(jnp.min(jnp.where(r == m1, idx, S)), 0, S - 1)
        r2 = jnp.where(idx == i1, -jnp.inf, r)
        m2 = jnp.max(r2)
        i2 = jnp.clip(jnp.min(jnp.where(r2 == m2, idx, S)), 0, S - 1)
        idx_s[0] = i1
        idx_s[1] = i2
        rsel_s[0] = m1
        rsel_s[1] = m2
        row16 = _iota((16, 128), 0)
        lane16 = _iota((16, 128), 1)
        xs = None
        for t, i in enumerate((i1, i2)):
            seg = i // L
            off = i - seg * L
            base = pl.multiple_of((off // 128) * 128, 128)
            cols = _unpack(xn_v[_rows(seg, D // 2), pl.ds(base, 128)])
            pick = jnp.where((row16 == t) & (lane16 == off - base), 1.0, 0.0)
            part = _dot_nt(pick.astype(BF16), cols)
            xs = part if xs is None else xs + part
        xs_v[...] = _pack(xs)
        y_v[...] = jnp.zeros(y_v.shape, F32)

    def ffn_hidden():
        xs = _unpack(xs_v[...])
        gt = _round_bf16(_dot(xs, wg_v[...]))
        up = _round_bf16(_dot(xs, wu_v[...]))
        hid = _round_bf16(_round_bf16(gt * jax.nn.sigmoid(gt)) * up)
        for t in range(2):
            for tile in range(FF // 128):
                hid_v[t, tile] = jnp.broadcast_to(
                    hid[t:t + 1, 128 * tile:128 * (tile + 1)], (8, 128))

    def ffn_down_chained():
        base = pl.multiple_of(step * (FT * 128), 128)
        link = [None, None]
        for b in range(D // 8):
            acc = [None, None]
            for tile in range(FT):
                w = wd_v[8 * b:8 * b + 8, pl.ds(base + 128 * tile, 128)].astype(F32)
                for t in range(2):
                    pr = w * hid_v[t, step * FT + tile]
                    if tile > 0:
                        acc[t] = acc[t] + pr
                    else:
                        acc[t] = pr if link[t] is None else pr + nothing(link[t])
            for t in range(2):
                rows = slice(8 * b, 8 * b + 8)
                y_v[t, rows, :] = y_v[t, rows, :] + acc[t]
                link[t] = acc[t]

    def ffn_down_looped():
        def down(tile, carry):
            col = step * FT + tile
            w = wd_v[:, pl.ds(pl.multiple_of(128 * col, 128), 128)].astype(F32)
            for t in range(2):
                y_v[t] = y_v[t] + w * hid_v[t, col][0:1, :]
            return carry

        lax.fori_loop(0, FT, down, 0)

    def masked_q_bits(g, hp, j):
        rid = _iota((64, 128), 0)
        mask = (rid >= (DH // 2) * hp) & (rid < (DH // 2) * (hp + 1))
        return jnp.where(mask, qt_v[_rows(step * NG + g, 64), 128 * j:128 * (j + 1)],
                         jnp.uint32(0))

    def keys(g, lo, hi):
        first = pl.multiple_of((step * NG + g) * (L // 2) + lo // 2, 8)
        return _unpack(k_v[pl.ds(first, (hi - lo) // 2), :])

    def causal_scores(g, hp, j):
        nk = 128 * (j + 1)
        st = _dot(keys(g, 0, nk), _unpack(masked_q_bits(g, hp, j)))
        diag = st[nk - 128:, :] + bias_v[...]
        return diag if j == 0 else jnp.concatenate([st[:nk - 128, :], diag], axis=0)

    def head_output(h, j, p, keep):
        o = _dot(_unpack(vt_v[_rows(step * H + h, 16), 0:128 * (j + 1)]), p)
        den = o[DH:DH + 1, :]
        inv = pl.reciprocal(den, approx=True)
        inv = inv * (2.0 - den * inv)
        return o[0:24, :] * (keep * inv)

    def single_probs(h, j):
        return jnp.exp2(causal_scores(*divmod(h, HPG), j)).astype(BF16)

    def pair_probs(pairs, j, flip):
        low = _iota((64, 128), 1) < 64
        qa, qb = {}, {}
        for h in pairs:
            g, hp = divmod(h, HPG)
            qa[h] = masked_q_bits(g, hp, j)
            qb[h] = pltpu.roll(masked_q_bits(g, hp + 1, j), 64, 1)
        off = {}
        if j > 0:
            for h in pairs:
                g = h // HPG
                for hh, q in ((h, qa[h]), (h + 1, qb[h])):
                    off[hh] = jnp.exp2(_dot(keys(g, 0, 128 * j), _unpack(q)))
        early, late = {}, {}
        for h in pairs:
            g = h // HPG
            k0 = 128 * j
            for which in ((0, 1) if flip else (1, 0)):
                if which == 0:
                    early[h] = _dot(keys(g, k0, k0 + 64),
                                    _unpack(jnp.where(low, qa[h], qb[h])))
                else:
                    late[h] = _dot(keys(g, k0, k0 + 128),
                                   _unpack(jnp.where(low, qb[h], qa[h])))
        probs = {}
        for h in pairs:
            p1 = jnp.exp2(early[h] + half_v[0])
            p2 = jnp.exp2(late[h][0:64, :])
            bottom = late[h][64:128, :]
            pa = jnp.concatenate(
                [jnp.where(low, p1, p2), jnp.exp2(bottom + half_v[1])], axis=0)
            pb = jnp.concatenate(
                [jnp.where(low, p2, p1), jnp.exp2(bottom + half_v[2])], axis=0)
            for hh, pd in ((h, pa), (h + 1, pb)):
                full = pd if j == 0 else jnp.concatenate([off[hh], pd], axis=0)
                probs[hh] = full.astype(BF16)
        return probs

    def attention_bounded():
        pairs = [g * HPG + hp for g in range(NG)
                 for hp in range(0, _heads_in_group(g) - 1, 2)]
        paired = set(pairs) | {h + 1 for h in pairs}
        singles = [h for h in range(H) if h not in paired]
        waves = [(pairs[i:i + 2], j) for i in range(0, len(pairs), 2) for j in range(NQT)]
        waves += [(None, j) for j in range(NQT)]

        def scores(w):
            grp, j = waves[w]
            if grp is None:
                return {h: single_probs(h, j) for h in singles}
            return pair_probs(grp, j, w % 2 == 1)

        def values(w, probs):
            grp, j = waves[w]
            for h, p in probs.items():
                o = head_output(h, j, p, 1.0 - gate_v[h:h + 1, :])
                if grp is not None and h - 1 in grp:
                    o = pltpu.roll(o, 64, 1)
                ot_v[step, DH * h:DH * (h + 1), 128 * j:128 * (j + 1)] = o[0:DH, :]

        pending = scores(0)
        for w in range(len(waves)):
            nxt = scores(w + 1) if w + 1 < len(waves) else None
            values(w, pending)
            pending = nxt
        ffn_down_chained()

    def attention_max_shifted():
        def one_tile(item, carry):
            h = item // NQT
            j = item - h * NQT
            g = h // HPG
            hp = h - g * HPG
            cols = pl.ds(pl.multiple_of(128 * j, 128), 128)
            rid = _iota((64, 128), 0)
            mask = (rid >= (DH // 2) * hp) & (rid < (DH // 2) * (hp + 1))
            qm = jnp.where(mask, qt_v[_rows(step * NG + g, 64), cols], jnp.uint32(0))
            st = _dot(keys(g, 0, L), _unpack(qm))
            future = _iota((L, 128), 0) > 128 * j + _iota((L, 128), 1)
            st = jnp.where(future, NEG, st)
            p = jnp.exp2(st - jnp.max(st, axis=0, keepdims=True)).astype(BF16)
            keep = 1.0 - gate_v[pl.ds(h, 1), :]
            oh_v[h, :, cols] = head_output(h, NQT - 1, p, keep)
            return carry

        def compact(q, carry):
            rows = jnp.concatenate([oh_v[4 * q + k, 0:DH, :] for k in range(4)], axis=0)
            ot_v[step, pl.ds(pl.multiple_of(4 * DH * q, 8), 4 * DH), :] = rows
            return carry

        lax.fori_loop(0, H * NQT, one_tile, 0)
        lax.fori_loop(0, H // 4, compact, 0)
        ffn_down_looped()

    def routed_columns():
        ys = []
        for t in range(2):
            y = _round_bf16(jnp.sum(y_v[t], axis=1, keepdims=True))
            rsel = jnp.full((1, 1), rsel_s[t], F32)
            ys.append(_round_bf16(y * _round_bf16(jax.nn.sigmoid(rsel))))
        return ys

    def output_copy(seg, n):
        return pltpu.make_async_copy(
            out_v.at[pl.ds(seg * D, D), pl.ds(128 * n, 128)],
            o_hbm.at[:, pl.ds(seg * L + 128 * n, 128)],
            out_sems.at[NQT * seg + n])

    def output_projection(seg, ys):
        heads_out = ot_v[seg, 0:D, :]
        if seg > 0:
            heads_out = heads_out + mem_v[seg - 1, 0:D, :]
        attn = _dot(_unpack(wot[...]), heads_out.astype(BF16))
        base = x_v[seg].astype(F32) + attn
        xn = _unpack(xn_v[_rows(seg, D // 2), :]).astype(F32)
        col = seg * L + _iota((1, L), 1)
        upd = (jnp.where(col == idx_s[0], ys[0], 0.0)
               + jnp.where(col == idx_s[1], ys[1], 0.0))
        result = base + (xn + upd)
        for n in range(NQT):
            cols = slice(128 * n, 128 * (n + 1))
            out_v[seg * D:(seg + 1) * D, cols] = result[:, cols].astype(BF16)
            output_copy(seg, n).start()

    col_blocks = [(c0, min(128, D - c0)) for c0 in range(0, D, 128)]

    def transpose_block(w_v, section, c0, n):
        r0 = (section * D + c0) // 2
        wall[r0:r0 + n // 2, :] = pltpu.bitcast(w_v[:, c0:c0 + n].T, U32)

    def project_block(section, c0, n, xn):
        r0 = (section * D + c0) // 2
        last = section == 2 and c0 + n == D
        hi = PROWS // 2 if last else r0 + n // 2
        return _dot(_unpack(wall[r0:hi, :]), xn)

    def query_half0(half):
        layer_norm(0, serial=False, tiles=[2 * half, 2 * half + 1])
        xn = _unpack(xn_v[0:D // 2, 256 * half:256 * (half + 1)])
        top = _dot(_unpack(wall[0:D // 4, :]), xn)
        if half == 0:
            for c0, n in col_blocks[3:]:
                transpose_block(wq_v, 0, c0, n)
        bottom = _dot(_unpack(wall[D // 4:D // 2, :]), xn)
        return jnp.concatenate([top, bottom], axis=0)

    def projections():
        qtiles = []
        for half in range(2):
            x0_copies[half].wait()
            if half == 1:
                cp_wk.wait()
            qtiles.append(query_half0(half))
        for c0, n in col_blocks:
            transpose_block(wk_v, 1, c0, n)
        parts = [jnp.concatenate(qtiles, axis=1)]
        xn0 = _unpack(xn_v[_rows(0, D // 2), :])
        parts += [project_block(1, c0, n, xn0) for c0, n in col_blocks[:EARLY_K]]
        cp_wv.wait()
        x_copies[1].wait()
        xn0 = _unpack(xn_v[_rows(0, D // 2), :])
        parts += [project_block(1, c0, n, xn0) for c0, n in col_blocks[EARLY_K:]]
        for c0, n in col_blocks:
            transpose_block(wv_v, 2, c0, n)
            parts.append(project_block(2, c0, n, xn0))
        layer_norm(1)
        _, pk, vg = store_qkv(0, jnp.concatenate(parts, axis=0))
        x_copies[2].wait()
        x_copies[3].wait()
        cp_wo.wait()

        layer_norm(2)
        pt = project(1)
        wot[...] = pltpu.bitcast(wo_v[...].T, U32)
        state1 = memory_update(None, pk, vg)
        pq1, pk, vg = store_qkv(1, pt)
        layer_norm(3)
        pt = project(2)
        state2 = memory_update(state1, pk, vg)
        pq2, pk, vg = store_qkv(2, pt)
        cp_wg.wait()
        cp_wu.wait()
        pt = project(3, router_first=True)
        pq3, _, _ = store_qkv(3, pt)
        route()
        ffn_hidden()
        state3 = memory_update(state2, pk, vg)
        memory_retrieve(1, state1, pq1)
        memory_retrieve(2, state2, pq2)
        memory_retrieve(3, state3, pq3)
        record_logit_bound()
        cp_wd.wait()

    @pl.when(step == 0)
    def _():
        for cp in (cp_wq, cp_wr, cp_beta, *x0_copies, cp_wk, cp_wv, x_copies[1],
                   x_copies[2], x_copies[3], cp_wo, cp_wg, cp_wu, cp_wd):
            cp.start()
        with _scope("sc_startup"):
            cp_wr.wait()
            cp_beta.wait()
            cp_wq.wait()
            init_constants()
            for c0, n in col_blocks[:3]:
                transpose_block(wq_v, 0, c0, n)
        with _scope("sc_projections"):
            projections()

    @pl.when(step < NSEG)
    def _():
        safe = safe_s[0] == 1

        @pl.when(safe)
        def _():
            with _scope("sc_attention"):
                attention_bounded()

        @pl.when(jnp.logical_not(safe))
        def _():
            attention_max_shifted()

    @pl.when(step == NSEG)
    def _():
        with _scope("sc_outproj"):
            ys = routed_columns()
            for seg in range(NSEG):
                output_projection(seg, ys)
            for seg in range(NSEG):
                for n in range(NQT):
                    output_copy(seg, n).wait()


@jax.jit
def pallas_parallel_sum__memory_aug_infini_attn__moe_arch_mod__prompt_kernel(
    A_x: jax.Array,
    A_wq: jax.Array,
    A_wk: jax.Array,
    A_wv: jax.Array,
    A_wo: jax.Array,
    A_beta: jax.Array,
    B_x: jax.Array,
    B_w_r: jax.Array,
    B_w_gate: jax.Array,
    B_w_up: jax.Array,
    B_w_down: jax.Array,
):
    del B_x
    vm = pltpu.VMEM
    scratch = [
        vm((NSEG, D, L), BF16),
        vm((D, D), BF16),
        vm((D, D), BF16),
        vm((D, D), BF16),
        vm((D, D), BF16),
        vm((H,), BF16),
        vm((D,), BF16),
        vm((D, FF), BF16),
        vm((D, FF), BF16),
        vm((D, FF), BF16),
        vm((PROWS // 2, D), U32),
        vm((D // 2, D), U32),
        vm((NSEG * D // 2, L), U32),
        vm((NSEG * NG * 64, L), U32),
        vm((NSEG * NG * L // 2, 128), U32),
        vm((NSEG * H * 16, L), U32),
        vm((NSEG - 1, D, L), F32),
        vm((8, L), F32),
        vm((8, D), U32),
        vm((2, D, 128), F32),
        vm((2, FF // 128, 8, 128), F32),
        pltpu.SMEM((2,), jnp.int32),
        pltpu.SMEM((2,), F32),
        pltpu.SMEM((1,), U32),
        pltpu.SMEM((1,), jnp.int32),
        vm((H, 128), F32),
        vm((NSEG, D, L), F32),
        vm((H, 24, L), F32),
        vm((128, 128), F32),
        vm((3, 64, 128), F32),
        vm((NSEG * D, L), BF16),
        pltpu.SemaphoreType.DMA((NSEG * NQT,)),
        pltpu.SemaphoreType.DMA((NSEG + 9 + 2,)),
    ]
    hbm = pl.BlockSpec(memory_space=pltpu.HBM)
    xt = jnp.transpose(A_x.reshape(S, D))
    out_t = pl.pallas_call(
        _kernel,
        grid=(NSEG + 1,),
        in_specs=[hbm] * 10,
        out_specs=hbm,
        out_shape=jax.ShapeDtypeStruct((D, S), BF16),
        scratch_shapes=scratch,
        compiler_params=pltpu.CompilerParams(
            dimension_semantics=("arbitrary",),
            vmem_limit_bytes=110 * 1024 * 1024,
        ),
        name="infini_moe",
    )(xt, A_wq, A_wk, A_wv, A_wo, A_beta, B_w_r, B_w_gate, B_w_up,
      jnp.transpose(B_w_down))
    return jnp.transpose(out_t).reshape(1, S, D)
```

```python
import contextlib

import jax
import jax.numpy as jnp
from jax import lax
from jax.experimental import pallas as pl
from jax.experimental.pallas import tpu as pltpu

S = 2048
D = 576
H = 32
DH = 18
NSEG = 4
L = 512
FF = 4608
NG = 5
HPG = 7
GW = HPG * DH
NQT = L // 128
PROWS = 3 * D + 16
RROW = 3 * D
EARLY_K = 1
FFN_FIRST_BLOCK = 3
FFN_PATTERN = (1, 2)
PBLOCK = 128
FT = FF // 128 // NSEG
LOG2E = 1.4426950408889634
QSCALE = DH ** -0.5 * LOG2E
NEG = -1e30
LN_EPS = 1.0013580322265625e-05
F32 = jnp.float32
BF16 = jnp.bfloat16
U32 = jnp.uint32

PROFILE_SCOPES = False

_NN = (((1,), (0,)), ((), ()))
_NT = (((1,), (1,)), ((), ()))


def _scope(name):
    return jax.named_scope(name) if PROFILE_SCOPES else contextlib.nullcontext()


def _dot(a, b):
    return lax.dot_general(a, b, _NN, preferred_element_type=F32)


def _dot_nt(a, b):
    return lax.dot_general(a, b, _NT, preferred_element_type=F32)


def _iota(shape, dim):
    return lax.broadcasted_iota(jnp.int32, shape, dim)


def _round_bf16(v):
    return v.astype(BF16).astype(F32)


def _pack(v):
    return pltpu.bitcast(v.astype(BF16), U32)


def _unpack(u):
    return pltpu.bitcast(u, BF16)


def _rows(index, size):
    if isinstance(index, int):
        return slice(index * size, (index + 1) * size)
    return pl.ds(pl.multiple_of(index * size, 8), size)


def _heads_in_group(g):
    return HPG if g < NG - 1 else H - HPG * (NG - 1)


def _memory_rows(g):
    used = _heads_in_group(g) * DH
    return (128, GW) if g < NG - 1 else (used + 8, used)


def _phi(t):
    return jnp.where(t > 0, t + 1.0, jnp.exp(t))


def _kernel(x_hbm, wq_hbm, wk_hbm, wv_hbm, wo_hbm, beta_hbm, wr_hbm,
            wg_hbm, wu_hbm, wd_hbm,
            o_hbm,
            x_v, wq_v, wk_v, wv_v, wo_v, beta_v, wr_v, wg_v, wu_v, wd_v,
            wall, wot, xn_v, qt_v, k_v, vt_v, mem_v,
            r_v, xs_v, y_v, hid_v, idx_s, rsel_s, zero_s, safe_s,
            gate_v, ot_v, oh_v, bias_v, half_v, out_v, out_sems,
            sems):
    step = pl.program_id(0)

    x_copies = [None] + [
        pltpu.make_async_copy(x_hbm.at[:, pl.ds(c * L, L)], x_v.at[c], sems.at[c])
        for c in range(1, NSEG)
    ]
    x0_copies = [
        pltpu.make_async_copy(x_hbm.at[:, pl.ds(256 * n, 256)],
                              x_v.at[0, :, pl.ds(256 * n, 256)],
                              sems.at[NSEG + 9 + n])
        for n in range(2)
    ]
    pairs = [(wq_hbm, wq_v), (wk_hbm, wk_v), (wv_hbm, wv_v), (wo_hbm, wo_v),
             (beta_hbm, beta_v), (wr_hbm, wr_v),
             (wg_hbm, wg_v), (wu_hbm, wu_v), (wd_hbm, wd_v)]
    (cp_wq, cp_wk, cp_wv, cp_wo, cp_beta, cp_wr, cp_wg, cp_wu, cp_wd) = [
        pltpu.make_async_copy(src, dst, sems.at[NSEG + i])
        for i, (src, dst) in enumerate(pairs)
    ]

    def nothing(v):
        return pltpu.bitcast(pltpu.bitcast(v, U32) & zero_s[0], F32)

    def layer_norm(c, serial=True, tiles=range(NQT)):
        link = None
        for n in tiles:
            cols = slice(128 * n, 128 * (n + 1))
            pivot = x_v[c, 0:16, cols].astype(F32)[0:1, :]
            pivot8 = jnp.broadcast_to(pivot, (8, 128))
            shift = pivot8
            s1 = s2 = None
            for i in range(D // 16):
                last = s1 if s1 is not None else link
                if serial and last is not None:
                    shift = pivot8 + nothing(last)
                x16 = x_v[c, 16 * i:16 * i + 16, cols].astype(F32)
                for k in range(2):
                    d = x16[8 * k:8 * k + 8, :] - shift
                    s1 = d if s1 is None else s1 + d
                    s2 = d * d if s2 is None else s2 + d * d
            dmean = jnp.sum(s1, axis=0, keepdims=True) * (1.0 / D)
            dsq = jnp.sum(s2, axis=0, keepdims=True) * (1.0 / D)
            var = jnp.maximum(dsq - dmean * dmean, 0.0)
            sd = _round_bf16(jnp.sqrt(_round_bf16(_round_bf16(var) + LN_EPS)))
            mean8 = jnp.broadcast_to(_round_bf16(pivot + dmean), (8, 128))
            inv8 = jnp.broadcast_to(1.0 / sd, (8, 128))
            center = mean8
            for i in range(D // 32):
                if serial and i > 0:
                    center = mean8 + nothing(link)
                x32 = x_v[c, 32 * i:32 * i + 32, cols].astype(F32)
                z = [(x32[8 * k:8 * k + 8, :] - center) * inv8 for k in range(4)]
                link = z[3]
                r0 = c * (D // 2) + 16 * i
                xn_v[r0:r0 + 16, cols] = _pack(jnp.concatenate(z, axis=0))

    def init_constants():
        gate = jax.nn.sigmoid(beta_v[...].astype(F32).reshape(1, H))
        on_diag = _iota((H, H), 0) == _iota((H, H), 1)
        gcol = jnp.sum(jnp.where(on_diag, gate, 0.0), axis=1, keepdims=True)
        gate_v[...] = jnp.broadcast_to(gcol, (H, 128))
        zero_s[0] = jnp.uint32(0)
        bias_v[...] = jnp.where(_iota((128, 128), 0) > _iota((128, 128), 1), NEG, 0.0)
        key, lane = _iota((64, 128), 0), _iota((64, 128), 1)
        future = key > (lane & 63)
        half_v[0] = jnp.where(future, NEG, 0.0)
        half_v[1] = jnp.where(future | (lane < 64), NEG, 0.0)
        half_v[2] = jnp.where(future | (lane >= 64), NEG, 0.0)
        router = jnp.broadcast_to(wr_v[...].astype(F32).reshape(1, D), (16, D))
        wall[RROW // 2:PROWS // 2, :] = _pack(
            jnp.where(_iota((16, D), 0) == 0, router, 0.0))

    def project(c):
        xn = _unpack(xn_v[_rows(c, D // 2), :])
        step_rows = PBLOCK // 2
        return jnp.concatenate(
            [_dot(_unpack(wall[r:min(r + step_rows, PROWS // 2), :]), xn)
             for r in range(0, PROWS // 2, step_rows)], axis=0)

    seen = [None]

    def record_logit_bound():
        big = (seen[0] >> 30) & 1
        safe_s[0] = (jnp.max(big.astype(jnp.int32)) == 0).astype(jnp.int32)

    def store_qkv(c, pt):
        if c < NSEG - 1:
            r_v[c:c + 1, :] = _round_bf16(pt[RROW:RROW + 1, :])
        tail_row = _iota((8, L), 0)
        for h in range(H):
            base = 2 * D + DH * h
            tail = jnp.where(tail_row < DH - 16, pt[base + 16:base + 24, :],
                             jnp.where(tail_row == DH - 16, 1.0, 0.0))
            blk = jnp.concatenate(
                [pt[base:base + 16, :], tail, jnp.zeros((8, L), F32)], axis=0)
            vt_v[_rows(c * H + h, 16), :] = _pack(blk)

        pqs, pks, vgs = [], [], []
        for g in range(NG):
            used = _heads_in_group(g) * DH
            qg = pt[GW * g:GW * g + 128, :]
            qs = qg * QSCALE
            qt_v[_rows(c * NG + g, 64), :] = _pack(qs)
            kg = pt[D + GW * g:D + GW * g + 128, :]
            for operand in (qs, kg):
                bits = pltpu.bitcast(operand, U32)
                for blk in range(0, 128 if g < NG - 1 else used, 8):
                    for col in range(0, L, 128):
                        piece = bits[blk:blk + 8, col:col + 128]
                        seen[0] = piece if seen[0] is None else seen[0] | piece
            k_v[_rows(c * NG + g, L // 2), :] = _pack(kg.T)
            pqs.append(_phi(qg).astype(BF16))
            if c < NSEG - 1:
                pks.append(_phi(kg).astype(BF16))
                lo = 2 * D + GW * g
                rows, zrow = _memory_rows(g)
                rid = _iota((rows, L), 0)
                vg = jnp.where(rid < used, pt[lo:lo + rows, :],
                               jnp.where(rid == zrow, 1.0, 0.0))
                vgs.append(vg.astype(BF16))
        return pqs, pks, vgs

    def memory_update(states, pks, vgs):
        out = []
        for g in range(NG):
            used = _heads_in_group(g) * DH
            rows, zrow = _memory_rows(g)
            row = _iota((rows, 128), 0)
            lane = _iota((rows, 128), 1)
            same_head = (row // DH) == (lane // DH)
            upd = _dot_nt(vgs[g], pks[g])
            keep = ((same_head & (row < used)) | (row == zrow)) & (lane < used)
            upd = jnp.where(keep, upd, 0.0)
            out.append(upd if states is None else states[g] + upd)
        return out

    def memory_retrieve(c, states, pqs):
        row8 = _iota((8, 128), 0)
        lane8 = _iota((8, 128), 1) // DH
        for g in range(NG):
            nh = _heads_in_group(g)
            rows, zrow = _memory_rows(g)
            st = states[g]
            mrows = jnp.where(_iota((rows, 128), 0) < zrow, st, 0.0)
            zrows = jnp.where(lane8 == row8, st[zrow:zrow + 1, :], 0.0)
            lhs = jnp.concatenate(
                [mrows, zrows, jnp.zeros((8, 128), F32)], axis=0).astype(BF16)
            ret = _dot(lhs, pqs[g])
            gsel = gate_v[HPG * g:HPG * g + 8, :] if g < NG - 1 else jnp.concatenate(
                [gate_v[HPG * g:H, :], jnp.zeros((8 - nh, 128), F32)], axis=0)
            gwide = jnp.concatenate([gsel] * NQT, axis=1)
            scale = gwide / (ret[rows:rows + 8, :] + 1e-6)
            out_rows = 128 if g < NG - 1 else nh * DH
            pieces = []
            for b in range(out_rows // 8):
                h0 = min((8 * b) // DH, nh - 1)
                h1 = min((8 * b + 7) // DH, nh - 1)
                sc = scale[h0:h0 + 1, :]
                if h1 != h0:
                    first = _iota((8, L), 0) < DH * h1 - 8 * b
                    sc = jnp.where(first, sc, scale[h1:h1 + 1, :])
                pieces.append(ret[8 * b:8 * b + 8, :] * sc)
            mem_v[c - 1, GW * g:GW * g + out_rows, :] = jnp.concatenate(pieces, axis=0)

    def route():
        r = r_v[0:NSEG, :]
        idx = _iota((NSEG, L), 0) * L + _iota((NSEG, L), 1)
        m1 = jnp.max(r)
        i1 = jnp.clip(jnp.min(jnp.where(r == m1, idx, S)), 0, S - 1)
        r2 = jnp.where(idx == i1, -jnp.inf, r)
        m2 = jnp.max(r2)
        i2 = jnp.clip(jnp.min(jnp.where(r2 == m2, idx, S)), 0, S - 1)
        idx_s[0] = i1
        idx_s[1] = i2
        rsel_s[0] = m1
        rsel_s[1] = m2
        row16 = _iota((16, 128), 0)
        lane16 = _iota((16, 128), 1)
        xs = None
        for t, i in enumerate((i1, i2)):
            seg = i // L
            off = i - seg * L
            base = pl.multiple_of((off // 128) * 128, 128)
            cols = _unpack(xn_v[_rows(seg, D // 2), pl.ds(base, 128)])
            pick = jnp.where((row16 == t) & (lane16 == off - base), 1.0, 0.0)
            part = _dot_nt(pick.astype(BF16), cols)
            xs = part if xs is None else xs + part
        xs_v[...] = _pack(xs)
        y_v[...] = jnp.zeros(y_v.shape, F32)

    def ffn_in_tile(w_ref, tile):
        return _dot(_unpack(xs_v[...]), w_ref[:, 128 * tile:128 * (tile + 1)])

    def store_ffn_hidden(gates, ups):
        for tile, (gt, up) in enumerate(zip(gates, ups)):
            gt = _round_bf16(gt)
            hid = _round_bf16(_round_bf16(gt * jax.nn.sigmoid(gt)) * _round_bf16(up))
            for t in range(2):
                hid_v[t, tile] = jnp.broadcast_to(hid[t:t + 1, :], (8, 128))

    def project_last_with_ffn():
        c = NSEG - 1
        xn = _unpack(xn_v[_rows(c, D // 2), :])
        router = _dot(_unpack(wall[RROW // 2:PROWS // 2, :]), xn)
        r_v[c:c + 1, :] = _round_bf16(router[0:1, :])
        todo = [(w_ref, tile) for w_ref in (wg_v, wu_v) for tile in range(FF // 128)]
        done = []
        blocks = []
        for i, r in enumerate(range(0, RROW // 2, PBLOCK // 2)):
            if i == FFN_FIRST_BLOCK:
                route()
            lhs = _unpack(wall[r:min(r + PBLOCK // 2, RROW // 2), :])
            tiles = []
            for n in range(NQT):
                tiles.append(_dot(lhs, xn[:, 128 * n:128 * (n + 1)]))
                if i >= FFN_FIRST_BLOCK:
                    for _ in range(min(FFN_PATTERN[n % len(FFN_PATTERN)], len(todo))):
                        done.append(ffn_in_tile(*todo.pop(0)))
            blocks.append(jnp.concatenate(tiles, axis=1))
        pt = jnp.concatenate(blocks + [router], axis=0)
        return pt, todo, done

    def ffn_down_chained():
        base = pl.multiple_of(step * (FT * 128), 128)
        link = [None, None]
        for b in range(D // 8):
            acc = [None, None]
            for tile in range(FT):
                w = wd_v[8 * b:8 * b + 8, pl.ds(base + 128 * tile, 128)].astype(F32)
                for t in range(2):
                    pr = w * hid_v[t, step * FT + tile]
                    if tile > 0:
                        acc[t] = acc[t] + pr
                    else:
                        acc[t] = pr if link[t] is None else pr + nothing(link[t])
            for t in range(2):
                rows = slice(8 * b, 8 * b + 8)
                y_v[t, rows, :] = y_v[t, rows, :] + acc[t]
                link[t] = acc[t]

    def ffn_down_looped():
        def down(tile, carry):
            col = step * FT + tile
            w = wd_v[:, pl.ds(pl.multiple_of(128 * col, 128), 128)].astype(F32)
            for t in range(2):
                y_v[t] = y_v[t] + w * hid_v[t, col][0:1, :]
            return carry

        lax.fori_loop(0, FT, down, 0)

    def masked_q_bits(g, hp, j):
        rid = _iota((64, 128), 0)
        mask = (rid >= (DH // 2) * hp) & (rid < (DH // 2) * (hp + 1))
        return jnp.where(mask, qt_v[_rows(step * NG + g, 64), 128 * j:128 * (j + 1)],
                         jnp.uint32(0))

    def keys(g, lo, hi):
        first = pl.multiple_of((step * NG + g) * (L // 2) + lo // 2, 8)
        return _unpack(k_v[pl.ds(first, (hi - lo) // 2), :])

    def causal_scores(g, hp, j):
        nk = 128 * (j + 1)
        st = _dot(keys(g, 0, nk), _unpack(masked_q_bits(g, hp, j)))
        diag = st[nk - 128:, :] + bias_v[...]
        return diag if j == 0 else jnp.concatenate([st[:nk - 128, :], diag], axis=0)

    def head_output(h, j, p, keep):
        o = _dot(_unpack(vt_v[_rows(step * H + h, 16), 0:128 * (j + 1)]), p)
        den = o[DH:DH + 1, :]
        inv = pl.reciprocal(den, approx=True)
        inv = inv * (2.0 - den * inv)
        return o[0:24, :] * (keep * inv)

    def single_probs(h, j):
        return jnp.exp2(causal_scores(*divmod(h, HPG), j)).astype(BF16)

    def pair_probs(pairs, j, flip):
        low = _iota((64, 128), 1) < 64
        qa, qb = {}, {}
        for h in pairs:
            g, hp = divmod(h, HPG)
            qa[h] = masked_q_bits(g, hp, j)
            qb[h] = pltpu.roll(masked_q_bits(g, hp + 1, j), 64, 1)
        off = {}
        if j > 0:
            for h in pairs:
                g = h // HPG
                for hh, q in ((h, qa[h]), (h + 1, qb[h])):
                    off[hh] = jnp.exp2(_dot(keys(g, 0, 128 * j), _unpack(q)))
        early, late = {}, {}
        for h in pairs:
            g = h // HPG
            k0 = 128 * j
            for which in ((0, 1) if flip else (1, 0)):
                if which == 0:
                    early[h] = _dot(keys(g, k0, k0 + 64),
                                    _unpack(jnp.where(low, qa[h], qb[h])))
                else:
                    late[h] = _dot(keys(g, k0, k0 + 128),
                                   _unpack(jnp.where(low, qb[h], qa[h])))
        probs = {}
        for h in pairs:
            p1 = jnp.exp2(early[h] + half_v[0])
            p2 = jnp.exp2(late[h][0:64, :])
            bottom = late[h][64:128, :]
            pa = jnp.concatenate(
                [jnp.where(low, p1, p2), jnp.exp2(bottom + half_v[1])], axis=0)
            pb = jnp.concatenate(
                [jnp.where(low, p2, p1), jnp.exp2(bottom + half_v[2])], axis=0)
            for hh, pd in ((h, pa), (h + 1, pb)):
                full = pd if j == 0 else jnp.concatenate([off[hh], pd], axis=0)
                probs[hh] = full.astype(BF16)
        return probs

    def attention_bounded():
        pairs = [g * HPG + hp for g in range(NG)
                 for hp in range(0, _heads_in_group(g) - 1, 2)]
        paired = set(pairs) | {h + 1 for h in pairs}
        singles = [h for h in range(H) if h not in paired]
        waves = [(pairs[i:i + 2], j) for i in range(0, len(pairs), 2) for j in range(NQT)]
        waves += [(None, j) for j in range(NQT)]

        def scores(w):
            grp, j = waves[w]
            if grp is None:
                return {h: single_probs(h, j) for h in singles}
            return pair_probs(grp, j, w % 2 == 1)

        def values(w, probs):
            grp, j = waves[w]
            for h, p in probs.items():
                o = head_output(h, j, p, 1.0 - gate_v[h:h + 1, :])
                if grp is not None and h - 1 in grp:
                    o = pltpu.roll(o, 64, 1)
                ot_v[step, DH * h:DH * (h + 1), 128 * j:128 * (j + 1)] = o[0:DH, :]

        pending = scores(0)
        for w in range(len(waves)):
            nxt = scores(w + 1) if w + 1 < len(waves) else None
            values(w, pending)
            pending = nxt
        ffn_down_chained()

    def attention_max_shifted():
        def one_tile(item, carry):
            h = item // NQT
            j = item - h * NQT
            g = h // HPG
            hp = h - g * HPG
            cols = pl.ds(pl.multiple_of(128 * j, 128), 128)
            rid = _iota((64, 128), 0)
            mask = (rid >= (DH // 2) * hp) & (rid < (DH // 2) * (hp + 1))
            qm = jnp.where(mask, qt_v[_rows(step * NG + g, 64), cols], jnp.uint32(0))
            st = _dot(keys(g, 0, L), _unpack(qm))
            future = _iota((L, 128), 0) > 128 * j + _iota((L, 128), 1)
            st = jnp.where(future, NEG, st)
            p = jnp.exp2(st - jnp.max(st, axis=0, keepdims=True)).astype(BF16)
            keep = 1.0 - gate_v[pl.ds(h, 1), :]
            oh_v[h, :, cols] = head_output(h, NQT - 1, p, keep)
            return carry

        def compact(q, carry):
            rows = jnp.concatenate([oh_v[4 * q + k, 0:DH, :] for k in range(4)], axis=0)
            ot_v[step, pl.ds(pl.multiple_of(4 * DH * q, 8), 4 * DH), :] = rows
            return carry

        lax.fori_loop(0, H * NQT, one_tile, 0)
        lax.fori_loop(0, H // 4, compact, 0)
        ffn_down_looped()

    def routed_columns():
        ys = []
        for t in range(2):
            y = _round_bf16(jnp.sum(y_v[t], axis=1, keepdims=True))
            rsel = jnp.full((1, 1), rsel_s[t], F32)
            ys.append(_round_bf16(y * _round_bf16(jax.nn.sigmoid(rsel))))
        return ys

    def output_copy(seg, n):
        return pltpu.make_async_copy(
            out_v.at[pl.ds(seg * D, D), pl.ds(128 * n, 128)],
            o_hbm.at[:, pl.ds(seg * L + 128 * n, 128)],
            out_sems.at[NQT * seg + n])

    def output_projection(seg, ys):
        heads_out = ot_v[seg, 0:D, :]
        if seg > 0:
            heads_out = heads_out + mem_v[seg - 1, 0:D, :]
        attn = _dot(_unpack(wot[...]), heads_out.astype(BF16))
        base = x_v[seg].astype(F32) + attn
        xn = _unpack(xn_v[_rows(seg, D // 2), :]).astype(F32)
        col = seg * L + _iota((1, L), 1)
        upd = (jnp.where(col == idx_s[0], ys[0], 0.0)
               + jnp.where(col == idx_s[1], ys[1], 0.0))
        result = base + (xn + upd)
        for n in range(NQT):
            cols = slice(128 * n, 128 * (n + 1))
            out_v[seg * D:(seg + 1) * D, cols] = result[:, cols].astype(BF16)
            output_copy(seg, n).start()

    col_blocks = [(c0, min(128, D - c0)) for c0 in range(0, D, 128)]

    def transpose_block(w_v, section, c0, n):
        r0 = (section * D + c0) // 2
        wall[r0:r0 + n // 2, :] = pltpu.bitcast(w_v[:, c0:c0 + n].T, U32)

    def project_block(section, c0, n, xn):
        r0 = (section * D + c0) // 2
        last = section == 2 and c0 + n == D
        hi = PROWS // 2 if last else r0 + n // 2
        return _dot(_unpack(wall[r0:hi, :]), xn)

    def query_half0(half):
        layer_norm(0, serial=False, tiles=[2 * half, 2 * half + 1])
        xn = _unpack(xn_v[0:D // 2, 256 * half:256 * (half + 1)])
        top = _dot(_unpack(wall[0:D // 4, :]), xn)
        if half == 0:
            for c0, n in col_blocks[3:]:
                transpose_block(wq_v, 0, c0, n)
        bottom = _dot(_unpack(wall[D // 4:D // 2, :]), xn)
        return jnp.concatenate([top, bottom], axis=0)

    def projections():
        qtiles = []
        for half in range(2):
            x0_copies[half].wait()
            if half == 1:
                cp_wk.wait()
            qtiles.append(query_half0(half))
        for c0, n in col_blocks:
            transpose_block(wk_v, 1, c0, n)
        parts = [jnp.concatenate(qtiles, axis=1)]
        xn0 = _unpack(xn_v[_rows(0, D // 2), :])
        parts += [project_block(1, c0, n, xn0) for c0, n in col_blocks[:EARLY_K]]
        cp_wv.wait()
        x_copies[1].wait()
        xn0 = _unpack(xn_v[_rows(0, D // 2), :])
        parts += [project_block(1, c0, n, xn0) for c0, n in col_blocks[EARLY_K:]]
        for c0, n in col_blocks:
            transpose_block(wv_v, 2, c0, n)
            parts.append(project_block(2, c0, n, xn0))
        layer_norm(1)
        _, pk, vg = store_qkv(0, jnp.concatenate(parts, axis=0))
        x_copies[2].wait()
        x_copies[3].wait()
        cp_wo.wait()

        layer_norm(2)
        pt = project(1)
        wot[...] = pltpu.bitcast(wo_v[...].T, U32)
        state1 = memory_update(None, pk, vg)
        pq1, pk, vg = store_qkv(1, pt)
        layer_norm(3)
        pt = project(2)
        state2 = memory_update(state1, pk, vg)
        pq2, pk, vg = store_qkv(2, pt)
        cp_wg.wait()
        cp_wu.wait()
        pt, todo, done = project_last_with_ffn()
        pq3, _, _ = store_qkv(3, pt)
        state3 = memory_update(state2, pk, vg)
        done += [ffn_in_tile(*item) for item in todo]
        store_ffn_hidden(done[:FF // 128], done[FF // 128:])
        memory_retrieve(1, state1, pq1)
        memory_retrieve(2, state2, pq2)
        memory_retrieve(3, state3, pq3)
        record_logit_bound()
        cp_wd.wait()

    @pl.when(step == 0)
    def _():
        for cp in (cp_wq, cp_wr, cp_beta, *x0_copies, cp_wk, cp_wv, x_copies[1],
                   x_copies[2], x_copies[3], cp_wo, cp_wg, cp_wu, cp_wd):
            cp.start()
        with _scope("sc_startup"):
            cp_wr.wait()
            cp_beta.wait()
            cp_wq.wait()
            init_constants()
            for c0, n in col_blocks[:3]:
                transpose_block(wq_v, 0, c0, n)
        with _scope("sc_projections"):
            projections()

    @pl.when(step < NSEG)
    def _():
        safe = safe_s[0] == 1

        @pl.when(safe)
        def _():
            with _scope("sc_attention"):
                attention_bounded()

        @pl.when(jnp.logical_not(safe))
        def _():
            attention_max_shifted()

    @pl.when(step == NSEG)
    def _():
        with _scope("sc_outproj"):
            ys = routed_columns()
            for seg in range(NSEG):
                output_projection(seg, ys)
            for seg in range(NSEG):
                for n in range(NQT):
                    output_copy(seg, n).wait()


@jax.jit
def pallas_parallel_sum__memory_aug_infini_attn__moe_arch_mod__prompt_kernel(
    A_x: jax.Array,
    A_wq: jax.Array,
    A_wk: jax.Array,
    A_wv: jax.Array,
    A_wo: jax.Array,
    A_beta: jax.Array,
    B_x: jax.Array,
    B_w_r: jax.Array,
    B_w_gate: jax.Array,
    B_w_up: jax.Array,
    B_w_down: jax.Array,
):
    del B_x
    vm = pltpu.VMEM
    scratch = [
        vm((NSEG, D, L), BF16),
        vm((D, D), BF16),
        vm((D, D), BF16),
        vm((D, D), BF16),
        vm((D, D), BF16),
        vm((H,), BF16),
        vm((D,), BF16),
        vm((D, FF), BF16),
        vm((D, FF), BF16),
        vm((D, FF), BF16),
        vm((PROWS // 2, D), U32),
        vm((D // 2, D), U32),
        vm((NSEG * D // 2, L), U32),
        vm((NSEG * NG * 64, L), U32),
        vm((NSEG * NG * L // 2, 128), U32),
        vm((NSEG * H * 16, L), U32),
        vm((NSEG - 1, D, L), F32),
        vm((8, L), F32),
        vm((8, D), U32),
        vm((2, D, 128), F32),
        vm((2, FF // 128, 8, 128), F32),
        pltpu.SMEM((2,), jnp.int32),
        pltpu.SMEM((2,), F32),
        pltpu.SMEM((1,), U32),
        pltpu.SMEM((1,), jnp.int32),
        vm((H, 128), F32),
        vm((NSEG, D, L), F32),
        vm((H, 24, L), F32),
        vm((128, 128), F32),
        vm((3, 64, 128), F32),
        vm((NSEG * D, L), BF16),
        pltpu.SemaphoreType.DMA((NSEG * NQT,)),
        pltpu.SemaphoreType.DMA((NSEG + 9 + 2,)),
    ]
    hbm = pl.BlockSpec(memory_space=pltpu.HBM)
    xt = jnp.transpose(A_x.reshape(S, D))
    out_t = pl.pallas_call(
        _kernel,
        grid=(NSEG + 1,),
        in_specs=[hbm] * 10,
        out_specs=hbm,
        out_shape=jax.ShapeDtypeStruct((D, S), BF16),
        scratch_shapes=scratch,
        compiler_params=pltpu.CompilerParams(
            dimension_semantics=("arbitrary",),
            vmem_limit_bytes=110 * 1024 * 1024,
        ),
        name="infini_moe",
    )(xt, A_wq, A_wk, A_wv, A_wo, A_beta, B_w_r, B_w_gate, B_w_up,
      jnp.transpose(B_w_down))
    return jnp.transpose(out_t).reshape(1, S, D)
```

```python
import contextlib

import jax
import jax.numpy as jnp
from jax import lax
from jax.experimental import pallas as pl
from jax.experimental.pallas import tpu as pltpu

S = 2048
D = 576
H = 32
DH = 18
NSEG = 4
L = 512
FF = 4608
NG = 5
HPG = 7
GW = HPG * DH
NQT = L // 128
PROWS = 3 * D + 16
RROW = 3 * D
EARLY_K = 1
FFN_FIRST_BLOCK = 3
FFN_PATTERN = (1, 2)
PBLOCK = 128
FT = FF // 128 // NSEG
LOG2E = 1.4426950408889634
QSCALE = DH ** -0.5 * LOG2E
NEG = -1e30
LN_EPS = 1.0013580322265625e-05
F32 = jnp.float32
BF16 = jnp.bfloat16
U32 = jnp.uint32

PROFILE_SCOPES = False

_NN = (((1,), (0,)), ((), ()))
_NT = (((1,), (1,)), ((), ()))


def _scope(name):
    return jax.named_scope(name) if PROFILE_SCOPES else contextlib.nullcontext()


def _dot(a, b):
    return lax.dot_general(a, b, _NN, preferred_element_type=F32)


def _dot_nt(a, b):
    return lax.dot_general(a, b, _NT, preferred_element_type=F32)


def _iota(shape, dim):
    return lax.broadcasted_iota(jnp.int32, shape, dim)


def _round_bf16(v):
    return v.astype(BF16).astype(F32)


def _pack(v):
    return pltpu.bitcast(v.astype(BF16), U32)


def _unpack(u):
    return pltpu.bitcast(u, BF16)


def _rows(index, size):
    if isinstance(index, int):
        return slice(index * size, (index + 1) * size)
    return pl.ds(pl.multiple_of(index * size, 8), size)


def _heads_in_group(g):
    return HPG if g < NG - 1 else H - HPG * (NG - 1)


def _memory_rows(g):
    used = _heads_in_group(g) * DH
    return (128, GW) if g < NG - 1 else (used + 8, used)


def _phi(t):
    return jnp.where(t > 0, t + 1.0, jnp.exp(t))


def _kernel(x_hbm, wq_hbm, wk_hbm, wv_hbm, wo_hbm, beta_hbm, wr_hbm,
            wg_hbm, wu_hbm, wd_hbm,
            o_hbm,
            x_v, wq_v, wk_v, wv_v, wo_v, beta_v, wr_v, wg_v, wu_v, wd_v,
            wall, wot, xn_v, qt_v, k_v, vt_v, mem_v, mscale_v,
            r_v, xs_v, y_v, hid_v, idx_s, rsel_s, zero_s, safe_s,
            gate_v, ot_v, oh_v, bias_v, half_v, out_v, out_sems,
            sems):
    step = pl.program_id(0)

    x_copies = [None] + [
        pltpu.make_async_copy(x_hbm.at[:, pl.ds(c * L, L)], x_v.at[c], sems.at[c])
        for c in range(1, NSEG)
    ]
    x0_copies = [
        pltpu.make_async_copy(x_hbm.at[:, pl.ds(256 * n, 256)],
                              x_v.at[0, :, pl.ds(256 * n, 256)],
                              sems.at[NSEG + 9 + n])
        for n in range(2)
    ]
    pairs = [(wq_hbm, wq_v), (wk_hbm, wk_v), (wv_hbm, wv_v), (wo_hbm, wo_v),
             (beta_hbm, beta_v), (wr_hbm, wr_v),
             (wg_hbm, wg_v), (wu_hbm, wu_v), (wd_hbm, wd_v)]
    (cp_wq, cp_wk, cp_wv, cp_wo, cp_beta, cp_wr, cp_wg, cp_wu, cp_wd) = [
        pltpu.make_async_copy(src, dst, sems.at[NSEG + i])
        for i, (src, dst) in enumerate(pairs)
    ]

    def nothing(v):
        return pltpu.bitcast(pltpu.bitcast(v, U32) & zero_s[0], F32)

    def layer_norm(c, serial=True, tiles=range(NQT)):
        link = None
        for n in tiles:
            cols = slice(128 * n, 128 * (n + 1))
            pivot = x_v[c, 0:16, cols].astype(F32)[0:1, :]
            pivot8 = jnp.broadcast_to(pivot, (8, 128))
            shift = pivot8
            s1 = s2 = None
            for i in range(D // 16):
                last = s1 if s1 is not None else link
                if serial and last is not None:
                    shift = pivot8 + nothing(last)
                x16 = x_v[c, 16 * i:16 * i + 16, cols].astype(F32)
                for k in range(2):
                    d = x16[8 * k:8 * k + 8, :] - shift
                    s1 = d if s1 is None else s1 + d
                    s2 = d * d if s2 is None else s2 + d * d
            dmean = jnp.sum(s1, axis=0, keepdims=True) * (1.0 / D)
            dsq = jnp.sum(s2, axis=0, keepdims=True) * (1.0 / D)
            var = jnp.maximum(dsq - dmean * dmean, 0.0)
            sd = _round_bf16(jnp.sqrt(_round_bf16(_round_bf16(var) + LN_EPS)))
            mean8 = jnp.broadcast_to(_round_bf16(pivot + dmean), (8, 128))
            inv8 = jnp.broadcast_to(1.0 / sd, (8, 128))
            center = mean8
            for i in range(D // 32):
                if serial and i > 0:
                    center = mean8 + nothing(link)
                x32 = x_v[c, 32 * i:32 * i + 32, cols].astype(F32)
                z = [(x32[8 * k:8 * k + 8, :] - center) * inv8 for k in range(4)]
                link = z[3]
                r0 = c * (D // 2) + 16 * i
                xn_v[r0:r0 + 16, cols] = _pack(jnp.concatenate(z, axis=0))

    def init_constants():
        gate = jax.nn.sigmoid(beta_v[...].astype(F32).reshape(1, H))
        on_diag = _iota((H, H), 0) == _iota((H, H), 1)
        gcol = jnp.sum(jnp.where(on_diag, gate, 0.0), axis=1, keepdims=True)
        gate_v[...] = jnp.broadcast_to(gcol, (H, 128))
        zero_s[0] = jnp.uint32(0)
        bias_v[...] = jnp.where(_iota((128, 128), 0) > _iota((128, 128), 1), NEG, 0.0)
        key, lane = _iota((64, 128), 0), _iota((64, 128), 1)
        future = key > (lane & 63)
        half_v[0] = jnp.where(future, NEG, 0.0)
        half_v[1] = jnp.where(future | (lane < 64), NEG, 0.0)
        half_v[2] = jnp.where(future | (lane >= 64), NEG, 0.0)
        router = jnp.broadcast_to(wr_v[...].astype(F32).reshape(1, D), (16, D))
        wall[RROW // 2:PROWS // 2, :] = _pack(
            jnp.where(_iota((16, D), 0) == 0, router, 0.0))

    def project(c):
        xn = _unpack(xn_v[_rows(c, D // 2), :])
        step_rows = PBLOCK // 2
        return jnp.concatenate(
            [_dot(_unpack(wall[r:min(r + step_rows, PROWS // 2), :]), xn)
             for r in range(0, PROWS // 2, step_rows)], axis=0)

    seen = [None]

    def record_logit_bound():
        big = (seen[0] >> 30) & 1
        safe_s[0] = (jnp.max(big.astype(jnp.int32)) == 0).astype(jnp.int32)

    def store_qkv(c, pt):
        if c < NSEG - 1:
            r_v[c:c + 1, :] = _round_bf16(pt[RROW:RROW + 1, :])
        tail_row = _iota((8, L), 0)
        for h in range(H):
            base = 2 * D + DH * h
            tail = jnp.where(tail_row < DH - 16, pt[base + 16:base + 24, :],
                             jnp.where(tail_row == DH - 16, 1.0, 0.0))
            blk = jnp.concatenate(
                [pt[base:base + 16, :], tail, jnp.zeros((8, L), F32)], axis=0)
            vt_v[_rows(c * H + h, 16), :] = _pack(blk)

        pqs, pks, vgs = [], [], []
        for g in range(NG):
            used = _heads_in_group(g) * DH
            qg = pt[GW * g:GW * g + 128, :]
            qs = qg * QSCALE
            qt_v[_rows(c * NG + g, 64), :] = _pack(qs)
            kg = pt[D + GW * g:D + GW * g + 128, :]
            for operand in (qs, kg):
                bits = pltpu.bitcast(operand, U32)
                for blk in range(0, 128 if g < NG - 1 else used, 8):
                    for col in range(0, L, 128):
                        piece = bits[blk:blk + 8, col:col + 128]
                        seen[0] = piece if seen[0] is None else seen[0] | piece
            k_v[_rows(c * NG + g, L // 2), :] = _pack(kg.T)
            pqs.append(_phi(qg).astype(BF16))
            if c < NSEG - 1:
                pks.append(_phi(kg).astype(BF16))
                lo = 2 * D + GW * g
                rows, zrow = _memory_rows(g)
                rid = _iota((rows, L), 0)
                vg = jnp.where(rid < used, pt[lo:lo + rows, :],
                               jnp.where(rid == zrow, 1.0, 0.0))
                vgs.append(vg.astype(BF16))
        return pqs, pks, vgs

    def memory_update(states, pks, vgs):
        out = []
        for g in range(NG):
            used = _heads_in_group(g) * DH
            rows, zrow = _memory_rows(g)
            row = _iota((rows, 128), 0)
            lane = _iota((rows, 128), 1)
            same_head = (row // DH) == (lane // DH)
            upd = _dot_nt(vgs[g], pks[g])
            keep = ((same_head & (row < used)) | (row == zrow)) & (lane < used)
            upd = jnp.where(keep, upd, 0.0)
            out.append(upd if states is None else states[g] + upd)
        return out

    def memory_retrieve(c, states, pqs):
        row8 = _iota((8, 128), 0)
        lane8 = _iota((8, 128), 1) // DH
        for g in range(NG):
            nh = _heads_in_group(g)
            rows, zrow = _memory_rows(g)
            st = states[g]
            mrows = jnp.where(_iota((rows, 128), 0) < zrow, st, 0.0)
            zrows = jnp.where(lane8 == row8, st[zrow:zrow + 1, :], 0.0)
            lhs = jnp.concatenate(
                [mrows, zrows, jnp.zeros((8, 128), F32)], axis=0).astype(BF16)
            ret = _dot(lhs, pqs[g])
            gsel = gate_v[HPG * g:HPG * g + 8, :] if g < NG - 1 else jnp.concatenate(
                [gate_v[HPG * g:H, :], jnp.zeros((8 - nh, 128), F32)], axis=0)
            gwide = jnp.concatenate([gsel] * NQT, axis=1)
            scale = gwide / (ret[rows:rows + 8, :] + 1e-6)
            out_rows = 128 if g < NG - 1 else nh * DH
            mem_v[c - 1, GW * g:GW * g + out_rows, :] = ret[0:out_rows, :]
            mscale_v[c - 1, HPG * g:HPG * g + 8, :] = scale

    def route():
        r = r_v[0:NSEG, :]
        idx = _iota((NSEG, L), 0) * L + _iota((NSEG, L), 1)
        m1 = jnp.max(r)
        i1 = jnp.clip(jnp.min(jnp.where(r == m1, idx, S)), 0, S - 1)
        r2 = jnp.where(idx == i1, -jnp.inf, r)
        m2 = jnp.max(r2)
        i2 = jnp.clip(jnp.min(jnp.where(r2 == m2, idx, S)), 0, S - 1)
        idx_s[0] = i1
        idx_s[1] = i2
        rsel_s[0] = m1
        rsel_s[1] = m2
        row16 = _iota((16, 128), 0)
        lane16 = _iota((16, 128), 1)
        xs = None
        for t, i in enumerate((i1, i2)):
            seg = i // L
            off = i - seg * L
            base = pl.multiple_of((off // 128) * 128, 128)
            cols = _unpack(xn_v[_rows(seg, D // 2), pl.ds(base, 128)])
            pick = jnp.where((row16 == t) & (lane16 == off - base), 1.0, 0.0)
            part = _dot_nt(pick.astype(BF16), cols)
            xs = part if xs is None else xs + part
        xs_v[...] = _pack(xs)
        y_v[...] = jnp.zeros(y_v.shape, F32)

    def ffn_in_tile(w_ref, tile):
        return _dot(_unpack(xs_v[...]), w_ref[:, 128 * tile:128 * (tile + 1)])

    def store_ffn_hidden(gates, ups):
        for tile, (gt, up) in enumerate(zip(gates, ups)):
            gt = _round_bf16(gt)
            hid = _round_bf16(_round_bf16(gt * jax.nn.sigmoid(gt)) * _round_bf16(up))
            for t in range(2):
                hid_v[t, tile] = jnp.broadcast_to(hid[t:t + 1, :], (8, 128))

    def project_last_with_ffn():
        c = NSEG - 1
        xn = _unpack(xn_v[_rows(c, D // 2), :])
        router = _dot(_unpack(wall[RROW // 2:PROWS // 2, :]), xn)
        r_v[c:c + 1, :] = _round_bf16(router[0:1, :])
        todo = [(w_ref, tile) for w_ref in (wg_v, wu_v) for tile in range(FF // 128)]
        done = []
        blocks = []
        for i, r in enumerate(range(0, RROW // 2, PBLOCK // 2)):
            if i == FFN_FIRST_BLOCK:
                route()
            lhs = _unpack(wall[r:min(r + PBLOCK // 2, RROW // 2), :])
            tiles = []
            for n in range(NQT):
                tiles.append(_dot(lhs, xn[:, 128 * n:128 * (n + 1)]))
                if i >= FFN_FIRST_BLOCK:
                    for _ in range(min(FFN_PATTERN[n % len(FFN_PATTERN)], len(todo))):
                        done.append(ffn_in_tile(*todo.pop(0)))
            blocks.append(jnp.concatenate(tiles, axis=1))
        pt = jnp.concatenate(blocks + [router], axis=0)
        return pt, todo, done

    def ffn_down_chained():
        base = pl.multiple_of(step * (FT * 128), 128)
        link = [None, None]
        for b in range(D // 8):
            acc = [None, None]
            for tile in range(FT):
                w = wd_v[8 * b:8 * b + 8, pl.ds(base + 128 * tile, 128)].astype(F32)
                for t in range(2):
                    pr = w * hid_v[t, step * FT + tile]
                    if tile > 0:
                        acc[t] = acc[t] + pr
                    else:
                        acc[t] = pr if link[t] is None else pr + nothing(link[t])
            for t in range(2):
                rows = slice(8 * b, 8 * b + 8)
                y_v[t, rows, :] = y_v[t, rows, :] + acc[t]
                link[t] = acc[t]

    def ffn_down_looped():
        def down(tile, carry):
            col = step * FT + tile
            w = wd_v[:, pl.ds(pl.multiple_of(128 * col, 128), 128)].astype(F32)
            for t in range(2):
                y_v[t] = y_v[t] + w * hid_v[t, col][0:1, :]
            return carry

        lax.fori_loop(0, FT, down, 0)

    def masked_q_bits(g, hp, j):
        rid = _iota((64, 128), 0)
        mask = (rid >= (DH // 2) * hp) & (rid < (DH // 2) * (hp + 1))
        return jnp.where(mask, qt_v[_rows(step * NG + g, 64), 128 * j:128 * (j + 1)],
                         jnp.uint32(0))

    def keys(g, lo, hi):
        first = pl.multiple_of((step * NG + g) * (L // 2) + lo // 2, 8)
        return _unpack(k_v[pl.ds(first, (hi - lo) // 2), :])

    def causal_scores(g, hp, j):
        nk = 128 * (j + 1)
        st = _dot(keys(g, 0, nk), _unpack(masked_q_bits(g, hp, j)))
        diag = st[nk - 128:, :] + bias_v[...]
        return diag if j == 0 else jnp.concatenate([st[:nk - 128, :], diag], axis=0)

    def head_output(h, j, p, keep):
        o = _dot(_unpack(vt_v[_rows(step * H + h, 16), 0:128 * (j + 1)]), p)
        den = o[DH:DH + 1, :]
        inv = pl.reciprocal(den, approx=True)
        inv = inv * (2.0 - den * inv)
        return o[0:24, :] * (keep * inv)

    def single_probs(h, j):
        return jnp.exp2(causal_scores(*divmod(h, HPG), j)).astype(BF16)

    def pair_probs(pairs, j, flip):
        low = _iota((64, 128), 1) < 64
        qa, qb = {}, {}
        for h in pairs:
            g, hp = divmod(h, HPG)
            qa[h] = masked_q_bits(g, hp, j)
            qb[h] = pltpu.roll(masked_q_bits(g, hp + 1, j), 64, 1)
        off = {}
        if j > 0:
            for h in pairs:
                g = h // HPG
                for hh, q in ((h, qa[h]), (h + 1, qb[h])):
                    off[hh] = jnp.exp2(_dot(keys(g, 0, 128 * j), _unpack(q)))
        early, late = {}, {}
        for h in pairs:
            g = h // HPG
            k0 = 128 * j
            for which in ((0, 1) if flip else (1, 0)):
                if which == 0:
                    early[h] = _dot(keys(g, k0, k0 + 64),
                                    _unpack(jnp.where(low, qa[h], qb[h])))
                else:
                    late[h] = _dot(keys(g, k0, k0 + 128),
                                   _unpack(jnp.where(low, qb[h], qa[h])))
        probs = {}
        for h in pairs:
            p1 = jnp.exp2(early[h] + half_v[0])
            p2 = jnp.exp2(late[h][0:64, :])
            bottom = late[h][64:128, :]
            pa = jnp.concatenate(
                [jnp.where(low, p1, p2), jnp.exp2(bottom + half_v[1])], axis=0)
            pb = jnp.concatenate(
                [jnp.where(low, p2, p1), jnp.exp2(bottom + half_v[2])], axis=0)
            for hh, pd in ((h, pa), (h + 1, pb)):
                full = pd if j == 0 else jnp.concatenate([off[hh], pd], axis=0)
                probs[hh] = full.astype(BF16)
        return probs

    def attention_bounded():
        pairs = [g * HPG + hp for g in range(NG)
                 for hp in range(0, _heads_in_group(g) - 1, 2)]
        paired = set(pairs) | {h + 1 for h in pairs}
        singles = [h for h in range(H) if h not in paired]
        waves = [(pairs[i:i + 2], j) for i in range(0, len(pairs), 2) for j in range(NQT)]
        waves += [(None, j) for j in range(NQT)]

        def scores(w):
            grp, j = waves[w]
            if grp is None:
                return {h: single_probs(h, j) for h in singles}
            return pair_probs(grp, j, w % 2 == 1)

        def values(w, probs):
            grp, j = waves[w]
            for h, p in probs.items():
                o = head_output(h, j, p, 1.0 - gate_v[h:h + 1, :])
                if grp is not None and h - 1 in grp:
                    o = pltpu.roll(o, 64, 1)
                ot_v[step, DH * h:DH * (h + 1), 128 * j:128 * (j + 1)] = o[0:DH, :]

        pending = scores(0)
        for w in range(len(waves)):
            nxt = scores(w + 1) if w + 1 < len(waves) else None
            values(w, pending)
            pending = nxt
        ffn_down_chained()

    def attention_max_shifted():
        def one_tile(item, carry):
            h = item // NQT
            j = item - h * NQT
            g = h // HPG
            hp = h - g * HPG
            cols = pl.ds(pl.multiple_of(128 * j, 128), 128)
            rid = _iota((64, 128), 0)
            mask = (rid >= (DH // 2) * hp) & (rid < (DH // 2) * (hp + 1))
            qm = jnp.where(mask, qt_v[_rows(step * NG + g, 64), cols], jnp.uint32(0))
            st = _dot(keys(g, 0, L), _unpack(qm))
            future = _iota((L, 128), 0) > 128 * j + _iota((L, 128), 1)
            st = jnp.where(future, NEG, st)
            p = jnp.exp2(st - jnp.max(st, axis=0, keepdims=True)).astype(BF16)
            keep = 1.0 - gate_v[pl.ds(h, 1), :]
            oh_v[h, :, cols] = head_output(h, NQT - 1, p, keep)
            return carry

        def compact(q, carry):
            rows = jnp.concatenate([oh_v[4 * q + k, 0:DH, :] for k in range(4)], axis=0)
            ot_v[step, pl.ds(pl.multiple_of(4 * DH * q, 8), 4 * DH), :] = rows
            return carry

        lax.fori_loop(0, H * NQT, one_tile, 0)
        lax.fori_loop(0, H // 4, compact, 0)
        ffn_down_looped()

    def routed_columns():
        ys = []
        for t in range(2):
            y = _round_bf16(jnp.sum(y_v[t], axis=1, keepdims=True))
            rsel = jnp.full((1, 1), rsel_s[t], F32)
            ys.append(_round_bf16(y * _round_bf16(jax.nn.sigmoid(rsel))))
        return ys

    def output_copy(seg, n):
        return pltpu.make_async_copy(
            out_v.at[pl.ds(seg * D, D), pl.ds(128 * n, 128)],
            o_hbm.at[:, pl.ds(seg * L + 128 * n, 128)],
            out_sems.at[NQT * seg + n])

    def output_projection(seg, ys):
        heads_out = ot_v[seg, 0:D, :]
        if seg > 0:
            pieces = []
            for b in range(D // 8):
                h0, h1 = (8 * b) // DH, (8 * b + 7) // DH
                sc = mscale_v[seg - 1, h0:h0 + 1, :]
                if h1 != h0:
                    first = _iota((8, L), 0) < DH * h1 - 8 * b
                    sc = jnp.where(first, sc, mscale_v[seg - 1, h1:h1 + 1, :])
                pieces.append(mem_v[seg - 1, 8 * b:8 * b + 8, :] * sc)
            heads_out = heads_out + jnp.concatenate(pieces, axis=0)
        attn = _dot(_unpack(wot[...]), heads_out.astype(BF16))
        base = x_v[seg].astype(F32) + attn
        xn = _unpack(xn_v[_rows(seg, D // 2), :]).astype(F32)
        col = seg * L + _iota((1, L), 1)
        upd = (jnp.where(col == idx_s[0], ys[0], 0.0)
               + jnp.where(col == idx_s[1], ys[1], 0.0))
        result = base + (xn + upd)
        for n in range(NQT):
            cols = slice(128 * n, 128 * (n + 1))
            out_v[seg * D:(seg + 1) * D, cols] = result[:, cols].astype(BF16)
            output_copy(seg, n).start()

    col_blocks = [(c0, min(128, D - c0)) for c0 in range(0, D, 128)]

    def transpose_block(w_v, section, c0, n):
        r0 = (section * D + c0) // 2
        wall[r0:r0 + n // 2, :] = pltpu.bitcast(w_v[:, c0:c0 + n].T, U32)

    def project_block(section, c0, n, xn):
        r0 = (section * D + c0) // 2
        last = section == 2 and c0 + n == D
        hi = PROWS // 2 if last else r0 + n // 2
        return _dot(_unpack(wall[r0:hi, :]), xn)

    def query_half0(half):
        layer_norm(0, serial=False, tiles=[2 * half, 2 * half + 1])
        xn = _unpack(xn_v[0:D // 2, 256 * half:256 * (half + 1)])
        top = _dot(_unpack(wall[0:D // 4, :]), xn)
        if half == 0:
            for c0, n in col_blocks[3:]:
                transpose_block(wq_v, 0, c0, n)
        bottom = _dot(_unpack(wall[D // 4:D // 2, :]), xn)
        return jnp.concatenate([top, bottom], axis=0)

    def projections():
        qtiles = []
        for half in range(2):
            x0_copies[half].wait()
            if half == 1:
                cp_wk.wait()
            qtiles.append(query_half0(half))
        for c0, n in col_blocks:
            transpose_block(wk_v, 1, c0, n)
        parts = [jnp.concatenate(qtiles, axis=1)]
        xn0 = _unpack(xn_v[_rows(0, D // 2), :])
        parts += [project_block(1, c0, n, xn0) for c0, n in col_blocks[:EARLY_K]]
        cp_wv.wait()
        x_copies[1].wait()
        xn0 = _unpack(xn_v[_rows(0, D // 2), :])
        parts += [project_block(1, c0, n, xn0) for c0, n in col_blocks[EARLY_K:]]
        for c0, n in col_blocks:
            transpose_block(wv_v, 2, c0, n)
            parts.append(project_block(2, c0, n, xn0))
        layer_norm(1)
        _, pk, vg = store_qkv(0, jnp.concatenate(parts, axis=0))
        x_copies[2].wait()
        x_copies[3].wait()
        cp_wo.wait()

        layer_norm(2)
        pt = project(1)
        wot[...] = pltpu.bitcast(wo_v[...].T, U32)
        state1 = memory_update(None, pk, vg)
        pq1, pk, vg = store_qkv(1, pt)
        layer_norm(3)
        pt = project(2)
        state2 = memory_update(state1, pk, vg)
        pq2, pk, vg = store_qkv(2, pt)
        cp_wg.wait()
        cp_wu.wait()
        pt, todo, done = project_last_with_ffn()
        pq3, _, _ = store_qkv(3, pt)
        state3 = memory_update(state2, pk, vg)
        done += [ffn_in_tile(*item) for item in todo]
        store_ffn_hidden(done[:FF // 128], done[FF // 128:])
        memory_retrieve(1, state1, pq1)
        memory_retrieve(2, state2, pq2)
        memory_retrieve(3, state3, pq3)
        record_logit_bound()
        cp_wd.wait()

    @pl.when(step == 0)
    def _():
        for cp in (cp_wq, cp_wr, cp_beta, *x0_copies, cp_wk, cp_wv, x_copies[1],
                   x_copies[2], x_copies[3], cp_wo, cp_wg, cp_wu, cp_wd):
            cp.start()
        with _scope("sc_startup"):
            cp_wr.wait()
            cp_beta.wait()
            cp_wq.wait()
            init_constants()
            for c0, n in col_blocks[:3]:
                transpose_block(wq_v, 0, c0, n)
        with _scope("sc_projections"):
            projections()

    @pl.when(step < NSEG)
    def _():
        safe = safe_s[0] == 1

        @pl.when(safe)
        def _():
            with _scope("sc_attention"):
                attention_bounded()

        @pl.when(jnp.logical_not(safe))
        def _():
            attention_max_shifted()

    @pl.when(step == NSEG)
    def _():
        with _scope("sc_outproj"):
            ys = routed_columns()
            for seg in range(NSEG):
                output_projection(seg, ys)
            for seg in range(NSEG):
                for n in range(NQT):
                    output_copy(seg, n).wait()


@jax.jit
def pallas_parallel_sum__memory_aug_infini_attn__moe_arch_mod__prompt_kernel(
    A_x: jax.Array,
    A_wq: jax.Array,
    A_wk: jax.Array,
    A_wv: jax.Array,
    A_wo: jax.Array,
    A_beta: jax.Array,
    B_x: jax.Array,
    B_w_r: jax.Array,
    B_w_gate: jax.Array,
    B_w_up: jax.Array,
    B_w_down: jax.Array,
):
    del B_x
    vm = pltpu.VMEM
    scratch = [
        vm((NSEG, D, L), BF16),
        vm((D, D), BF16),
        vm((D, D), BF16),
        vm((D, D), BF16),
        vm((D, D), BF16),
        vm((H,), BF16),
        vm((D,), BF16),
        vm((D, FF), BF16),
        vm((D, FF), BF16),
        vm((D, FF), BF16),
        vm((PROWS // 2, D), U32),
        vm((D // 2, D), U32),
        vm((NSEG * D // 2, L), U32),
        vm((NSEG * NG * 64, L), U32),
        vm((NSEG * NG * L // 2, 128), U32),
        vm((NSEG * H * 16, L), U32),
        vm((NSEG - 1, D, L), F32),
        vm((NSEG - 1, H + 8, L), F32),
        vm((8, L), F32),
        vm((8, D), U32),
        vm((2, D, 128), F32),
        vm((2, FF // 128, 8, 128), F32),
        pltpu.SMEM((2,), jnp.int32),
        pltpu.SMEM((2,), F32),
        pltpu.SMEM((1,), U32),
        pltpu.SMEM((1,), jnp.int32),
        vm((H, 128), F32),
        vm((NSEG, D, L), F32),
        vm((H, 24, L), F32),
        vm((128, 128), F32),
        vm((3, 64, 128), F32),
        vm((NSEG * D, L), BF16),
        pltpu.SemaphoreType.DMA((NSEG * NQT,)),
        pltpu.SemaphoreType.DMA((NSEG + 9 + 2,)),
    ]
    hbm = pl.BlockSpec(memory_space=pltpu.HBM)
    xt = jnp.transpose(A_x.reshape(S, D))
    out_t = pl.pallas_call(
        _kernel,
        grid=(NSEG + 1,),
        in_specs=[hbm] * 10,
        out_specs=hbm,
        out_shape=jax.ShapeDtypeStruct((D, S), BF16),
        scratch_shapes=scratch,
        compiler_params=pltpu.CompilerParams(
            dimension_semantics=("arbitrary",),
            vmem_limit_bytes=110 * 1024 * 1024,
        ),
        name="infini_moe",
    )(xt, A_wq, A_wk, A_wv, A_wo, A_beta, B_w_r, B_w_gate, B_w_up,
      jnp.transpose(B_w_down))
    return jnp.transpose(out_t).reshape(1, S, D)
```

```python
import contextlib

import jax
import jax.numpy as jnp
from jax import lax
from jax.experimental import pallas as pl
from jax.experimental.pallas import tpu as pltpu

S = 2048
D = 576
H = 32
DH = 18
NSEG = 4
L = 512
FF = 4608
NG = 5
HPG = 7
GW = HPG * DH
NQT = L // 128
PROWS = 3 * D + 16
RROW = 3 * D
EARLY_K = 1
FFN_FIRST_BLOCK = 3
FFN_PATTERN = (1, 2)
PBLOCK = 128
FT = FF // 128 // NSEG
LOG2E = 1.4426950408889634
QSCALE = DH ** -0.5 * LOG2E
NEG = -1e30
LN_EPS = 1.0013580322265625e-05
F32 = jnp.float32
BF16 = jnp.bfloat16
U32 = jnp.uint32

PROFILE_SCOPES = False

_NN = (((1,), (0,)), ((), ()))
_NT = (((1,), (1,)), ((), ()))


def _scope(name):
    return jax.named_scope(name) if PROFILE_SCOPES else contextlib.nullcontext()


def _dot(a, b):
    return lax.dot_general(a, b, _NN, preferred_element_type=F32)


def _dot_nt(a, b):
    return lax.dot_general(a, b, _NT, preferred_element_type=F32)


def _iota(shape, dim):
    return lax.broadcasted_iota(jnp.int32, shape, dim)


def _round_bf16(v):
    return v.astype(BF16).astype(F32)


def _pack(v):
    return pltpu.bitcast(v.astype(BF16), U32)


def _unpack(u):
    return pltpu.bitcast(u, BF16)


def _rows(index, size):
    if isinstance(index, int):
        return slice(index * size, (index + 1) * size)
    return pl.ds(pl.multiple_of(index * size, 8), size)


def _heads_in_group(g):
    return HPG if g < NG - 1 else H - HPG * (NG - 1)


def _memory_rows(g):
    used = _heads_in_group(g) * DH
    return (128, GW) if g < NG - 1 else (used + 8, used)


def _phi(t):
    return jnp.where(t > 0, t + 1.0, jnp.exp(t))


def _kernel(x_hbm, wq_hbm, wk_hbm, wv_hbm, wo_hbm, beta_hbm, wr_hbm,
            wg_hbm, wu_hbm, wd_hbm,
            o_hbm,
            x_v, wq_v, wk_v, wv_v, wo_v, beta_v, wr_v, wg_v, wu_v, wd_v,
            wall, wot, xn_v, qt_v, k_v, vt_v, mem_v, mden_v,
            r_v, xs_v, y_v, hid_v, idx_s, rsel_s, zero_s, safe_s,
            gate_v, ot_v, oh_v, bias_v, half_v, out_v, out_sems,
            sems):
    step = pl.program_id(0)

    x_copies = [None] + [
        pltpu.make_async_copy(x_hbm.at[:, pl.ds(c * L, L)], x_v.at[c], sems.at[c])
        for c in range(1, NSEG)
    ]
    x0_copies = [
        pltpu.make_async_copy(x_hbm.at[:, pl.ds(256 * n, 256)],
                              x_v.at[0, :, pl.ds(256 * n, 256)],
                              sems.at[NSEG + 9 + n])
        for n in range(2)
    ]
    pairs = [(wq_hbm, wq_v), (wk_hbm, wk_v), (wv_hbm, wv_v), (wo_hbm, wo_v),
             (beta_hbm, beta_v), (wr_hbm, wr_v),
             (wg_hbm, wg_v), (wu_hbm, wu_v), (wd_hbm, wd_v)]
    (cp_wq, cp_wk, cp_wv, cp_wo, cp_beta, cp_wr, cp_wg, cp_wu, cp_wd) = [
        pltpu.make_async_copy(src, dst, sems.at[NSEG + i])
        for i, (src, dst) in enumerate(pairs)
    ]

    def nothing(v):
        return pltpu.bitcast(pltpu.bitcast(v, U32) & zero_s[0], F32)

    def layer_norm(c, serial=True, tiles=range(NQT)):
        link = None
        for n in tiles:
            cols = slice(128 * n, 128 * (n + 1))
            pivot = x_v[c, 0:16, cols].astype(F32)[0:1, :]
            pivot8 = jnp.broadcast_to(pivot, (8, 128))
            shift = pivot8
            s1 = s2 = None
            for i in range(D // 16):
                last = s1 if s1 is not None else link
                if serial and last is not None:
                    shift = pivot8 + nothing(last)
                x16 = x_v[c, 16 * i:16 * i + 16, cols].astype(F32)
                for k in range(2):
                    d = x16[8 * k:8 * k + 8, :] - shift
                    s1 = d if s1 is None else s1 + d
                    s2 = d * d if s2 is None else s2 + d * d
            dmean = jnp.sum(s1, axis=0, keepdims=True) * (1.0 / D)
            dsq = jnp.sum(s2, axis=0, keepdims=True) * (1.0 / D)
            var = jnp.maximum(dsq - dmean * dmean, 0.0)
            sd = _round_bf16(jnp.sqrt(_round_bf16(_round_bf16(var) + LN_EPS)))
            mean8 = jnp.broadcast_to(_round_bf16(pivot + dmean), (8, 128))
            inv8 = jnp.broadcast_to(1.0 / sd, (8, 128))
            center = mean8
            for i in range(D // 32):
                if serial and i > 0:
                    center = mean8 + nothing(link)
                x32 = x_v[c, 32 * i:32 * i + 32, cols].astype(F32)
                z = [(x32[8 * k:8 * k + 8, :] - center) * inv8 for k in range(4)]
                link = z[3]
                r0 = c * (D // 2) + 16 * i
                xn_v[r0:r0 + 16, cols] = _pack(jnp.concatenate(z, axis=0))

    def init_constants():
        gate = jax.nn.sigmoid(beta_v[...].astype(F32).reshape(1, H))
        on_diag = _iota((H, H), 0) == _iota((H, H), 1)
        gcol = jnp.sum(jnp.where(on_diag, gate, 0.0), axis=1, keepdims=True)
        gate_v[...] = jnp.broadcast_to(gcol, (H, 128))
        zero_s[0] = jnp.uint32(0)
        bias_v[...] = jnp.where(_iota((128, 128), 0) > _iota((128, 128), 1), NEG, 0.0)
        key, lane = _iota((64, 128), 0), _iota((64, 128), 1)
        future = key > (lane & 63)
        half_v[0] = jnp.where(future, NEG, 0.0)
        half_v[1] = jnp.where(future | (lane < 64), NEG, 0.0)
        half_v[2] = jnp.where(future | (lane >= 64), NEG, 0.0)
        router = jnp.broadcast_to(wr_v[...].astype(F32).reshape(1, D), (16, D))
        wall[RROW // 2:PROWS // 2, :] = _pack(
            jnp.where(_iota((16, D), 0) == 0, router, 0.0))

    def project(c):
        xn = _unpack(xn_v[_rows(c, D // 2), :])
        step_rows = PBLOCK // 2
        return jnp.concatenate(
            [_dot(_unpack(wall[r:min(r + step_rows, PROWS // 2), :]), xn)
             for r in range(0, PROWS // 2, step_rows)], axis=0)

    seen = [None]

    def record_logit_bound():
        big = (seen[0] >> 30) & 1
        safe_s[0] = (jnp.max(big.astype(jnp.int32)) == 0).astype(jnp.int32)

    def store_qkv(c, pt):
        if c < NSEG - 1:
            r_v[c:c + 1, :] = _round_bf16(pt[RROW:RROW + 1, :])
        tail_row = _iota((8, L), 0)
        for h in range(H):
            base = 2 * D + DH * h
            tail = jnp.where(tail_row < DH - 16, pt[base + 16:base + 24, :],
                             jnp.where(tail_row == DH - 16, 1.0, 0.0))
            blk = jnp.concatenate(
                [pt[base:base + 16, :], tail, jnp.zeros((8, L), F32)], axis=0)
            vt_v[_rows(c * H + h, 16), :] = _pack(blk)

        pqs, pks, vgs = [], [], []
        for g in range(NG):
            used = _heads_in_group(g) * DH
            qg = pt[GW * g:GW * g + 128, :]
            qs = qg * QSCALE
            qt_v[_rows(c * NG + g, 64), :] = _pack(qs)
            kg = pt[D + GW * g:D + GW * g + 128, :]
            for operand in (qs, kg):
                bits = pltpu.bitcast(operand, U32)
                for blk in range(0, 128 if g < NG - 1 else used, 8):
                    for col in range(0, L, 128):
                        piece = bits[blk:blk + 8, col:col + 128]
                        seen[0] = piece if seen[0] is None else seen[0] | piece
            k_v[_rows(c * NG + g, L // 2), :] = _pack(kg.T)
            pqs.append(_phi(qg).astype(BF16))
            if c < NSEG - 1:
                pks.append(_phi(kg).astype(BF16))
                lo = 2 * D + GW * g
                rows, zrow = _memory_rows(g)
                rid = _iota((rows, L), 0)
                vg = jnp.where(rid < used, pt[lo:lo + rows, :],
                               jnp.where(rid == zrow, 1.0, 0.0))
                vgs.append(vg.astype(BF16))
        return pqs, pks, vgs

    def memory_update(states, pks, vgs):
        out = []
        for g in range(NG):
            used = _heads_in_group(g) * DH
            rows, zrow = _memory_rows(g)
            row = _iota((rows, 128), 0)
            lane = _iota((rows, 128), 1)
            same_head = (row // DH) == (lane // DH)
            upd = _dot_nt(vgs[g], pks[g])
            keep = ((same_head & (row < used)) | (row == zrow)) & (lane < used)
            upd = jnp.where(keep, upd, 0.0)
            out.append(upd if states is None else states[g] + upd)
        return out

    def memory_retrieve(c, states, pqs):
        row8 = _iota((8, 128), 0)
        lane8 = _iota((8, 128), 1) // DH
        for g in range(NG):
            nh = _heads_in_group(g)
            rows, zrow = _memory_rows(g)
            st = states[g]
            mrows = jnp.where(_iota((rows, 128), 0) < zrow, st, 0.0)
            zrows = jnp.where(lane8 == row8, st[zrow:zrow + 1, :], 0.0)
            lhs = jnp.concatenate(
                [mrows, zrows, jnp.zeros((8, 128), F32)], axis=0).astype(BF16)
            ret = _dot(lhs, pqs[g])
            out_rows = 128 if g < NG - 1 else nh * DH
            mem_v[c - 1, GW * g:GW * g + out_rows, :] = ret[0:out_rows, :]
            mden_v[c - 1, HPG * g:HPG * g + 8, :] = ret[rows:rows + 8, :]

    def route():
        r = r_v[0:NSEG, :]
        idx = _iota((NSEG, L), 0) * L + _iota((NSEG, L), 1)
        m1 = jnp.max(r)
        i1 = jnp.clip(jnp.min(jnp.where(r == m1, idx, S)), 0, S - 1)
        r2 = jnp.where(idx == i1, -jnp.inf, r)
        m2 = jnp.max(r2)
        i2 = jnp.clip(jnp.min(jnp.where(r2 == m2, idx, S)), 0, S - 1)
        idx_s[0] = i1
        idx_s[1] = i2
        rsel_s[0] = m1
        rsel_s[1] = m2
        row16 = _iota((16, 128), 0)
        lane16 = _iota((16, 128), 1)
        xs = None
        for t, i in enumerate((i1, i2)):
            seg = i // L
            off = i - seg * L
            base = pl.multiple_of((off // 128) * 128, 128)
            cols = _unpack(xn_v[_rows(seg, D // 2), pl.ds(base, 128)])
            pick = jnp.where((row16 == t) & (lane16 == off - base), 1.0, 0.0)
            part = _dot_nt(pick.astype(BF16), cols)
            xs = part if xs is None else xs + part
        xs_v[...] = _pack(xs)
        y_v[...] = jnp.zeros(y_v.shape, F32)

    def ffn_in_tile(w_ref, tile):
        return _dot(_unpack(xs_v[...]), w_ref[:, 128 * tile:128 * (tile + 1)])

    def store_ffn_hidden(gates, ups):
        for tile, (gt, up) in enumerate(zip(gates, ups)):
            gt = _round_bf16(gt)
            hid = _round_bf16(_round_bf16(gt * jax.nn.sigmoid(gt)) * _round_bf16(up))
            for t in range(2):
                hid_v[t, tile] = jnp.broadcast_to(hid[t:t + 1, :], (8, 128))

    def project_last_with_ffn():
        c = NSEG - 1
        xn = _unpack(xn_v[_rows(c, D // 2), :])
        router = _dot(_unpack(wall[RROW // 2:PROWS // 2, :]), xn)
        r_v[c:c + 1, :] = _round_bf16(router[0:1, :])
        todo = [(w_ref, tile) for w_ref in (wg_v, wu_v) for tile in range(FF // 128)]
        done = []
        blocks = []
        for i, r in enumerate(range(0, RROW // 2, PBLOCK // 2)):
            if i == FFN_FIRST_BLOCK:
                route()
            lhs = _unpack(wall[r:min(r + PBLOCK // 2, RROW // 2), :])
            tiles = []
            for n in range(NQT):
                tiles.append(_dot(lhs, xn[:, 128 * n:128 * (n + 1)]))
                if i >= FFN_FIRST_BLOCK:
                    for _ in range(min(FFN_PATTERN[n % len(FFN_PATTERN)], len(todo))):
                        done.append(ffn_in_tile(*todo.pop(0)))
            blocks.append(jnp.concatenate(tiles, axis=1))
        pt = jnp.concatenate(blocks + [router], axis=0)
        return pt, todo, done

    def ffn_down_chained():
        base = pl.multiple_of(step * (FT * 128), 128)
        hid = [[hid_v[t, step * FT + tile] for tile in range(FT)] for t in range(2)]
        link = [None, None]
        for b in range(D // 8):
            acc = [None, None]
            for tile in range(FT):
                w = wd_v[8 * b:8 * b + 8, pl.ds(base + 128 * tile, 128)].astype(F32)
                for t in range(2):
                    pr = w * hid[t][tile]
                    if tile > 0:
                        acc[t] = acc[t] + pr
                    else:
                        acc[t] = pr if link[t] is None else pr + nothing(link[t])
            for t in range(2):
                rows = slice(8 * b, 8 * b + 8)
                y_v[t, rows, :] = y_v[t, rows, :] + acc[t]
                link[t] = acc[t]

    def ffn_down_looped():
        def down(tile, carry):
            col = step * FT + tile
            w = wd_v[:, pl.ds(pl.multiple_of(128 * col, 128), 128)].astype(F32)
            for t in range(2):
                y_v[t] = y_v[t] + w * hid_v[t, col][0:1, :]
            return carry

        lax.fori_loop(0, FT, down, 0)

    def masked_q_bits(g, hp, j):
        rid = _iota((64, 128), 0)
        mask = (rid >= (DH // 2) * hp) & (rid < (DH // 2) * (hp + 1))
        return jnp.where(mask, qt_v[_rows(step * NG + g, 64), 128 * j:128 * (j + 1)],
                         jnp.uint32(0))

    def keys(g, lo, hi):
        first = pl.multiple_of((step * NG + g) * (L // 2) + lo // 2, 8)
        return _unpack(k_v[pl.ds(first, (hi - lo) // 2), :])

    def causal_scores(g, hp, j):
        nk = 128 * (j + 1)
        st = _dot(keys(g, 0, nk), _unpack(masked_q_bits(g, hp, j)))
        diag = st[nk - 128:, :] + bias_v[...]
        return diag if j == 0 else jnp.concatenate([st[:nk - 128, :], diag], axis=0)

    def head_output(h, j, p, keep):
        o = _dot(_unpack(vt_v[_rows(step * H + h, 16), 0:128 * (j + 1)]), p)
        den = o[DH:DH + 1, :]
        inv = pl.reciprocal(den, approx=True)
        inv = inv * (2.0 - den * inv)
        return o[0:24, :] * (keep * inv)

    def single_probs(h, j):
        return jnp.exp2(causal_scores(*divmod(h, HPG), j)).astype(BF16)

    def pair_probs(pairs, j, flip):
        low = _iota((64, 128), 1) < 64
        qa, qb = {}, {}
        for h in pairs:
            g, hp = divmod(h, HPG)
            qa[h] = masked_q_bits(g, hp, j)
            qb[h] = pltpu.roll(masked_q_bits(g, hp + 1, j), 64, 1)
        off = {}
        if j > 0:
            for h in pairs:
                g = h // HPG
                for hh, q in ((h, qa[h]), (h + 1, qb[h])):
                    off[hh] = jnp.exp2(_dot(keys(g, 0, 128 * j), _unpack(q)))
        early, late = {}, {}
        for h in pairs:
            g = h // HPG
            k0 = 128 * j
            for which in ((0, 1) if flip else (1, 0)):
                if which == 0:
                    early[h] = _dot(keys(g, k0, k0 + 64),
                                    _unpack(jnp.where(low, qa[h], qb[h])))
                else:
                    late[h] = _dot(keys(g, k0, k0 + 128),
                                   _unpack(jnp.where(low, qb[h], qa[h])))
        probs = {}
        for h in pairs:
            p1 = jnp.exp2(early[h] + half_v[0])
            p2 = jnp.exp2(late[h][0:64, :])
            bottom = late[h][64:128, :]
            pa = jnp.concatenate(
                [jnp.where(low, p1, p2), jnp.exp2(bottom + half_v[1])], axis=0)
            pb = jnp.concatenate(
                [jnp.where(low, p2, p1), jnp.exp2(bottom + half_v[2])], axis=0)
            for hh, pd in ((h, pa), (h + 1, pb)):
                full = pd if j == 0 else jnp.concatenate([off[hh], pd], axis=0)
                probs[hh] = full.astype(BF16)
        return probs

    def attention_bounded():
        pairs = [g * HPG + hp for g in range(NG)
                 for hp in range(0, _heads_in_group(g) - 1, 2)]
        paired = set(pairs) | {h + 1 for h in pairs}
        singles = [h for h in range(H) if h not in paired]
        waves = [(pairs[i:i + 2], j) for i in range(0, len(pairs), 2) for j in range(NQT)]
        waves += [(None, j) for j in range(NQT)]

        def scores(w):
            grp, j = waves[w]
            if grp is None:
                return {h: single_probs(h, j) for h in singles}
            return pair_probs(grp, j, w % 2 == 1)

        def values(w, probs):
            grp, j = waves[w]
            for h, p in probs.items():
                o = head_output(h, j, p, 1.0 - gate_v[h:h + 1, :])
                if grp is not None and h - 1 in grp:
                    o = pltpu.roll(o, 64, 1)
                ot_v[step, DH * h:DH * (h + 1), 128 * j:128 * (j + 1)] = o[0:DH, :]

        pending = scores(0)
        for w in range(len(waves)):
            nxt = scores(w + 1) if w + 1 < len(waves) else None
            values(w, pending)
            pending = nxt
        ffn_down_chained()

    def attention_max_shifted():
        def one_tile(item, carry):
            h = item // NQT
            j = item - h * NQT
            g = h // HPG
            hp = h - g * HPG
            cols = pl.ds(pl.multiple_of(128 * j, 128), 128)
            rid = _iota((64, 128), 0)
            mask = (rid >= (DH // 2) * hp) & (rid < (DH // 2) * (hp + 1))
            qm = jnp.where(mask, qt_v[_rows(step * NG + g, 64), cols], jnp.uint32(0))
            st = _dot(keys(g, 0, L), _unpack(qm))
            future = _iota((L, 128), 0) > 128 * j + _iota((L, 128), 1)
            st = jnp.where(future, NEG, st)
            p = jnp.exp2(st - jnp.max(st, axis=0, keepdims=True)).astype(BF16)
            keep = 1.0 - gate_v[pl.ds(h, 1), :]
            oh_v[h, :, cols] = head_output(h, NQT - 1, p, keep)
            return carry

        def compact(q, carry):
            rows = jnp.concatenate([oh_v[4 * q + k, 0:DH, :] for k in range(4)], axis=0)
            ot_v[step, pl.ds(pl.multiple_of(4 * DH * q, 8), 4 * DH), :] = rows
            return carry

        lax.fori_loop(0, H * NQT, one_tile, 0)
        lax.fori_loop(0, H // 4, compact, 0)
        ffn_down_looped()

    def routed_columns():
        ys = []
        for t in range(2):
            y = _round_bf16(jnp.sum(y_v[t], axis=1, keepdims=True))
            rsel = jnp.full((1, 1), rsel_s[t], F32)
            ys.append(_round_bf16(y * _round_bf16(jax.nn.sigmoid(rsel))))
        return ys

    def output_copy(seg, n):
        return pltpu.make_async_copy(
            out_v.at[pl.ds(seg * D, D), pl.ds(128 * n, 128)],
            o_hbm.at[:, pl.ds(seg * L + 128 * n, 128)],
            out_sems.at[NQT * seg + n])

    def output_projection(seg, ys):
        heads_out = ot_v[seg, 0:D, :]
        if seg > 0:
            gates = jnp.concatenate([gate_v[...]] * NQT, axis=1)
            scale = gates / (mden_v[seg - 1, 0:H, :] + 1e-6)
            pieces = []
            for b in range(D // 8):
                h0, h1 = (8 * b) // DH, (8 * b + 7) // DH
                sc = scale[h0:h0 + 1, :]
                if h1 != h0:
                    first = _iota((8, L), 0) < DH * h1 - 8 * b
                    sc = jnp.where(first, sc, scale[h1:h1 + 1, :])
                pieces.append(mem_v[seg - 1, 8 * b:8 * b + 8, :] * sc)
            heads_out = heads_out + jnp.concatenate(pieces, axis=0)
        attn = _dot(_unpack(wot[...]), heads_out.astype(BF16))
        base = x_v[seg].astype(F32) + attn
        xn = _unpack(xn_v[_rows(seg, D // 2), :]).astype(F32)
        col = seg * L + _iota((1, L), 1)
        upd = (jnp.where(col == idx_s[0], ys[0], 0.0)
               + jnp.where(col == idx_s[1], ys[1], 0.0))
        result = base + (xn + upd)
        for n in range(NQT):
            cols = slice(128 * n, 128 * (n + 1))
            out_v[seg * D:(seg + 1) * D, cols] = result[:, cols].astype(BF16)
            output_copy(seg, n).start()

    col_blocks = [(c0, min(128, D - c0)) for c0 in range(0, D, 128)]

    def transpose_block(w_v, section, c0, n):
        r0 = (section * D + c0) // 2
        wall[r0:r0 + n // 2, :] = pltpu.bitcast(w_v[:, c0:c0 + n].T, U32)

    def project_block(section, c0, n, xn):
        r0 = (section * D + c0) // 2
        last = section == 2 and c0 + n == D
        hi = PROWS // 2 if last else r0 + n // 2
        return _dot(_unpack(wall[r0:hi, :]), xn)

    def query_half0(half):
        layer_norm(0, serial=False, tiles=[2 * half, 2 * half + 1])
        xn = _unpack(xn_v[0:D // 2, 256 * half:256 * (half + 1)])
        top = _dot(_unpack(wall[0:D // 4, :]), xn)
        if half == 0:
            for c0, n in col_blocks[3:]:
                transpose_block(wq_v, 0, c0, n)
        bottom = _dot(_unpack(wall[D // 4:D // 2, :]), xn)
        return jnp.concatenate([top, bottom], axis=0)

    def projections():
        qtiles = []
        for half in range(2):
            x0_copies[half].wait()
            if half == 1:
                cp_wk.wait()
            qtiles.append(query_half0(half))
        for c0, n in col_blocks:
            transpose_block(wk_v, 1, c0, n)
        parts = [jnp.concatenate(qtiles, axis=1)]
        xn0 = _unpack(xn_v[_rows(0, D // 2), :])
        parts += [project_block(1, c0, n, xn0) for c0, n in col_blocks[:EARLY_K]]
        cp_wv.wait()
        x_copies[1].wait()
        xn0 = _unpack(xn_v[_rows(0, D // 2), :])
        parts += [project_block(1, c0, n, xn0) for c0, n in col_blocks[EARLY_K:]]
        for c0, n in col_blocks:
            transpose_block(wv_v, 2, c0, n)
            parts.append(project_block(2, c0, n, xn0))
        layer_norm(1)
        _, pk, vg = store_qkv(0, jnp.concatenate(parts, axis=0))
        x_copies[2].wait()
        x_copies[3].wait()
        cp_wo.wait()

        layer_norm(2)
        pt = project(1)
        wot[...] = pltpu.bitcast(wo_v[...].T, U32)
        state1 = memory_update(None, pk, vg)
        pq1, pk, vg = store_qkv(1, pt)
        layer_norm(3)
        pt = project(2)
        state2 = memory_update(state1, pk, vg)
        pq2, pk, vg = store_qkv(2, pt)
        cp_wg.wait()
        cp_wu.wait()
        pt, todo, done = project_last_with_ffn()
        pq3, _, _ = store_qkv(3, pt)
        state3 = memory_update(state2, pk, vg)
        done += [ffn_in_tile(*item) for item in todo]
        store_ffn_hidden(done[:FF // 128], done[FF // 128:])
        memory_retrieve(1, state1, pq1)
        memory_retrieve(2, state2, pq2)
        memory_retrieve(3, state3, pq3)
        record_logit_bound()
        cp_wd.wait()

    @pl.when(step == 0)
    def _():
        for cp in (cp_wq, cp_wr, cp_beta, *x0_copies, cp_wk, cp_wv, x_copies[1],
                   x_copies[2], x_copies[3], cp_wo, cp_wg, cp_wu, cp_wd):
            cp.start()
        with _scope("sc_startup"):
            cp_wr.wait()
            cp_beta.wait()
            cp_wq.wait()
            init_constants()
            for c0, n in col_blocks[:3]:
                transpose_block(wq_v, 0, c0, n)
        with _scope("sc_projections"):
            projections()

    @pl.when(step < NSEG)
    def _():
        safe = safe_s[0] == 1

        @pl.when(safe)
        def _():
            with _scope("sc_attention"):
                attention_bounded()

        @pl.when(jnp.logical_not(safe))
        def _():
            attention_max_shifted()

    @pl.when(step == NSEG)
    def _():
        with _scope("sc_outproj"):
            ys = routed_columns()
            for seg in range(NSEG):
                output_projection(seg, ys)
            for seg in range(NSEG):
                for n in range(NQT):
                    output_copy(seg, n).wait()


@jax.jit
def pallas_parallel_sum__memory_aug_infini_attn__moe_arch_mod__prompt_kernel(
    A_x: jax.Array,
    A_wq: jax.Array,
    A_wk: jax.Array,
    A_wv: jax.Array,
    A_wo: jax.Array,
    A_beta: jax.Array,
    B_x: jax.Array,
    B_w_r: jax.Array,
    B_w_gate: jax.Array,
    B_w_up: jax.Array,
    B_w_down: jax.Array,
):
    del B_x
    vm = pltpu.VMEM
    scratch = [
        vm((NSEG, D, L), BF16),
        vm((D, D), BF16),
        vm((D, D), BF16),
        vm((D, D), BF16),
        vm((D, D), BF16),
        vm((H,), BF16),
        vm((D,), BF16),
        vm((D, FF), BF16),
        vm((D, FF), BF16),
        vm((D, FF), BF16),
        vm((PROWS // 2, D), U32),
        vm((D // 2, D), U32),
        vm((NSEG * D // 2, L), U32),
        vm((NSEG * NG * 64, L), U32),
        vm((NSEG * NG * L // 2, 128), U32),
        vm((NSEG * H * 16, L), U32),
        vm((NSEG - 1, D, L), F32),
        vm((NSEG - 1, H + 8, L), F32),
        vm((8, L), F32),
        vm((8, D), U32),
        vm((2, D, 128), F32),
        vm((2, FF // 128, 8, 128), F32),
        pltpu.SMEM((2,), jnp.int32),
        pltpu.SMEM((2,), F32),
        pltpu.SMEM((1,), U32),
        pltpu.SMEM((1,), jnp.int32),
        vm((H, 128), F32),
        vm((NSEG, D, L), F32),
        vm((H, 24, L), F32),
        vm((128, 128), F32),
        vm((3, 64, 128), F32),
        vm((NSEG * D, L), BF16),
        pltpu.SemaphoreType.DMA((NSEG * NQT,)),
        pltpu.SemaphoreType.DMA((NSEG + 9 + 2,)),
    ]
    hbm = pl.BlockSpec(memory_space=pltpu.HBM)
    xt = jnp.transpose(A_x.reshape(S, D))
    out_t = pl.pallas_call(
        _kernel,
        grid=(NSEG + 1,),
        in_specs=[hbm] * 10,
        out_specs=hbm,
        out_shape=jax.ShapeDtypeStruct((D, S), BF16),
        scratch_shapes=scratch,
        compiler_params=pltpu.CompilerParams(
            dimension_semantics=("arbitrary",),
            vmem_limit_bytes=110 * 1024 * 1024,
        ),
        name="infini_moe",
    )(xt, A_wq, A_wk, A_wv, A_wo, A_beta, B_w_r, B_w_gate, B_w_up,
      jnp.transpose(B_w_down))
    return jnp.transpose(out_t).reshape(1, S, D)
```

```python
import contextlib

import jax
import jax.numpy as jnp
from jax import lax
from jax.experimental import pallas as pl
from jax.experimental.pallas import tpu as pltpu

S = 2048
D = 576
H = 32
DH = 18
NSEG = 4
L = 512
FF = 4608
NG = 5
HPG = 7
GW = HPG * DH
NQT = L // 128
PROWS = 3 * D + 16
RROW = 3 * D
EARLY_K = 1
FFN_FIRST_BLOCK = 3
FFN_PATTERN = (1, 2)
LOOKAHEAD = 2
PBLOCK = 128
FT = FF // 128 // NSEG
LOG2E = 1.4426950408889634
QSCALE = DH ** -0.5 * LOG2E
NEG = -1e30
LN_EPS = 1.0013580322265625e-05
F32 = jnp.float32
BF16 = jnp.bfloat16
U32 = jnp.uint32

PROFILE_SCOPES = False

_NN = (((1,), (0,)), ((), ()))
_NT = (((1,), (1,)), ((), ()))


def _scope(name):
    return jax.named_scope(name) if PROFILE_SCOPES else contextlib.nullcontext()


def _dot(a, b):
    return lax.dot_general(a, b, _NN, preferred_element_type=F32)


def _dot_nt(a, b):
    return lax.dot_general(a, b, _NT, preferred_element_type=F32)


def _iota(shape, dim):
    return lax.broadcasted_iota(jnp.int32, shape, dim)


def _round_bf16(v):
    return v.astype(BF16).astype(F32)


def _pack(v):
    return pltpu.bitcast(v.astype(BF16), U32)


def _unpack(u):
    return pltpu.bitcast(u, BF16)


def _rows(index, size):
    if isinstance(index, int):
        return slice(index * size, (index + 1) * size)
    return pl.ds(pl.multiple_of(index * size, 8), size)


def _heads_in_group(g):
    return HPG if g < NG - 1 else H - HPG * (NG - 1)


def _memory_rows(g):
    used = _heads_in_group(g) * DH
    return (128, GW) if g < NG - 1 else (used + 8, used)


def _phi(t):
    return jnp.where(t > 0, t + 1.0, jnp.exp(t))


def _kernel(x_hbm, wq_hbm, wk_hbm, wv_hbm, wo_hbm, beta_hbm, wr_hbm,
            wg_hbm, wu_hbm, wd_hbm,
            o_hbm,
            x_v, wq_v, wk_v, wv_v, wo_v, beta_v, wr_v, wg_v, wu_v, wd_v,
            wall, wot, xn_v, qt_v, k_v, vt_v, mem_v, mden_v,
            r_v, xs_v, y_v, hid_v, idx_s, rsel_s, zero_s, safe_s,
            gate_v, ot_v, oh_v, bias_v, half_v, quarter_v, out_v, out_sems,
            sems):
    step = pl.program_id(0)

    x_copies = [None] + [
        pltpu.make_async_copy(x_hbm.at[:, pl.ds(c * L, L)], x_v.at[c], sems.at[c])
        for c in range(1, NSEG)
    ]
    x0_copies = [
        pltpu.make_async_copy(x_hbm.at[:, pl.ds(256 * n, 256)],
                              x_v.at[0, :, pl.ds(256 * n, 256)],
                              sems.at[NSEG + 9 + n])
        for n in range(2)
    ]
    pairs = [(wq_hbm, wq_v), (wk_hbm, wk_v), (wv_hbm, wv_v), (wo_hbm, wo_v),
             (beta_hbm, beta_v), (wr_hbm, wr_v),
             (wg_hbm, wg_v), (wu_hbm, wu_v), (wd_hbm, wd_v)]
    (cp_wq, cp_wk, cp_wv, cp_wo, cp_beta, cp_wr, cp_wg, cp_wu, cp_wd) = [
        pltpu.make_async_copy(src, dst, sems.at[NSEG + i])
        for i, (src, dst) in enumerate(pairs)
    ]

    def nothing(v):
        return pltpu.bitcast(pltpu.bitcast(v, U32) & zero_s[0], F32)

    def layer_norm(c, serial=True, tiles=range(NQT)):
        link = None
        for n in tiles:
            cols = slice(128 * n, 128 * (n + 1))
            pivot = x_v[c, 0:16, cols].astype(F32)[0:1, :]
            pivot8 = jnp.broadcast_to(pivot, (8, 128))
            shift = pivot8
            s1 = s2 = None
            for i in range(D // 16):
                last = s1 if s1 is not None else link
                if serial and last is not None:
                    shift = pivot8 + nothing(last)
                x16 = x_v[c, 16 * i:16 * i + 16, cols].astype(F32)
                for k in range(2):
                    d = x16[8 * k:8 * k + 8, :] - shift
                    s1 = d if s1 is None else s1 + d
                    s2 = d * d if s2 is None else s2 + d * d
            dmean = jnp.sum(s1, axis=0, keepdims=True) * (1.0 / D)
            dsq = jnp.sum(s2, axis=0, keepdims=True) * (1.0 / D)
            var = jnp.maximum(dsq - dmean * dmean, 0.0)
            sd = _round_bf16(jnp.sqrt(_round_bf16(_round_bf16(var) + LN_EPS)))
            mean8 = jnp.broadcast_to(_round_bf16(pivot + dmean), (8, 128))
            inv8 = jnp.broadcast_to(1.0 / sd, (8, 128))
            center = mean8
            for i in range(D // 32):
                if serial and i > 0:
                    center = mean8 + nothing(link)
                x32 = x_v[c, 32 * i:32 * i + 32, cols].astype(F32)
                z = [(x32[8 * k:8 * k + 8, :] - center) * inv8 for k in range(4)]
                link = z[3]
                r0 = c * (D // 2) + 16 * i
                xn_v[r0:r0 + 16, cols] = _pack(jnp.concatenate(z, axis=0))

    def init_constants():
        gate = jax.nn.sigmoid(beta_v[...].astype(F32).reshape(1, H))
        on_diag = _iota((H, H), 0) == _iota((H, H), 1)
        gcol = jnp.sum(jnp.where(on_diag, gate, 0.0), axis=1, keepdims=True)
        gate_v[...] = jnp.broadcast_to(gcol, (H, 128))
        zero_s[0] = jnp.uint32(0)
        bias_v[...] = jnp.where(_iota((128, 128), 0) > _iota((128, 128), 1), NEG, 0.0)
        key, lane = _iota((64, 128), 0), _iota((64, 128), 1)
        future = key > (lane & 63)
        half_v[0] = jnp.where(future, NEG, 0.0)
        half_v[1] = jnp.where(future | (lane < 64), NEG, 0.0)
        half_v[2] = jnp.where(future | (lane >= 64), NEG, 0.0)
        quarter_v[...] = jnp.where(
            _iota((32, 128), 0) > (_iota((32, 128), 1) & 31), NEG, 0.0)
        router = jnp.broadcast_to(wr_v[...].astype(F32).reshape(1, D), (16, D))
        wall[RROW // 2:PROWS // 2, :] = _pack(
            jnp.where(_iota((16, D), 0) == 0, router, 0.0))

    def project(c):
        xn = _unpack(xn_v[_rows(c, D // 2), :])
        step_rows = PBLOCK // 2
        return jnp.concatenate(
            [_dot(_unpack(wall[r:min(r + step_rows, PROWS // 2), :]), xn)
             for r in range(0, PROWS // 2, step_rows)], axis=0)

    seen = [None]

    def record_logit_bound():
        big = (seen[0] >> 30) & 1
        safe_s[0] = (jnp.max(big.astype(jnp.int32)) == 0).astype(jnp.int32)

    def store_qkv(c, pt):
        if c < NSEG - 1:
            r_v[c:c + 1, :] = _round_bf16(pt[RROW:RROW + 1, :])
        tail_row = _iota((8, L), 0)
        for h in range(H):
            base = 2 * D + DH * h
            tail = jnp.where(tail_row < DH - 16, pt[base + 16:base + 24, :],
                             jnp.where(tail_row == DH - 16, 1.0, 0.0))
            blk = jnp.concatenate(
                [pt[base:base + 16, :], tail, jnp.zeros((8, L), F32)], axis=0)
            vt_v[_rows(c * H + h, 16), :] = _pack(blk)

        pqs, pks, vgs = [], [], []
        for g in range(NG):
            used = _heads_in_group(g) * DH
            qg = pt[GW * g:GW * g + 128, :]
            qs = qg * QSCALE
            qt_v[_rows(c * NG + g, 64), :] = _pack(qs)
            kg = pt[D + GW * g:D + GW * g + 128, :]
            for operand in (qs, kg):
                bits = pltpu.bitcast(operand, U32)
                for blk in range(0, 128 if g < NG - 1 else used, 8):
                    for col in range(0, L, 128):
                        piece = bits[blk:blk + 8, col:col + 128]
                        seen[0] = piece if seen[0] is None else seen[0] | piece
            k_v[_rows(c * NG + g, L // 2), :] = _pack(kg.T)
            pqs.append(_phi(qg).astype(BF16))
            if c < NSEG - 1:
                pks.append(_phi(kg).astype(BF16))
                lo = 2 * D + GW * g
                rows, zrow = _memory_rows(g)
                rid = _iota((rows, L), 0)
                vg = jnp.where(rid < used, pt[lo:lo + rows, :],
                               jnp.where(rid == zrow, 1.0, 0.0))
                vgs.append(vg.astype(BF16))
        return pqs, pks, vgs

    def memory_update(states, pks, vgs):
        out = []
        for g in range(NG):
            used = _heads_in_group(g) * DH
            rows, zrow = _memory_rows(g)
            row = _iota((rows, 128), 0)
            lane = _iota((rows, 128), 1)
            same_head = (row // DH) == (lane // DH)
            upd = _dot_nt(vgs[g], pks[g])
            keep = ((same_head & (row < used)) | (row == zrow)) & (lane < used)
            upd = jnp.where(keep, upd, 0.0)
            out.append(upd if states is None else states[g] + upd)
        return out

    def memory_retrieve(c, states, pqs):
        row8 = _iota((8, 128), 0)
        lane8 = _iota((8, 128), 1) // DH
        for g in range(NG):
            nh = _heads_in_group(g)
            rows, zrow = _memory_rows(g)
            st = states[g]
            mrows = jnp.where(_iota((rows, 128), 0) < zrow, st, 0.0)
            zrows = jnp.where(lane8 == row8, st[zrow:zrow + 1, :], 0.0)
            lhs = jnp.concatenate(
                [mrows, zrows, jnp.zeros((8, 128), F32)], axis=0).astype(BF16)
            ret = _dot(lhs, pqs[g])
            out_rows = 128 if g < NG - 1 else nh * DH
            mem_v[c - 1, GW * g:GW * g + out_rows, :] = ret[0:out_rows, :]
            mden_v[c - 1, HPG * g:HPG * g + 8, :] = ret[rows:rows + 8, :]

    def route():
        r = r_v[0:NSEG, :]
        idx = _iota((NSEG, L), 0) * L + _iota((NSEG, L), 1)
        m1 = jnp.max(r)
        i1 = jnp.clip(jnp.min(jnp.where(r == m1, idx, S)), 0, S - 1)
        r2 = jnp.where(idx == i1, -jnp.inf, r)
        m2 = jnp.max(r2)
        i2 = jnp.clip(jnp.min(jnp.where(r2 == m2, idx, S)), 0, S - 1)
        idx_s[0] = i1
        idx_s[1] = i2
        rsel_s[0] = m1
        rsel_s[1] = m2
        row16 = _iota((16, 128), 0)
        lane16 = _iota((16, 128), 1)
        xs = None
        for t, i in enumerate((i1, i2)):
            seg = i // L
            off = i - seg * L
            base = pl.multiple_of((off // 128) * 128, 128)
            cols = _unpack(xn_v[_rows(seg, D // 2), pl.ds(base, 128)])
            pick = jnp.where((row16 == t) & (lane16 == off - base), 1.0, 0.0)
            part = _dot_nt(pick.astype(BF16), cols)
            xs = part if xs is None else xs + part
        xs_v[...] = _pack(xs)
        y_v[...] = jnp.zeros(y_v.shape, F32)

    def ffn_in_tile(w_ref, tile):
        return _dot(_unpack(xs_v[...]), w_ref[:, 128 * tile:128 * (tile + 1)])

    def store_ffn_hidden(gates, ups):
        for tile, (gt, up) in enumerate(zip(gates, ups)):
            gt = _round_bf16(gt)
            hid = _round_bf16(_round_bf16(gt * jax.nn.sigmoid(gt)) * _round_bf16(up))
            for t in range(2):
                hid_v[t, tile] = jnp.broadcast_to(hid[t:t + 1, :], (8, 128))

    def project_last_with_ffn():
        c = NSEG - 1
        xn = _unpack(xn_v[_rows(c, D // 2), :])
        router = _dot(_unpack(wall[RROW // 2:PROWS // 2, :]), xn)
        r_v[c:c + 1, :] = _round_bf16(router[0:1, :])
        todo = [(w_ref, tile) for w_ref in (wg_v, wu_v) for tile in range(FF // 128)]
        done = []
        blocks = []
        for i, r in enumerate(range(0, RROW // 2, PBLOCK // 2)):
            if i == FFN_FIRST_BLOCK:
                route()
            lhs = _unpack(wall[r:min(r + PBLOCK // 2, RROW // 2), :])
            tiles = []
            for n in range(NQT):
                tiles.append(_dot(lhs, xn[:, 128 * n:128 * (n + 1)]))
                if i >= FFN_FIRST_BLOCK:
                    for _ in range(min(FFN_PATTERN[n % len(FFN_PATTERN)], len(todo))):
                        done.append(ffn_in_tile(*todo.pop(0)))
            blocks.append(jnp.concatenate(tiles, axis=1))
        pt = jnp.concatenate(blocks + [router], axis=0)
        return pt, todo, done

    def ffn_down_chained():
        base = pl.multiple_of(step * (FT * 128), 128)
        hid = [[hid_v[t, step * FT + tile] for tile in range(FT)] for t in range(2)]
        link = [None, None]
        for b in range(D // 8):
            acc = [None, None]
            for tile in range(FT):
                w = wd_v[8 * b:8 * b + 8, pl.ds(base + 128 * tile, 128)].astype(F32)
                for t in range(2):
                    pr = w * hid[t][tile]
                    if tile > 0:
                        acc[t] = acc[t] + pr
                    else:
                        acc[t] = pr if link[t] is None else pr + nothing(link[t])
            for t in range(2):
                rows = slice(8 * b, 8 * b + 8)
                y_v[t, rows, :] = y_v[t, rows, :] + acc[t]
                link[t] = acc[t]

    def ffn_down_looped():
        def down(tile, carry):
            col = step * FT + tile
            w = wd_v[:, pl.ds(pl.multiple_of(128 * col, 128), 128)].astype(F32)
            for t in range(2):
                y_v[t] = y_v[t] + w * hid_v[t, col][0:1, :]
            return carry

        lax.fori_loop(0, FT, down, 0)

    def masked_q_bits(g, hp, j):
        rid = _iota((64, 128), 0)
        mask = (rid >= (DH // 2) * hp) & (rid < (DH // 2) * (hp + 1))
        return jnp.where(mask, qt_v[_rows(step * NG + g, 64), 128 * j:128 * (j + 1)],
                         jnp.uint32(0))

    def keys(g, lo, hi):
        first = pl.multiple_of((step * NG + g) * (L // 2) + lo // 2, 8)
        return _unpack(k_v[pl.ds(first, (hi - lo) // 2), :])

    def causal_scores(g, hp, j):
        nk = 128 * (j + 1)
        st = _dot(keys(g, 0, nk), _unpack(masked_q_bits(g, hp, j)))
        diag = st[nk - 128:, :] + bias_v[...]
        return diag if j == 0 else jnp.concatenate([st[:nk - 128, :], diag], axis=0)

    def head_output(h, j, p, keep):
        o = _dot(_unpack(vt_v[_rows(step * H + h, 16), 0:128 * (j + 1)]), p)
        den = o[DH:DH + 1, :]
        inv = pl.reciprocal(den, approx=True)
        inv = inv * (2.0 - den * inv)
        return o[0:24, :] * (keep * inv)

    def single_probs(h, j):
        return jnp.exp2(causal_scores(*divmod(h, HPG), j)).astype(BF16)

    def pair_probs(pairs, j, flip):
        low = _iota((64, 128), 1) < 64
        qa, qb = {}, {}
        for h in pairs:
            g, hp = divmod(h, HPG)
            qa[h] = masked_q_bits(g, hp, j)
            qb[h] = pltpu.roll(masked_q_bits(g, hp + 1, j), 64, 1)
        off = {}
        if j > 0:
            for h in pairs:
                g = h // HPG
                for hh, q in ((h, qa[h]), (h + 1, qb[h])):
                    off[hh] = jnp.exp2(_dot(keys(g, 0, 128 * j), _unpack(q)))
        early, late = {}, {}
        for h in pairs:
            g = h // HPG
            k0 = 128 * j
            for which in ((0, 1) if flip else (1, 0)):
                if which == 0:
                    early[h] = _dot(keys(g, k0, k0 + 64),
                                    _unpack(jnp.where(low, qa[h], qb[h])))
                else:
                    late[h] = _dot(keys(g, k0, k0 + 128),
                                   _unpack(jnp.where(low, qb[h], qa[h])))
        probs = {}
        for h in pairs:
            p1 = jnp.exp2(early[h] + half_v[0])
            p2 = jnp.exp2(late[h][0:64, :])
            bottom = late[h][64:128, :]
            pa = jnp.concatenate(
                [jnp.where(low, p1, p2), jnp.exp2(bottom + half_v[1])], axis=0)
            pb = jnp.concatenate(
                [jnp.where(low, p2, p1), jnp.exp2(bottom + half_v[2])], axis=0)
            for hh, pd in ((h, pa), (h + 1, pb)):
                full = pd if j == 0 else jnp.concatenate([off[hh], pd], axis=0)
                probs[hh] = full.astype(BF16)
        return probs

    def quad_probs(h0, j, turn):
        g, hp = divmod(h0, HPG)
        q = [masked_q_bits(g, hp, j)] + [
            pltpu.roll(masked_q_bits(g, hp + x, j), 32 * x, 1) for x in range(1, 4)]
        off = [jnp.exp2(_dot(keys(g, 0, 128 * j), _unpack(q[x]))) for x in range(4)
               ] if j > 0 else None
        lane_q = _iota((64, 128), 1) // 32
        k0 = 128 * j
        e = [None] * 4
        for i in [(turn + n) % 4 for n in range(4)]:
            w = q[(3 - i) % 4]
            for lam in range(3):
                w = jnp.where(lane_q == lam, q[(lam - i) % 4], w)
            st = _dot(keys(g, k0, k0 + 32 * (i + 1)), _unpack(w))
            last = st[32 * i:, :] + quarter_v[...]
            st = last if i == 0 else jnp.concatenate([st[:32 * i, :], last], axis=0)
            e[i] = jnp.exp2(st)
        lane_q = _iota((32, 128), 1) // 32
        probs = {}
        for x in range(4):
            blocks = []
            for r in range(4):
                blk = e[0][0:32, :] if r == 0 else jnp.zeros((32, 128), F32)
                for i in range(max(r, 1), 4):
                    blk = jnp.where(lane_q == (i + x) % 4, e[i][32 * r:32 * (r + 1), :], blk)
                blocks.append(blk)
            full = jnp.concatenate(([off[x]] if j > 0 else []) + blocks, axis=0)
            probs[h0 + x] = full.astype(BF16)
        return probs

    def attention_bounded():
        quads = [g * HPG for g in range(NG)]
        pairs = [g * HPG + 4 for g in range(NG - 1)]
        singles = [g * HPG + 6 for g in range(NG - 1)]
        rotation = {h + x: 32 * x for h in quads for x in range(4)}
        rotation.update({h + 1: 64 for h in pairs})
        waves = [("quad", h, j) for h in quads for j in range(NQT)]
        waves += [("pairs", pairs[i:i + 2], j) for i in (0, 2) for j in range(NQT)]
        waves += [("singles", singles, j) for j in range(NQT)]

        def scores(w):
            kind, grp, j = waves[w]
            if kind == "quad":
                return quad_probs(grp, j, w % 4)
            if kind == "pairs":
                return pair_probs(grp, j, w % 2 == 1)
            return {h: single_probs(h, j) for h in grp}

        def values(w, probs):
            j = waves[w][2]
            for h, p in probs.items():
                o = head_output(h, j, p, 1.0 - gate_v[h:h + 1, :])
                if rotation.get(h, 0):
                    o = pltpu.roll(o, 128 - rotation[h], 1)
                ot_v[step, DH * h:DH * (h + 1), 128 * j:128 * (j + 1)] = o[0:DH, :]

        pending = {}
        for w in range(len(waves) + LOOKAHEAD):
            if w < len(waves):
                pending[w] = scores(w)
            if w >= LOOKAHEAD:
                values(w - LOOKAHEAD, pending.pop(w - LOOKAHEAD))
        ffn_down_chained()

    def attention_max_shifted():
        def one_tile(item, carry):
            h = item // NQT
            j = item - h * NQT
            g = h // HPG
            hp = h - g * HPG
            cols = pl.ds(pl.multiple_of(128 * j, 128), 128)
            rid = _iota((64, 128), 0)
            mask = (rid >= (DH // 2) * hp) & (rid < (DH // 2) * (hp + 1))
            qm = jnp.where(mask, qt_v[_rows(step * NG + g, 64), cols], jnp.uint32(0))
            st = _dot(keys(g, 0, L), _unpack(qm))
            future = _iota((L, 128), 0) > 128 * j + _iota((L, 128), 1)
            st = jnp.where(future, NEG, st)
            p = jnp.exp2(st - jnp.max(st, axis=0, keepdims=True)).astype(BF16)
            keep = 1.0 - gate_v[pl.ds(h, 1), :]
            oh_v[h, :, cols] = head_output(h, NQT - 1, p, keep)
            return carry

        def compact(q, carry):
            rows = jnp.concatenate([oh_v[4 * q + k, 0:DH, :] for k in range(4)], axis=0)
            ot_v[step, pl.ds(pl.multiple_of(4 * DH * q, 8), 4 * DH), :] = rows
            return carry

        lax.fori_loop(0, H * NQT, one_tile, 0)
        lax.fori_loop(0, H // 4, compact, 0)
        ffn_down_looped()

    def routed_columns():
        ys = []
        for t in range(2):
            y = _round_bf16(jnp.sum(y_v[t], axis=1, keepdims=True))
            rsel = jnp.full((1, 1), rsel_s[t], F32)
            ys.append(_round_bf16(y * _round_bf16(jax.nn.sigmoid(rsel))))
        return ys

    def output_copy(seg, n):
        return pltpu.make_async_copy(
            out_v.at[pl.ds(seg * D, D), pl.ds(128 * n, 128)],
            o_hbm.at[:, pl.ds(seg * L + 128 * n, 128)],
            out_sems.at[NQT * seg + n])

    def output_projection(seg, ys):
        heads_out = ot_v[seg, 0:D, :]
        if seg > 0:
            gates = jnp.concatenate([gate_v[...]] * NQT, axis=1)
            scale = gates / (mden_v[seg - 1, 0:H, :] + 1e-6)
            pieces = []
            for b in range(D // 8):
                h0, h1 = (8 * b) // DH, (8 * b + 7) // DH
                sc = scale[h0:h0 + 1, :]
                if h1 != h0:
                    first = _iota((8, L), 0) < DH * h1 - 8 * b
                    sc = jnp.where(first, sc, scale[h1:h1 + 1, :])
                pieces.append(mem_v[seg - 1, 8 * b:8 * b + 8, :] * sc)
            heads_out = heads_out + jnp.concatenate(pieces, axis=0)
        attn = _dot(_unpack(wot[...]), heads_out.astype(BF16))
        base = x_v[seg].astype(F32) + attn
        xn = _unpack(xn_v[_rows(seg, D // 2), :]).astype(F32)
        col = seg * L + _iota((1, L), 1)
        upd = (jnp.where(col == idx_s[0], ys[0], 0.0)
               + jnp.where(col == idx_s[1], ys[1], 0.0))
        result = base + (xn + upd)
        for n in range(NQT):
            cols = slice(128 * n, 128 * (n + 1))
            out_v[seg * D:(seg + 1) * D, cols] = result[:, cols].astype(BF16)
            output_copy(seg, n).start()

    col_blocks = [(c0, min(128, D - c0)) for c0 in range(0, D, 128)]

    def transpose_block(w_v, section, c0, n):
        r0 = (section * D + c0) // 2
        wall[r0:r0 + n // 2, :] = pltpu.bitcast(w_v[:, c0:c0 + n].T, U32)

    def project_block(section, c0, n, xn):
        r0 = (section * D + c0) // 2
        last = section == 2 and c0 + n == D
        hi = PROWS // 2 if last else r0 + n // 2
        return _dot(_unpack(wall[r0:hi, :]), xn)

    def query_half0(half):
        layer_norm(0, serial=False, tiles=[2 * half, 2 * half + 1])
        xn = _unpack(xn_v[0:D // 2, 256 * half:256 * (half + 1)])
        top = _dot(_unpack(wall[0:D // 4, :]), xn)
        if half == 0:
            for c0, n in col_blocks[3:]:
                transpose_block(wq_v, 0, c0, n)
        bottom = _dot(_unpack(wall[D // 4:D // 2, :]), xn)
        return jnp.concatenate([top, bottom], axis=0)

    def projections():
        qtiles = []
        for half in range(2):
            x0_copies[half].wait()
            if half == 1:
                cp_wk.wait()
            qtiles.append(query_half0(half))
        for c0, n in col_blocks:
            transpose_block(wk_v, 1, c0, n)
        parts = [jnp.concatenate(qtiles, axis=1)]
        xn0 = _unpack(xn_v[_rows(0, D // 2), :])
        parts += [project_block(1, c0, n, xn0) for c0, n in col_blocks[:EARLY_K]]
        cp_wv.wait()
        x_copies[1].wait()
        xn0 = _unpack(xn_v[_rows(0, D // 2), :])
        parts += [project_block(1, c0, n, xn0) for c0, n in col_blocks[EARLY_K:]]
        for c0, n in col_blocks:
            transpose_block(wv_v, 2, c0, n)
            parts.append(project_block(2, c0, n, xn0))
        layer_norm(1)
        _, pk, vg = store_qkv(0, jnp.concatenate(parts, axis=0))
        x_copies[2].wait()
        x_copies[3].wait()
        cp_wo.wait()

        layer_norm(2)
        pt = project(1)
        wot[...] = pltpu.bitcast(wo_v[...].T, U32)
        state1 = memory_update(None, pk, vg)
        pq1, pk, vg = store_qkv(1, pt)
        layer_norm(3)
        pt = project(2)
        state2 = memory_update(state1, pk, vg)
        pq2, pk, vg = store_qkv(2, pt)
        cp_wg.wait()
        cp_wu.wait()
        pt, todo, done = project_last_with_ffn()
        pq3, _, _ = store_qkv(3, pt)
        state3 = memory_update(state2, pk, vg)
        done += [ffn_in_tile(*item) for item in todo]
        store_ffn_hidden(done[:FF // 128], done[FF // 128:])
        memory_retrieve(1, state1, pq1)
        memory_retrieve(2, state2, pq2)
        memory_retrieve(3, state3, pq3)
        record_logit_bound()
        cp_wd.wait()

    @pl.when(step == 0)
    def _():
        for cp in (cp_wq, cp_wr, cp_beta, *x0_copies, cp_wk, cp_wv, x_copies[1],
                   x_copies[2], x_copies[3], cp_wo, cp_wg, cp_wu, cp_wd):
            cp.start()
        with _scope("sc_startup"):
            cp_wr.wait()
            cp_beta.wait()
            cp_wq.wait()
            init_constants()
            for c0, n in col_blocks[:3]:
                transpose_block(wq_v, 0, c0, n)
        with _scope("sc_projections"):
            projections()

    @pl.when(step < NSEG)
    def _():
        safe = safe_s[0] == 1

        @pl.when(safe)
        def _():
            with _scope("sc_attention"):
                attention_bounded()

        @pl.when(jnp.logical_not(safe))
        def _():
            attention_max_shifted()

    @pl.when(step == NSEG)
    def _():
        with _scope("sc_outproj"):
            ys = routed_columns()
            for seg in range(NSEG):
                output_projection(seg, ys)
            for seg in range(NSEG):
                for n in range(NQT):
                    output_copy(seg, n).wait()


@jax.jit
def pallas_parallel_sum__memory_aug_infini_attn__moe_arch_mod__prompt_kernel(
    A_x: jax.Array,
    A_wq: jax.Array,
    A_wk: jax.Array,
    A_wv: jax.Array,
    A_wo: jax.Array,
    A_beta: jax.Array,
    B_x: jax.Array,
    B_w_r: jax.Array,
    B_w_gate: jax.Array,
    B_w_up: jax.Array,
    B_w_down: jax.Array,
):
    del B_x
    vm = pltpu.VMEM
    scratch = [
        vm((NSEG, D, L), BF16),
        vm((D, D), BF16),
        vm((D, D), BF16),
        vm((D, D), BF16),
        vm((D, D), BF16),
        vm((H,), BF16),
        vm((D,), BF16),
        vm((D, FF), BF16),
        vm((D, FF), BF16),
        vm((D, FF), BF16),
        vm((PROWS // 2, D), U32),
        vm((D // 2, D), U32),
        vm((NSEG * D // 2, L), U32),
        vm((NSEG * NG * 64, L), U32),
        vm((NSEG * NG * L // 2, 128), U32),
        vm((NSEG * H * 16, L), U32),
        vm((NSEG - 1, D, L), F32),
        vm((NSEG - 1, H + 8, L), F32),
        vm((8, L), F32),
        vm((8, D), U32),
        vm((2, D, 128), F32),
        vm((2, FF // 128, 8, 128), F32),
        pltpu.SMEM((2,), jnp.int32),
        pltpu.SMEM((2,), F32),
        pltpu.SMEM((1,), U32),
        pltpu.SMEM((1,), jnp.int32),
        vm((H, 128), F32),
        vm((NSEG, D, L), F32),
        vm((H, 24, L), F32),
        vm((128, 128), F32),
        vm((3, 64, 128), F32),
        vm((32, 128), F32),
        vm((NSEG * D, L), BF16),
        pltpu.SemaphoreType.DMA((NSEG * NQT,)),
        pltpu.SemaphoreType.DMA((NSEG + 9 + 2,)),
    ]
    hbm = pl.BlockSpec(memory_space=pltpu.HBM)
    xt = jnp.transpose(A_x.reshape(S, D))
    out_t = pl.pallas_call(
        _kernel,
        grid=(NSEG + 1,),
        in_specs=[hbm] * 10,
        out_specs=hbm,
        out_shape=jax.ShapeDtypeStruct((D, S), BF16),
        scratch_shapes=scratch,
        compiler_params=pltpu.CompilerParams(
            dimension_semantics=("arbitrary",),
            vmem_limit_bytes=110 * 1024 * 1024,
        ),
        name="infini_moe",
    )(xt, A_wq, A_wk, A_wv, A_wo, A_beta, B_w_r, B_w_gate, B_w_up,
      jnp.transpose(B_w_down))
    return jnp.transpose(out_t).reshape(1, S, D)
```

```python
import contextlib

import jax
import jax.numpy as jnp
from jax import lax
from jax.experimental import pallas as pl
from jax.experimental.pallas import tpu as pltpu

S = 2048
D = 576
H = 32
DH = 18
NSEG = 4
L = 512
FF = 4608
HPG = 4
NG = H // HPG
GW = HPG * DH
MROWS = GW + 8
QROWS = 40
NQT = L // 128
PROWS = 3 * D + 16
RROW = 3 * D
EARLY_K = 1
FFN_FIRST_BLOCK = 3
FFN_PATTERN = (1, 2)
LOOKAHEAD = 2
PBLOCK = 128
FT = FF // 128 // NSEG
LOG2E = 1.4426950408889634
QSCALE = DH ** -0.5 * LOG2E
NEG = -1e30
LN_EPS = 1.0013580322265625e-05
F32 = jnp.float32
BF16 = jnp.bfloat16
U32 = jnp.uint32

PROFILE_SCOPES = False

_NN = (((1,), (0,)), ((), ()))
_NT = (((1,), (1,)), ((), ()))


def _scope(name):
    return jax.named_scope(name) if PROFILE_SCOPES else contextlib.nullcontext()


def _dot(a, b):
    return lax.dot_general(a, b, _NN, preferred_element_type=F32)


def _dot_nt(a, b):
    return lax.dot_general(a, b, _NT, preferred_element_type=F32)


def _iota(shape, dim):
    return lax.broadcasted_iota(jnp.int32, shape, dim)


def _round_bf16(v):
    return v.astype(BF16).astype(F32)


def _pack(v):
    return pltpu.bitcast(v.astype(BF16), U32)


def _unpack(u):
    return pltpu.bitcast(u, BF16)


def _rows(index, size):
    if isinstance(index, int):
        return slice(index * size, (index + 1) * size)
    return pl.ds(pl.multiple_of(index * size, 8), size)


def _phi(t):
    return jnp.where(t > 0, t + 1.0, jnp.exp(t))


def _kernel(x_hbm, wq_hbm, wk_hbm, wv_hbm, wo_hbm, beta_hbm, wr_hbm,
            wg_hbm, wu_hbm, wd_hbm,
            o_hbm,
            x_v, wq_v, wk_v, wv_v, wo_v, beta_v, wr_v, wg_v, wu_v, wd_v,
            wall, wot, xn_v, qt_v, k_v, vt_v, mem_v, mden_v,
            r_v, xs_v, y_v, hid_v, idx_s, rsel_s, zero_s, safe_s,
            gate_v, ot_v, oh_v, quarter_v, out_v, out_sems,
            sems):
    step = pl.program_id(0)

    x_copies = [None] + [
        pltpu.make_async_copy(x_hbm.at[:, pl.ds(c * L, L)], x_v.at[c], sems.at[c])
        for c in range(1, NSEG)
    ]
    x0_copies = [
        pltpu.make_async_copy(x_hbm.at[:, pl.ds(256 * n, 256)],
                              x_v.at[0, :, pl.ds(256 * n, 256)],
                              sems.at[NSEG + 9 + n])
        for n in range(2)
    ]
    pairs = [(wq_hbm, wq_v), (wk_hbm, wk_v), (wv_hbm, wv_v), (wo_hbm, wo_v),
             (beta_hbm, beta_v), (wr_hbm, wr_v),
             (wg_hbm, wg_v), (wu_hbm, wu_v), (wd_hbm, wd_v)]
    (cp_wq, cp_wk, cp_wv, cp_wo, cp_beta, cp_wr, cp_wg, cp_wu, cp_wd) = [
        pltpu.make_async_copy(src, dst, sems.at[NSEG + i])
        for i, (src, dst) in enumerate(pairs)
    ]

    def nothing(v):
        return pltpu.bitcast(pltpu.bitcast(v, U32) & zero_s[0], F32)

    def layer_norm(c, serial=True, tiles=range(NQT)):
        link = None
        for n in tiles:
            cols = slice(128 * n, 128 * (n + 1))
            pivot = x_v[c, 0:16, cols].astype(F32)[0:1, :]
            pivot8 = jnp.broadcast_to(pivot, (8, 128))
            shift = pivot8
            s1 = s2 = None
            for i in range(D // 16):
                last = s1 if s1 is not None else link
                if serial and last is not None:
                    shift = pivot8 + nothing(last)
                x16 = x_v[c, 16 * i:16 * i + 16, cols].astype(F32)
                for k in range(2):
                    d = x16[8 * k:8 * k + 8, :] - shift
                    s1 = d if s1 is None else s1 + d
                    s2 = d * d if s2 is None else s2 + d * d
            dmean = jnp.sum(s1, axis=0, keepdims=True) * (1.0 / D)
            dsq = jnp.sum(s2, axis=0, keepdims=True) * (1.0 / D)
            var = jnp.maximum(dsq - dmean * dmean, 0.0)
            sd = _round_bf16(jnp.sqrt(_round_bf16(_round_bf16(var) + LN_EPS)))
            mean8 = jnp.broadcast_to(_round_bf16(pivot + dmean), (8, 128))
            inv8 = jnp.broadcast_to(1.0 / sd, (8, 128))
            center = mean8
            for i in range(D // 32):
                if serial and i > 0:
                    center = mean8 + nothing(link)
                x32 = x_v[c, 32 * i:32 * i + 32, cols].astype(F32)
                z = [(x32[8 * k:8 * k + 8, :] - center) * inv8 for k in range(4)]
                link = z[3]
                r0 = c * (D // 2) + 16 * i
                xn_v[r0:r0 + 16, cols] = _pack(jnp.concatenate(z, axis=0))

    def init_constants():
        gate = jax.nn.sigmoid(beta_v[...].astype(F32).reshape(1, H))
        on_diag = _iota((H, H), 0) == _iota((H, H), 1)
        gcol = jnp.sum(jnp.where(on_diag, gate, 0.0), axis=1, keepdims=True)
        gate_v[...] = jnp.broadcast_to(gcol, (H, 128))
        zero_s[0] = jnp.uint32(0)
        quarter_v[...] = jnp.where(
            _iota((32, 128), 0) > (_iota((32, 128), 1) & 31), NEG, 0.0)
        router = jnp.broadcast_to(wr_v[...].astype(F32).reshape(1, D), (16, D))
        wall[RROW // 2:PROWS // 2, :] = _pack(
            jnp.where(_iota((16, D), 0) == 0, router, 0.0))

    def project(c):
        xn = _unpack(xn_v[_rows(c, D // 2), :])
        step_rows = PBLOCK // 2
        return jnp.concatenate(
            [_dot(_unpack(wall[r:min(r + step_rows, PROWS // 2), :]), xn)
             for r in range(0, PROWS // 2, step_rows)], axis=0)

    seen = [None]

    def record_logit_bound():
        big = (seen[0] >> 30) & 1
        safe_s[0] = (jnp.max(big.astype(jnp.int32)) == 0).astype(jnp.int32)

    def store_qkv(c, pt):
        if c < NSEG - 1:
            r_v[c:c + 1, :] = _round_bf16(pt[RROW:RROW + 1, :])
        tail_row = _iota((8, L), 0)
        for h in range(H):
            base = 2 * D + DH * h
            tail = jnp.where(tail_row < DH - 16, pt[base + 16:base + 24, :],
                             jnp.where(tail_row == DH - 16, 1.0, 0.0))
            blk = jnp.concatenate(
                [pt[base:base + 16, :], tail, jnp.zeros((8, L), F32)], axis=0)
            vt_v[_rows(c * H + h, 16), :] = _pack(blk)

        pqs, pks, vgs = [], [], []
        for g in range(NG):
            qg = pt[GW * g:GW * g + 128, :]
            qs = qg[0:2 * QROWS, :] * QSCALE
            qt_v[_rows(c * NG + g, QROWS), :] = _pack(qs)
            kg = pt[D + GW * g:D + GW * g + 128, :]
            for operand in (qs, kg):
                bits = pltpu.bitcast(operand[0:GW, :], U32)
                for blk in range(0, GW, 8):
                    for col in range(0, L, 128):
                        piece = bits[blk:blk + 8, col:col + 128]
                        seen[0] = piece if seen[0] is None else seen[0] | piece
            k_v[_rows(c * NG + g, L // 2), :] = _pack(kg.T)
            pqs.append(_phi(qg).astype(BF16))
            if c < NSEG - 1:
                pks.append(_phi(kg).astype(BF16))
                lo = 2 * D + GW * g
                rid = _iota((MROWS, L), 0)
                vg = jnp.where(rid < GW, pt[lo:lo + MROWS, :],
                               jnp.where(rid == GW, 1.0, 0.0))
                vgs.append(vg.astype(BF16))
        return pqs, pks, vgs

    def memory_update(states, pks, vgs):
        row = _iota((MROWS, 128), 0)
        lane = _iota((MROWS, 128), 1)
        keep = (((row // DH) == (lane // DH)) | (row == GW)) & (row <= GW) & (lane < GW)
        out = []
        for g in range(NG):
            upd = jnp.where(keep, _dot_nt(vgs[g], pks[g]), 0.0)
            out.append(upd if states is None else states[g] + upd)
        return out

    def memory_retrieve(c, states, pqs):
        row8 = _iota((8, 128), 0)
        lane8 = _iota((8, 128), 1) // DH
        for g in range(NG):
            st = states[g]
            mrows = jnp.where(_iota((MROWS, 128), 0) < GW, st, 0.0)
            zrows = jnp.where(lane8 == row8, st[GW:GW + 1, :], 0.0)
            lhs = jnp.concatenate(
                [mrows, zrows, jnp.zeros((8, 128), F32)], axis=0).astype(BF16)
            ret = _dot(lhs, pqs[g])
            mem_v[c - 1, GW * g:GW * (g + 1), :] = ret[0:GW, :]
            mden_v[c - 1, HPG * g:HPG * g + 8, :] = ret[MROWS:MROWS + 8, :]

    def route():
        r = r_v[0:NSEG, :]
        idx = _iota((NSEG, L), 0) * L + _iota((NSEG, L), 1)
        m1 = jnp.max(r)
        i1 = jnp.clip(jnp.min(jnp.where(r == m1, idx, S)), 0, S - 1)
        r2 = jnp.where(idx == i1, -jnp.inf, r)
        m2 = jnp.max(r2)
        i2 = jnp.clip(jnp.min(jnp.where(r2 == m2, idx, S)), 0, S - 1)
        idx_s[0] = i1
        idx_s[1] = i2
        rsel_s[0] = m1
        rsel_s[1] = m2
        row16 = _iota((16, 128), 0)
        lane16 = _iota((16, 128), 1)
        xs = None
        for t, i in enumerate((i1, i2)):
            seg = i // L
            off = i - seg * L
            base = pl.multiple_of((off // 128) * 128, 128)
            cols = _unpack(xn_v[_rows(seg, D // 2), pl.ds(base, 128)])
            pick = jnp.where((row16 == t) & (lane16 == off - base), 1.0, 0.0)
            part = _dot_nt(pick.astype(BF16), cols)
            xs = part if xs is None else xs + part
        xs_v[...] = _pack(xs)
        y_v[...] = jnp.zeros(y_v.shape, F32)

    def ffn_in_tile(w_ref, tile):
        return _dot(_unpack(xs_v[...]), w_ref[:, 128 * tile:128 * (tile + 1)])

    def store_ffn_hidden(gates, ups):
        for tile, (gt, up) in enumerate(zip(gates, ups)):
            gt = _round_bf16(gt)
            hid = _round_bf16(_round_bf16(gt * jax.nn.sigmoid(gt)) * _round_bf16(up))
            for t in range(2):
                hid_v[t, tile] = jnp.broadcast_to(hid[t:t + 1, :], (8, 128))

    def project_last_with_ffn():
        c = NSEG - 1
        xn = _unpack(xn_v[_rows(c, D // 2), :])
        router = _dot(_unpack(wall[RROW // 2:PROWS // 2, :]), xn)
        r_v[c:c + 1, :] = _round_bf16(router[0:1, :])
        todo = [(w_ref, tile) for w_ref in (wg_v, wu_v) for tile in range(FF // 128)]
        done = []
        blocks = []
        for i, r in enumerate(range(0, RROW // 2, PBLOCK // 2)):
            if i == FFN_FIRST_BLOCK:
                route()
            lhs = _unpack(wall[r:min(r + PBLOCK // 2, RROW // 2), :])
            tiles = []
            for n in range(NQT):
                tiles.append(_dot(lhs, xn[:, 128 * n:128 * (n + 1)]))
                if i >= FFN_FIRST_BLOCK:
                    for _ in range(min(FFN_PATTERN[n % len(FFN_PATTERN)], len(todo))):
                        done.append(ffn_in_tile(*todo.pop(0)))
            blocks.append(jnp.concatenate(tiles, axis=1))
        pt = jnp.concatenate(blocks + [router], axis=0)
        return pt, todo, done

    def ffn_down_chained():
        base = pl.multiple_of(step * (FT * 128), 128)
        hid = [[hid_v[t, step * FT + tile] for tile in range(FT)] for t in range(2)]
        link = [None, None]
        for b in range(D // 8):
            acc = [None, None]
            for tile in range(FT):
                w = wd_v[8 * b:8 * b + 8, pl.ds(base + 128 * tile, 128)].astype(F32)
                for t in range(2):
                    pr = w * hid[t][tile]
                    if tile > 0:
                        acc[t] = acc[t] + pr
                    else:
                        acc[t] = pr if link[t] is None else pr + nothing(link[t])
            for t in range(2):
                rows = slice(8 * b, 8 * b + 8)
                y_v[t, rows, :] = y_v[t, rows, :] + acc[t]
                link[t] = acc[t]

    def ffn_down_looped():
        def down(tile, carry):
            col = step * FT + tile
            w = wd_v[:, pl.ds(pl.multiple_of(128 * col, 128), 128)].astype(F32)
            for t in range(2):
                y_v[t] = y_v[t] + w * hid_v[t, col][0:1, :]
            return carry

        lax.fori_loop(0, FT, down, 0)

    def masked_q_bits(g, hp, cols):
        rid = _iota((QROWS, 128), 0)
        mask = (rid >= (DH // 2) * hp) & (rid < (DH // 2) * (hp + 1))
        kept = jnp.where(mask, qt_v[_rows(step * NG + g, QROWS), cols], jnp.uint32(0))
        return jnp.concatenate([kept, jnp.zeros((64 - QROWS, 128), U32)], axis=0)

    def keys(g, lo, hi):
        first = pl.multiple_of((step * NG + g) * (L // 2) + lo // 2, 8)
        return _unpack(k_v[pl.ds(first, (hi - lo) // 2), :])

    def head_output(h, j, p, keep):
        o = _dot(_unpack(vt_v[_rows(step * H + h, 16), 0:128 * (j + 1)]), p)
        den = o[DH:DH + 1, :]
        inv = pl.reciprocal(den, approx=True)
        inv = inv * (2.0 - den * inv)
        return o[0:24, :] * (keep * inv)

    def group_probs(g, j, turn):
        cols = slice(128 * j, 128 * (j + 1))
        q = [masked_q_bits(g, 0, cols)] + [
            pltpu.roll(masked_q_bits(g, x, cols), 32 * x, 1) for x in range(1, 4)]
        off = [jnp.exp2(_dot(keys(g, 0, 128 * j), _unpack(q[x]))) for x in range(4)
               ] if j > 0 else None
        lane_q = _iota((64, 128), 1) // 32
        k0 = 128 * j
        e = [None] * 4
        for i in [(turn + n) % 4 for n in range(4)]:
            w = q[(3 - i) % 4]
            for lam in range(3):
                w = jnp.where(lane_q == lam, q[(lam - i) % 4], w)
            st = _dot(keys(g, k0, k0 + 32 * (i + 1)), _unpack(w))
            last = st[32 * i:, :] + quarter_v[...]
            st = last if i == 0 else jnp.concatenate([st[:32 * i, :], last], axis=0)
            e[i] = jnp.exp2(st)
        lane_q = _iota((32, 128), 1) // 32
        probs = {}
        for x in range(4):
            blocks = []
            for r in range(4):
                blk = e[0][0:32, :] if r == 0 else jnp.zeros((32, 128), F32)
                for i in range(max(r, 1), 4):
                    blk = jnp.where(lane_q == (i + x) % 4, e[i][32 * r:32 * (r + 1), :], blk)
                blocks.append(blk)
            full = jnp.concatenate(([off[x]] if j > 0 else []) + blocks, axis=0)
            probs[HPG * g + x] = full.astype(BF16)
        return probs

    def attention_bounded():
        waves = [(g, j) for g in range(NG) for j in range(NQT)]

        def scores(w):
            return group_probs(*waves[w], w % 4)

        def values(w, probs):
            j = waves[w][1]
            for h, p in probs.items():
                o = head_output(h, j, p, 1.0 - gate_v[h:h + 1, :])
                if h % HPG:
                    o = pltpu.roll(o, 128 - 32 * (h % HPG), 1)
                ot_v[step, DH * h:DH * (h + 1), 128 * j:128 * (j + 1)] = o[0:DH, :]

        pending = {}
        for w in range(len(waves) + LOOKAHEAD):
            if w < len(waves):
                pending[w] = scores(w)
            if w >= LOOKAHEAD:
                values(w - LOOKAHEAD, pending.pop(w - LOOKAHEAD))
        ffn_down_chained()

    def attention_max_shifted():
        def one_tile(item, carry):
            h = item // NQT
            j = item - h * NQT
            g = h // HPG
            hp = h - g * HPG
            cols = pl.ds(pl.multiple_of(128 * j, 128), 128)
            st = _dot(keys(g, 0, L), _unpack(masked_q_bits(g, hp, cols)))
            future = _iota((L, 128), 0) > 128 * j + _iota((L, 128), 1)
            st = jnp.where(future, NEG, st)
            p = jnp.exp2(st - jnp.max(st, axis=0, keepdims=True)).astype(BF16)
            keep = 1.0 - gate_v[pl.ds(h, 1), :]
            oh_v[h, :, cols] = head_output(h, NQT - 1, p, keep)
            return carry

        def compact(q, carry):
            rows = jnp.concatenate([oh_v[4 * q + k, 0:DH, :] for k in range(4)], axis=0)
            ot_v[step, pl.ds(pl.multiple_of(4 * DH * q, 8), 4 * DH), :] = rows
            return carry

        lax.fori_loop(0, H * NQT, one_tile, 0)
        lax.fori_loop(0, H // 4, compact, 0)
        ffn_down_looped()

    def routed_columns():
        ys = []
        for t in range(2):
            y = _round_bf16(jnp.sum(y_v[t], axis=1, keepdims=True))
            rsel = jnp.full((1, 1), rsel_s[t], F32)
            ys.append(_round_bf16(y * _round_bf16(jax.nn.sigmoid(rsel))))
        return ys

    def output_copy(seg, n):
        return pltpu.make_async_copy(
            out_v.at[pl.ds(seg * D, D), pl.ds(128 * n, 128)],
            o_hbm.at[:, pl.ds(seg * L + 128 * n, 128)],
            out_sems.at[NQT * seg + n])

    def output_projection(seg, ys):
        heads_out = ot_v[seg, 0:D, :]
        if seg > 0:
            gates = jnp.concatenate([gate_v[...]] * NQT, axis=1)
            scale = gates / (mden_v[seg - 1, 0:H, :] + 1e-6)
            pieces = []
            for b in range(D // 8):
                h0, h1 = (8 * b) // DH, (8 * b + 7) // DH
                sc = scale[h0:h0 + 1, :]
                if h1 != h0:
                    first = _iota((8, L), 0) < DH * h1 - 8 * b
                    sc = jnp.where(first, sc, scale[h1:h1 + 1, :])
                pieces.append(mem_v[seg - 1, 8 * b:8 * b + 8, :] * sc)
            heads_out = heads_out + jnp.concatenate(pieces, axis=0)
        attn = _dot(_unpack(wot[...]), heads_out.astype(BF16))
        base = x_v[seg].astype(F32) + attn
        xn = _unpack(xn_v[_rows(seg, D // 2), :]).astype(F32)
        col = seg * L + _iota((1, L), 1)
        upd = (jnp.where(col == idx_s[0], ys[0], 0.0)
               + jnp.where(col == idx_s[1], ys[1], 0.0))
        result = base + (xn + upd)
        for n in range(NQT):
            cols = slice(128 * n, 128 * (n + 1))
            out_v[seg * D:(seg + 1) * D, cols] = result[:, cols].astype(BF16)
            output_copy(seg, n).start()

    col_blocks = [(c0, min(128, D - c0)) for c0 in range(0, D, 128)]

    def transpose_block(w_v, section, c0, n):
        r0 = (section * D + c0) // 2
        wall[r0:r0 + n // 2, :] = pltpu.bitcast(w_v[:, c0:c0 + n].T, U32)

    def project_block(section, c0, n, xn):
        r0 = (section * D + c0) // 2
        last = section == 2 and c0 + n == D
        hi = PROWS // 2 if last else r0 + n // 2
        return _dot(_unpack(wall[r0:hi, :]), xn)

    def query_half0(half):
        layer_norm(0, serial=False, tiles=[2 * half, 2 * half + 1])
        xn = _unpack(xn_v[0:D // 2, 256 * half:256 * (half + 1)])
        top = _dot(_unpack(wall[0:D // 4, :]), xn)
        if half == 0:
            for c0, n in col_blocks[3:]:
                transpose_block(wq_v, 0, c0, n)
        bottom = _dot(_unpack(wall[D // 4:D // 2, :]), xn)
        return jnp.concatenate([top, bottom], axis=0)

    def projections():
        qtiles = []
        for half in range(2):
            x0_copies[half].wait()
            if half == 1:
                cp_wk.wait()
            qtiles.append(query_half0(half))
        for c0, n in col_blocks:
            transpose_block(wk_v, 1, c0, n)
        parts = [jnp.concatenate(qtiles, axis=1)]
        xn0 = _unpack(xn_v[_rows(0, D // 2), :])
        parts += [project_block(1, c0, n, xn0) for c0, n in col_blocks[:EARLY_K]]
        cp_wv.wait()
        x_copies[1].wait()
        xn0 = _unpack(xn_v[_rows(0, D // 2), :])
        parts += [project_block(1, c0, n, xn0) for c0, n in col_blocks[EARLY_K:]]
        for c0, n in col_blocks:
            transpose_block(wv_v, 2, c0, n)
            parts.append(project_block(2, c0, n, xn0))
        layer_norm(1)
        _, pk, vg = store_qkv(0, jnp.concatenate(parts, axis=0))
        x_copies[2].wait()
        x_copies[3].wait()
        cp_wo.wait()

        layer_norm(2)
        pt = project(1)
        wot[...] = pltpu.bitcast(wo_v[...].T, U32)
        state1 = memory_update(None, pk, vg)
        pq1, pk, vg = store_qkv(1, pt)
        layer_norm(3)
        pt = project(2)
        state2 = memory_update(state1, pk, vg)
        pq2, pk, vg = store_qkv(2, pt)
        cp_wg.wait()
        cp_wu.wait()
        pt, todo, done = project_last_with_ffn()
        pq3, _, _ = store_qkv(3, pt)
        state3 = memory_update(state2, pk, vg)
        done += [ffn_in_tile(*item) for item in todo]
        store_ffn_hidden(done[:FF // 128], done[FF // 128:])
        memory_retrieve(1, state1, pq1)
        memory_retrieve(2, state2, pq2)
        memory_retrieve(3, state3, pq3)
        record_logit_bound()
        cp_wd.wait()

    @pl.when(step == 0)
    def _():
        for cp in (cp_wq, cp_wr, cp_beta, *x0_copies, cp_wk, cp_wv, x_copies[1],
                   x_copies[2], x_copies[3], cp_wo, cp_wg, cp_wu, cp_wd):
            cp.start()
        with _scope("sc_startup"):
            cp_wr.wait()
            cp_beta.wait()
            cp_wq.wait()
            init_constants()
            for c0, n in col_blocks[:3]:
                transpose_block(wq_v, 0, c0, n)
        with _scope("sc_projections"):
            projections()

    @pl.when(step < NSEG)
    def _():
        safe = safe_s[0] == 1

        @pl.when(safe)
        def _():
            with _scope("sc_attention"):
                attention_bounded()

        @pl.when(jnp.logical_not(safe))
        def _():
            attention_max_shifted()

    @pl.when(step == NSEG)
    def _():
        with _scope("sc_outproj"):
            ys = routed_columns()
            for seg in range(NSEG):
                output_projection(seg, ys)
            for seg in range(NSEG):
                for n in range(NQT):
                    output_copy(seg, n).wait()


@jax.jit
def pallas_parallel_sum__memory_aug_infini_attn__moe_arch_mod__prompt_kernel(
    A_x: jax.Array,
    A_wq: jax.Array,
    A_wk: jax.Array,
    A_wv: jax.Array,
    A_wo: jax.Array,
    A_beta: jax.Array,
    B_x: jax.Array,
    B_w_r: jax.Array,
    B_w_gate: jax.Array,
    B_w_up: jax.Array,
    B_w_down: jax.Array,
):
    del B_x
    vm = pltpu.VMEM
    scratch = [
        vm((NSEG, D, L), BF16),
        vm((D, D), BF16),
        vm((D, D), BF16),
        vm((D, D), BF16),
        vm((D, D), BF16),
        vm((H,), BF16),
        vm((D,), BF16),
        vm((D, FF), BF16),
        vm((D, FF), BF16),
        vm((D, FF), BF16),
        vm((PROWS // 2, D), U32),
        vm((D // 2, D), U32),
        vm((NSEG * D // 2, L), U32),
        vm((NSEG * NG * QROWS, L), U32),
        vm((NSEG * NG * L // 2, 128), U32),
        vm((NSEG * H * 16, L), U32),
        vm((NSEG - 1, D, L), F32),
        vm((NSEG - 1, H + 8, L), F32),
        vm((8, L), F32),
        vm((8, D), U32),
        vm((2, D, 128), F32),
        vm((2, FF // 128, 8, 128), F32),
        pltpu.SMEM((2,), jnp.int32),
        pltpu.SMEM((2,), F32),
        pltpu.SMEM((1,), U32),
        pltpu.SMEM((1,), jnp.int32),
        vm((H, 128), F32),
        vm((NSEG, D, L), F32),
        vm((H, 24, L), F32),
        vm((32, 128), F32),
        vm((NSEG * D, L), BF16),
        pltpu.SemaphoreType.DMA((NSEG * NQT,)),
        pltpu.SemaphoreType.DMA((NSEG + 9 + 2,)),
    ]
    hbm = pl.BlockSpec(memory_space=pltpu.HBM)
    xt = jnp.transpose(A_x.reshape(S, D))
    out_t = pl.pallas_call(
        _kernel,
        grid=(NSEG + 1,),
        in_specs=[hbm] * 10,
        out_specs=hbm,
        out_shape=jax.ShapeDtypeStruct((D, S), BF16),
        scratch_shapes=scratch,
        compiler_params=pltpu.CompilerParams(
            dimension_semantics=("arbitrary",),
            vmem_limit_bytes=110 * 1024 * 1024,
        ),
        name="infini_moe",
    )(xt, A_wq, A_wk, A_wv, A_wo, A_beta, B_w_r, B_w_gate, B_w_up,
      jnp.transpose(B_w_down))
    return jnp.transpose(out_t).reshape(1, S, D)
```

```python
import contextlib

import jax
import jax.numpy as jnp
from jax import lax
from jax.experimental import pallas as pl
from jax.experimental.pallas import tpu as pltpu

S = 2048
D = 576
H = 32
DH = 18
NSEG = 4
L = 512
FF = 4608
HPG = 4
NG = H // HPG
GW = HPG * DH
MROWS = GW + 8
QROWS = 40
NQT = L // 128
PROWS = 3 * D + 16
RROW = 3 * D
EARLY_K = 1
FFN_FIRST_BLOCK = 2
FFN_PATTERN = (1, 2)
LOOKAHEAD = 2
PBLOCK = 128
FT = FF // 128 // NSEG
LOG2E = 1.4426950408889634
QSCALE = DH ** -0.5 * LOG2E
NEG = -1e30
LN_EPS = 1.0013580322265625e-05
F32 = jnp.float32
BF16 = jnp.bfloat16
U32 = jnp.uint32

PROFILE_SCOPES = False

_NN = (((1,), (0,)), ((), ()))
_NT = (((1,), (1,)), ((), ()))


def _scope(name):
    return jax.named_scope(name) if PROFILE_SCOPES else contextlib.nullcontext()


def _dot(a, b):
    return lax.dot_general(a, b, _NN, preferred_element_type=F32)


def _dot_nt(a, b):
    return lax.dot_general(a, b, _NT, preferred_element_type=F32)


def _iota(shape, dim):
    return lax.broadcasted_iota(jnp.int32, shape, dim)


def _round_bf16(v):
    return v.astype(BF16).astype(F32)


def _pack(v):
    return pltpu.bitcast(v.astype(BF16), U32)


def _unpack(u):
    return pltpu.bitcast(u, BF16)


def _rows(index, size):
    if isinstance(index, int):
        return slice(index * size, (index + 1) * size)
    return pl.ds(pl.multiple_of(index * size, 8), size)


def _phi(t):
    return jnp.where(t > 0, t + 1.0, jnp.exp(t))


def _kernel(x_hbm, wq_hbm, wk_hbm, wv_hbm, wo_hbm, beta_hbm, wr_hbm,
            wg_hbm, wu_hbm, wd_hbm,
            o_hbm,
            x_v, wq_v, wk_v, wv_v, wo_v, beta_v, wr_v, wg_v, wu_v, wd_v,
            wall, wot, xn_v, qt_v, k_v, vt_v, mem_v, mden_v,
            r_v, xs_v, y_v, hid_v, idx_s, rsel_s, zero_s, safe_s,
            gate_v, ot_v, oh_v, quarter_v, out_v, out_sems,
            sems):
    step = pl.program_id(0)

    x_copies = [None] + [
        pltpu.make_async_copy(x_hbm.at[:, pl.ds(c * L, L)], x_v.at[c], sems.at[c])
        for c in range(1, NSEG)
    ]
    x0_copies = [
        pltpu.make_async_copy(x_hbm.at[:, pl.ds(256 * n, 256)],
                              x_v.at[0, :, pl.ds(256 * n, 256)],
                              sems.at[NSEG + 9 + n])
        for n in range(2)
    ]
    pairs = [(wq_hbm, wq_v), (wk_hbm, wk_v), (wv_hbm, wv_v), (wo_hbm, wo_v),
             (beta_hbm, beta_v), (wr_hbm, wr_v),
             (wg_hbm, wg_v), (wu_hbm, wu_v), (wd_hbm, wd_v)]
    (cp_wq, cp_wk, cp_wv, cp_wo, cp_beta, cp_wr, cp_wg, cp_wu, cp_wd) = [
        pltpu.make_async_copy(src, dst, sems.at[NSEG + i])
        for i, (src, dst) in enumerate(pairs)
    ]

    def nothing(v):
        return pltpu.bitcast(pltpu.bitcast(v, U32) & zero_s[0], F32)

    def layer_norm(c, serial=True, tiles=range(NQT)):
        link = None
        for n in tiles:
            cols = slice(128 * n, 128 * (n + 1))
            pivot = x_v[c, 0:16, cols].astype(F32)[0:1, :]
            pivot8 = jnp.broadcast_to(pivot, (8, 128))
            shift = pivot8
            s1 = s2 = None
            for i in range(D // 16):
                last = s1 if s1 is not None else link
                if serial and last is not None:
                    shift = pivot8 + nothing(last)
                x16 = x_v[c, 16 * i:16 * i + 16, cols].astype(F32)
                for k in range(2):
                    d = x16[8 * k:8 * k + 8, :] - shift
                    s1 = d if s1 is None else s1 + d
                    s2 = d * d if s2 is None else s2 + d * d
            dmean = jnp.sum(s1, axis=0, keepdims=True) * (1.0 / D)
            dsq = jnp.sum(s2, axis=0, keepdims=True) * (1.0 / D)
            var = jnp.maximum(dsq - dmean * dmean, 0.0)
            sd = _round_bf16(jnp.sqrt(_round_bf16(_round_bf16(var) + LN_EPS)))
            mean8 = jnp.broadcast_to(_round_bf16(pivot + dmean), (8, 128))
            inv8 = jnp.broadcast_to(1.0 / sd, (8, 128))
            center = mean8
            for i in range(D // 32):
                if serial and i > 0:
                    center = mean8 + nothing(link)
                x32 = x_v[c, 32 * i:32 * i + 32, cols].astype(F32)
                z = [(x32[8 * k:8 * k + 8, :] - center) * inv8 for k in range(4)]
                link = z[3]
                r0 = c * (D // 2) + 16 * i
                xn_v[r0:r0 + 16, cols] = _pack(jnp.concatenate(z, axis=0))

    def init_constants():
        gate = jax.nn.sigmoid(beta_v[...].astype(F32).reshape(1, H))
        on_diag = _iota((H, H), 0) == _iota((H, H), 1)
        gcol = jnp.sum(jnp.where(on_diag, gate, 0.0), axis=1, keepdims=True)
        gate_v[...] = jnp.broadcast_to(gcol, (H, 128))
        zero_s[0] = jnp.uint32(0)
        quarter_v[...] = jnp.where(
            _iota((32, 128), 0) > (_iota((32, 128), 1) & 31), NEG, 0.0)
        router = jnp.broadcast_to(wr_v[...].astype(F32).reshape(1, D), (16, D))
        wall[RROW // 2:PROWS // 2, :] = _pack(
            jnp.where(_iota((16, D), 0) == 0, router, 0.0))

    def project(c):
        xn = _unpack(xn_v[_rows(c, D // 2), :])
        step_rows = PBLOCK // 2
        return jnp.concatenate(
            [_dot(_unpack(wall[r:min(r + step_rows, PROWS // 2), :]), xn)
             for r in range(0, PROWS // 2, step_rows)], axis=0)

    seen = [None]

    def record_logit_bound():
        big = (seen[0] >> 30) & 1
        safe_s[0] = (jnp.max(big.astype(jnp.int32)) == 0).astype(jnp.int32)

    def feature_map(window):
        return jnp.concatenate(
            [_phi(window[0:MROWS, :]), jnp.zeros((128 - MROWS, L), F32)],
            axis=0).astype(BF16)

    def store_qkv(c, pt):
        if c < NSEG - 1:
            r_v[c:c + 1, :] = _round_bf16(pt[RROW:RROW + 1, :])
        tail_row = _iota((8, L), 0)
        for h in range(H):
            base = 2 * D + DH * h
            tail = jnp.where(tail_row < DH - 16, pt[base + 16:base + 24, :],
                             jnp.where(tail_row == DH - 16, 1.0, 0.0))
            blk = jnp.concatenate(
                [pt[base:base + 16, :], tail, jnp.zeros((8, L), F32)], axis=0)
            vt_v[_rows(c * H + h, 16), :] = _pack(blk)

        pqs, pks, vgs = [], [], []
        for g in range(NG):
            qg = pt[GW * g:GW * g + 2 * QROWS, :]
            qs = qg * QSCALE
            qt_v[_rows(c * NG + g, QROWS), :] = _pack(qs)
            kg = pt[D + GW * g:D + GW * g + 128, :]
            for operand in (qs, kg):
                bits = pltpu.bitcast(operand[0:GW, :], U32)
                for blk in range(0, GW, 8):
                    for col in range(0, L, 128):
                        piece = bits[blk:blk + 8, col:col + 128]
                        seen[0] = piece if seen[0] is None else seen[0] | piece
            k_v[_rows(c * NG + g, L // 2), :] = _pack(kg.T)
            pqs.append(feature_map(qg))
            if c < NSEG - 1:
                pks.append(feature_map(kg))
                lo = 2 * D + GW * g
                rid = _iota((MROWS, L), 0)
                vg = jnp.where(rid < GW, pt[lo:lo + MROWS, :],
                               jnp.where(rid == GW, 1.0, 0.0))
                vgs.append(vg.astype(BF16))
        return pqs, pks, vgs

    def memory_update(states, pks, vgs):
        row = _iota((MROWS, 128), 0)
        lane = _iota((MROWS, 128), 1)
        keep = (((row // DH) == (lane // DH)) | (row == GW)) & (row <= GW) & (lane < GW)
        out = []
        for g in range(NG):
            upd = jnp.where(keep, _dot_nt(vgs[g], pks[g]), 0.0)
            out.append(upd if states is None else states[g] + upd)
        return out

    def memory_retrieve(c, states, pqs):
        row8 = _iota((8, 128), 0)
        lane8 = _iota((8, 128), 1) // DH
        for g in range(NG):
            st = states[g]
            mrows = jnp.where(_iota((MROWS, 128), 0) < GW, st, 0.0)
            zrows = jnp.where(lane8 == row8, st[GW:GW + 1, :], 0.0)
            lhs = jnp.concatenate(
                [mrows, zrows, jnp.zeros((8, 128), F32)], axis=0).astype(BF16)
            ret = _dot(lhs, pqs[g])
            mem_v[c - 1, GW * g:GW * (g + 1), :] = ret[0:GW, :]
            mden_v[c - 1, HPG * g:HPG * g + 8, :] = ret[MROWS:MROWS + 8, :]

    def route():
        r = r_v[0:NSEG, :]
        idx = _iota((NSEG, L), 0) * L + _iota((NSEG, L), 1)
        m1 = jnp.max(r)
        i1 = jnp.clip(jnp.min(jnp.where(r == m1, idx, S)), 0, S - 1)
        r2 = jnp.where(idx == i1, -jnp.inf, r)
        m2 = jnp.max(r2)
        i2 = jnp.clip(jnp.min(jnp.where(r2 == m2, idx, S)), 0, S - 1)
        idx_s[0] = i1
        idx_s[1] = i2
        rsel_s[0] = m1
        rsel_s[1] = m2
        row16 = _iota((16, 128), 0)
        lane16 = _iota((16, 128), 1)
        xs = None
        for t, i in enumerate((i1, i2)):
            seg = i // L
            off = i - seg * L
            base = pl.multiple_of((off // 128) * 128, 128)
            cols = _unpack(xn_v[_rows(seg, D // 2), pl.ds(base, 128)])
            pick = jnp.where((row16 == t) & (lane16 == off - base), 1.0, 0.0)
            part = _dot_nt(pick.astype(BF16), cols)
            xs = part if xs is None else xs + part
        xs_v[...] = _pack(xs)
        y_v[...] = jnp.zeros(y_v.shape, F32)

    def ffn_in_tile(w_ref, tile):
        return _dot(_unpack(xs_v[...]), w_ref[:, 128 * tile:128 * (tile + 1)])

    def store_ffn_hidden(gates, ups):
        for tile, (gt, up) in enumerate(zip(gates, ups)):
            gt = _round_bf16(gt)
            hid = _round_bf16(_round_bf16(gt * jax.nn.sigmoid(gt)) * _round_bf16(up))
            for t in range(2):
                hid_v[t, tile] = jnp.broadcast_to(hid[t:t + 1, :], (8, 128))

    def project_last_with_ffn():
        c = NSEG - 1
        xn = _unpack(xn_v[_rows(c, D // 2), :])
        router = _dot(_unpack(wall[RROW // 2:PROWS // 2, :]), xn)
        r_v[c:c + 1, :] = _round_bf16(router[0:1, :])
        todo = [(w_ref, tile) for w_ref in (wg_v, wu_v) for tile in range(FF // 128)]
        done = []
        blocks = []
        for i, r in enumerate(range(0, RROW // 2, PBLOCK // 2)):
            if i == FFN_FIRST_BLOCK:
                route()
            lhs = _unpack(wall[r:min(r + PBLOCK // 2, RROW // 2), :])
            tiles = []
            for n in range(NQT):
                tiles.append(_dot(lhs, xn[:, 128 * n:128 * (n + 1)]))
                if i >= FFN_FIRST_BLOCK:
                    for _ in range(min(FFN_PATTERN[n % len(FFN_PATTERN)], len(todo))):
                        done.append(ffn_in_tile(*todo.pop(0)))
            blocks.append(jnp.concatenate(tiles, axis=1))
        pt = jnp.concatenate(blocks + [router], axis=0)
        return pt, todo, done

    def ffn_down_chained():
        base = pl.multiple_of(step * (FT * 128), 128)
        hid = [[hid_v[t, step * FT + tile] for tile in range(FT)] for t in range(2)]
        link = [None, None]
        for b in range(D // 8):
            acc = [None, None]
            for tile in range(FT):
                w = wd_v[8 * b:8 * b + 8, pl.ds(base + 128 * tile, 128)].astype(F32)
                for t in range(2):
                    pr = w * hid[t][tile]
                    if tile > 0:
                        acc[t] = acc[t] + pr
                    else:
                        acc[t] = pr if link[t] is None else pr + nothing(link[t])
            for t in range(2):
                rows = slice(8 * b, 8 * b + 8)
                y_v[t, rows, :] = y_v[t, rows, :] + acc[t]
                link[t] = acc[t]

    def ffn_down_looped():
        def down(tile, carry):
            col = step * FT + tile
            w = wd_v[:, pl.ds(pl.multiple_of(128 * col, 128), 128)].astype(F32)
            for t in range(2):
                y_v[t] = y_v[t] + w * hid_v[t, col][0:1, :]
            return carry

        lax.fori_loop(0, FT, down, 0)

    def masked_q_bits(g, hp, cols):
        rid = _iota((QROWS, 128), 0)
        mask = (rid >= (DH // 2) * hp) & (rid < (DH // 2) * (hp + 1))
        kept = jnp.where(mask, qt_v[_rows(step * NG + g, QROWS), cols], jnp.uint32(0))
        return jnp.concatenate([kept, jnp.zeros((64 - QROWS, 128), U32)], axis=0)

    def keys(g, lo, hi):
        first = pl.multiple_of((step * NG + g) * (L // 2) + lo // 2, 8)
        return _unpack(k_v[pl.ds(first, (hi - lo) // 2), :])

    def head_output(h, j, p, keep):
        o = _dot(_unpack(vt_v[_rows(step * H + h, 16), 0:128 * (j + 1)]), p)
        den = o[DH:DH + 1, :]
        inv = pl.reciprocal(den, approx=True)
        inv = inv * (2.0 - den * inv)
        return o[0:24, :] * (keep * inv)

    def group_probs(g, j, turn):
        cols = slice(128 * j, 128 * (j + 1))
        q = [masked_q_bits(g, 0, cols)] + [
            pltpu.roll(masked_q_bits(g, x, cols), 32 * x, 1) for x in range(1, 4)]
        off = [jnp.exp2(_dot(keys(g, 0, 128 * j), _unpack(q[x]))) for x in range(4)
               ] if j > 0 else None
        lane_q = _iota((64, 128), 1) // 32
        k0 = 128 * j
        e = [None] * 4
        for i in [(turn + n) % 4 for n in range(4)]:
            w = q[(3 - i) % 4]
            for lam in range(3):
                w = jnp.where(lane_q == lam, q[(lam - i) % 4], w)
            st = _dot(keys(g, k0, k0 + 32 * (i + 1)), _unpack(w))
            last = st[32 * i:, :] + quarter_v[...]
            st = last if i == 0 else jnp.concatenate([st[:32 * i, :], last], axis=0)
            e[i] = jnp.exp2(st)
        lane_q = _iota((32, 128), 1) // 32
        probs = {}
        for x in range(4):
            blocks = []
            for r in range(4):
                blk = e[0][0:32, :] if r == 0 else jnp.zeros((32, 128), F32)
                for i in range(max(r, 1), 4):
                    blk = jnp.where(lane_q == (i + x) % 4, e[i][32 * r:32 * (r + 1), :], blk)
                blocks.append(blk)
            full = jnp.concatenate(([off[x]] if j > 0 else []) + blocks, axis=0)
            probs[HPG * g + x] = full.astype(BF16)
        return probs

    def attention_bounded():
        waves = [(g, j) for g in range(NG) for j in range(NQT)]

        def scores(w):
            return group_probs(*waves[w], w % 4)

        def values(w, probs):
            j = waves[w][1]
            for h, p in probs.items():
                o = head_output(h, j, p, 1.0 - gate_v[h:h + 1, :])
                if h % HPG:
                    o = pltpu.roll(o, 128 - 32 * (h % HPG), 1)
                ot_v[step, DH * h:DH * (h + 1), 128 * j:128 * (j + 1)] = o[0:DH, :]

        pending = {}
        for w in range(len(waves) + LOOKAHEAD):
            if w < len(waves):
                pending[w] = scores(w)
            if w >= LOOKAHEAD:
                values(w - LOOKAHEAD, pending.pop(w - LOOKAHEAD))
        ffn_down_chained()

    def attention_max_shifted():
        def one_tile(item, carry):
            h = item // NQT
            j = item - h * NQT
            g = h // HPG
            hp = h - g * HPG
            cols = pl.ds(pl.multiple_of(128 * j, 128), 128)
            st = _dot(keys(g, 0, L), _unpack(masked_q_bits(g, hp, cols)))
            future = _iota((L, 128), 0) > 128 * j + _iota((L, 128), 1)
            st = jnp.where(future, NEG, st)
            p = jnp.exp2(st - jnp.max(st, axis=0, keepdims=True)).astype(BF16)
            keep = 1.0 - gate_v[pl.ds(h, 1), :]
            oh_v[h, :, cols] = head_output(h, NQT - 1, p, keep)
            return carry

        def compact(q, carry):
            rows = jnp.concatenate([oh_v[4 * q + k, 0:DH, :] for k in range(4)], axis=0)
            ot_v[step, pl.ds(pl.multiple_of(4 * DH * q, 8), 4 * DH), :] = rows
            return carry

        lax.fori_loop(0, H * NQT, one_tile, 0)
        lax.fori_loop(0, H // 4, compact, 0)
        ffn_down_looped()

    def routed_columns():
        ys = []
        for t in range(2):
            y = _round_bf16(jnp.sum(y_v[t], axis=1, keepdims=True))
            rsel = jnp.full((1, 1), rsel_s[t], F32)
            ys.append(_round_bf16(y * _round_bf16(jax.nn.sigmoid(rsel))))
        return ys

    def output_copy(seg, n):
        return pltpu.make_async_copy(
            out_v.at[pl.ds(seg * D, D), pl.ds(128 * n, 128)],
            o_hbm.at[:, pl.ds(seg * L + 128 * n, 128)],
            out_sems.at[NQT * seg + n])

    def output_projection(seg, ys):
        heads_out = ot_v[seg, 0:D, :]
        if seg > 0:
            gates = jnp.concatenate([gate_v[...]] * NQT, axis=1)
            scale = gates / (mden_v[seg - 1, 0:H, :] + 1e-6)
            pieces = []
            for b in range(D // 8):
                h0, h1 = (8 * b) // DH, (8 * b + 7) // DH
                sc = scale[h0:h0 + 1, :]
                if h1 != h0:
                    first = _iota((8, L), 0) < DH * h1 - 8 * b
                    sc = jnp.where(first, sc, scale[h1:h1 + 1, :])
                pieces.append(mem_v[seg - 1, 8 * b:8 * b + 8, :] * sc)
            heads_out = heads_out + jnp.concatenate(pieces, axis=0)
        attn = _dot(_unpack(wot[...]), heads_out.astype(BF16))
        base = x_v[seg].astype(F32) + attn
        xn = _unpack(xn_v[_rows(seg, D // 2), :]).astype(F32)
        col = seg * L + _iota((1, L), 1)
        upd = (jnp.where(col == idx_s[0], ys[0], 0.0)
               + jnp.where(col == idx_s[1], ys[1], 0.0))
        result = base + (xn + upd)
        for n in range(NQT):
            cols = slice(128 * n, 128 * (n + 1))
            out_v[seg * D:(seg + 1) * D, cols] = result[:, cols].astype(BF16)
            output_copy(seg, n).start()

    col_blocks = [(c0, min(128, D - c0)) for c0 in range(0, D, 128)]

    def transpose_block(w_v, section, c0, n):
        r0 = (section * D + c0) // 2
        wall[r0:r0 + n // 2, :] = pltpu.bitcast(w_v[:, c0:c0 + n].T, U32)

    def project_block(section, c0, n, xn):
        r0 = (section * D + c0) // 2
        last = section == 2 and c0 + n == D
        hi = PROWS // 2 if last else r0 + n // 2
        return _dot(_unpack(wall[r0:hi, :]), xn)

    def query_half0(half):
        layer_norm(0, serial=False, tiles=[2 * half, 2 * half + 1])
        xn = _unpack(xn_v[0:D // 2, 256 * half:256 * (half + 1)])
        top = _dot(_unpack(wall[0:D // 4, :]), xn)
        if half == 0:
            for c0, n in col_blocks[3:]:
                transpose_block(wq_v, 0, c0, n)
        bottom = _dot(_unpack(wall[D // 4:D // 2, :]), xn)
        return jnp.concatenate([top, bottom], axis=0)

    def projections():
        qtiles = []
        for half in range(2):
            x0_copies[half].wait()
            if half == 1:
                cp_wk.wait()
            qtiles.append(query_half0(half))
        for c0, n in col_blocks:
            transpose_block(wk_v, 1, c0, n)
        parts = [jnp.concatenate(qtiles, axis=1)]
        xn0 = _unpack(xn_v[_rows(0, D // 2), :])
        parts += [project_block(1, c0, n, xn0) for c0, n in col_blocks[:EARLY_K]]
        cp_wv.wait()
        x_copies[1].wait()
        xn0 = _unpack(xn_v[_rows(0, D // 2), :])
        parts += [project_block(1, c0, n, xn0) for c0, n in col_blocks[EARLY_K:]]
        for c0, n in col_blocks:
            transpose_block(wv_v, 2, c0, n)
            parts.append(project_block(2, c0, n, xn0))
        layer_norm(1)
        _, pk, vg = store_qkv(0, jnp.concatenate(parts, axis=0))
        x_copies[2].wait()
        x_copies[3].wait()
        cp_wo.wait()

        layer_norm(2)
        pt = project(1)
        wot[...] = pltpu.bitcast(wo_v[...].T, U32)
        state1 = memory_update(None, pk, vg)
        pq1, pk, vg = store_qkv(1, pt)
        layer_norm(3)
        pt = project(2)
        state2 = memory_update(state1, pk, vg)
        pq2, pk, vg = store_qkv(2, pt)
        cp_wg.wait()
        cp_wu.wait()
        pt, todo, done = project_last_with_ffn()
        pq3, _, _ = store_qkv(3, pt)
        state3 = memory_update(state2, pk, vg)
        done += [ffn_in_tile(*item) for item in todo]
        store_ffn_hidden(done[:FF // 128], done[FF // 128:])
        memory_retrieve(1, state1, pq1)
        memory_retrieve(2, state2, pq2)
        memory_retrieve(3, state3, pq3)
        record_logit_bound()
        cp_wd.wait()

    @pl.when(step == 0)
    def _():
        for cp in (cp_wq, cp_wr, cp_beta, *x0_copies, cp_wk, cp_wv, x_copies[1],
                   x_copies[2], x_copies[3], cp_wo, cp_wg, cp_wu, cp_wd):
            cp.start()
        with _scope("sc_startup"):
            cp_wr.wait()
            cp_beta.wait()
            cp_wq.wait()
            init_constants()
            for c0, n in col_blocks[:3]:
                transpose_block(wq_v, 0, c0, n)
        with _scope("sc_projections"):
            projections()

    @pl.when(step < NSEG)
    def _():
        safe = safe_s[0] == 1

        @pl.when(safe)
        def _():
            with _scope("sc_attention"):
                attention_bounded()

        @pl.when(jnp.logical_not(safe))
        def _():
            attention_max_shifted()

    @pl.when(step == NSEG)
    def _():
        with _scope("sc_outproj"):
            ys = routed_columns()
            for seg in range(NSEG):
                output_projection(seg, ys)
            for seg in range(NSEG):
                for n in range(NQT):
                    output_copy(seg, n).wait()


@jax.jit
def pallas_parallel_sum__memory_aug_infini_attn__moe_arch_mod__prompt_kernel(
    A_x: jax.Array,
    A_wq: jax.Array,
    A_wk: jax.Array,
    A_wv: jax.Array,
    A_wo: jax.Array,
    A_beta: jax.Array,
    B_x: jax.Array,
    B_w_r: jax.Array,
    B_w_gate: jax.Array,
    B_w_up: jax.Array,
    B_w_down: jax.Array,
):
    del B_x
    vm = pltpu.VMEM
    scratch = [
        vm((NSEG, D, L), BF16),
        vm((D, D), BF16),
        vm((D, D), BF16),
        vm((D, D), BF16),
        vm((D, D), BF16),
        vm((H,), BF16),
        vm((D,), BF16),
        vm((D, FF), BF16),
        vm((D, FF), BF16),
        vm((D, FF), BF16),
        vm((PROWS // 2, D), U32),
        vm((D // 2, D), U32),
        vm((NSEG * D // 2, L), U32),
        vm((NSEG * NG * QROWS, L), U32),
        vm((NSEG * NG * L // 2, 128), U32),
        vm((NSEG * H * 16, L), U32),
        vm((NSEG - 1, D, L), F32),
        vm((NSEG - 1, H + 8, L), F32),
        vm((8, L), F32),
        vm((8, D), U32),
        vm((2, D, 128), F32),
        vm((2, FF // 128, 8, 128), F32),
        pltpu.SMEM((2,), jnp.int32),
        pltpu.SMEM((2,), F32),
        pltpu.SMEM((1,), U32),
        pltpu.SMEM((1,), jnp.int32),
        vm((H, 128), F32),
        vm((NSEG, D, L), F32),
        vm((H, 24, L), F32),
        vm((32, 128), F32),
        vm((NSEG * D, L), BF16),
        pltpu.SemaphoreType.DMA((NSEG * NQT,)),
        pltpu.SemaphoreType.DMA((NSEG + 9 + 2,)),
    ]
    hbm = pl.BlockSpec(memory_space=pltpu.HBM)
    xt = jnp.transpose(A_x.reshape(S, D))
    out_t = pl.pallas_call(
        _kernel,
        grid=(NSEG + 1,),
        in_specs=[hbm] * 10,
        out_specs=hbm,
        out_shape=jax.ShapeDtypeStruct((D, S), BF16),
        scratch_shapes=scratch,
        compiler_params=pltpu.CompilerParams(
            dimension_semantics=("arbitrary",),
            vmem_limit_bytes=110 * 1024 * 1024,
        ),
        name="infini_moe",
    )(xt, A_wq, A_wk, A_wv, A_wo, A_beta, B_w_r, B_w_gate, B_w_up,
      jnp.transpose(B_w_down))
    return jnp.transpose(out_t).reshape(1, S, D)
```
